```python
import jax
import jax.numpy as jnp

def _softmax(x, axis=-1):
    return jax.nn.softmax(x, axis=axis)

def _gelu(x):
    return jax.nn.gelu(x, approximate=True)

def _silu(x):
    return jax.nn.silu(x)

def _sigmoid(x):
    return jax.nn.sigmoid(x)

def _layernorm(x, axis=-1, eps=1e-05):
    m = jnp.mean(x, axis=axis, keepdims=True)
    v = jnp.var(x, axis=axis, keepdims=True)
    return (x - m) / jnp.sqrt(v + eps)

def _scatter_add(tgt, idx, src, axis=0):
    return tgt.at[idx].add(src)

def _segment_sum(src, seg, n):
    return jax.ops.segment_sum(src, seg, n)

class _Rng:

    def __init__(self, key):
        self._k = key

    def _next(self):
        self._k, sub = jax.random.split(self._k)
        return sub

    def normal(self, shape):
        return jax.random.normal(self._next(), shape, dtype=jnp.bfloat16)

    def randint(self, lo, hi, shape):
        return jax.random.randint(self._next(), shape, lo, hi, dtype=jnp.int32)

    def uniform(self, shape, lo=0.0, hi=1.0):
        return jax.random.uniform(self._next(), shape, jnp.bfloat16, lo, hi)

    def permutation(self, n):
        return jax.random.permutation(self._next(), n)
kernel_name = 'adaLN_cond__memory_aug_recurrent_mem_tr__glu_gated_swiglu__prompt'

def setup_inputs():
    _rng = _Rng(jax.random.key(int.from_bytes(__import__("os").urandom(4), "little")))
    _w = lambda a: (lambda t: t.astype(jnp.bfloat16) if jnp.issubdtype(t.dtype, jnp.floating) else t)(jnp.asarray(a))

    def _A_setup():
        B, S, Dm = (1, 2048, 1024)
        H, Dh = (32, 128)
        M, seg = (8, 32)
        seg = min(seg, S)
        S = S // seg * seg
        return {'x': _w((lambda *s: _rng.normal(s) * 0.05)(B, S, Dm)), 'mem0': _w((lambda *s: _rng.normal(s) * 0.05)(B, M, Dm)), 'Wq': _w((lambda *s: _rng.normal(s) * 0.05)(Dm, H, Dh) * Dm ** (-0.5)), 'Wk': _w((lambda *s: _rng.normal(s) * 0.05)(Dm, H, Dh) * Dm ** (-0.5)), 'Wv': _w((lambda *s: _rng.normal(s) * 0.05)(Dm, H, Dh) * Dm ** (-0.5)), 'Wo': _w((lambda *s: _rng.normal(s) * 0.05)(H, Dh, Dm) * (H * Dh) ** (-0.5)), 'seg_len': seg}
    _A_in = _A_setup()

    def _B_setup():
        B, S, D, F = (1, 2048, 1024, 3584)
        return {'x': _w((lambda *s: _rng.normal(s) * 0.05)(B, S, D)), 'w1': _w((lambda *s: _rng.normal(s) * 0.05)(D, F) * (2.0 / D) ** 0.5), 'w3': _w((lambda *s: _rng.normal(s) * 0.05)(D, F) * (2.0 / D) ** 0.5), 'w2': _w((lambda *s: _rng.normal(s) * 0.05)(F, D) * (2.0 / F) ** 0.5)}
    _B_in = _B_setup()
    return {'A_x': _A_in['x'], 'A_mem0': _A_in['mem0'], 'A_Wq': _A_in['Wq'], 'A_Wk': _A_in['Wk'], 'A_Wv': _A_in['Wv'], 'A_Wo': _A_in['Wo'], 'A_seg_len': _A_in['seg_len'], 'B_x': _B_in['x'], 'B_w1': _B_in['w1'], 'B_w3': _B_in['w3'], 'B_w2': _B_in['w2'], 'c': _w((lambda *s: _rng.normal(s) * 0.05)(1, 1024)), 'w_mod': _w((lambda *s: _rng.normal(s) * 0.05)(1024, 6 * 1024) * 1024 ** (-0.5))}

def reference(A_x, A_mem0, A_Wq, A_Wk, A_Wv, A_Wo, A_seg_len, B_x, B_w1, B_w3, B_w2, c, w_mod):

    def _A_ref(x, mem0, Wq, Wk, Wv, Wo, seg_len):
        B, S, Dm = x.shape
        H, Dh = (Wq.shape[1], Wq.shape[2])
        M = mem0.shape[1]
        scale = Dh ** (-0.5)
        n_seg = S // seg_len
        L = M + seg_len
        idx = jnp.arange(L)
        mask = (idx[:, None] < M) | (idx[:, None] >= idx[None, :])
        mem = mem0
        outs = []
        for s in range(n_seg):
            xs = x[:, s * seg_len:(s + 1) * seg_len, :].copy()
            h = jnp.concatenate([mem, xs], axis=1)
            q = jnp.einsum('btd,dhe->bhte', h, Wq)
            k = jnp.einsum('btd,dhe->bhte', h, Wk)
            v = jnp.einsum('btd,dhe->bhte', h, Wv)
            scores = jnp.einsum('bhqe,bhke->bhqk', q, k) * scale
            scores = jnp.where(mask[None, None], scores, -1000000000.0)
            p = _softmax(scores, axis=-1)
            o = jnp.einsum('bhqk,bhke->bhqe', p, v)
            o = jnp.einsum('bhte,hed->btd', o, Wo)
            mem = o[:, :M, :].copy()
            outs.append(o[:, M:, :])
        return jnp.concatenate(outs, axis=1)

    def _B_ref(x, w1, w3, w2):
        gate = jnp.einsum('bsd,df->bsf', x, w1)
        up = jnp.einsum('bsd,df->bsf', x, w3)
        h = _silu(gate) * up
        out = jnp.einsum('bsf,fd->bsd', h, w2)
        return out
    x = A_x
    mod = (_silu(c) @ w_mod).reshape(c.shape[0], 6, 1, -1)
    sa, ca, ga, sb, cb, gb = (mod[:, 0].copy(), mod[:, 1].copy(), mod[:, 2].copy(), mod[:, 3].copy(), mod[:, 4].copy(), mod[:, 5].copy())
    h = _layernorm(x, axis=-1) * (1 + ca) + sa
    x = x + ga * _A_ref(h, A_mem0, A_Wq, A_Wk, A_Wv, A_Wo, A_seg_len)
    h = _layernorm(x, axis=-1) * (1 + cb) + sb
    x = x + gb * _B_ref(h, B_w1, B_w3, B_w2)
    return x
```

```python
import functools

import jax
import jax.numpy as jnp
from jax import lax
import jax.experimental.pallas as pl
import jax.experimental.pallas.tpu as pltpu

BF16 = jnp.bfloat16
F32 = jnp.float32
U32 = jnp.uint32

S = 2048
D = 1024
H = 32
DH = 128
F = 3584
M = 8
SEG = 32
NSEG = S // SEG
XR = 24
PRO = S - XR * NSEG
RING = 544
ORING = 576
OOFF = 256
PAD = 48
NC = D // 128
NF = F // 128
FB = 128
EPS = 1e-5
SCALE = DH ** -0.5


def _dot(a, b):
    return jnp.dot(a, b, preferred_element_type=F32)


def _w(ref32, i):
    return pltpu.bitcast(ref32[i], BF16)


def _ln_mod(x, shift, scale1):
    mu = jnp.mean(x, axis=-1, keepdims=True)
    xc = x - mu
    var = jnp.mean(xc * xc, axis=-1, keepdims=True)
    return xc * lax.rsqrt(var + EPS) * scale1 + shift


def _kernel(x_hbm, mem0_hbm, wq_hbm, wk_hbm, wv_hbm, wo_hbm, w1_hbm, w3_hbm,
            w2_hbm, c_hbm, wmod_hbm, out_hbm,
            wq_s, wk_s, wv_s, wo_s, xbuf, hbuf, qring, kring, vring,
            mod_s, mem_s, ax_s, hn_s, c_s, m0_s, sems):
    wq32 = wq_s.bitcast(U32)
    wk32 = wk_s.bitcast(U32)
    wv32 = wv_s.bitcast(U32)
    wo32 = wo_s.bitcast(U32)

    SEM_X0, SEM_X1, SEM_C, SEM_M0 = 0, 1, 2, 3
    SEM_WO = 4
    SEM_ST = SEM_WO + NC
    SEM_WM = SEM_ST + 12
    SEM_W1 = SEM_WM + 48
    SEM_W3 = SEM_W1 + NF
    SEM_W2 = SEM_W3 + NF
    SEM_OUT = SEM_W2 + NC

    cp_x0 = pltpu.make_async_copy(x_hbm.at[pl.ds(0, PRO)],
                                  xbuf.at[pl.ds(PAD, PRO)], sems.at[SEM_X0])
    cp_x1 = pltpu.make_async_copy(x_hbm.at[pl.ds(PRO, S - PRO)],
                                  xbuf.at[pl.ds(PAD + PRO, S - PRO)],
                                  sems.at[SEM_X1])
    cp_c = pltpu.make_async_copy(c_hbm, c_s, sems.at[SEM_C])
    cp_m0 = pltpu.make_async_copy(mem0_hbm, m0_s, sems.at[SEM_M0])
    cp_wo = [pltpu.make_async_copy(wo_hbm.at[:, pl.ds(c * 128, 128)],
                                   wo_s.at[c], sems.at[SEM_WO + c])
             for c in range(NC)]

    def mod_row(i):
        return mod_s[pl.ds(i, 1), :]

    def prologue(stq, stk, stv, wm_s):
        wm32 = wm_s.bitcast(U32)
        srcs = (wq_hbm, wk_hbm, wv_hbm)
        stages = (stq, stk, stv)
        dsts = (wq_s, wk_s, wv_s)

        def cp_st(j, g):
            return pltpu.make_async_copy(
                srcs[j].at[:, pl.ds(g * 8, 8), :], stages[j].at[g],
                sems.at[SEM_ST + j * 4 + g])

        cp_wm = [pltpu.make_async_copy(wmod_hbm.at[:, pl.ds(i * 128, 128)],
                                       wm_s.at[i], sems.at[SEM_WM + i])
                 for i in range(48)]

        cp_c.start()
        cp_m0.start()
        cp_x0.start()
        cp_st(0, 0).start()
        for i in range(16):
            cp_wm[i].start()
        cp_st(1, 0).start()
        cp_st(2, 0).start()
        for g in range(1, 4):
            for j in range(3):
                cp_st(j, g).start()
        cp_x1.start()
        for i in range(16, 48):
            cp_wm[i].start()
        for c in range(NC):
            cp_wo[c].start()

        xbuf[pl.ds(0, PAD), :] = jnp.zeros((PAD, D), BF16)
        ax_s[...] = jnp.zeros((XR, D), F32)

        def relayout(j, g):
            st, dst = stages[j], dsts[j]
            for db in range(8):
                blk = st[g, pl.ds(db * 128, 128), :, :]
                dst[pl.ds(g * 8, 8), pl.ds(db * 128, 128), :] = (
                    jnp.swapaxes(blk, 0, 1))

        cp_st(0, 0).wait()
        relayout(0, 0)

        cp_c.wait()
        cf = c_s[...].astype(F32)
        sc = (cf * jax.nn.sigmoid(cf)).astype(BF16)
        sc8 = jnp.broadcast_to(sc, (8, D))

        def mod_part(lo, hi):
            for i in range(lo, hi):
                cp_wm[i].wait()
            for k in range(lo // NC, hi // NC):
                parts = [_dot(sc8, _w(wm32, k * NC + c))[0:1, :]
                         for c in range(NC)]
                row = jnp.concatenate(parts, axis=1)
                if k in (1, 4):
                    row = row + 1.0
                mod_s[pl.ds(k, 1), :] = row

        mod_part(0, 16)
        cp_x0.wait()

        def ln1_body(i, carry):
            r = pl.multiple_of(PAD + i * 64, 8)
            xv = xbuf[pl.ds(r, 64), :].astype(F32)
            hbuf[pl.ds(r, 64), :] = _ln_mod(xv, mod_row(0), mod_row(1)).astype(BF16)
            return carry

        lax.fori_loop(0, PRO // 64, ln1_body, 0)

        def bulk(w32, ring, g):
            for mb in range(PRO // 128):
                lhs = hbuf[pl.ds(PAD + mb * 128, 128), :]
                for hh in range(8):
                    h = g * 8 + hh
                    ring[h, pl.ds(mb * 128, 128), :] = (
                        _dot(lhs, _w(w32, h)).astype(BF16))

        def grp_body(g, carry):
            cp_st(1, g).wait()
            relayout(1, g)
            bulk(wq32, qring, g)
            cp_st(2, g).wait()
            relayout(2, g)
            bulk(wk32, kring, g)
            gn = jnp.minimum(g + 1, 3)

            @pl.when(g < 3)
            def _():
                cp_st(0, gn).wait()

            relayout(0, gn)
            bulk(wv32, vring, g)
            return carry

        lax.fori_loop(0, 4, grp_body, 0)

        mod_part(16, 48)
        cp_x1.wait()
        cp_m0.wait()
        mem_s[...] = m0_s[...].astype(F32)
        xv = xbuf[pl.ds(PAD + PRO, XR), :].astype(F32)
        hn_s[...] = _ln_mod(xv, mod_row(0), mod_row(1))

    pl.run_scoped(
        prologue,
        pltpu.VMEM((4, D, 8, DH), BF16),
        pltpu.VMEM((4, D, 8, DH), BF16),
        pltpu.VMEM((4, D, 8, DH), BF16),
        pltpu.VMEM((48, D, 128), BF16),
    )

    def rest(w1_s, w3_s, w2_s, oring):
        w132 = w1_s.bitcast(U32)
        w332 = w3_s.bitcast(U32)
        w232 = w2_s.bitcast(U32)
        q32 = qring.bitcast(U32)
        k32 = kring.bitcast(U32)
        v32 = vring.bitcast(U32)

        cp_w1 = [pltpu.make_async_copy(w1_hbm.at[:, pl.ds(f * 128, 128)],
                                       w1_s.at[f], sems.at[SEM_W1 + f])
                 for f in range(NF)]
        cp_w3 = [pltpu.make_async_copy(w3_hbm.at[:, pl.ds(f * 128, 128)],
                                       w3_s.at[f], sems.at[SEM_W3 + f])
                 for f in range(NF)]
        cp_w2 = [pltpu.make_async_copy(w2_hbm.at[:, pl.ds(c * 128, 128)],
                                       w2_s.at[c], sems.at[SEM_W2 + c])
                 for c in range(NC)]
        for cp in cp_w1 + cp_w3 + cp_w2:
            cp.start()
        for c in range(NC):
            cp_wo[c].wait()

        oring[:, pl.ds(OOFF - XR, XR), :] = jnp.zeros((H, XR, DH), BF16)

        def post_attn(a, r, n):
            x1 = xbuf[pl.ds(r, n), :].astype(F32) + mod_row(2) * a
            x1 = x1.astype(BF16)
            xbuf[pl.ds(r, n), :] = x1
            hbuf[pl.ds(r, n), :] = _ln_mod(
                x1.astype(F32), mod_row(3), mod_row(4)).astype(BF16)

        row = lax.broadcasted_iota(jnp.int32, (48, 48), 0)
        col = lax.broadcasted_iota(jnp.int32, (48, 48), 1)
        mask = (col < SEG + M) & ((row >= SEG) | (col >= SEG) | (col <= row))
        fill = jnp.where(col < SEG + M, -1e9, -jnp.inf).astype(F32)

        def step(s, carry):
            lhs = jnp.concatenate([hn_s[...], mem_s[...]], axis=0).astype(BF16)

            post_attn(ax_s[...], pl.multiple_of(XR * s, 8), XR)
            rn = pl.multiple_of(
                PAD + jnp.minimum(PRO + XR * (s + 1), S - XR), 8)
            hn_s[...] = _ln_mod(xbuf[pl.ds(rn, XR), :].astype(F32),
                                mod_row(0), mod_row(1))

            wpos = [pl.multiple_of(lax.rem(PRO + XR * s + 8 * j, RING), 8)
                    for j in range(XR // 8)]
            rpos = pl.multiple_of(lax.rem(s, RING // SEG) * (SEG // 2), 16)
            opos = [pl.multiple_of(
                lax.rem(XR * s - XR + 8 * j + OOFF, ORING), 8)
                for j in range(XR // 8)]
            owr = pl.multiple_of(lax.rem(SEG * s + OOFF, ORING), SEG)
            zpad = jnp.zeros((8, DH), F32)

            lhs_o = []
            for h in range(H):
                full = []
                for w32, ring, r32 in ((wq32, qring, q32), (wk32, kring, k32),
                                       (wv32, vring, v32)):
                    t = _dot(lhs, _w(w32, h))
                    for j in range(XR // 8):
                        ring[h, pl.ds(wpos[j], 8), :] = (
                            t[8 * j:8 * j + 8].astype(BF16))
                    tail = jnp.concatenate([t[XR:], zpad], axis=0).astype(BF16)
                    tx = pltpu.bitcast(r32[h, pl.ds(rpos, SEG // 2), :], BF16)
                    full.append(jnp.concatenate([tx, tail], axis=0))
                q, k, v = full
                sc = lax.dot_general(q, k, (((1,), (1,)), ((), ())),
                                     preferred_element_type=F32)
                sc = jnp.where(mask, sc * SCALE, fill)
                mx = jnp.max(sc, axis=-1, keepdims=True)
                e = jnp.exp(sc - mx)
                l = jnp.sum(e, axis=-1, keepdims=True)
                o = _dot(e.astype(BF16), v) / l
                ox = [oring[h, pl.ds(opos[j], 8), :] for j in range(XR // 8)]
                last = jnp.concatenate(
                    [ox[2].astype(F32), o[SEG:SEG + M]], axis=0).astype(BF16)
                lhs_o.append(jnp.concatenate([ox[0], ox[1], last], axis=0))
                oring[h, pl.ds(owr, SEG), :] = o[:SEG].astype(BF16)
            lo = jnp.concatenate(lhs_o, axis=1)
            for c in range(NC):
                a = _dot(lo, _w(wo32, c))
                ax_s[:, pl.ds(c * 128, 128)] = a[:XR]
                mem_s[:, pl.ds(c * 128, 128)] = a[XR:]
            return carry

        lax.fori_loop(0, NSEG, step, 0)

        post_attn(ax_s[...], XR * NSEG, XR)
        done = XR * (NSEG - 1)

        def wo_bulk(r, n):
            p = r - done + (done + OOFF) % ORING
            if not isinstance(p, int):
                p = pl.multiple_of(p, 8)
            lo = jnp.concatenate(
                [oring[h, pl.ds(p, n), :] for h in range(H)], axis=1)
            a = jnp.concatenate(
                [_dot(lo, _w(wo32, c)) for c in range(NC)], axis=1)
            rr = PAD + r
            if not isinstance(rr, int):
                rr = pl.multiple_of(rr, 8)
            post_attn(a, rr, n)

        def wo_body(i, carry):
            wo_bulk(done + i * 128, 128)
            return carry

        lax.fori_loop(0, 4, wo_body, 0)
        wo_bulk(done + 512, S - done - 512)

        for cp in cp_w1 + cp_w3 + cp_w2:
            cp.wait()

        def cp_out(i):
            r = i * FB
            rb = PAD + r
            if not isinstance(i, int):
                r = pl.multiple_of(r, FB)
                rb = pl.multiple_of(rb, 8)
            return pltpu.make_async_copy(xbuf.at[pl.ds(rb, FB)],
                                         out_hbm.at[pl.ds(r, FB)],
                                         sems.at[SEM_OUT + i])

        def ffn_body(i, carry):
            r = pl.multiple_of(PAD + i * FB, 8)
            hv = hbuf[pl.ds(r, FB), :]
            act = []
            for f in range(NF):
                g = _dot(hv, _w(w132, f))
                u = _dot(hv, _w(w332, f))
                act.append((g * jax.nn.sigmoid(g) * u).astype(BF16))
            av = jnp.concatenate(act, axis=1)
            for c in range(NC):
                y = _dot(av, _w(w232, c))
                cs = pl.ds(c * 128, 128)
                x2 = xbuf[pl.ds(r, FB), cs].astype(F32) + mod_s[pl.ds(5, 1), cs] * y
                xbuf[pl.ds(r, FB), cs] = x2.astype(BF16)
            cp_out(i).start()
            return carry

        lax.fori_loop(0, S // FB, ffn_body, 0)
        for i in range(S // FB):
            cp_out(i).wait()

    pl.run_scoped(
        rest,
        pltpu.VMEM((NF, D, 128), BF16),
        pltpu.VMEM((NF, D, 128), BF16),
        pltpu.VMEM((NC, F, 128), BF16),
        pltpu.VMEM((H, ORING, DH), BF16),
    )


@functools.partial(jax.jit, static_argnames=("A_seg_len",))
def pallas_adaLN_cond__memory_aug_recurrent_mem_tr__glu_gated_swiglu__prompt_kernel(
    A_x: jax.Array,
    A_mem0: jax.Array,
    A_Wq: jax.Array,
    A_Wk: jax.Array,
    A_Wv: jax.Array,
    A_Wo: jax.Array,
    A_seg_len,
    B_x: jax.Array,
    B_w1: jax.Array,
    B_w3: jax.Array,
    B_w2: jax.Array,
    c: jax.Array,
    w_mod: jax.Array,
):
    del B_x
    assert A_seg_len == SEG
    assert A_x.shape == (1, S, D) and A_mem0.shape == (1, M, D)
    assert A_Wq.shape == (D, H, DH) and B_w1.shape == (D, F)

    n_sems = 4 + NC + 12 + 48 + NF + NF + NC + S // FB
    any_spec = pl.BlockSpec(memory_space=pl.ANY)
    out = pl.pallas_call(
        _kernel,
        out_shape=jax.ShapeDtypeStruct((S, D), BF16),
        in_specs=[any_spec] * 11,
        out_specs=any_spec,
        scratch_shapes=[
            pltpu.VMEM((H, D, DH), BF16),
            pltpu.VMEM((H, D, DH), BF16),
            pltpu.VMEM((H, D, DH), BF16),
            pltpu.VMEM((NC, H * DH, 128), BF16),
            pltpu.VMEM((PAD + S, D), BF16),
            pltpu.VMEM((PAD + S, D), BF16),
            pltpu.VMEM((H, RING, DH), BF16),
            pltpu.VMEM((H, RING, DH), BF16),
            pltpu.VMEM((H, RING, DH), BF16),
            pltpu.VMEM((8, D), F32),
            pltpu.VMEM((M, D), F32),
            pltpu.VMEM((XR, D), F32),
            pltpu.VMEM((XR, D), F32),
            pltpu.VMEM((1, D), BF16),
            pltpu.VMEM((M, D), BF16),
            pltpu.SemaphoreType.DMA((n_sems,)),
        ],
        compiler_params=pltpu.CompilerParams(
            vmem_limit_bytes=120 * 1024 * 1024),
        name="adaln_memtr_swiglu",
    )(
        A_x.reshape(S, D),
        A_mem0.reshape(M, D),
        A_Wq, A_Wk, A_Wv,
        A_Wo.reshape(H * DH, D),
        B_w1, B_w3, B_w2, c, w_mod,
    )
    return out.reshape(1, S, D)
```

```python
import functools

import jax
import jax.numpy as jnp
from jax import lax
import jax.experimental.pallas as pl
import jax.experimental.pallas.tpu as pltpu

BF16 = jnp.bfloat16
F32 = jnp.float32
U32 = jnp.uint32

S = 2048
D = 1024
H = 32
DH = 128
F = 3584
M = 8
SEG = 32
NSEG = S // SEG
XR = 24
PRO = S - XR * NSEG
RING = 544
ORING = 576
OOFF = 256
PAD = 48
NC = D // 128
NF = F // 128
FB = 128
NQ = SEG + M
EPS = 1e-5
SCALE = DH ** -0.5


def _dot(a, b):
    return jnp.dot(a, b, preferred_element_type=F32)


def _w(ref32, i):
    return pltpu.bitcast(ref32[i], BF16)


def _ln_mod(x, shift, scale1):
    mu = jnp.mean(x, axis=-1, keepdims=True)
    xc = x - mu
    var = jnp.mean(xc * xc, axis=-1, keepdims=True)
    return xc * lax.rsqrt(var + EPS) * scale1 + shift


def _kernel(x_hbm, mem0_hbm, wq_hbm, wk_hbm, wv_hbm, wo_hbm, w1_hbm, w3_hbm,
            w2_hbm, c_hbm, wmod_hbm, out_hbm,
            wq_s, wk_s, wv_s, wo_s, xbuf, hbuf, qring, kring, vring,
            mod_s, mem_s, ax_s, hn_s, c_s, m0_s, sems):
    wq32 = wq_s.bitcast(U32)
    wk32 = wk_s.bitcast(U32)
    wv32 = wv_s.bitcast(U32)
    wo32 = wo_s.bitcast(U32)

    SEM_X0, SEM_X1, SEM_C, SEM_M0 = 0, 1, 2, 3
    SEM_WO = 4
    SEM_ST = SEM_WO + NC
    SEM_WM = SEM_ST + 12
    SEM_W1 = SEM_WM + 48
    SEM_W3 = SEM_W1 + NF
    SEM_W2 = SEM_W3 + NF
    SEM_OUT = SEM_W2 + NC

    cp_x0 = pltpu.make_async_copy(x_hbm.at[pl.ds(0, PRO)],
                                  xbuf.at[pl.ds(PAD, PRO)], sems.at[SEM_X0])
    cp_x1 = pltpu.make_async_copy(x_hbm.at[pl.ds(PRO, S - PRO)],
                                  xbuf.at[pl.ds(PAD + PRO, S - PRO)],
                                  sems.at[SEM_X1])
    cp_c = pltpu.make_async_copy(c_hbm, c_s, sems.at[SEM_C])
    cp_m0 = pltpu.make_async_copy(mem0_hbm, m0_s, sems.at[SEM_M0])
    cp_wo = [pltpu.make_async_copy(wo_hbm.at[:, pl.ds(c * 128, 128)],
                                   wo_s.at[c], sems.at[SEM_WO + c])
             for c in range(NC)]

    def mod_row(i):
        return mod_s[pl.ds(i, 1), :]

    def prologue(stq, stk, stv, wm_s):
        wm32 = wm_s.bitcast(U32)
        srcs = (wq_hbm, wk_hbm, wv_hbm)
        stages = (stq, stk, stv)
        dsts = (wq_s, wk_s, wv_s)

        def cp_st(j, g):
            return pltpu.make_async_copy(
                srcs[j].at[:, pl.ds(g * 8, 8), :], stages[j].at[g],
                sems.at[SEM_ST + j * 4 + g])

        cp_wm = [pltpu.make_async_copy(wmod_hbm.at[:, pl.ds(i * 128, 128)],
                                       wm_s.at[i], sems.at[SEM_WM + i])
                 for i in range(48)]

        cp_c.start()
        cp_m0.start()
        cp_x0.start()
        cp_st(0, 0).start()
        for i in range(16):
            cp_wm[i].start()
        cp_st(1, 0).start()
        cp_st(2, 0).start()
        for g in range(1, 4):
            for j in range(3):
                cp_st(j, g).start()
        cp_x1.start()
        for i in range(16, 48):
            cp_wm[i].start()
        for c in range(NC):
            cp_wo[c].start()

        xbuf[pl.ds(0, PAD), :] = jnp.zeros((PAD, D), BF16)
        ax_s[...] = jnp.zeros((XR, D), F32)

        def relayout(j, g):
            st, dst = stages[j], dsts[j]
            for db in range(8):
                blk = st[g, pl.ds(db * 128, 128), :, :]
                dst[pl.ds(g * 8, 8), pl.ds(db * 128, 128), :] = (
                    jnp.swapaxes(blk, 0, 1))

        cp_st(0, 0).wait()
        relayout(0, 0)

        cp_c.wait()
        cf = c_s[...].astype(F32)
        sc = (cf * jax.nn.sigmoid(cf)).astype(BF16)
        sc8 = jnp.broadcast_to(sc, (8, D))

        def mod_part(lo, hi):
            for i in range(lo, hi):
                cp_wm[i].wait()
            for k in range(lo // NC, hi // NC):
                parts = [_dot(sc8, _w(wm32, k * NC + c))[0:1, :]
                         for c in range(NC)]
                row = jnp.concatenate(parts, axis=1)
                if k in (1, 4):
                    row = row + 1.0
                mod_s[pl.ds(k, 1), :] = row

        mod_part(0, 16)
        cp_x0.wait()

        def ln1_body(i, carry):
            r = pl.multiple_of(PAD + i * 64, 8)
            xv = xbuf[pl.ds(r, 64), :].astype(F32)
            hbuf[pl.ds(r, 64), :] = _ln_mod(xv, mod_row(0), mod_row(1)).astype(BF16)
            return carry

        lax.fori_loop(0, PRO // 64, ln1_body, 0)

        def bulk(w32, ring, g):
            for mb in range(PRO // 128):
                lhs = hbuf[pl.ds(PAD + mb * 128, 128), :]
                for hh in range(8):
                    h = g * 8 + hh
                    ring[h, pl.ds(mb * 128, 128), :] = (
                        _dot(lhs, _w(w32, h)).astype(BF16))

        def grp_body(g, carry):
            cp_st(1, g).wait()
            relayout(1, g)
            bulk(wq32, qring, g)
            cp_st(2, g).wait()
            relayout(2, g)
            bulk(wk32, kring, g)
            gn = jnp.minimum(g + 1, 3)

            @pl.when(g < 3)
            def _():
                cp_st(0, gn).wait()

            relayout(0, gn)
            bulk(wv32, vring, g)
            return carry

        lax.fori_loop(0, 4, grp_body, 0)

        mod_part(16, 48)
        cp_x1.wait()
        cp_m0.wait()
        mem_s[...] = m0_s[...].astype(F32)
        xv = xbuf[pl.ds(PAD + PRO, XR), :].astype(F32)
        hn_s[...] = _ln_mod(xv, mod_row(0), mod_row(1))

    pl.run_scoped(
        prologue,
        pltpu.VMEM((4, D, 8, DH), BF16),
        pltpu.VMEM((4, D, 8, DH), BF16),
        pltpu.VMEM((4, D, 8, DH), BF16),
        pltpu.VMEM((48, D, 128), BF16),
    )

    def rest(w1_s, w3_s, w2_s, oring):
        w132 = w1_s.bitcast(U32)
        w332 = w3_s.bitcast(U32)
        w232 = w2_s.bitcast(U32)
        q32 = qring.bitcast(U32)
        k32 = kring.bitcast(U32)
        v32 = vring.bitcast(U32)

        cp_w1 = [pltpu.make_async_copy(w1_hbm.at[:, pl.ds(f * 128, 128)],
                                       w1_s.at[f], sems.at[SEM_W1 + f])
                 for f in range(NF)]
        cp_w3 = [pltpu.make_async_copy(w3_hbm.at[:, pl.ds(f * 128, 128)],
                                       w3_s.at[f], sems.at[SEM_W3 + f])
                 for f in range(NF)]
        cp_w2 = [pltpu.make_async_copy(w2_hbm.at[:, pl.ds(c * 128, 128)],
                                       w2_s.at[c], sems.at[SEM_W2 + c])
                 for c in range(NC)]
        for cp in cp_w1 + cp_w3 + cp_w2:
            cp.start()
        for c in range(NC):
            cp_wo[c].wait()

        oring[:, pl.ds(OOFF - XR, XR), :] = jnp.zeros((H, XR, DH), BF16)

        def post_attn(a, r, n):
            x1 = xbuf[pl.ds(r, n), :].astype(F32) + mod_row(2) * a
            x1 = x1.astype(BF16)
            xbuf[pl.ds(r, n), :] = x1
            hbuf[pl.ds(r, n), :] = _ln_mod(
                x1.astype(F32), mod_row(3), mod_row(4)).astype(BF16)

        row = lax.broadcasted_iota(jnp.int32, (NQ, 48), 0)
        col = lax.broadcasted_iota(jnp.int32, (NQ, 48), 1)
        mask = (col < SEG + M) & ((row >= SEG) | (col >= SEG) | (col <= row))
        fill = jnp.where(col < SEG + M, -1e9, -jnp.inf).astype(F32)

        def step(s, carry):
            lhs = jnp.concatenate([hn_s[...], mem_s[...]], axis=0).astype(BF16)

            post_attn(ax_s[...], pl.multiple_of(XR * s, 8), XR)
            rn = pl.multiple_of(
                PAD + jnp.minimum(PRO + XR * (s + 1), S - XR), 8)
            hn_s[...] = _ln_mod(xbuf[pl.ds(rn, XR), :].astype(F32),
                                mod_row(0), mod_row(1))

            wpos = [pl.multiple_of(lax.rem(PRO + XR * s + 8 * j, RING), 8)
                    for j in range(XR // 8)]
            rpos = pl.multiple_of(lax.rem(s, RING // SEG) * (SEG // 2), 16)
            opos = [pl.multiple_of(
                lax.rem(XR * s - XR + 8 * j + OOFF, ORING), 8)
                for j in range(XR // 8)]
            owr = pl.multiple_of(lax.rem(SEG * s + OOFF, ORING), SEG)
            zpad = jnp.zeros((8, DH), F32)

            tails = {}
            xq, xk, xv = {}, {}, {}
            es, ls = {}, {}
            lhs_o = {}

            def seg_rows(r32, h):
                return pltpu.bitcast(r32[h, pl.ds(rpos, SEG // 2), :], BF16)

            def loads(hq, hv):
                if 0 <= hq < H:
                    xq[hq] = seg_rows(q32, hq)
                    xk[hq] = seg_rows(k32, hq)
                if 0 <= hv < H:
                    xv[hv] = seg_rows(v32, hv)

            def proj(h):
                tl = []
                for w32, ring in ((wq32, qring), (wk32, kring), (wv32, vring)):
                    t = _dot(lhs, _w(w32, h))
                    for j in range(XR // 8):
                        ring[h, pl.ds(wpos[j], 8), :] = (
                            t[8 * j:8 * j + 8].astype(BF16))
                    tl.append(jnp.concatenate([t[XR:], zpad], axis=0).astype(BF16))
                tails[h] = tl

            def qk(h):
                q = jnp.concatenate([xq.pop(h), tails[h][0]], axis=0)
                k = jnp.concatenate([xk.pop(h), tails[h][1]], axis=0)
                sc = lax.dot_general(q, k, (((1,), (1,)), ((), ())),
                                     preferred_element_type=F32)[:NQ]
                sc = jnp.where(mask, sc * SCALE, fill)
                mx = jnp.max(sc, axis=-1, keepdims=True)
                e = jnp.exp(sc - mx)
                ls[h] = jnp.sum(e, axis=-1, keepdims=True)
                es[h] = e.astype(BF16)

            def pv(h):
                v = jnp.concatenate([xv.pop(h), tails.pop(h)[2]], axis=0)
                o = _dot(es.pop(h), v) / ls.pop(h)
                ox = [oring[h, pl.ds(opos[j], 8), :] for j in range(XR // 8)]
                last = jnp.concatenate(
                    [ox[2].astype(F32), o[SEG:SEG + M]], axis=0).astype(BF16)
                lhs_o[h] = jnp.concatenate([ox[0], ox[1], last], axis=0)
                oring[h, pl.ds(owr, SEG), :] = o[:SEG].astype(BF16)

            def wo_part(c, h0, h1):
                lo = jnp.concatenate([lhs_o[h] for h in range(h0, h1)], axis=1)
                w = pltpu.bitcast(wo32[c, pl.ds(h0 * 64, (h1 - h0) * 64), :], BF16)
                return _dot(lo, w)

            for t in range(H):
                loads(t - 1, t - 3)
                proj(t)
                if t >= 1:
                    qk(t - 1)
                if t >= 3:
                    pv(t - 3)
            HA = H - 4
            acc = {}
            loads(H - 1, H - 3)
            for c in (0, 1):
                acc[c] = wo_part(c, 0, HA)
            qk(H - 1)
            pv(H - 3)
            loads(-1, H - 2)
            for c in (2, 3):
                acc[c] = wo_part(c, 0, HA)
            pv(H - 2)
            loads(-1, H - 1)
            for c in (4, 5):
                acc[c] = wo_part(c, 0, HA)
            pv(H - 1)
            for c in (6, 7):
                acc[c] = wo_part(c, 0, HA)
            for c in range(NC):
                a = acc[c] + wo_part(c, HA, H)
                ax_s[:, pl.ds(c * 128, 128)] = a[:XR]
                mem_s[:, pl.ds(c * 128, 128)] = a[XR:]
            return carry

        lax.fori_loop(0, NSEG, step, 0)

        post_attn(ax_s[...], XR * NSEG, XR)
        done = XR * (NSEG - 1)

        def wo_bulk(r, n):
            p = r - done + (done + OOFF) % ORING
            if not isinstance(p, int):
                p = pl.multiple_of(p, 8)
            lo = jnp.concatenate(
                [oring[h, pl.ds(p, n), :] for h in range(H)], axis=1)
            a = jnp.concatenate(
                [_dot(lo, _w(wo32, c)) for c in range(NC)], axis=1)
            rr = PAD + r
            if not isinstance(rr, int):
                rr = pl.multiple_of(rr, 8)
            post_attn(a, rr, n)

        def wo_body(i, carry):
            wo_bulk(done + i * 128, 128)
            return carry

        lax.fori_loop(0, 4, wo_body, 0)
        wo_bulk(done + 512, S - done - 512)

        for cp in cp_w1 + cp_w3 + cp_w2:
            cp.wait()

        def cp_out(i):
            r = i * FB
            rb = PAD + r
            if not isinstance(i, int):
                r = pl.multiple_of(r, FB)
                rb = pl.multiple_of(rb, 8)
            return pltpu.make_async_copy(xbuf.at[pl.ds(rb, FB)],
                                         out_hbm.at[pl.ds(r, FB)],
                                         sems.at[SEM_OUT + i])

        def ffn_body(i, carry):
            r = pl.multiple_of(PAD + i * FB, 8)
            hv = hbuf[pl.ds(r, FB), :]
            act = []
            for f in range(NF):
                g = _dot(hv, _w(w132, f))
                u = _dot(hv, _w(w332, f))
                act.append((g * jax.nn.sigmoid(g) * u).astype(BF16))
            av = jnp.concatenate(act, axis=1)
            for c in range(NC):
                y = _dot(av, _w(w232, c))
                cs = pl.ds(c * 128, 128)
                x2 = xbuf[pl.ds(r, FB), cs].astype(F32) + mod_s[pl.ds(5, 1), cs] * y
                xbuf[pl.ds(r, FB), cs] = x2.astype(BF16)
            cp_out(i).start()
            return carry

        lax.fori_loop(0, S // FB, ffn_body, 0)
        for i in range(S // FB):
            cp_out(i).wait()

    pl.run_scoped(
        rest,
        pltpu.VMEM((NF, D, 128), BF16),
        pltpu.VMEM((NF, D, 128), BF16),
        pltpu.VMEM((NC, F, 128), BF16),
        pltpu.VMEM((H, ORING, DH), BF16),
    )


@functools.partial(jax.jit, static_argnames=("A_seg_len",))
def pallas_adaLN_cond__memory_aug_recurrent_mem_tr__glu_gated_swiglu__prompt_kernel(
    A_x: jax.Array,
    A_mem0: jax.Array,
    A_Wq: jax.Array,
    A_Wk: jax.Array,
    A_Wv: jax.Array,
    A_Wo: jax.Array,
    A_seg_len,
    B_x: jax.Array,
    B_w1: jax.Array,
    B_w3: jax.Array,
    B_w2: jax.Array,
    c: jax.Array,
    w_mod: jax.Array,
):
    del B_x
    assert A_seg_len == SEG
    assert A_x.shape == (1, S, D) and A_mem0.shape == (1, M, D)
    assert A_Wq.shape == (D, H, DH) and B_w1.shape == (D, F)

    n_sems = 4 + NC + 12 + 48 + NF + NF + NC + S // FB
    any_spec = pl.BlockSpec(memory_space=pl.ANY)
    out = pl.pallas_call(
        _kernel,
        out_shape=jax.ShapeDtypeStruct((S, D), BF16),
        in_specs=[any_spec] * 11,
        out_specs=any_spec,
        scratch_shapes=[
            pltpu.VMEM((H, D, DH), BF16),
            pltpu.VMEM((H, D, DH), BF16),
            pltpu.VMEM((H, D, DH), BF16),
            pltpu.VMEM((NC, H * DH, 128), BF16),
            pltpu.VMEM((PAD + S, D), BF16),
            pltpu.VMEM((PAD + S, D), BF16),
            pltpu.VMEM((H, RING, DH), BF16),
            pltpu.VMEM((H, RING, DH), BF16),
            pltpu.VMEM((H, RING, DH), BF16),
            pltpu.VMEM((8, D), F32),
            pltpu.VMEM((M, D), F32),
            pltpu.VMEM((XR, D), F32),
            pltpu.VMEM((XR, D), F32),
            pltpu.VMEM((1, D), BF16),
            pltpu.VMEM((M, D), BF16),
            pltpu.SemaphoreType.DMA((n_sems,)),
        ],
        compiler_params=pltpu.CompilerParams(
            vmem_limit_bytes=120 * 1024 * 1024),
        name="adaln_memtr_swiglu",
    )(
        A_x.reshape(S, D),
        A_mem0.reshape(M, D),
        A_Wq, A_Wk, A_Wv,
        A_Wo.reshape(H * DH, D),
        B_w1, B_w3, B_w2, c, w_mod,
    )
    return out.reshape(1, S, D)
```

```python
import functools

import jax
import jax.numpy as jnp
from jax import lax
import jax.experimental.pallas as pl
import jax.experimental.pallas.tpu as pltpu

BF16 = jnp.bfloat16
F32 = jnp.float32
U32 = jnp.uint32

S = 2048
D = 1024
H = 32
DH = 128
F = 3584
M = 8
SEG = 32
NSEG = S // SEG
XR = 24
PRO = S - XR * NSEG
RING = 544
ORING = 576
OOFF = 256
PAD = 48
NC = D // 128
NF = F // 128
FB = 128
NQ = SEG + M
EPS = 1e-5
SCALE = DH ** -0.5


def _dot(a, b):
    return jnp.dot(a, b, preferred_element_type=F32)


def _w(ref32, i):
    return pltpu.bitcast(ref32[i], BF16)


def _ln_mod(x, shift, scale1):
    mu = jnp.mean(x, axis=-1, keepdims=True)
    xc = x - mu
    var = jnp.mean(xc * xc, axis=-1, keepdims=True)
    return xc * lax.rsqrt(var + EPS) * scale1 + shift


def _kernel(x_hbm, mem0_hbm, wq_hbm, wk_hbm, wv_hbm, wo_hbm, w1_hbm, w3_hbm,
            w2_hbm, c_hbm, wmod_hbm, out_hbm,
            wq_s, wk_s, wv_s, wo_s, xbuf, hbuf, qring, kring, vring,
            mod_s, mem_s, ax_s, hn_s, c_s, m0_s, sems):
    wq32 = wq_s.bitcast(U32)
    wk32 = wk_s.bitcast(U32)
    wv32 = wv_s.bitcast(U32)
    wo32 = wo_s.bitcast(U32)

    SEM_X0, SEM_X1, SEM_C, SEM_M0 = 0, 1, 2, 3
    SEM_WO = 4
    SEM_ST = SEM_WO + NC
    SEM_WM = SEM_ST + 12
    SEM_W1 = SEM_WM + 48
    SEM_W3 = SEM_W1 + NF
    SEM_W2 = SEM_W3 + NF
    SEM_OUT = SEM_W2 + NC

    cp_x0 = pltpu.make_async_copy(x_hbm.at[pl.ds(0, PRO)],
                                  xbuf.at[pl.ds(PAD, PRO)], sems.at[SEM_X0])
    cp_x1 = pltpu.make_async_copy(x_hbm.at[pl.ds(PRO, S - PRO)],
                                  xbuf.at[pl.ds(PAD + PRO, S - PRO)],
                                  sems.at[SEM_X1])
    cp_c = pltpu.make_async_copy(c_hbm, c_s, sems.at[SEM_C])
    cp_m0 = pltpu.make_async_copy(mem0_hbm, m0_s, sems.at[SEM_M0])
    cp_wo = [pltpu.make_async_copy(wo_hbm.at[:, pl.ds(c * 128, 128)],
                                   wo_s.at[c], sems.at[SEM_WO + c])
             for c in range(NC)]

    def mod_row(i):
        return mod_s[pl.ds(i, 1), :]

    def prologue(stq, stk, stv, wm_s):
        wm32 = wm_s.bitcast(U32)
        srcs = (wq_hbm, wk_hbm, wv_hbm)
        stages = (stq, stk, stv)
        dsts = (wq_s, wk_s, wv_s)

        def cp_st(j, g):
            return pltpu.make_async_copy(
                srcs[j].at[:, pl.ds(g * 8, 8), :], stages[j].at[g],
                sems.at[SEM_ST + j * 4 + g])

        cp_wm = [pltpu.make_async_copy(wmod_hbm.at[:, pl.ds(i * 128, 128)],
                                       wm_s.at[i], sems.at[SEM_WM + i])
                 for i in range(48)]

        cp_c.start()
        cp_m0.start()
        cp_x0.start()
        cp_st(0, 0).start()
        for i in range(16):
            cp_wm[i].start()
        cp_st(1, 0).start()
        cp_st(2, 0).start()
        for g in range(1, 4):
            for j in range(3):
                cp_st(j, g).start()
        cp_x1.start()
        for i in range(16, 48):
            cp_wm[i].start()
        for c in range(NC):
            cp_wo[c].start()

        xbuf[pl.ds(0, PAD), :] = jnp.zeros((PAD, D), BF16)
        ax_s[...] = jnp.zeros((XR, D), F32)

        def relayout(j, g):
            st, dst = stages[j], dsts[j]
            for db in range(8):
                blk = st[g, pl.ds(db * 128, 128), :, :]
                dst[pl.ds(g * 8, 8), pl.ds(db * 128, 128), :] = (
                    jnp.swapaxes(blk, 0, 1))

        cp_st(0, 0).wait()
        relayout(0, 0)

        cp_c.wait()
        cf = c_s[...].astype(F32)
        sc = (cf * jax.nn.sigmoid(cf)).astype(BF16)
        sc8 = jnp.broadcast_to(sc, (8, D))

        def mod_part(lo, hi):
            for i in range(lo, hi):
                cp_wm[i].wait()
            for k in range(lo // NC, hi // NC):
                parts = [_dot(sc8, _w(wm32, k * NC + c))[0:1, :]
                         for c in range(NC)]
                row = jnp.concatenate(parts, axis=1)
                if k in (1, 4):
                    row = row + 1.0
                mod_s[pl.ds(k, 1), :] = row

        mod_part(0, 16)
        cp_x0.wait()

        def ln1_body(i, carry):
            r = pl.multiple_of(PAD + i * 64, 8)
            xv = xbuf[pl.ds(r, 64), :].astype(F32)
            hbuf[pl.ds(r, 64), :] = _ln_mod(xv, mod_row(0), mod_row(1)).astype(BF16)
            return carry

        lax.fori_loop(0, PRO // 64, ln1_body, 0)

        def bulk(w32, ring, g):
            for mb in range(PRO // 128):
                lhs = hbuf[pl.ds(PAD + mb * 128, 128), :]
                for hh in range(8):
                    h = g * 8 + hh
                    ring[h, pl.ds(mb * 128, 128), :] = (
                        _dot(lhs, _w(w32, h)).astype(BF16))

        def grp_body(g, carry):
            cp_st(1, g).wait()
            relayout(1, g)
            bulk(wq32, qring, g)
            cp_st(2, g).wait()
            relayout(2, g)
            bulk(wk32, kring, g)
            gn = jnp.minimum(g + 1, 3)

            @pl.when(g < 3)
            def _():
                cp_st(0, gn).wait()

            relayout(0, gn)
            bulk(wv32, vring, g)
            return carry

        lax.fori_loop(0, 4, grp_body, 0)

        mod_part(16, 48)
        cp_x1.wait()
        cp_m0.wait()
        mem_s[...] = m0_s[...].astype(F32)
        xv = xbuf[pl.ds(PAD + PRO, XR), :].astype(F32)
        hn_s[...] = _ln_mod(xv, mod_row(0), mod_row(1))

    pl.run_scoped(
        prologue,
        pltpu.VMEM((4, D, 8, DH), BF16),
        pltpu.VMEM((4, D, 8, DH), BF16),
        pltpu.VMEM((4, D, 8, DH), BF16),
        pltpu.VMEM((48, D, 128), BF16),
    )

    def rest(w1_s, w3_s, w2_s, oring):
        w132 = w1_s.bitcast(U32)
        w332 = w3_s.bitcast(U32)
        w232 = w2_s.bitcast(U32)
        q32 = qring.bitcast(U32)
        k32 = kring.bitcast(U32)
        v32 = vring.bitcast(U32)

        cp_w1 = [pltpu.make_async_copy(w1_hbm.at[:, pl.ds(f * 128, 128)],
                                       w1_s.at[f], sems.at[SEM_W1 + f])
                 for f in range(NF)]
        cp_w3 = [pltpu.make_async_copy(w3_hbm.at[:, pl.ds(f * 128, 128)],
                                       w3_s.at[f], sems.at[SEM_W3 + f])
                 for f in range(NF)]
        cp_w2 = [pltpu.make_async_copy(w2_hbm.at[:, pl.ds(c * 128, 128)],
                                       w2_s.at[c], sems.at[SEM_W2 + c])
                 for c in range(NC)]
        for cp in cp_w1 + cp_w3 + cp_w2:
            cp.start()
        for c in range(NC):
            cp_wo[c].wait()

        oring[:, pl.ds(OOFF - XR, XR), :] = jnp.zeros((H, XR, DH), BF16)

        def post_attn(a, r, n):
            x1 = xbuf[pl.ds(r, n), :].astype(F32) + mod_row(2) * a
            x1 = x1.astype(BF16)
            xbuf[pl.ds(r, n), :] = x1
            hbuf[pl.ds(r, n), :] = _ln_mod(
                x1.astype(F32), mod_row(3), mod_row(4)).astype(BF16)

        row = lax.broadcasted_iota(jnp.int32, (NQ, 48), 0)
        col = lax.broadcasted_iota(jnp.int32, (NQ, 48), 1)
        mask = (col < SEG + M) & ((row >= SEG) | (col >= SEG) | (col <= row))
        fill = jnp.where(col < SEG + M, -1e9, -jnp.inf).astype(F32)

        def step(s, carry):
            lhs = jnp.concatenate([hn_s[...], mem_s[...]], axis=0).astype(BF16)

            post_attn(ax_s[...], pl.multiple_of(XR * s, 8), XR)
            rn = pl.multiple_of(
                PAD + jnp.minimum(PRO + XR * (s + 1), S - XR), 8)
            hn_s[...] = _ln_mod(xbuf[pl.ds(rn, XR), :].astype(F32),
                                mod_row(0), mod_row(1))

            wpos = [pl.multiple_of(lax.rem(PRO + XR * s + 8 * j, RING), 8)
                    for j in range(XR // 8)]
            rpos = pl.multiple_of(lax.rem(s, RING // SEG) * (SEG // 2), 16)
            opos = [pl.multiple_of(
                lax.rem(XR * s - XR + 8 * j + OOFF, ORING), 8)
                for j in range(XR // 8)]
            owr = pl.multiple_of(lax.rem(SEG * s + OOFF, ORING), SEG)
            zpad = jnp.zeros((8, DH), F32)

            tails = {}
            xq, xk, xv = {}, {}, {}
            es, rs = {}, {}

            def pad16(a, b):
                return jnp.concatenate([a, b], axis=0).astype(BF16)

            lhs_o = {}

            def seg_rows(r32, h):
                return pltpu.bitcast(r32[h, pl.ds(rpos, SEG // 2), :], BF16)

            def loads(hq, hv):
                if 0 <= hq < H:
                    xq[hq] = seg_rows(q32, hq)
                    xk[hq] = seg_rows(k32, hq)
                if 0 <= hv < H:
                    xv[hv] = seg_rows(v32, hv)

            def proj(h):
                tl = []
                for w32, ring in ((wq32, qring), (wk32, kring), (wv32, vring)):
                    t = _dot(lhs, _w(w32, h))
                    for j in range(XR // 8):
                        ring[h, pl.ds(wpos[j], 8), :] = (
                            t[8 * j:8 * j + 8].astype(BF16))
                    tl.append(t[XR:])
                tails[h] = tl

            def qk(h):
                q = jnp.concatenate([xq.pop(h), pad16(tails[h][0], zpad)], axis=0)
                k = jnp.concatenate([xk.pop(h), pad16(tails[h][1], zpad)], axis=0)
                sc = lax.dot_general(q, k, (((1,), (1,)), ((), ())),
                                     preferred_element_type=F32)[:NQ]
                sc = jnp.where(mask, sc * SCALE, fill)
                mx = jnp.max(sc, axis=-1, keepdims=True)
                e = jnp.exp(sc - mx)
                l = jnp.sum(e, axis=-1, keepdims=True)
                r = pl.reciprocal(l, approx=True)
                es[h] = (e * r).astype(BF16)
                rs[h] = jnp.broadcast_to(r[SEG:], (M, DH))

            def pv(h):
                v = jnp.concatenate(
                    [xv.pop(h), pad16(tails.pop(h)[2], rs.pop(h))], axis=0)
                o = _dot(es.pop(h), v)
                ox = [oring[h, pl.ds(opos[j], 8), :] for j in range(XR // 8)]
                last = jnp.concatenate(
                    [ox[2].astype(F32), o[SEG:SEG + M]], axis=0).astype(BF16)
                lhs_o[h] = jnp.concatenate([ox[0], ox[1], last], axis=0)
                oring[h, pl.ds(owr, SEG), :] = o[:SEG].astype(BF16)

            def wo_part(c, h0, h1):
                lo = jnp.concatenate([lhs_o[h] for h in range(h0, h1)], axis=1)
                w = pltpu.bitcast(wo32[c, pl.ds(h0 * 64, (h1 - h0) * 64), :], BF16)
                return _dot(lo, w)

            PD = 4
            for t in range(H):
                loads(t - 1, t - PD)
                proj(t)
                if t >= 1:
                    qk(t - 1)
                if t >= PD:
                    pv(t - PD)
            HA = H - 4
            acc = {}
            loads(H - 1, H - 4)
            acc[0] = wo_part(0, 0, HA)
            qk(H - 1)
            pv(H - 4)
            loads(-1, H - 3)
            acc[1] = wo_part(1, 0, HA)
            pv(H - 3)
            loads(-1, H - 2)
            acc[2] = wo_part(2, 0, HA)
            pv(H - 2)
            loads(-1, H - 1)
            for c in (3, 4):
                acc[c] = wo_part(c, 0, HA)
            pv(H - 1)
            for c in (5, 6, 7):
                acc[c] = wo_part(c, 0, HA)
            for c in range(NC):
                a = wo_part(c, HA, H) + acc[c]
                ax_s[:, pl.ds(c * 128, 128)] = a[:XR]
                mem_s[:, pl.ds(c * 128, 128)] = a[XR:]
            return carry

        lax.fori_loop(0, NSEG, step, 0)

        post_attn(ax_s[...], XR * NSEG, XR)
        done = XR * (NSEG - 1)

        def wo_bulk(r, n):
            p = r - done + (done + OOFF) % ORING
            if not isinstance(p, int):
                p = pl.multiple_of(p, 8)
            lo = jnp.concatenate(
                [oring[h, pl.ds(p, n), :] for h in range(H)], axis=1)
            a = jnp.concatenate(
                [_dot(lo, _w(wo32, c)) for c in range(NC)], axis=1)
            rr = PAD + r
            if not isinstance(rr, int):
                rr = pl.multiple_of(rr, 8)
            post_attn(a, rr, n)

        def wo_body(i, carry):
            wo_bulk(done + i * 128, 128)
            return carry

        lax.fori_loop(0, 4, wo_body, 0)
        wo_bulk(done + 512, S - done - 512)

        for cp in cp_w1 + cp_w3 + cp_w2:
            cp.wait()

        def cp_out(i):
            r = i * FB
            rb = PAD + r
            if not isinstance(i, int):
                r = pl.multiple_of(r, FB)
                rb = pl.multiple_of(rb, 8)
            return pltpu.make_async_copy(xbuf.at[pl.ds(rb, FB)],
                                         out_hbm.at[pl.ds(r, FB)],
                                         sems.at[SEM_OUT + i])

        def ffn_body(i, carry):
            r = pl.multiple_of(PAD + i * FB, 8)
            hv = hbuf[pl.ds(r, FB), :]
            act = []
            for f in range(NF):
                g = _dot(hv, _w(w132, f))
                u = _dot(hv, _w(w332, f))
                act.append((g * jax.nn.sigmoid(g) * u).astype(BF16))
            av = jnp.concatenate(act, axis=1)
            for c in range(NC):
                y = _dot(av, _w(w232, c))
                cs = pl.ds(c * 128, 128)
                x2 = xbuf[pl.ds(r, FB), cs].astype(F32) + mod_s[pl.ds(5, 1), cs] * y
                xbuf[pl.ds(r, FB), cs] = x2.astype(BF16)
            cp_out(i).start()
            return carry

        lax.fori_loop(0, S // FB, ffn_body, 0)
        for i in range(S // FB):
            cp_out(i).wait()

    pl.run_scoped(
        rest,
        pltpu.VMEM((NF, D, 128), BF16),
        pltpu.VMEM((NF, D, 128), BF16),
        pltpu.VMEM((NC, F, 128), BF16),
        pltpu.VMEM((H, ORING, DH), BF16),
    )


@functools.partial(jax.jit, static_argnames=("A_seg_len",))
def pallas_adaLN_cond__memory_aug_recurrent_mem_tr__glu_gated_swiglu__prompt_kernel(
    A_x: jax.Array,
    A_mem0: jax.Array,
    A_Wq: jax.Array,
    A_Wk: jax.Array,
    A_Wv: jax.Array,
    A_Wo: jax.Array,
    A_seg_len,
    B_x: jax.Array,
    B_w1: jax.Array,
    B_w3: jax.Array,
    B_w2: jax.Array,
    c: jax.Array,
    w_mod: jax.Array,
):
    del B_x
    assert A_seg_len == SEG
    assert A_x.shape == (1, S, D) and A_mem0.shape == (1, M, D)
    assert A_Wq.shape == (D, H, DH) and B_w1.shape == (D, F)

    n_sems = 4 + NC + 12 + 48 + NF + NF + NC + S // FB
    any_spec = pl.BlockSpec(memory_space=pl.ANY)
    out = pl.pallas_call(
        _kernel,
        out_shape=jax.ShapeDtypeStruct((S, D), BF16),
        in_specs=[any_spec] * 11,
        out_specs=any_spec,
        scratch_shapes=[
            pltpu.VMEM((H, D, DH), BF16),
            pltpu.VMEM((H, D, DH), BF16),
            pltpu.VMEM((H, D, DH), BF16),
            pltpu.VMEM((NC, H * DH, 128), BF16),
            pltpu.VMEM((PAD + S, D), BF16),
            pltpu.VMEM((PAD + S, D), BF16),
            pltpu.VMEM((H, RING, DH), BF16),
            pltpu.VMEM((H, RING, DH), BF16),
            pltpu.VMEM((H, RING, DH), BF16),
            pltpu.VMEM((8, D), F32),
            pltpu.VMEM((M, D), F32),
            pltpu.VMEM((XR, D), F32),
            pltpu.VMEM((XR, D), F32),
            pltpu.VMEM((1, D), BF16),
            pltpu.VMEM((M, D), BF16),
            pltpu.SemaphoreType.DMA((n_sems,)),
        ],
        compiler_params=pltpu.CompilerParams(
            vmem_limit_bytes=120 * 1024 * 1024),
        name="adaln_memtr_swiglu",
    )(
        A_x.reshape(S, D),
        A_mem0.reshape(M, D),
        A_Wq, A_Wk, A_Wv,
        A_Wo.reshape(H * DH, D),
        B_w1, B_w3, B_w2, c, w_mod,
    )
    return out.reshape(1, S, D)
```

```python
import functools

import jax
import jax.numpy as jnp
from jax import lax
import jax.experimental.pallas as pl
import jax.experimental.pallas.tpu as pltpu

BF16 = jnp.bfloat16
F32 = jnp.float32
U32 = jnp.uint32

S = 2048
D = 1024
H = 32
DH = 128
F = 3584
M = 8
SEG = 32
NSEG = S // SEG
XR = 24
PRO = S - XR * NSEG
RING = 544
ORING = 576
OOFF = 256
PAD = 48
NC = D // 128
NF = F // 128
FB = 128
NU = 3 * H // 2
UPI = 6
NQ = SEG + M
EPS = 1e-5
SCALE = DH ** -0.5


def _dot(a, b):
    return jnp.dot(a, b, preferred_element_type=F32)


def _w(ref32, i):
    return pltpu.bitcast(ref32[i], BF16)


def _ln(x):
    mu = jnp.mean(x, axis=-1, keepdims=True)
    xc = x - mu
    var = jnp.mean(xc * xc, axis=-1, keepdims=True)
    return xc * lax.rsqrt(var + EPS)


def _ln_mod(x, shift, scale1):
    return _ln(x) * scale1 + shift


def _kernel(x_hbm, mem0_hbm, wq_hbm, wk_hbm, wv_hbm, wo_hbm, w1_hbm, w3_hbm,
            w2_hbm, c_hbm, wmod_hbm, out_hbm,
            wq32, wk32, wv32, wo_s, xbuf, hbuf, qring, kring, vring,
            mod_s, mem_s, ax_s, hn_s, c_s, m0_s, sems):
    wo32 = wo_s.bitcast(U32)

    SEM_X0, SEM_X1, SEM_C, SEM_M0 = 0, 1, 2, 3
    SEM_WO = 4
    SEM_ST = SEM_WO + NC
    SEM_WM = SEM_ST + NU
    SEM_W1 = SEM_WM + 48
    SEM_W3 = SEM_W1 + NF
    SEM_W2 = SEM_W3 + NF
    SEM_OUT = SEM_W2 + NC

    cp_x0 = pltpu.make_async_copy(x_hbm.at[pl.ds(0, PRO)],
                                  xbuf.at[pl.ds(PAD, PRO)], sems.at[SEM_X0])
    cp_x1 = pltpu.make_async_copy(x_hbm.at[pl.ds(PRO, S - PRO)],
                                  xbuf.at[pl.ds(PAD + PRO, S - PRO)],
                                  sems.at[SEM_X1])
    cp_c = pltpu.make_async_copy(c_hbm, c_s, sems.at[SEM_C])
    cp_m0 = pltpu.make_async_copy(mem0_hbm, m0_s, sems.at[SEM_M0])
    cp_wo = [pltpu.make_async_copy(wo_hbm.at[:, pl.ds(c * 128, 128)],
                                   wo_s.at[c], sems.at[SEM_WO + c])
             for c in range(NC)]

    def mod_row(i):
        return mod_s[pl.ds(i, 1), :]

    def prologue(st, wm_s, xn_s):
        wm32 = wm_s.bitcast(U32)
        srcs = (wq_hbm.bitcast(U32), wk_hbm.bitcast(U32), wv_hbm.bitcast(U32))
        dsts = (wq32, wk32, wv32)
        rings = (qring, kring, vring)

        def cp_st(j, s):
            return pltpu.make_async_copy(
                srcs[j].at[:, s, :], st.at[3 * s + j],
                sems.at[SEM_ST + 3 * s + j])

        cp_wm = [pltpu.make_async_copy(wmod_hbm.at[:, pl.ds(i * 128, 128)],
                                       wm_s.at[i], sems.at[SEM_WM + i])
                 for i in range(48)]

        cp_c.start()
        cp_m0.start()
        cp_x0.start()
        for i in range(16):
            cp_wm[i].start()
        for u in range(NU):
            cp_st(u % 3, u // 3).start()
        cp_x1.start()
        for i in range(16, 48):
            cp_wm[i].start()
        for c in range(NC):
            cp_wo[c].start()

        xbuf[pl.ds(0, PAD), :] = jnp.zeros((PAD, D), BF16)
        ax_s[...] = jnp.zeros((XR, D), F32)

        cp_c.wait()
        cf = c_s[...].astype(F32)
        sc = (cf * jax.nn.sigmoid(cf)).astype(BF16)
        sc8 = jnp.broadcast_to(sc, (8, D))

        cp_x0.wait()

        def ln_body(i, carry):
            r = pl.multiple_of(i * 64, 64)
            xv = xbuf[pl.ds(pl.multiple_of(PAD + r, 8), 64), :].astype(F32)
            xn_s[pl.ds(r, 64), :] = _ln(xv)
            return carry

        lax.fori_loop(0, PRO // 64, ln_body, 0)

        def mod_part(lo, hi, chunk):
            for c0 in range(lo, hi, chunk):
                for i in range(c0, c0 + chunk):
                    cp_wm[i].wait()
                for i in range(c0, c0 + chunk):
                    k, c = divmod(i, NC)
                    part = _dot(sc8, _w(wm32, i))[0:1, :]
                    if k in (1, 4):
                        part = part + 1.0
                    mod_s[pl.ds(k, 1), pl.ds(c * 128, 128)] = part

        mod_part(0, 16, 4)

        def relayout(j, s):
            u = 3 * s + j
            for db in range(8):
                ev = st[u, pl.ds(db * 128, 64, stride=2), :]
                od = st[u, pl.ds(db * 128 + 1, 64, stride=2), :]
                rows = pl.ds(db * 64, 64)
                dsts[j][2 * s, rows, :] = (ev & U32(0xFFFF)) | (od << 16)
                dsts[j][2 * s + 1, rows, :] = (ev >> 16) | (od & U32(0xFFFF0000))

        def bulk(j, s, first=False):
            for mb in range(PRO // 128):
                rows = pl.ds(PAD + mb * 128, 128)
                if first:
                    lhs = (xn_s[pl.ds(mb * 128, 128), :] * mod_row(1)
                           + mod_row(0)).astype(BF16)
                    hbuf[rows, :] = lhs
                else:
                    lhs = hbuf[rows, :]
                for hh in range(2):
                    h = 2 * s + hh
                    rings[j][h, pl.ds(mb * 128, 128), :] = (
                        _dot(lhs, _w(dsts[j], h)).astype(BF16))

        cp_st(0, 0).wait()
        relayout(0, 0)
        for u in range(UPI):
            cp_st((u + 1) % 3, (u + 1) // 3).wait()
            relayout((u + 1) % 3, (u + 1) // 3)
            bulk(u % 3, u // 3, first=(u == 0))

        def grp_body(it, carry):
            s0 = it * (UPI // 3)
            last = NU // UPI - 1
            sn = jnp.minimum(s0 + UPI // 3, H // 2 - 1)
            for u in range(1, UPI):
                cp_st(u % 3, s0 + u // 3).wait()

            @pl.when(it < last)
            def _():
                cp_st(0, sn).wait()

            for u in range(UPI):
                if u + 1 < UPI:
                    relayout((u + 1) % 3, s0 + (u + 1) // 3)
                else:
                    relayout(0, sn)
                bulk(u % 3, s0 + u // 3)
            return carry

        lax.fori_loop(1, NU // UPI, grp_body, 0)

        mod_part(16, 48, 32)
        cp_x1.wait()
        cp_m0.wait()
        mem_s[...] = m0_s[...].astype(F32)
        xv = xbuf[pl.ds(PAD + PRO, XR), :].astype(F32)
        hn_s[...] = _ln_mod(xv, mod_row(0), mod_row(1))

    pl.run_scoped(
        prologue,
        pltpu.VMEM((NU, D, DH), U32),
        pltpu.VMEM((48, D, 128), BF16),
        pltpu.VMEM((PRO, D), F32),
    )

    def rest(w1_s, w3_s, w2_s, oring):
        w132 = w1_s.bitcast(U32)
        w332 = w3_s.bitcast(U32)
        w232 = w2_s.bitcast(U32)
        q32 = qring.bitcast(U32)
        k32 = kring.bitcast(U32)
        v32 = vring.bitcast(U32)

        cp_w1 = [pltpu.make_async_copy(w1_hbm.at[:, pl.ds(f * 128, 128)],
                                       w1_s.at[f], sems.at[SEM_W1 + f])
                 for f in range(NF)]
        cp_w3 = [pltpu.make_async_copy(w3_hbm.at[:, pl.ds(f * 128, 128)],
                                       w3_s.at[f], sems.at[SEM_W3 + f])
                 for f in range(NF)]
        cp_w2 = [pltpu.make_async_copy(w2_hbm.at[:, pl.ds(c * 128, 128)],
                                       w2_s.at[c], sems.at[SEM_W2 + c])
                 for c in range(NC)]
        for cp in cp_w1 + cp_w3 + cp_w2:
            cp.start()
        for c in range(NC):
            cp_wo[c].wait()

        oring[:, pl.ds(OOFF - XR, XR), :] = jnp.zeros((H, XR, DH), BF16)

        def post_attn(a, r, n):
            x1 = xbuf[pl.ds(r, n), :].astype(F32) + mod_row(2) * a
            x1 = x1.astype(BF16)
            xbuf[pl.ds(r, n), :] = x1
            hbuf[pl.ds(r, n), :] = _ln_mod(
                x1.astype(F32), mod_row(3), mod_row(4)).astype(BF16)

        row = lax.broadcasted_iota(jnp.int32, (NQ, 48), 0)
        col = lax.broadcasted_iota(jnp.int32, (NQ, 48), 1)
        mask = (col < SEG + M) & ((row >= SEG) | (col >= SEG) | (col <= row))
        fill = jnp.where(col < SEG + M, -1e9, -jnp.inf).astype(F32)

        def step(s, carry):
            lhs = jnp.concatenate([hn_s[...], mem_s[...]], axis=0).astype(BF16)

            post_attn(ax_s[...], pl.multiple_of(XR * s, 8), XR)
            rn = pl.multiple_of(
                PAD + jnp.minimum(PRO + XR * (s + 1), S - XR), 8)
            hn_s[...] = _ln_mod(xbuf[pl.ds(rn, XR), :].astype(F32),
                                mod_row(0), mod_row(1))

            wpos = [pl.multiple_of(lax.rem(PRO + XR * s + 8 * j, RING), 8)
                    for j in range(XR // 8)]
            rpos = pl.multiple_of(lax.rem(s, RING // SEG) * (SEG // 2), 16)
            opos = [pl.multiple_of(
                lax.rem(XR * s - XR + 8 * j + OOFF, ORING), 8)
                for j in range(XR // 8)]
            owr = pl.multiple_of(lax.rem(SEG * s + OOFF, ORING), SEG)
            zpad = jnp.zeros((8, DH), F32)

            tails = {}
            xq, xk, xv = {}, {}, {}
            es, rs = {}, {}

            def pad16(a, b):
                return jnp.concatenate([a, b], axis=0).astype(BF16)

            lhs_o = {}

            def seg_rows(r32, h):
                return pltpu.bitcast(r32[h, pl.ds(rpos, SEG // 2), :], BF16)

            def loads(hq, hv):
                if 0 <= hq < H:
                    xq[hq] = seg_rows(q32, hq)
                    xk[hq] = seg_rows(k32, hq)
                if 0 <= hv < H:
                    xv[hv] = seg_rows(v32, hv)

            def proj(h):
                tl = []
                for w32, ring in ((wq32, qring), (wk32, kring), (wv32, vring)):
                    t = _dot(lhs, _w(w32, h))
                    for j in range(XR // 8):
                        ring[h, pl.ds(wpos[j], 8), :] = (
                            t[8 * j:8 * j + 8].astype(BF16))
                    tl.append(t[XR:])
                tails[h] = tl

            def qk(h):
                q = jnp.concatenate([xq.pop(h), pad16(tails[h][0], zpad)], axis=0)
                k = jnp.concatenate([xk.pop(h), pad16(tails[h][1], zpad)], axis=0)
                sc = lax.dot_general(q, k, (((1,), (1,)), ((), ())),
                                     preferred_element_type=F32)[:NQ]
                sc = jnp.where(mask, sc * SCALE, fill)
                mx = jnp.max(sc, axis=-1, keepdims=True)
                e = jnp.exp(sc - mx)
                l = jnp.sum(e, axis=-1, keepdims=True)
                r = pl.reciprocal(l, approx=True)
                es[h] = (e * r).astype(BF16)
                rs[h] = jnp.broadcast_to(r[SEG:], (M, DH))

            def pv(h):
                v = jnp.concatenate(
                    [xv.pop(h), pad16(tails.pop(h)[2], rs.pop(h))], axis=0)
                o = _dot(es.pop(h), v)
                ox = [oring[h, pl.ds(opos[j], 8), :] for j in range(XR // 8)]
                last = jnp.concatenate(
                    [ox[2].astype(F32), o[SEG:SEG + M]], axis=0).astype(BF16)
                lhs_o[h] = jnp.concatenate([ox[0], ox[1], last], axis=0)
                oring[h, pl.ds(owr, SEG), :] = o[:SEG].astype(BF16)

            def wo_part(c, h0, h1):
                lo = jnp.concatenate([lhs_o[h] for h in range(h0, h1)], axis=1)
                w = pltpu.bitcast(wo32[c, pl.ds(h0 * 64, (h1 - h0) * 64), :], BF16)
                return _dot(lo, w)

            PD = 4
            for t in range(H):
                loads(t - 1, t - PD)
                proj(t)
                if t >= 1:
                    qk(t - 1)
                if t >= PD:
                    pv(t - PD)
            HA = H - 4
            acc = {}
            loads(H - 1, H - 4)
            acc[0] = wo_part(0, 0, HA)
            qk(H - 1)
            pv(H - 4)
            loads(-1, H - 3)
            acc[1] = wo_part(1, 0, HA)
            pv(H - 3)
            loads(-1, H - 2)
            acc[2] = wo_part(2, 0, HA)
            pv(H - 2)
            loads(-1, H - 1)
            for c in (3, 4):
                acc[c] = wo_part(c, 0, HA)
            pv(H - 1)
            for c in (5, 6, 7):
                acc[c] = wo_part(c, 0, HA)
            for c in range(NC):
                a = wo_part(c, HA, H) + acc[c]
                ax_s[:, pl.ds(c * 128, 128)] = a[:XR]
                mem_s[:, pl.ds(c * 128, 128)] = a[XR:]
            return carry

        lax.fori_loop(0, NSEG, step, 0)

        post_attn(ax_s[...], XR * NSEG, XR)
        done = XR * (NSEG - 1)

        def wo_bulk(r, n):
            p = r - done + (done + OOFF) % ORING
            if not isinstance(p, int):
                p = pl.multiple_of(p, 8)
            lo = jnp.concatenate(
                [oring[h, pl.ds(p, n), :] for h in range(H)], axis=1)
            a = jnp.concatenate(
                [_dot(lo, _w(wo32, c)) for c in range(NC)], axis=1)
            rr = PAD + r
            if not isinstance(rr, int):
                rr = pl.multiple_of(rr, 8)
            post_attn(a, rr, n)

        def wo_body(i, carry):
            wo_bulk(done + i * 128, 128)
            return carry

        lax.fori_loop(0, 4, wo_body, 0)
        wo_bulk(done + 512, S - done - 512)

        for cp in cp_w1 + cp_w3 + cp_w2:
            cp.wait()

        def cp_out(i):
            r = i * FB
            rb = PAD + r
            if not isinstance(i, int):
                r = pl.multiple_of(r, FB)
                rb = pl.multiple_of(rb, 8)
            return pltpu.make_async_copy(xbuf.at[pl.ds(rb, FB)],
                                         out_hbm.at[pl.ds(r, FB)],
                                         sems.at[SEM_OUT + i])

        def ffn_body(i, carry):
            r = pl.multiple_of(PAD + i * FB, 8)
            hv = hbuf[pl.ds(r, FB), :]
            act = []
            for f in range(NF):
                g = _dot(hv, _w(w132, f))
                u = _dot(hv, _w(w332, f))
                act.append((g * jax.nn.sigmoid(g) * u).astype(BF16))
            av = jnp.concatenate(act, axis=1)
            for c in range(NC):
                y = _dot(av, _w(w232, c))
                cs = pl.ds(c * 128, 128)
                x2 = xbuf[pl.ds(r, FB), cs].astype(F32) + mod_s[pl.ds(5, 1), cs] * y
                xbuf[pl.ds(r, FB), cs] = x2.astype(BF16)
            cp_out(i).start()
            return carry

        lax.fori_loop(0, S // FB, ffn_body, 0)
        for i in range(S // FB):
            cp_out(i).wait()

    pl.run_scoped(
        rest,
        pltpu.VMEM((NF, D, 128), BF16),
        pltpu.VMEM((NF, D, 128), BF16),
        pltpu.VMEM((NC, F, 128), BF16),
        pltpu.VMEM((H, ORING, DH), BF16),
    )


@functools.partial(jax.jit, static_argnames=("A_seg_len",))
def pallas_adaLN_cond__memory_aug_recurrent_mem_tr__glu_gated_swiglu__prompt_kernel(
    A_x: jax.Array,
    A_mem0: jax.Array,
    A_Wq: jax.Array,
    A_Wk: jax.Array,
    A_Wv: jax.Array,
    A_Wo: jax.Array,
    A_seg_len,
    B_x: jax.Array,
    B_w1: jax.Array,
    B_w3: jax.Array,
    B_w2: jax.Array,
    c: jax.Array,
    w_mod: jax.Array,
):
    del B_x
    assert A_seg_len == SEG
    assert A_x.shape == (1, S, D) and A_mem0.shape == (1, M, D)
    assert A_Wq.shape == (D, H, DH) and B_w1.shape == (D, F)

    n_sems = 4 + NC + NU + 48 + NF + NF + NC + S // FB
    any_spec = pl.BlockSpec(memory_space=pl.ANY)
    out = pl.pallas_call(
        _kernel,
        out_shape=jax.ShapeDtypeStruct((S, D), BF16),
        in_specs=[any_spec] * 11,
        out_specs=any_spec,
        scratch_shapes=[
            pltpu.VMEM((H, D // 2, DH), U32),
            pltpu.VMEM((H, D // 2, DH), U32),
            pltpu.VMEM((H, D // 2, DH), U32),
            pltpu.VMEM((NC, H * DH, 128), BF16),
            pltpu.VMEM((PAD + S, D), BF16),
            pltpu.VMEM((PAD + S, D), BF16),
            pltpu.VMEM((H, RING, DH), BF16),
            pltpu.VMEM((H, RING, DH), BF16),
            pltpu.VMEM((H, RING, DH), BF16),
            pltpu.VMEM((8, D), F32),
            pltpu.VMEM((M, D), F32),
            pltpu.VMEM((XR, D), F32),
            pltpu.VMEM((XR, D), F32),
            pltpu.VMEM((1, D), BF16),
            pltpu.VMEM((M, D), BF16),
            pltpu.SemaphoreType.DMA((n_sems,)),
        ],
        compiler_params=pltpu.CompilerParams(
            vmem_limit_bytes=120 * 1024 * 1024),
        name="adaln_memtr_swiglu",
    )(
        A_x.reshape(S, D),
        A_mem0.reshape(M, D),
        A_Wq, A_Wk, A_Wv,
        A_Wo.reshape(H * DH, D),
        B_w1, B_w3, B_w2, c, w_mod,
    )
    return out.reshape(1, S, D)
```

```python
import functools

import jax
import jax.numpy as jnp
from jax import lax
import jax.experimental.pallas as pl
import jax.experimental.pallas.tpu as pltpu

BF16 = jnp.bfloat16
F32 = jnp.float32
U32 = jnp.uint32

S = 2048
D = 1024
H = 32
DH = 128
F = 3584
M = 8
SEG = 32
NSEG = S // SEG
XR = 24
PRO = S - XR * NSEG
RING = 544
ORING = 576
OOFF = 256
PAD = 48
NC = D // 128
NF = F // 128
FB = 128
NU = 3 * H // 2
NU0 = 40
UPI = 6
NQ = SEG + M
EPS = 1e-5
SCALE = DH ** -0.5


def _dot(a, b):
    return jnp.dot(a, b, preferred_element_type=F32)


def _w(ref32, i):
    return pltpu.bitcast(ref32[i], BF16)


def _ln(x):
    mu = jnp.mean(x, axis=-1, keepdims=True)
    xc = x - mu
    var = jnp.mean(xc * xc, axis=-1, keepdims=True)
    return xc * lax.rsqrt(var + EPS)


def _ln_mod(x, shift, scale1):
    return _ln(x) * scale1 + shift


def _kernel(x_hbm, mem0_hbm, wq_hbm, wk_hbm, wv_hbm, wo_hbm, w1_hbm, w3_hbm,
            w2_hbm, c_hbm, wmod_hbm, out_hbm,
            wq32, wk32, wv32, wo_s, xbuf, hbuf, qring, kring, vring,
            mod_s, mem_s, ax_s, hn_s, c_s, m0_s, sems):
    wo32 = wo_s.bitcast(U32)

    SEM_X0, SEM_X1, SEM_C, SEM_M0 = 0, 1, 2, 3
    SEM_WO = 4
    SEM_ST = SEM_WO + NC
    SEM_WM = SEM_ST + NU
    SEM_W1 = SEM_WM + 48
    SEM_W3 = SEM_W1 + NF
    SEM_W2 = SEM_W3 + NF
    SEM_OUT = SEM_W2 + NC

    cp_x0 = pltpu.make_async_copy(x_hbm.at[pl.ds(0, PRO)],
                                  xbuf.at[pl.ds(PAD, PRO)], sems.at[SEM_X0])
    cp_x1 = pltpu.make_async_copy(x_hbm.at[pl.ds(PRO, S - PRO)],
                                  xbuf.at[pl.ds(PAD + PRO, S - PRO)],
                                  sems.at[SEM_X1])
    cp_c = pltpu.make_async_copy(c_hbm, c_s, sems.at[SEM_C])
    cp_m0 = pltpu.make_async_copy(mem0_hbm, m0_s, sems.at[SEM_M0])
    cp_wo = [pltpu.make_async_copy(wo_hbm.at[:, pl.ds(c * 128, 128)],
                                   wo_s.at[c], sems.at[SEM_WO + c])
             for c in range(NC)]

    def mod_row(i):
        return mod_s[pl.ds(i, 1), :]

    def prologue(st, wm_s, xn_s):
        wm32 = wm_s.bitcast(U32)
        srcs = (wq_hbm.bitcast(U32), wk_hbm.bitcast(U32), wv_hbm.bitcast(U32))
        dsts = (wq32, wk32, wv32)
        rings = (qring, kring, vring)

        def cp_st(j, s):
            return pltpu.make_async_copy(
                srcs[j].at[:, s, :], st.at[3 * s + j],
                sems.at[SEM_ST + 3 * s + j])

        def cp_wm(i):
            col = i * 128 if isinstance(i, int) else pl.multiple_of(i * 128, 128)
            return pltpu.make_async_copy(wmod_hbm.at[:, pl.ds(col, 128)],
                                         wm_s.at[i], sems.at[SEM_WM + i])

        cp_c.start()
        cp_m0.start()
        cp_x0.start()
        for i in range(16):
            cp_wm(i).start()
        for u in range(NU0):
            cp_st(u % 3, u // 3).start()

        xbuf[pl.ds(0, PAD), :] = jnp.zeros((PAD, D), BF16)
        ax_s[...] = jnp.zeros((XR, D), F32)

        cp_c.wait()
        cf = c_s[...].astype(F32)
        sc = (cf * jax.nn.sigmoid(cf)).astype(BF16)
        sc8 = jnp.broadcast_to(sc, (8, D))

        cp_x0.wait()

        def ln_body(i, carry):
            r = pl.multiple_of(i * 64, 64)
            xv = xbuf[pl.ds(pl.multiple_of(PAD + r, 8), 64), :].astype(F32)
            xn_s[pl.ds(r, 64), :] = _ln(xv)
            return carry

        lax.fori_loop(0, PRO // 64, ln_body, 0)

        def mod_part(lo, hi, chunk):
            for c0 in range(lo, hi, chunk):
                for i in range(c0, c0 + chunk):
                    cp_wm(i).wait()
                for i in range(c0, c0 + chunk):
                    k, c = divmod(i, NC)
                    part = _dot(sc8, _w(wm32, i))[0:1, :]
                    if k in (1, 4):
                        part = part + 1.0
                    mod_s[pl.ds(k, 1), pl.ds(c * 128, 128)] = part

        mod_part(0, 16, 4)

        def relayout(j, s):
            u = 3 * s + j
            for db in range(8):
                ev = st[u, pl.ds(db * 128, 64, stride=2), :]
                od = st[u, pl.ds(db * 128 + 1, 64, stride=2), :]
                rows = pl.ds(db * 64, 64)
                dsts[j][2 * s, rows, :] = (ev & U32(0xFFFF)) | (od << 16)
                dsts[j][2 * s + 1, rows, :] = (ev >> 16) | (od & U32(0xFFFF0000))

        def bulk(j, s, first=False):
            for mb in range(PRO // 128):
                rows = pl.ds(PAD + mb * 128, 128)
                if first:
                    lhs = (xn_s[pl.ds(mb * 128, 128), :] * mod_row(1)
                           + mod_row(0)).astype(BF16)
                    hbuf[rows, :] = lhs
                else:
                    lhs = hbuf[rows, :]
                for hh in range(2):
                    h = 2 * s + hh
                    rings[j][h, pl.ds(mb * 128, 128), :] = (
                        _dot(lhs, _w(dsts[j], h)).astype(BF16))

        for u in range(NU0, NU):
            cp_st(u % 3, u // 3).start()
        cp_x1.start()
        for c in range(NC):
            cp_wo[c].start()

        cp_st(0, 0).wait()
        relayout(0, 0)
        for u in range(UPI):
            cp_st((u + 1) % 3, (u + 1) // 3).wait()
            relayout((u + 1) % 3, (u + 1) // 3)
            bulk(u % 3, u // 3, first=(u == 0))

        def grp_body(it, carry):
            s0 = it * (UPI // 3)
            last = NU // UPI - 1
            sn = jnp.minimum(s0 + UPI // 3, H // 2 - 1)
            for u in range(1, UPI):
                cp_st(u % 3, s0 + u // 3).wait()

            @pl.when(it < last)
            def _():
                cp_st(0, sn).wait()

            @pl.when(it <= 4)
            def _():
                for k in range(8):
                    cp_wm(8 + 8 * it + k).start()

            for u in range(UPI):
                if u + 1 < UPI:
                    relayout((u + 1) % 3, s0 + (u + 1) // 3)
                else:
                    relayout(0, sn)
                bulk(u % 3, s0 + u // 3)
            return carry

        lax.fori_loop(1, NU // UPI, grp_body, 0)

        mod_part(16, 48, 32)
        cp_x1.wait()
        cp_m0.wait()
        mem_s[...] = m0_s[...].astype(F32)
        xv = xbuf[pl.ds(PAD + PRO, XR), :].astype(F32)
        hn_s[...] = _ln_mod(xv, mod_row(0), mod_row(1))

    pl.run_scoped(
        prologue,
        pltpu.VMEM((NU, D, DH), U32),
        pltpu.VMEM((48, D, 128), BF16),
        pltpu.VMEM((PRO, D), F32),
    )

    def rest(w1_s, w3_s, w2_s, oring):
        w132 = w1_s.bitcast(U32)
        w332 = w3_s.bitcast(U32)
        w232 = w2_s.bitcast(U32)
        q32 = qring.bitcast(U32)
        k32 = kring.bitcast(U32)
        v32 = vring.bitcast(U32)

        cp_w1 = [pltpu.make_async_copy(w1_hbm.at[:, pl.ds(f * 128, 128)],
                                       w1_s.at[f], sems.at[SEM_W1 + f])
                 for f in range(NF)]
        cp_w3 = [pltpu.make_async_copy(w3_hbm.at[:, pl.ds(f * 128, 128)],
                                       w3_s.at[f], sems.at[SEM_W3 + f])
                 for f in range(NF)]
        cp_w2 = [pltpu.make_async_copy(w2_hbm.at[:, pl.ds(c * 128, 128)],
                                       w2_s.at[c], sems.at[SEM_W2 + c])
                 for c in range(NC)]
        for cp in cp_w1 + cp_w3 + cp_w2:
            cp.start()
        for c in range(NC):
            cp_wo[c].wait()

        oring[:, pl.ds(OOFF - XR, XR), :] = jnp.zeros((H, XR, DH), BF16)

        def post_attn(a, r, n):
            x1 = xbuf[pl.ds(r, n), :].astype(F32) + mod_row(2) * a
            x1 = x1.astype(BF16)
            xbuf[pl.ds(r, n), :] = x1
            hbuf[pl.ds(r, n), :] = _ln_mod(
                x1.astype(F32), mod_row(3), mod_row(4)).astype(BF16)

        row = lax.broadcasted_iota(jnp.int32, (NQ, 48), 0)
        col = lax.broadcasted_iota(jnp.int32, (NQ, 48), 1)
        mask = (col < SEG + M) & ((row >= SEG) | (col >= SEG) | (col <= row))
        fill = jnp.where(col < SEG + M, -1e9, -jnp.inf).astype(F32)

        def step(s, carry):
            lhs = jnp.concatenate([hn_s[...], mem_s[...]], axis=0).astype(BF16)

            post_attn(ax_s[...], pl.multiple_of(XR * s, 8), XR)
            rn = pl.multiple_of(
                PAD + jnp.minimum(PRO + XR * (s + 1), S - XR), 8)
            hn_s[...] = _ln_mod(xbuf[pl.ds(rn, XR), :].astype(F32),
                                mod_row(0), mod_row(1))

            wpos = [pl.multiple_of(lax.rem(PRO + XR * s + 8 * j, RING), 8)
                    for j in range(XR // 8)]
            rpos = pl.multiple_of(lax.rem(s, RING // SEG) * (SEG // 2), 16)
            opos = [pl.multiple_of(
                lax.rem(XR * s - XR + 8 * j + OOFF, ORING), 8)
                for j in range(XR // 8)]
            owr = pl.multiple_of(lax.rem(SEG * s + OOFF, ORING), SEG)
            zpad = jnp.zeros((8, DH), F32)

            tails = {}
            xq, xk, xv = {}, {}, {}
            es, rs = {}, {}

            def pad16(a, b):
                return jnp.concatenate([a, b], axis=0).astype(BF16)

            lhs_o = {}

            def seg_rows(r32, h):
                return pltpu.bitcast(r32[h, pl.ds(rpos, SEG // 2), :], BF16)

            def loads(hq, hv):
                if 0 <= hq < H:
                    xq[hq] = seg_rows(q32, hq)
                    xk[hq] = seg_rows(k32, hq)
                if 0 <= hv < H:
                    xv[hv] = seg_rows(v32, hv)

            def proj(h):
                tl = []
                for w32, ring in ((wq32, qring), (wk32, kring), (wv32, vring)):
                    t = _dot(lhs, _w(w32, h))
                    for j in range(XR // 8):
                        ring[h, pl.ds(wpos[j], 8), :] = (
                            t[8 * j:8 * j + 8].astype(BF16))
                    tl.append(t[XR:])
                tails[h] = tl

            def qk(h):
                q = jnp.concatenate([xq.pop(h), pad16(tails[h][0], zpad)], axis=0)
                k = jnp.concatenate([xk.pop(h), pad16(tails[h][1], zpad)], axis=0)
                sc = lax.dot_general(q, k, (((1,), (1,)), ((), ())),
                                     preferred_element_type=F32)[:NQ]
                sc = jnp.where(mask, sc * SCALE, fill)
                mx = jnp.max(sc, axis=-1, keepdims=True)
                e = jnp.exp(sc - mx)
                l = jnp.sum(e, axis=-1, keepdims=True)
                r = pl.reciprocal(l, approx=True)
                es[h] = (e * r).astype(BF16)
                rs[h] = jnp.broadcast_to(r[SEG:], (M, DH))

            def pv(h):
                v = jnp.concatenate(
                    [xv.pop(h), pad16(tails.pop(h)[2], rs.pop(h))], axis=0)
                o = _dot(es.pop(h), v)
                ox = [oring[h, pl.ds(opos[j], 8), :] for j in range(XR // 8)]
                last = jnp.concatenate(
                    [ox[2].astype(F32), o[SEG:SEG + M]], axis=0).astype(BF16)
                lhs_o[h] = jnp.concatenate([ox[0], ox[1], last], axis=0)
                oring[h, pl.ds(owr, SEG), :] = o[:SEG].astype(BF16)

            def wo_part(c, h0, h1):
                lo = jnp.concatenate([lhs_o[h] for h in range(h0, h1)], axis=1)
                w = pltpu.bitcast(wo32[c, pl.ds(h0 * 64, (h1 - h0) * 64), :], BF16)
                return _dot(lo, w)

            PD = 4
            for t in range(H):
                loads(t - 1, t - PD)
                proj(t)
                if t >= 1:
                    qk(t - 1)
                if t >= PD:
                    pv(t - PD)
            HA = H - 4
            acc = {}
            loads(H - 1, H - 4)
            acc[0] = wo_part(0, 0, HA)
            qk(H - 1)
            pv(H - 4)
            loads(-1, H - 3)
            acc[1] = wo_part(1, 0, HA)
            pv(H - 3)
            loads(-1, H - 2)
            acc[2] = wo_part(2, 0, HA)
            pv(H - 2)
            loads(-1, H - 1)
            for c in (3, 4):
                acc[c] = wo_part(c, 0, HA)
            pv(H - 1)
            for c in (5, 6, 7):
                acc[c] = wo_part(c, 0, HA)
            for c in range(NC):
                a = wo_part(c, HA, H) + acc[c]
                ax_s[:, pl.ds(c * 128, 128)] = a[:XR]
                mem_s[:, pl.ds(c * 128, 128)] = a[XR:]
            return carry

        lax.fori_loop(0, NSEG, step, 0)

        post_attn(ax_s[...], XR * NSEG, XR)
        done = XR * (NSEG - 1)

        def wo_bulk(r, n):
            p = r - done + (done + OOFF) % ORING
            if not isinstance(p, int):
                p = pl.multiple_of(p, 8)
            lo = jnp.concatenate(
                [oring[h, pl.ds(p, n), :] for h in range(H)], axis=1)
            a = jnp.concatenate(
                [_dot(lo, _w(wo32, c)) for c in range(NC)], axis=1)
            rr = PAD + r
            if not isinstance(rr, int):
                rr = pl.multiple_of(rr, 8)
            post_attn(a, rr, n)

        def wo_body(i, carry):
            wo_bulk(done + i * 128, 128)
            return carry

        lax.fori_loop(0, 4, wo_body, 0)
        wo_bulk(done + 512, S - done - 512)

        for cp in cp_w1 + cp_w3 + cp_w2:
            cp.wait()

        def cp_out(i):
            r = i * FB
            rb = PAD + r
            if not isinstance(i, int):
                r = pl.multiple_of(r, FB)
                rb = pl.multiple_of(rb, 8)
            return pltpu.make_async_copy(xbuf.at[pl.ds(rb, FB)],
                                         out_hbm.at[pl.ds(r, FB)],
                                         sems.at[SEM_OUT + i])

        def ffn_body(i, carry):
            r = pl.multiple_of(PAD + i * FB, 8)
            hv = hbuf[pl.ds(r, FB), :]
            act = []
            for f in range(NF):
                g = _dot(hv, _w(w132, f))
                u = _dot(hv, _w(w332, f))
                act.append((g * jax.nn.sigmoid(g) * u).astype(BF16))
            av = jnp.concatenate(act, axis=1)
            for c in range(NC):
                y = _dot(av, _w(w232, c))
                cs = pl.ds(c * 128, 128)
                x2 = xbuf[pl.ds(r, FB), cs].astype(F32) + mod_s[pl.ds(5, 1), cs] * y
                xbuf[pl.ds(r, FB), cs] = x2.astype(BF16)
            cp_out(i).start()
            return carry

        lax.fori_loop(0, S // FB, ffn_body, 0)
        for i in range(S // FB):
            cp_out(i).wait()

    pl.run_scoped(
        rest,
        pltpu.VMEM((NF, D, 128), BF16),
        pltpu.VMEM((NF, D, 128), BF16),
        pltpu.VMEM((NC, F, 128), BF16),
        pltpu.VMEM((H, ORING, DH), BF16),
    )


@functools.partial(jax.jit, static_argnames=("A_seg_len",))
def pallas_adaLN_cond__memory_aug_recurrent_mem_tr__glu_gated_swiglu__prompt_kernel(
    A_x: jax.Array,
    A_mem0: jax.Array,
    A_Wq: jax.Array,
    A_Wk: jax.Array,
    A_Wv: jax.Array,
    A_Wo: jax.Array,
    A_seg_len,
    B_x: jax.Array,
    B_w1: jax.Array,
    B_w3: jax.Array,
    B_w2: jax.Array,
    c: jax.Array,
    w_mod: jax.Array,
):
    del B_x
    assert A_seg_len == SEG
    assert A_x.shape == (1, S, D) and A_mem0.shape == (1, M, D)
    assert A_Wq.shape == (D, H, DH) and B_w1.shape == (D, F)

    n_sems = 4 + NC + NU + 48 + NF + NF + NC + S // FB
    any_spec = pl.BlockSpec(memory_space=pl.ANY)
    out = pl.pallas_call(
        _kernel,
        out_shape=jax.ShapeDtypeStruct((S, D), BF16),
        in_specs=[any_spec] * 11,
        out_specs=any_spec,
        scratch_shapes=[
            pltpu.VMEM((H, D // 2, DH), U32),
            pltpu.VMEM((H, D // 2, DH), U32),
            pltpu.VMEM((H, D // 2, DH), U32),
            pltpu.VMEM((NC, H * DH, 128), BF16),
            pltpu.VMEM((PAD + S, D), BF16),
            pltpu.VMEM((PAD + S, D), BF16),
            pltpu.VMEM((H, RING, DH), BF16),
            pltpu.VMEM((H, RING, DH), BF16),
            pltpu.VMEM((H, RING, DH), BF16),
            pltpu.VMEM((8, D), F32),
            pltpu.VMEM((M, D), F32),
            pltpu.VMEM((XR, D), F32),
            pltpu.VMEM((XR, D), F32),
            pltpu.VMEM((1, D), BF16),
            pltpu.VMEM((M, D), BF16),
            pltpu.SemaphoreType.DMA((n_sems,)),
        ],
        compiler_params=pltpu.CompilerParams(
            vmem_limit_bytes=120 * 1024 * 1024),
        name="adaln_memtr_swiglu",
    )(
        A_x.reshape(S, D),
        A_mem0.reshape(M, D),
        A_Wq, A_Wk, A_Wv,
        A_Wo.reshape(H * DH, D),
        B_w1, B_w3, B_w2, c, w_mod,
    )
    return out.reshape(1, S, D)
```

```python
import functools

import jax
import jax.numpy as jnp
from jax import lax
import jax.experimental.pallas as pl
import jax.experimental.pallas.tpu as pltpu

BF16 = jnp.bfloat16
F32 = jnp.float32
U32 = jnp.uint32

S = 2048
D = 1024
H = 32
DH = 128
F = 3584
M = 8
SEG = 32
NSEG = S // SEG
XR = 24
PRO = S - XR * NSEG
RING = 544
ORING = 576
OOFF = 256
PAD = 48
NC = D // 128
NF = F // 128
FB = 128
NU = 3 * H // 2
NU0 = 40
UPI = 6
NP = 2 * (SEG + M)
EPS = 1e-5
SCALE = DH ** -0.5


def _dot(a, b):
    return jnp.dot(a, b, preferred_element_type=F32)


def _w(ref32, i):
    return pltpu.bitcast(ref32[i], BF16)


def _ln(x):
    mu = jnp.mean(x, axis=-1, keepdims=True)
    xc = x - mu
    var = jnp.mean(xc * xc, axis=-1, keepdims=True)
    return xc * lax.rsqrt(var + EPS)


def _ln_mod(x, shift, scale1):
    return _ln(x) * scale1 + shift


def _kernel(x_hbm, mem0_hbm, wq_hbm, wk_hbm, wv_hbm, wo_hbm, w1_hbm, w3_hbm,
            w2_hbm, c_hbm, wmod_hbm, out_hbm,
            wq32, wk32, wv32, wo_s, xbuf, hbuf, qring, kring, vring,
            mod_s, mem_s, ax_s, hn_s, c_s, m0_s, sems):
    wo32 = wo_s.bitcast(U32)

    SEM_X0, SEM_X1, SEM_C, SEM_M0 = 0, 1, 2, 3
    SEM_WO = 4
    SEM_ST = SEM_WO + NC
    SEM_WM = SEM_ST + NU
    SEM_W1 = SEM_WM + 48
    SEM_W3 = SEM_W1 + NF
    SEM_W2 = SEM_W3 + NF
    SEM_OUT = SEM_W2 + NC

    cp_x0 = pltpu.make_async_copy(x_hbm.at[pl.ds(0, PRO)],
                                  xbuf.at[pl.ds(PAD, PRO)], sems.at[SEM_X0])
    cp_x1 = pltpu.make_async_copy(x_hbm.at[pl.ds(PRO, S - PRO)],
                                  xbuf.at[pl.ds(PAD + PRO, S - PRO)],
                                  sems.at[SEM_X1])
    cp_c = pltpu.make_async_copy(c_hbm, c_s, sems.at[SEM_C])
    cp_m0 = pltpu.make_async_copy(mem0_hbm, m0_s, sems.at[SEM_M0])
    cp_wo = [pltpu.make_async_copy(wo_hbm.at[:, pl.ds(c * 128, 128)],
                                   wo_s.at[c], sems.at[SEM_WO + c])
             for c in range(NC)]

    def mod_row(i):
        return mod_s[pl.ds(i, 1), :]

    def prologue(st, wm_s, xn_s):
        wm32 = wm_s.bitcast(U32)
        srcs = (wq_hbm.bitcast(U32), wk_hbm.bitcast(U32), wv_hbm.bitcast(U32))
        dsts = (wq32, wk32, wv32)
        rings = (qring, kring, vring)

        def cp_st(j, s):
            return pltpu.make_async_copy(
                srcs[j].at[:, s, :], st.at[3 * s + j],
                sems.at[SEM_ST + 3 * s + j])

        def cp_wm(i):
            col = i * 128 if isinstance(i, int) else pl.multiple_of(i * 128, 128)
            return pltpu.make_async_copy(wmod_hbm.at[:, pl.ds(col, 128)],
                                         wm_s.at[i], sems.at[SEM_WM + i])

        cp_c.start()
        cp_m0.start()
        cp_x0.start()
        for i in range(16):
            cp_wm(i).start()
        for u in range(NU0):
            cp_st(u % 3, u // 3).start()

        xbuf[pl.ds(0, PAD), :] = jnp.zeros((PAD, D), BF16)
        ax_s[...] = jnp.zeros((XR, D), F32)

        cp_c.wait()
        cf = c_s[...].astype(F32)
        sc = (cf * jax.nn.sigmoid(cf)).astype(BF16)
        sc8 = jnp.broadcast_to(sc, (8, D))

        cp_x0.wait()

        def ln_body(i, carry):
            r = pl.multiple_of(i * 64, 64)
            xv = xbuf[pl.ds(pl.multiple_of(PAD + r, 8), 64), :].astype(F32)
            xn_s[pl.ds(r, 64), :] = _ln(xv)
            return carry

        lax.fori_loop(0, PRO // 64, ln_body, 0)

        def mod_part(lo, hi, chunk):
            for c0 in range(lo, hi, chunk):
                for i in range(c0, c0 + chunk):
                    cp_wm(i).wait()
                for i in range(c0, c0 + chunk):
                    k, c = divmod(i, NC)
                    part = _dot(sc8, _w(wm32, i))[0:1, :]
                    if k in (1, 4):
                        part = part + 1.0
                    mod_s[pl.ds(k, 1), pl.ds(c * 128, 128)] = part

        mod_part(0, 16, 4)

        def relayout(j, s):
            u = 3 * s + j
            for db in range(8):
                ev = st[u, pl.ds(db * 128, 64, stride=2), :]
                od = st[u, pl.ds(db * 128 + 1, 64, stride=2), :]
                rows = pl.ds(db * 64, 64)
                dsts[j][2 * s, rows, :] = (ev & U32(0xFFFF)) | (od << 16)
                dsts[j][2 * s + 1, rows, :] = (ev >> 16) | (od & U32(0xFFFF0000))

        def bulk(j, s, first=False):
            for mb in range(PRO // 128):
                rows = pl.ds(PAD + mb * 128, 128)
                if first:
                    lhs = (xn_s[pl.ds(mb * 128, 128), :] * mod_row(1)
                           + mod_row(0)).astype(BF16)
                    hbuf[rows, :] = lhs
                else:
                    lhs = hbuf[rows, :]
                for hh in range(2):
                    h = 2 * s + hh
                    rings[j][h, pl.ds(mb * 128, 128), :] = (
                        _dot(lhs, _w(dsts[j], h)).astype(BF16))

        for u in range(NU0, NU):
            cp_st(u % 3, u // 3).start()
        cp_x1.start()
        for c in range(NC):
            cp_wo[c].start()

        cp_st(0, 0).wait()
        relayout(0, 0)
        for u in range(UPI):
            cp_st((u + 1) % 3, (u + 1) // 3).wait()
            relayout((u + 1) % 3, (u + 1) // 3)
            bulk(u % 3, u // 3, first=(u == 0))

        def grp_body(it, carry):
            s0 = it * (UPI // 3)
            last = NU // UPI - 1
            sn = jnp.minimum(s0 + UPI // 3, H // 2 - 1)
            for u in range(1, UPI):
                cp_st(u % 3, s0 + u // 3).wait()

            @pl.when(it < last)
            def _():
                cp_st(0, sn).wait()

            @pl.when(it <= 4)
            def _():
                for k in range(8):
                    cp_wm(8 + 8 * it + k).start()

            for u in range(UPI):
                if u + 1 < UPI:
                    relayout((u + 1) % 3, s0 + (u + 1) // 3)
                else:
                    relayout(0, sn)
                bulk(u % 3, s0 + u // 3)
            return carry

        lax.fori_loop(1, NU // UPI, grp_body, 0)

        mod_part(16, 48, 32)
        cp_x1.wait()
        cp_m0.wait()
        mem_s[...] = m0_s[...].astype(F32)
        xv = xbuf[pl.ds(PAD + PRO, XR), :].astype(F32)
        hn_s[...] = _ln_mod(xv, mod_row(0), mod_row(1))

    pl.run_scoped(
        prologue,
        pltpu.VMEM((NU, D, DH), U32),
        pltpu.VMEM((48, D, 128), BF16),
        pltpu.VMEM((PRO, D), F32),
    )

    def rest(w1_s, w3_s, w2_s, oring):
        w132 = w1_s.bitcast(U32)
        w332 = w3_s.bitcast(U32)
        w232 = w2_s.bitcast(U32)
        q32 = qring.bitcast(U32)
        k32 = kring.bitcast(U32)
        v32 = vring.bitcast(U32)

        cp_w1 = [pltpu.make_async_copy(w1_hbm.at[:, pl.ds(f * 128, 128)],
                                       w1_s.at[f], sems.at[SEM_W1 + f])
                 for f in range(NF)]
        cp_w3 = [pltpu.make_async_copy(w3_hbm.at[:, pl.ds(f * 128, 128)],
                                       w3_s.at[f], sems.at[SEM_W3 + f])
                 for f in range(NF)]
        cp_w2 = [pltpu.make_async_copy(w2_hbm.at[:, pl.ds(c * 128, 128)],
                                       w2_s.at[c], sems.at[SEM_W2 + c])
                 for c in range(NC)]
        for cp in cp_w1 + cp_w3 + cp_w2:
            cp.start()
        for c in range(NC):
            cp_wo[c].wait()

        oring[:, pl.ds(OOFF - XR, XR), :] = jnp.zeros((H, XR, DH), BF16)

        def post_attn(a, r, n):
            x1 = xbuf[pl.ds(r, n), :].astype(F32) + mod_row(2) * a
            x1 = x1.astype(BF16)
            xbuf[pl.ds(r, n), :] = x1
            hbuf[pl.ds(r, n), :] = _ln_mod(
                x1.astype(F32), mod_row(3), mod_row(4)).astype(BF16)

        row = lax.broadcasted_iota(jnp.int32, (NP, NP), 0)
        col = lax.broadcasted_iota(jnp.int32, (NP, NP), 1)

        def second(i):
            return ((i >= SEG) & (i < 2 * SEG)) | (i >= 2 * SEG + M)

        same = second(row) == second(col)
        mask = same & ((row >= 2 * SEG) | (col >= 2 * SEG) | (col <= row))
        fill = jnp.where(same, -1e9, -jnp.inf).astype(F32)

        def step(s, carry):
            lhs = jnp.concatenate([hn_s[...], mem_s[...]], axis=0).astype(BF16)

            post_attn(ax_s[...], pl.multiple_of(XR * s, 8), XR)
            rn = pl.multiple_of(
                PAD + jnp.minimum(PRO + XR * (s + 1), S - XR), 8)
            hn_s[...] = _ln_mod(xbuf[pl.ds(rn, XR), :].astype(F32),
                                mod_row(0), mod_row(1))

            wpos = [pl.multiple_of(lax.rem(PRO + XR * s + 8 * j, RING), 8)
                    for j in range(XR // 8)]
            rpos = pl.multiple_of(lax.rem(s, RING // SEG) * (SEG // 2), 16)
            opos = [pl.multiple_of(
                lax.rem(XR * s - XR + 8 * j + OOFF, ORING), 8)
                for j in range(XR // 8)]
            owr = pl.multiple_of(lax.rem(SEG * s + OOFF, ORING), SEG)

            tails = {}
            xs = {}
            ps = {}
            lhs_o = {}

            def load(j, p):
                r32 = (q32, k32, v32)[j]
                xs[j, p] = [
                    pltpu.bitcast(r32[h, pl.ds(rpos, SEG // 2), :], BF16)
                    for h in (2 * p, 2 * p + 1)]

            def operand(j, p):
                tail = jnp.concatenate(
                    [tails.pop((j, 2 * p)), tails.pop((j, 2 * p + 1))], axis=0)
                return jnp.concatenate(
                    xs.pop((j, p)) + [tail.astype(BF16)], axis=0)

            def proj(h):
                for j, (w32, ring) in enumerate(
                        ((wq32, qring), (wk32, kring), (wv32, vring))):
                    t = _dot(lhs, _w(w32, h))
                    for i in range(XR // 8):
                        ring[h, pl.ds(wpos[i], 8), :] = (
                            t[8 * i:8 * i + 8].astype(BF16))
                    tails[j, h] = t[XR:]

            def qk(p):
                sc = lax.dot_general(operand(0, p), operand(1, p),
                                     (((1,), (1,)), ((), ())),
                                     preferred_element_type=F32)
                sc = jnp.where(mask, sc * SCALE, fill)
                mx = jnp.max(sc, axis=-1, keepdims=True)
                e = jnp.exp(sc - mx)
                l = jnp.sum(e, axis=-1, keepdims=True)
                ps[p] = (e * pl.reciprocal(l, approx=True)).astype(BF16)

            def pv(p):
                o = _dot(ps.pop(p), operand(2, p))
                for i, h in enumerate((2 * p, 2 * p + 1)):
                    ox = [oring[h, pl.ds(opos[k], 8), :] for k in range(XR // 8)]
                    om = o[2 * SEG + M * i:2 * SEG + M * (i + 1)]
                    last = jnp.concatenate(
                        [ox[2].astype(F32), om], axis=0).astype(BF16)
                    lhs_o[h] = jnp.concatenate([ox[0], ox[1], last], axis=0)
                for i, h in enumerate((2 * p, 2 * p + 1)):
                    oring[h, pl.ds(owr, SEG), :] = (
                        o[SEG * i:SEG * (i + 1)].astype(BF16))

            def wo_part(c, h0, h1):
                lo = jnp.concatenate([lhs_o[h] for h in range(h0, h1)], axis=1)
                w = pltpu.bitcast(wo32[c, pl.ds(h0 * 64, (h1 - h0) * 64), :], BF16)
                return _dot(lo, w)

            NPR = H // 2
            for t in range(NPR):
                if t >= 1:
                    load(0, t - 1)
                    load(1, t - 1)
                proj(2 * t)
                if t >= 1:
                    qk(t - 1)
                if t >= 2:
                    load(2, t - 2)
                proj(2 * t + 1)
                if t >= 2:
                    pv(t - 2)
            HA = H - 4
            acc = {}
            load(0, NPR - 1)
            load(1, NPR - 1)
            load(2, NPR - 2)
            acc[0] = wo_part(0, 0, HA)
            qk(NPR - 1)
            acc[1] = wo_part(1, 0, HA)
            pv(NPR - 2)
            load(2, NPR - 1)
            for c in (2, 3, 4):
                acc[c] = wo_part(c, 0, HA)
            pv(NPR - 1)
            for c in (5, 6, 7):
                acc[c] = wo_part(c, 0, HA)
            for c in range(NC):
                a = wo_part(c, HA, H) + acc[c]
                ax_s[:, pl.ds(c * 128, 128)] = a[:XR]
                mem_s[:, pl.ds(c * 128, 128)] = a[XR:]
            return carry

        lax.fori_loop(0, NSEG, step, 0)

        post_attn(ax_s[...], XR * NSEG, XR)
        done = XR * (NSEG - 1)

        def wo_bulk(r, n):
            p = r - done + (done + OOFF) % ORING
            if not isinstance(p, int):
                p = pl.multiple_of(p, 8)
            lo = jnp.concatenate(
                [oring[h, pl.ds(p, n), :] for h in range(H)], axis=1)
            a = jnp.concatenate(
                [_dot(lo, _w(wo32, c)) for c in range(NC)], axis=1)
            rr = PAD + r
            if not isinstance(rr, int):
                rr = pl.multiple_of(rr, 8)
            post_attn(a, rr, n)

        def wo_body(i, carry):
            wo_bulk(done + i * 128, 128)
            return carry

        lax.fori_loop(0, 4, wo_body, 0)
        wo_bulk(done + 512, S - done - 512)

        for cp in cp_w1 + cp_w3 + cp_w2:
            cp.wait()

        def cp_out(i):
            r = i * FB
            rb = PAD + r
            if not isinstance(i, int):
                r = pl.multiple_of(r, FB)
                rb = pl.multiple_of(rb, 8)
            return pltpu.make_async_copy(xbuf.at[pl.ds(rb, FB)],
                                         out_hbm.at[pl.ds(r, FB)],
                                         sems.at[SEM_OUT + i])

        def ffn_body(i, carry):
            r = pl.multiple_of(PAD + i * FB, 8)
            hv = hbuf[pl.ds(r, FB), :]
            act = []
            for f in range(NF):
                g = _dot(hv, _w(w132, f))
                u = _dot(hv, _w(w332, f))
                act.append((g * jax.nn.sigmoid(g) * u).astype(BF16))
            av = jnp.concatenate(act, axis=1)
            for c in range(NC):
                y = _dot(av, _w(w232, c))
                cs = pl.ds(c * 128, 128)
                x2 = xbuf[pl.ds(r, FB), cs].astype(F32) + mod_s[pl.ds(5, 1), cs] * y
                xbuf[pl.ds(r, FB), cs] = x2.astype(BF16)
            cp_out(i).start()
            return carry

        lax.fori_loop(0, S // FB, ffn_body, 0)
        for i in range(S // FB):
            cp_out(i).wait()

    pl.run_scoped(
        rest,
        pltpu.VMEM((NF, D, 128), BF16),
        pltpu.VMEM((NF, D, 128), BF16),
        pltpu.VMEM((NC, F, 128), BF16),
        pltpu.VMEM((H, ORING, DH), BF16),
    )


@functools.partial(jax.jit, static_argnames=("A_seg_len",))
def pallas_adaLN_cond__memory_aug_recurrent_mem_tr__glu_gated_swiglu__prompt_kernel(
    A_x: jax.Array,
    A_mem0: jax.Array,
    A_Wq: jax.Array,
    A_Wk: jax.Array,
    A_Wv: jax.Array,
    A_Wo: jax.Array,
    A_seg_len,
    B_x: jax.Array,
    B_w1: jax.Array,
    B_w3: jax.Array,
    B_w2: jax.Array,
    c: jax.Array,
    w_mod: jax.Array,
):
    del B_x
    assert A_seg_len == SEG
    assert A_x.shape == (1, S, D) and A_mem0.shape == (1, M, D)
    assert A_Wq.shape == (D, H, DH) and B_w1.shape == (D, F)

    n_sems = 4 + NC + NU + 48 + NF + NF + NC + S // FB
    any_spec = pl.BlockSpec(memory_space=pl.ANY)
    out = pl.pallas_call(
        _kernel,
        out_shape=jax.ShapeDtypeStruct((S, D), BF16),
        in_specs=[any_spec] * 11,
        out_specs=any_spec,
        scratch_shapes=[
            pltpu.VMEM((H, D // 2, DH), U32),
            pltpu.VMEM((H, D // 2, DH), U32),
            pltpu.VMEM((H, D // 2, DH), U32),
            pltpu.VMEM((NC, H * DH, 128), BF16),
            pltpu.VMEM((PAD + S, D), BF16),
            pltpu.VMEM((PAD + S, D), BF16),
            pltpu.VMEM((H, RING, DH), BF16),
            pltpu.VMEM((H, RING, DH), BF16),
            pltpu.VMEM((H, RING, DH), BF16),
            pltpu.VMEM((8, D), F32),
            pltpu.VMEM((M, D), F32),
            pltpu.VMEM((XR, D), F32),
            pltpu.VMEM((XR, D), F32),
            pltpu.VMEM((1, D), BF16),
            pltpu.VMEM((M, D), BF16),
            pltpu.SemaphoreType.DMA((n_sems,)),
        ],
        compiler_params=pltpu.CompilerParams(
            vmem_limit_bytes=120 * 1024 * 1024),
        name="adaln_memtr_swiglu",
    )(
        A_x.reshape(S, D),
        A_mem0.reshape(M, D),
        A_Wq, A_Wk, A_Wv,
        A_Wo.reshape(H * DH, D),
        B_w1, B_w3, B_w2, c, w_mod,
    )
    return out.reshape(1, S, D)
```

```python
import functools

import jax
import jax.numpy as jnp
from jax import lax
import jax.experimental.pallas as pl
import jax.experimental.pallas.tpu as pltpu

BF16 = jnp.bfloat16
F32 = jnp.float32
U32 = jnp.uint32

S = 2048
D = 1024
H = 32
DH = 128
F = 3584
M = 8
SEG = 32
NSEG = S // SEG
XR = 24
PRO = S - XR * NSEG
RING = 544
ORING = 576
OOFF = 256
PAD = 48
NC = D // 128
NF = F // 128
FB = 128
NU = 3 * H // 2
NU0 = 40
UPI = 6
NP = 2 * (SEG + M)
EPS = 1e-5
SCALE = DH ** -0.5


def _dot(a, b):
    return jnp.dot(a, b, preferred_element_type=F32)


def _w(ref32, i):
    return pltpu.bitcast(ref32[i], BF16)


def _wrap(i, n):
    return jnp.where(i >= n, i - n, i)


def _ln(x):
    mu = jnp.mean(x, axis=-1, keepdims=True)
    xc = x - mu
    var = jnp.mean(xc * xc, axis=-1, keepdims=True)
    return xc * lax.rsqrt(var + EPS)


def _ln_mod(x, shift, scale1):
    return _ln(x) * scale1 + shift


def _kernel(x_hbm, mem0_hbm, wq_hbm, wk_hbm, wv_hbm, wo_hbm, w1_hbm, w3_hbm,
            w2_hbm, c_hbm, wmod_hbm, out_hbm,
            wq32, wk32, wv32, wo_s, xbuf, hbuf, qring, kring, vring,
            mod_s, mem_s, ax_s, hn_s, c_s, m0_s, sems):
    wo32 = wo_s.bitcast(U32)

    SEM_X0, SEM_X1, SEM_C, SEM_M0 = 0, 1, 2, 3
    SEM_WO = 4
    SEM_ST = SEM_WO + NC
    SEM_WM = SEM_ST + NU
    SEM_W1 = SEM_WM + 48
    SEM_W3 = SEM_W1 + NF
    SEM_W2 = SEM_W3 + NF
    SEM_OUT = SEM_W2 + NC

    cp_x0 = pltpu.make_async_copy(x_hbm.at[pl.ds(0, PRO)],
                                  xbuf.at[pl.ds(PAD, PRO)], sems.at[SEM_X0])
    cp_x1 = pltpu.make_async_copy(x_hbm.at[pl.ds(PRO, S - PRO)],
                                  xbuf.at[pl.ds(PAD + PRO, S - PRO)],
                                  sems.at[SEM_X1])
    cp_c = pltpu.make_async_copy(c_hbm, c_s, sems.at[SEM_C])
    cp_m0 = pltpu.make_async_copy(mem0_hbm, m0_s, sems.at[SEM_M0])
    cp_wo = [pltpu.make_async_copy(wo_hbm.at[:, pl.ds(c * 128, 128)],
                                   wo_s.at[c], sems.at[SEM_WO + c])
             for c in range(NC)]

    def mod_row(i):
        return mod_s[pl.ds(i, 1), :]

    def prologue(st, wm_s, xn_s):
        wm32 = wm_s.bitcast(U32)
        srcs = (wq_hbm.bitcast(U32), wk_hbm.bitcast(U32), wv_hbm.bitcast(U32))
        dsts = (wq32, wk32, wv32)
        rings = (qring, kring, vring)

        def cp_st(j, s):
            return pltpu.make_async_copy(
                srcs[j].at[:, s, :], st.at[3 * s + j],
                sems.at[SEM_ST + 3 * s + j])

        def cp_wm(i):
            col = i * 128 if isinstance(i, int) else pl.multiple_of(i * 128, 128)
            return pltpu.make_async_copy(wmod_hbm.at[:, pl.ds(col, 128)],
                                         wm_s.at[i], sems.at[SEM_WM + i])

        cp_c.start()
        cp_m0.start()
        cp_x0.start()
        for i in range(16):
            cp_wm(i).start()
        for u in range(NU0):
            cp_st(u % 3, u // 3).start()

        xbuf[pl.ds(0, PAD), :] = jnp.zeros((PAD, D), BF16)
        ax_s[...] = jnp.zeros((XR, D), F32)

        cp_c.wait()
        cf = c_s[...].astype(F32)
        sc = (cf * jax.nn.sigmoid(cf)).astype(BF16)
        sc8 = jnp.broadcast_to(sc, (8, D))

        cp_x0.wait()

        def ln_body(i, carry):
            r = pl.multiple_of(i * 64, 64)
            xv = xbuf[pl.ds(pl.multiple_of(PAD + r, 8), 64), :].astype(F32)
            xn_s[pl.ds(r, 64), :] = _ln(xv)
            return carry

        lax.fori_loop(0, PRO // 64, ln_body, 0)

        def mod_part(lo, hi, chunk):
            for c0 in range(lo, hi, chunk):
                for i in range(c0, c0 + chunk):
                    cp_wm(i).wait()
                for i in range(c0, c0 + chunk):
                    k, c = divmod(i, NC)
                    part = _dot(sc8, _w(wm32, i))[0:1, :]
                    if k in (1, 4):
                        part = part + 1.0
                    mod_s[pl.ds(k, 1), pl.ds(c * 128, 128)] = part

        mod_part(0, 16, 4)

        def relayout(j, s):
            u = 3 * s + j
            for db in range(8):
                ev = st[u, pl.ds(db * 128, 64, stride=2), :]
                od = st[u, pl.ds(db * 128 + 1, 64, stride=2), :]
                rows = pl.ds(db * 64, 64)
                dsts[j][2 * s, rows, :] = (ev & U32(0xFFFF)) | (od << 16)
                dsts[j][2 * s + 1, rows, :] = (ev >> 16) | (od & U32(0xFFFF0000))

        def bulk(j, s, first=False):
            for mb in range(PRO // 128):
                rows = pl.ds(PAD + mb * 128, 128)
                if first:
                    lhs = (xn_s[pl.ds(mb * 128, 128), :] * mod_row(1)
                           + mod_row(0)).astype(BF16)
                    hbuf[rows, :] = lhs
                else:
                    lhs = hbuf[rows, :]
                for hh in range(2):
                    h = 2 * s + hh
                    rings[j][h, pl.ds(mb * 128, 128), :] = (
                        _dot(lhs, _w(dsts[j], h)).astype(BF16))

        for u in range(NU0, NU):
            cp_st(u % 3, u // 3).start()
        cp_x1.start()
        for c in range(NC):
            cp_wo[c].start()

        cp_st(0, 0).wait()
        relayout(0, 0)
        for u in range(UPI):
            cp_st((u + 1) % 3, (u + 1) // 3).wait()
            relayout((u + 1) % 3, (u + 1) // 3)
            bulk(u % 3, u // 3, first=(u == 0))

        def grp_body(it, carry):
            s0 = it * (UPI // 3)
            last = NU // UPI - 1
            sn = jnp.minimum(s0 + UPI // 3, H // 2 - 1)
            for u in range(1, UPI):
                cp_st(u % 3, s0 + u // 3).wait()

            @pl.when(it < last)
            def _():
                cp_st(0, sn).wait()

            @pl.when(it <= 4)
            def _():
                for k in range(8):
                    cp_wm(8 + 8 * it + k).start()

            for u in range(UPI):
                if u + 1 < UPI:
                    relayout((u + 1) % 3, s0 + (u + 1) // 3)
                else:
                    relayout(0, sn)
                bulk(u % 3, s0 + u // 3)
            return carry

        lax.fori_loop(1, NU // UPI, grp_body, 0)

        mod_part(16, 48, 32)
        cp_x1.wait()
        cp_m0.wait()
        mem_s[...] = m0_s[...].astype(F32)
        xv = xbuf[pl.ds(PAD + PRO, XR), :].astype(F32)
        hn_s[...] = _ln_mod(xv, mod_row(0), mod_row(1))

    pl.run_scoped(
        prologue,
        pltpu.VMEM((NU, D, DH), U32),
        pltpu.VMEM((48, D, 128), BF16),
        pltpu.VMEM((PRO, D), F32),
    )

    def rest(w1_s, w3_s, w2_s, oring):
        w132 = w1_s.bitcast(U32)
        w332 = w3_s.bitcast(U32)
        w232 = w2_s.bitcast(U32)
        q32 = qring.bitcast(U32)
        k32 = kring.bitcast(U32)
        v32 = vring.bitcast(U32)

        cp_w1 = [pltpu.make_async_copy(w1_hbm.at[:, pl.ds(f * 128, 128)],
                                       w1_s.at[f], sems.at[SEM_W1 + f])
                 for f in range(NF)]
        cp_w3 = [pltpu.make_async_copy(w3_hbm.at[:, pl.ds(f * 128, 128)],
                                       w3_s.at[f], sems.at[SEM_W3 + f])
                 for f in range(NF)]
        cp_w2 = [pltpu.make_async_copy(w2_hbm.at[:, pl.ds(c * 128, 128)],
                                       w2_s.at[c], sems.at[SEM_W2 + c])
                 for c in range(NC)]
        for cp in cp_w1 + cp_w3 + cp_w2:
            cp.start()
        for c in range(NC):
            cp_wo[c].wait()

        oring[:, pl.ds(OOFF - XR, XR), :] = jnp.zeros((H, XR, DH), BF16)

        def post_attn(a, r, n):
            x1 = xbuf[pl.ds(r, n), :].astype(F32) + mod_row(2) * a
            x1 = x1.astype(BF16)
            xbuf[pl.ds(r, n), :] = x1
            hbuf[pl.ds(r, n), :] = _ln_mod(
                x1.astype(F32), mod_row(3), mod_row(4)).astype(BF16)

        row = lax.broadcasted_iota(jnp.int32, (NP, NP), 0)
        col = lax.broadcasted_iota(jnp.int32, (NP, NP), 1)

        def second(i):
            return ((i >= SEG) & (i < 2 * SEG)) | (i >= 2 * SEG + M)

        same = second(row) == second(col)
        mask = same & ((row >= 2 * SEG) | (col >= 2 * SEG) | (col <= row))
        fill = jnp.where(same, -1e9, -jnp.inf).astype(F32)

        def step(s, carry):
            lhs = jnp.concatenate([hn_s[...], mem_s[...]], axis=0).astype(BF16)

            post_attn(ax_s[...], pl.multiple_of(XR * s, 8), XR)
            rn = pl.multiple_of(
                PAD + jnp.minimum(PRO + XR * (s + 1), S - XR), 8)
            hn_s[...] = _ln_mod(xbuf[pl.ds(rn, XR), :].astype(F32),
                                mod_row(0), mod_row(1))

            wp, rp, op, ow = carry
            wpos = [pl.multiple_of(_wrap(wp + 8 * j, RING), 8)
                    for j in range(XR // 8)]
            rpos = pl.multiple_of(rp, SEG // 2)
            opos = [pl.multiple_of(_wrap(op + 8 * j, ORING), 8)
                    for j in range(XR // 8)]
            owr = pl.multiple_of(ow, SEG)

            tails = {}
            xs = {}
            ps = {}
            lhs_o = {}

            def load(j, p):
                r32 = (q32, k32, v32)[j]
                xs[j, p] = [
                    pltpu.bitcast(r32[h, pl.ds(rpos, SEG // 2), :], BF16)
                    for h in (2 * p, 2 * p + 1)]

            def operand(j, p):
                tail = jnp.concatenate(
                    [tails.pop((j, 2 * p)), tails.pop((j, 2 * p + 1))], axis=0)
                return jnp.concatenate(
                    xs.pop((j, p)) + [tail.astype(BF16)], axis=0)

            def proj(h):
                for j, (w32, ring) in enumerate(
                        ((wq32, qring), (wk32, kring), (wv32, vring))):
                    t = _dot(lhs, _w(w32, h))
                    for i in range(XR // 8):
                        ring[h, pl.ds(wpos[i], 8), :] = (
                            t[8 * i:8 * i + 8].astype(BF16))
                    tails[j, h] = t[XR:]

            def qk(p):
                sc = lax.dot_general(operand(0, p), operand(1, p),
                                     (((1,), (1,)), ((), ())),
                                     preferred_element_type=F32)
                sc = jnp.where(mask, sc * SCALE, fill)
                mx = jnp.max(sc, axis=-1, keepdims=True)
                e = jnp.exp(sc - mx)
                l = jnp.sum(e, axis=-1, keepdims=True)
                ps[p] = (e * pl.reciprocal(l, approx=True)).astype(BF16)

            def pv(p):
                o = _dot(ps.pop(p), operand(2, p))
                for i, h in enumerate((2 * p, 2 * p + 1)):
                    ox = [oring[h, pl.ds(opos[k], 8), :] for k in range(XR // 8)]
                    om = o[2 * SEG + M * i:2 * SEG + M * (i + 1)]
                    last = jnp.concatenate(
                        [ox[2].astype(F32), om], axis=0).astype(BF16)
                    lhs_o[h] = jnp.concatenate([ox[0], ox[1], last], axis=0)
                for i, h in enumerate((2 * p, 2 * p + 1)):
                    oring[h, pl.ds(owr, SEG), :] = (
                        o[SEG * i:SEG * (i + 1)].astype(BF16))

            def wo_part(c, h0, h1):
                lo = jnp.concatenate([lhs_o[h] for h in range(h0, h1)], axis=1)
                w = pltpu.bitcast(wo32[c, pl.ds(h0 * 64, (h1 - h0) * 64), :], BF16)
                return _dot(lo, w)

            NPR = H // 2
            for t in range(NPR):
                if t >= 1:
                    load(0, t - 1)
                    load(1, t - 1)
                proj(2 * t)
                if t >= 1:
                    qk(t - 1)
                if t >= 2:
                    load(2, t - 2)
                proj(2 * t + 1)
                if t >= 2:
                    pv(t - 2)
            HA = H - 4
            acc = {}
            load(0, NPR - 1)
            load(1, NPR - 1)
            load(2, NPR - 2)
            acc[0] = wo_part(0, 0, HA)
            qk(NPR - 1)
            acc[1] = wo_part(1, 0, HA)
            pv(NPR - 2)
            load(2, NPR - 1)
            for c in (2, 3, 4):
                acc[c] = wo_part(c, 0, HA)
            pv(NPR - 1)
            for c in (5, 6, 7):
                acc[c] = wo_part(c, 0, HA)
            for c in range(NC):
                a = wo_part(c, HA, H) + acc[c]
                ax_s[:, pl.ds(c * 128, 128)] = a[:XR]
                mem_s[:, pl.ds(c * 128, 128)] = a[XR:]
            return (_wrap(wp + XR, RING), _wrap(rp + SEG // 2, RING // 2),
                    _wrap(op + XR, ORING), _wrap(ow + SEG, ORING))

        lax.fori_loop(0, NSEG, step,
                      (jnp.int32(PRO), jnp.int32(0), jnp.int32(OOFF - XR),
                       jnp.int32(OOFF)))

        post_attn(ax_s[...], XR * NSEG, XR)
        done = XR * (NSEG - 1)

        def wo_bulk(r, n):
            p = r - done + (done + OOFF) % ORING
            if not isinstance(p, int):
                p = pl.multiple_of(p, 8)
            lo = jnp.concatenate(
                [oring[h, pl.ds(p, n), :] for h in range(H)], axis=1)
            a = jnp.concatenate(
                [_dot(lo, _w(wo32, c)) for c in range(NC)], axis=1)
            rr = PAD + r
            if not isinstance(rr, int):
                rr = pl.multiple_of(rr, 8)
            post_attn(a, rr, n)

        def wo_body(i, carry):
            wo_bulk(done + i * 128, 128)
            return carry

        lax.fori_loop(0, 4, wo_body, 0)
        wo_bulk(done + 512, S - done - 512)

        for cp in cp_w1 + cp_w3 + cp_w2:
            cp.wait()

        def cp_out(i):
            r = i * FB
            rb = PAD + r
            if not isinstance(i, int):
                r = pl.multiple_of(r, FB)
                rb = pl.multiple_of(rb, 8)
            return pltpu.make_async_copy(xbuf.at[pl.ds(rb, FB)],
                                         out_hbm.at[pl.ds(r, FB)],
                                         sems.at[SEM_OUT + i])

        def ffn_body(i, carry):
            r = pl.multiple_of(PAD + i * FB, 8)
            hv = hbuf[pl.ds(r, FB), :]
            act = []
            for f in range(NF):
                g = _dot(hv, _w(w132, f))
                u = _dot(hv, _w(w332, f))
                act.append((g * jax.nn.sigmoid(g) * u).astype(BF16))
            av = jnp.concatenate(act, axis=1)
            for c in range(NC):
                y = _dot(av, _w(w232, c))
                cs = pl.ds(c * 128, 128)
                x2 = xbuf[pl.ds(r, FB), cs].astype(F32) + mod_s[pl.ds(5, 1), cs] * y
                xbuf[pl.ds(r, FB), cs] = x2.astype(BF16)
            cp_out(i).start()
            return carry

        lax.fori_loop(0, S // FB, ffn_body, 0)
        for i in range(S // FB):
            cp_out(i).wait()

    pl.run_scoped(
        rest,
        pltpu.VMEM((NF, D, 128), BF16),
        pltpu.VMEM((NF, D, 128), BF16),
        pltpu.VMEM((NC, F, 128), BF16),
        pltpu.VMEM((H, ORING, DH), BF16),
    )


@functools.partial(jax.jit, static_argnames=("A_seg_len",))
def pallas_adaLN_cond__memory_aug_recurrent_mem_tr__glu_gated_swiglu__prompt_kernel(
    A_x: jax.Array,
    A_mem0: jax.Array,
    A_Wq: jax.Array,
    A_Wk: jax.Array,
    A_Wv: jax.Array,
    A_Wo: jax.Array,
    A_seg_len,
    B_x: jax.Array,
    B_w1: jax.Array,
    B_w3: jax.Array,
    B_w2: jax.Array,
    c: jax.Array,
    w_mod: jax.Array,
):
    del B_x
    assert A_seg_len == SEG
    assert A_x.shape == (1, S, D) and A_mem0.shape == (1, M, D)
    assert A_Wq.shape == (D, H, DH) and B_w1.shape == (D, F)

    n_sems = 4 + NC + NU + 48 + NF + NF + NC + S // FB
    any_spec = pl.BlockSpec(memory_space=pl.ANY)
    out = pl.pallas_call(
        _kernel,
        out_shape=jax.ShapeDtypeStruct((S, D), BF16),
        in_specs=[any_spec] * 11,
        out_specs=any_spec,
        scratch_shapes=[
            pltpu.VMEM((H, D // 2, DH), U32),
            pltpu.VMEM((H, D // 2, DH), U32),
            pltpu.VMEM((H, D // 2, DH), U32),
            pltpu.VMEM((NC, H * DH, 128), BF16),
            pltpu.VMEM((PAD + S, D), BF16),
            pltpu.VMEM((PAD + S, D), BF16),
            pltpu.VMEM((H, RING, DH), BF16),
            pltpu.VMEM((H, RING, DH), BF16),
            pltpu.VMEM((H, RING, DH), BF16),
            pltpu.VMEM((8, D), F32),
            pltpu.VMEM((M, D), F32),
            pltpu.VMEM((XR, D), F32),
            pltpu.VMEM((XR, D), F32),
            pltpu.VMEM((1, D), BF16),
            pltpu.VMEM((M, D), BF16),
            pltpu.SemaphoreType.DMA((n_sems,)),
        ],
        compiler_params=pltpu.CompilerParams(
            vmem_limit_bytes=120 * 1024 * 1024),
        name="adaln_memtr_swiglu",
    )(
        A_x.reshape(S, D),
        A_mem0.reshape(M, D),
        A_Wq, A_Wk, A_Wv,
        A_Wo.reshape(H * DH, D),
        B_w1, B_w3, B_w2, c, w_mod,
    )
    return out.reshape(1, S, D)
```

```python
import functools

import jax
import jax.numpy as jnp
from jax import lax
import jax.experimental.pallas as pl
import jax.experimental.pallas.tpu as pltpu

BF16 = jnp.bfloat16
F32 = jnp.float32
U32 = jnp.uint32

S = 2048
D = 1024
H = 32
DH = 128
F = 3584
M = 8
SEG = 32
NSEG = S // SEG
XR = 24
PRO = S - XR * NSEG
RING = 544
ORING = 576
OOFF = 256
PAD = 48
NC = D // 128
NF = F // 128
FB = 128
UNROLL = 4
NU = 3 * H // 2
NU0 = 40
UPI = 6
NP = 2 * (SEG + M)
EPS = 1e-5
SCALE = DH ** -0.5


def _dot(a, b):
    return jnp.dot(a, b, preferred_element_type=F32)


def _w(ref32, i):
    return pltpu.bitcast(ref32[i], BF16)


def _wrap(i, n):
    return jnp.where(i >= n, i - n, i)


def _ln(x):
    mu = jnp.mean(x, axis=-1, keepdims=True)
    xc = x - mu
    var = jnp.mean(xc * xc, axis=-1, keepdims=True)
    return xc * lax.rsqrt(var + EPS)


def _ln_mod(x, shift, scale1):
    return _ln(x) * scale1 + shift


def _kernel(x_hbm, mem0_hbm, wq_hbm, wk_hbm, wv_hbm, wo_hbm, w1_hbm, w3_hbm,
            w2_hbm, c_hbm, wmod_hbm, out_hbm,
            wq32, wk32, wv32, wo_s, xh, qring, kring, vring,
            mod_s, mem_s, ax_s, hn_s, c_s, m0_s, sems):
    wo32 = wo_s.bitcast(U32)
    xbuf = xh.at[0]
    hbuf = xh.at[1]

    SEM_X0, SEM_X1, SEM_C, SEM_M0 = 0, 1, 2, 3
    SEM_WO = 4
    SEM_ST = SEM_WO + NC
    SEM_WM = SEM_ST + NU
    SEM_W1 = SEM_WM + 48
    SEM_W3 = SEM_W1 + NF
    SEM_W2 = SEM_W3 + NF
    SEM_OUT = SEM_W2 + NC

    cp_x0 = pltpu.make_async_copy(x_hbm.at[pl.ds(0, PRO)],
                                  xbuf.at[pl.ds(PAD, PRO)], sems.at[SEM_X0])
    cp_x1 = pltpu.make_async_copy(x_hbm.at[pl.ds(PRO, S - PRO)],
                                  xbuf.at[pl.ds(PAD + PRO, S - PRO)],
                                  sems.at[SEM_X1])
    cp_c = pltpu.make_async_copy(c_hbm, c_s, sems.at[SEM_C])
    cp_m0 = pltpu.make_async_copy(mem0_hbm, m0_s, sems.at[SEM_M0])
    cp_wo = [pltpu.make_async_copy(wo_hbm.at[:, pl.ds(c * 128, 128)],
                                   wo_s.at[c], sems.at[SEM_WO + c])
             for c in range(NC)]

    def mod_row(i):
        return mod_s[pl.ds(i, 1), :]

    def prologue(st, wm_s, xn_s):
        wm32 = wm_s.bitcast(U32)
        srcs = (wq_hbm.bitcast(U32), wk_hbm.bitcast(U32), wv_hbm.bitcast(U32))
        dsts = (wq32, wk32, wv32)
        rings = (qring, kring, vring)

        def cp_st(j, s):
            return pltpu.make_async_copy(
                srcs[j].at[:, s, :], st.at[3 * s + j],
                sems.at[SEM_ST + 3 * s + j])

        def cp_wm(i):
            col = i * 128 if isinstance(i, int) else pl.multiple_of(i * 128, 128)
            return pltpu.make_async_copy(wmod_hbm.at[:, pl.ds(col, 128)],
                                         wm_s.at[i], sems.at[SEM_WM + i])

        cp_c.start()
        cp_m0.start()
        cp_x0.start()
        for i in range(16):
            cp_wm(i).start()
        for u in range(NU0):
            cp_st(u % 3, u // 3).start()

        xbuf[pl.ds(0, PAD), :] = jnp.zeros((PAD, D), BF16)
        ax_s[...] = jnp.zeros((XR, D), F32)

        cp_c.wait()
        cf = c_s[...].astype(F32)
        sc = (cf * jax.nn.sigmoid(cf)).astype(BF16)
        sc8 = jnp.broadcast_to(sc, (8, D))

        cp_x0.wait()

        def ln_body(i, carry):
            r = pl.multiple_of(i * 64, 64)
            xv = xbuf[pl.ds(pl.multiple_of(PAD + r, 8), 64), :].astype(F32)
            xn_s[pl.ds(r, 64), :] = _ln(xv)
            return carry

        lax.fori_loop(0, PRO // 64, ln_body, 0)

        def mod_part(lo, hi, chunk):
            for c0 in range(lo, hi, chunk):
                for i in range(c0, c0 + chunk):
                    cp_wm(i).wait()
                for i in range(c0, c0 + chunk):
                    k, c = divmod(i, NC)
                    part = _dot(sc8, _w(wm32, i))[0:1, :]
                    if k in (1, 4):
                        part = part + 1.0
                    mod_s[pl.ds(k, 1), pl.ds(c * 128, 128)] = part

        mod_part(0, 16, 4)

        def relayout(j, s):
            u = 3 * s + j
            for db in range(8):
                ev = st[u, pl.ds(db * 128, 64, stride=2), :]
                od = st[u, pl.ds(db * 128 + 1, 64, stride=2), :]
                rows = pl.ds(db * 64, 64)
                dsts[j][2 * s, rows, :] = (ev & U32(0xFFFF)) | (od << 16)
                dsts[j][2 * s + 1, rows, :] = (ev >> 16) | (od & U32(0xFFFF0000))

        def bulk(j, s, first=False):
            for mb in range(PRO // 128):
                rows = pl.ds(PAD + mb * 128, 128)
                if first:
                    lhs = (xn_s[pl.ds(mb * 128, 128), :] * mod_row(1)
                           + mod_row(0)).astype(BF16)
                    hbuf[rows, :] = lhs
                else:
                    lhs = hbuf[rows, :]
                for hh in range(2):
                    h = 2 * s + hh
                    rings[j][h, pl.ds(mb * 128, 128), :] = (
                        _dot(lhs, _w(dsts[j], h)).astype(BF16))

        for u in range(NU0, NU):
            cp_st(u % 3, u // 3).start()
        cp_x1.start()
        for c in range(NC):
            cp_wo[c].start()

        cp_st(0, 0).wait()
        relayout(0, 0)
        for u in range(UPI):
            cp_st((u + 1) % 3, (u + 1) // 3).wait()
            relayout((u + 1) % 3, (u + 1) // 3)
            bulk(u % 3, u // 3, first=(u == 0))

        def grp_body(it, carry):
            s0 = it * (UPI // 3)
            last = NU // UPI - 1
            sn = jnp.minimum(s0 + UPI // 3, H // 2 - 1)
            for u in range(1, UPI):
                cp_st(u % 3, s0 + u // 3).wait()

            @pl.when(it < last)
            def _():
                cp_st(0, sn).wait()

            @pl.when(it <= 4)
            def _():
                for k in range(8):
                    cp_wm(8 + 8 * it + k).start()

            for u in range(UPI):
                if u + 1 < UPI:
                    relayout((u + 1) % 3, s0 + (u + 1) // 3)
                else:
                    relayout(0, sn)
                bulk(u % 3, s0 + u // 3)
            return carry

        lax.fori_loop(1, NU // UPI, grp_body, 0)

        mod_part(16, 48, 32)
        cp_x1.wait()
        cp_m0.wait()
        mem_s[...] = m0_s[...].astype(F32)
        xv = xbuf[pl.ds(PAD + PRO, XR), :].astype(F32)
        hn_s[...] = _ln_mod(xv, mod_row(0), mod_row(1))

    pl.run_scoped(
        prologue,
        pltpu.VMEM((NU, D, DH), U32),
        pltpu.VMEM((48, D, 128), BF16),
        pltpu.VMEM((PRO, D), F32),
    )

    def rest(w1_s, w3_s, w2_s, oring):
        w132 = w1_s.bitcast(U32)
        w332 = w3_s.bitcast(U32)
        w232 = w2_s.bitcast(U32)
        q32 = qring.bitcast(U32)
        k32 = kring.bitcast(U32)
        v32 = vring.bitcast(U32)

        cp_w1 = [pltpu.make_async_copy(w1_hbm.at[:, pl.ds(f * 128, 128)],
                                       w1_s.at[f], sems.at[SEM_W1 + f])
                 for f in range(NF)]
        cp_w3 = [pltpu.make_async_copy(w3_hbm.at[:, pl.ds(f * 128, 128)],
                                       w3_s.at[f], sems.at[SEM_W3 + f])
                 for f in range(NF)]
        cp_w2 = [pltpu.make_async_copy(w2_hbm.at[:, pl.ds(c * 128, 128)],
                                       w2_s.at[c], sems.at[SEM_W2 + c])
                 for c in range(NC)]
        for cp in cp_w1 + cp_w3 + cp_w2:
            cp.start()
        for c in range(NC):
            cp_wo[c].wait()

        oring[:, pl.ds(OOFF - XR, XR), :] = jnp.zeros((H, XR, DH), BF16)

        def post_attn(a, r, n):
            x1 = xbuf[pl.ds(r, n), :].astype(F32) + mod_row(2) * a
            x1 = x1.astype(BF16)
            xbuf[pl.ds(r, n), :] = x1
            hbuf[pl.ds(r, n), :] = _ln_mod(
                x1.astype(F32), mod_row(3), mod_row(4)).astype(BF16)

        row = lax.broadcasted_iota(jnp.int32, (NP, NP), 0)
        col = lax.broadcasted_iota(jnp.int32, (NP, NP), 1)

        def second(i):
            return ((i >= SEG) & (i < 2 * SEG)) | (i >= 2 * SEG + M)

        same = second(row) == second(col)
        mask = same & ((row >= 2 * SEG) | (col >= 2 * SEG) | (col <= row))
        fill = jnp.where(same, -1e9, -jnp.inf).astype(F32)

        def step(s, carry, mem, split):
            lhs_c = [jnp.concatenate([hn_s[:, pl.ds(c * 128, 128)], mem[c]],
                                     axis=0).astype(BF16) for c in range(NC)]
            lhs = jnp.concatenate(lhs_c, axis=1)

            post_attn(ax_s[...], pl.multiple_of(XR * s, 8), XR)
            rn = pl.multiple_of(
                PAD + jnp.minimum(PRO + XR * (s + 1), S - XR), 8)
            hn_s[...] = _ln_mod(xbuf[pl.ds(rn, XR), :].astype(F32),
                                mod_row(0), mod_row(1))

            wp, rp, op, ow = carry
            wpos = [pl.multiple_of(_wrap(wp + 8 * j, RING), 8)
                    for j in range(XR // 8)]
            rpos = pl.multiple_of(rp, SEG // 2)
            opos = [pl.multiple_of(_wrap(op + 8 * j, ORING), 8)
                    for j in range(XR // 8)]
            owr = pl.multiple_of(ow, SEG)

            tails = {}
            xs = {}
            ps = {}
            lhs_o = {}

            def load(j, p):
                r32 = (q32, k32, v32)[j]
                xs[j, p] = [
                    pltpu.bitcast(r32[h, pl.ds(rpos, SEG // 2), :], BF16)
                    for h in (2 * p, 2 * p + 1)]

            def operand(j, p):
                tail = jnp.concatenate(
                    [tails.pop((j, 2 * p)), tails.pop((j, 2 * p + 1))], axis=0)
                return jnp.concatenate(
                    xs.pop((j, p)) + [tail.astype(BF16)], axis=0)

            low = {}
            if split:
                lhs_lo = jnp.concatenate(lhs_c[:NC // 2], axis=1)
                lhs_hi = jnp.concatenate(lhs_c[NC // 2:], axis=1)
                for h in range(2):
                    for j, w32 in enumerate((wq32, wk32, wv32)):
                        low[j, h] = _dot(lhs_lo, pltpu.bitcast(
                            w32[h, pl.ds(0, D // 4), :], BF16))

            def proj(h):
                for j, (w32, ring) in enumerate(
                        ((wq32, qring), (wk32, kring), (wv32, vring))):
                    if (j, h) in low:
                        t = _dot(lhs_hi, pltpu.bitcast(
                            w32[h, pl.ds(D // 4, D // 4), :], BF16)) + low[j, h]
                    else:
                        t = _dot(lhs, _w(w32, h))
                    for i in range(XR // 8):
                        ring[h, pl.ds(wpos[i], 8), :] = (
                            t[8 * i:8 * i + 8].astype(BF16))
                    tails[j, h] = t[XR:]

            def qk(p):
                sc = lax.dot_general(operand(0, p), operand(1, p),
                                     (((1,), (1,)), ((), ())),
                                     preferred_element_type=F32)
                sc = jnp.where(mask, sc * SCALE, fill)
                mx = jnp.max(sc, axis=-1, keepdims=True)
                e = jnp.exp(sc - mx)
                l = jnp.sum(e, axis=-1, keepdims=True)
                ps[p] = (e * pl.reciprocal(l, approx=True)).astype(BF16)

            def pv(p):
                o = _dot(ps.pop(p), operand(2, p))
                for i, h in enumerate((2 * p, 2 * p + 1)):
                    ox = [oring[h, pl.ds(opos[k], 8), :] for k in range(XR // 8)]
                    om = o[2 * SEG + M * i:2 * SEG + M * (i + 1)]
                    last = jnp.concatenate(
                        [ox[2].astype(F32), om], axis=0).astype(BF16)
                    lhs_o[h] = jnp.concatenate([ox[0], ox[1], last], axis=0)
                for i, h in enumerate((2 * p, 2 * p + 1)):
                    oring[h, pl.ds(owr, SEG), :] = (
                        o[SEG * i:SEG * (i + 1)].astype(BF16))

            def wo_part(c, h0, h1):
                lo = jnp.concatenate([lhs_o[h] for h in range(h0, h1)], axis=1)
                w = pltpu.bitcast(wo32[c, pl.ds(h0 * 64, (h1 - h0) * 64), :], BF16)
                return _dot(lo, w)

            NPR = H // 2
            for t in range(NPR):
                if t >= 1:
                    load(0, t - 1)
                    load(1, t - 1)
                proj(2 * t)
                if t >= 1:
                    qk(t - 1)
                if t >= 2:
                    load(2, t - 2)
                proj(2 * t + 1)
                if t >= 2:
                    pv(t - 2)
            HA = H - 4
            acc = {}
            load(0, NPR - 1)
            load(1, NPR - 1)
            load(2, NPR - 2)
            acc[0] = wo_part(0, 0, HA)
            qk(NPR - 1)
            acc[1] = wo_part(1, 0, HA)
            pv(NPR - 2)
            load(2, NPR - 1)
            for c in (2, 3, 4):
                acc[c] = wo_part(c, 0, HA)
            pv(NPR - 1)
            for c in (5, 6, 7):
                acc[c] = wo_part(c, 0, HA)
            mem_new = []
            for c in range(NC):
                a = wo_part(c, HA, H) + acc[c]
                ax_s[:, pl.ds(c * 128, 128)] = a[:XR]
                mem_new.append(a[XR:])
            return (_wrap(wp + XR, RING), _wrap(rp + SEG // 2, RING // 2),
                    _wrap(op + XR, ORING), _wrap(ow + SEG, ORING)), mem_new

        def steps(i, carry):
            mem = [mem_s[:, pl.ds(c * 128, 128)] for c in range(NC)]
            for u in range(UNROLL):
                carry, mem = step(i * UNROLL + u, carry, mem, split=u > 0)
            for c in range(NC):
                mem_s[:, pl.ds(c * 128, 128)] = mem[c]
            return carry

        lax.fori_loop(0, NSEG // UNROLL, steps,
                      (jnp.int32(PRO), jnp.int32(0), jnp.int32(OOFF - XR),
                       jnp.int32(OOFF)))

        post_attn(ax_s[...], XR * NSEG, XR)
        done = XR * (NSEG - 1)

        def wo_bulk(r, n):
            p = r - done + (done + OOFF) % ORING
            if not isinstance(p, int):
                p = pl.multiple_of(p, 8)
            lo = jnp.concatenate(
                [oring[h, pl.ds(p, n), :] for h in range(H)], axis=1)
            a = jnp.concatenate(
                [_dot(lo, _w(wo32, c)) for c in range(NC)], axis=1)
            rr = PAD + r
            if not isinstance(rr, int):
                rr = pl.multiple_of(rr, 8)
            post_attn(a, rr, n)

        def wo_body(i, carry):
            wo_bulk(done + i * 128, 128)
            return carry

        lax.fori_loop(0, 4, wo_body, 0)
        wo_bulk(done + 512, S - done - 512)

        for cp in cp_w1 + cp_w3 + cp_w2:
            cp.wait()

        def cp_out(i):
            r = i * FB
            rb = PAD + r
            if not isinstance(i, int):
                r = pl.multiple_of(r, FB)
                rb = pl.multiple_of(rb, 8)
            return pltpu.make_async_copy(xbuf.at[pl.ds(rb, FB)],
                                         out_hbm.at[pl.ds(r, FB)],
                                         sems.at[SEM_OUT + i])

        def ffn_body(i, carry):
            r = pl.multiple_of(PAD + i * FB, 8)
            hv = hbuf[pl.ds(r, FB), :]
            act = []
            for f in range(NF):
                g = _dot(hv, _w(w132, f))
                u = _dot(hv, _w(w332, f))
                act.append((g * jax.nn.sigmoid(g) * u).astype(BF16))
            av = jnp.concatenate(act, axis=1)
            for c in range(NC):
                y = _dot(av, _w(w232, c))
                cs = pl.ds(c * 128, 128)
                x2 = xbuf[pl.ds(r, FB), cs].astype(F32) + mod_s[pl.ds(5, 1), cs] * y
                xbuf[pl.ds(r, FB), cs] = x2.astype(BF16)
            cp_out(i).start()
            return carry

        lax.fori_loop(0, S // FB, ffn_body, 0)
        for i in range(S // FB):
            cp_out(i).wait()

    pl.run_scoped(
        rest,
        pltpu.VMEM((NF, D, 128), BF16),
        pltpu.VMEM((NF, D, 128), BF16),
        pltpu.VMEM((NC, F, 128), BF16),
        pltpu.VMEM((H, ORING, DH), BF16),
    )


@functools.partial(jax.jit, static_argnames=("A_seg_len",))
def pallas_adaLN_cond__memory_aug_recurrent_mem_tr__glu_gated_swiglu__prompt_kernel(
    A_x: jax.Array,
    A_mem0: jax.Array,
    A_Wq: jax.Array,
    A_Wk: jax.Array,
    A_Wv: jax.Array,
    A_Wo: jax.Array,
    A_seg_len,
    B_x: jax.Array,
    B_w1: jax.Array,
    B_w3: jax.Array,
    B_w2: jax.Array,
    c: jax.Array,
    w_mod: jax.Array,
):
    del B_x
    assert A_seg_len == SEG
    assert A_x.shape == (1, S, D) and A_mem0.shape == (1, M, D)
    assert A_Wq.shape == (D, H, DH) and B_w1.shape == (D, F)

    n_sems = 4 + NC + NU + 48 + NF + NF + NC + S // FB
    any_spec = pl.BlockSpec(memory_space=pl.ANY)
    out = pl.pallas_call(
        _kernel,
        out_shape=jax.ShapeDtypeStruct((S, D), BF16),
        in_specs=[any_spec] * 11,
        out_specs=any_spec,
        scratch_shapes=[
            pltpu.VMEM((H, D // 2, DH), U32),
            pltpu.VMEM((H, D // 2, DH), U32),
            pltpu.VMEM((H, D // 2, DH), U32),
            pltpu.VMEM((NC, H * DH, 128), BF16),
            pltpu.VMEM((2, PAD + S, D), BF16),
            pltpu.VMEM((H, RING, DH), BF16),
            pltpu.VMEM((H, RING, DH), BF16),
            pltpu.VMEM((H, RING, DH), BF16),
            pltpu.VMEM((8, D), F32),
            pltpu.VMEM((M, D), F32),
            pltpu.VMEM((XR, D), F32),
            pltpu.VMEM((XR, D), F32),
            pltpu.VMEM((1, D), BF16),
            pltpu.VMEM((M, D), BF16),
            pltpu.SemaphoreType.DMA((n_sems,)),
        ],
        compiler_params=pltpu.CompilerParams(
            vmem_limit_bytes=120 * 1024 * 1024),
        name="adaln_memtr_swiglu",
    )(
        A_x.reshape(S, D),
        A_mem0.reshape(M, D),
        A_Wq, A_Wk, A_Wv,
        A_Wo.reshape(H * DH, D),
        B_w1, B_w3, B_w2, c, w_mod,
    )
    return out.reshape(1, S, D)
```

```python
import functools

import jax
import jax.numpy as jnp
from jax import lax
import jax.experimental.pallas as pl
import jax.experimental.pallas.tpu as pltpu

BF16 = jnp.bfloat16
F32 = jnp.float32
U32 = jnp.uint32

S = 2048
D = 1024
H = 32
DH = 128
F = 3584
M = 8
SEG = 32
NSEG = S // SEG
XR = 24
PRO = S - XR * NSEG
RING = 544
ORING = 576
OOFF = 256
PAD = 48
NC = D // 128
NF = F // 128
FB = 128
UNROLL = 4
NU = 3 * H // 2
NU0 = 40
UPI = 6
NP = 2 * (SEG + M)
EPS = 1e-5
SEM_FIRST, SEM_LATE, SEM_WM2, SEM_FFN, SEM_OUT = 0, 1, 2, 3, 4
SEM_WM1 = 5
SEM_U0 = SEM_WM1 + 4
SEM_IT = SEM_U0 + 5 - 1
NSEMS = SEM_IT + NU // UPI
U0_GROUP = (0, 1, 2, 3, 3, 4, 4)
SCALE = DH ** -0.5


def _dot(a, b):
    return jnp.dot(a, b, preferred_element_type=F32)


def _w(ref32, i):
    return pltpu.bitcast(ref32[i], BF16)


def _wrap(i, n):
    return jnp.where(i >= n, i - n, i)


def _ln(x):
    mu = jnp.mean(x, axis=-1, keepdims=True)
    xc = x - mu
    var = jnp.mean(xc * xc, axis=-1, keepdims=True)
    return xc * lax.rsqrt(var + EPS)


def _ln_mod(x, shift, scale1):
    return _ln(x) * scale1 + shift


def _kernel(x_hbm, mem0_hbm, wq_hbm, wk_hbm, wv_hbm, wo_hbm, w1_hbm, w3_hbm,
            w2_hbm, c_hbm, wmod_hbm, out_hbm,
            wq32, wk32, wv32, wo_s, xh, qring, kring, vring,
            mod_s, mem_s, ax_s, hn_s, c_s, m0_s, sems):
    wo32 = wo_s.bitcast(U32)
    xbuf = xh.at[0]
    hbuf = xh.at[1]

    cp_x0 = pltpu.make_async_copy(x_hbm.at[pl.ds(0, PRO)],
                                  xbuf.at[pl.ds(PAD, PRO)], sems.at[SEM_FIRST])
    cp_c = pltpu.make_async_copy(c_hbm, c_s, sems.at[SEM_FIRST])
    cp_late = [
        pltpu.make_async_copy(mem0_hbm, m0_s, sems.at[SEM_LATE]),
        pltpu.make_async_copy(x_hbm.at[pl.ds(PRO, S - PRO)],
                              xbuf.at[pl.ds(PAD + PRO, S - PRO)],
                              sems.at[SEM_LATE]),
    ] + [pltpu.make_async_copy(wo_hbm.at[:, pl.ds(c * 128, 128)],
                               wo_s.at[c], sems.at[SEM_LATE])
         for c in range(NC)]

    def mod_row(i):
        return mod_s[pl.ds(i, 1), :]

    def prologue(st, wm_s, xn_s):
        wm32 = wm_s.bitcast(U32)
        srcs = (wq_hbm.bitcast(U32), wk_hbm.bitcast(U32), wv_hbm.bitcast(U32))
        dsts = (wq32, wk32, wv32)
        rings = (qring, kring, vring)

        def cp_st(j, s, sem):
            return pltpu.make_async_copy(srcs[j].at[:, s, :], st.at[3 * s + j],
                                         sems.at[sem])

        def cp_unit(u):
            sem = (SEM_U0 + U0_GROUP[u] if u <= UPI
                   else SEM_IT + (u - 1) // UPI)
            return cp_st(u % 3, u // 3, sem)

        def cp_wm(i):
            if isinstance(i, int):
                col = i * 128
                sem = SEM_WM1 + i // 4 if i < 16 else SEM_WM2
            else:
                col = pl.multiple_of(i * 128, 128)
                sem = SEM_WM2
            return pltpu.make_async_copy(wmod_hbm.at[:, pl.ds(col, 128)],
                                         wm_s.at[i], sems.at[sem])

        cp_c.start()
        cp_x0.start()
        for i in range(16):
            cp_wm(i).start()
        for u in range(NU0):
            cp_unit(u).start()

        xbuf[pl.ds(0, PAD), :] = jnp.zeros((PAD, D), BF16)
        ax_s[...] = jnp.zeros((XR, D), F32)

        cp_c.wait()
        cp_x0.wait()
        cf = c_s[...].astype(F32)
        sc = (cf * jax.nn.sigmoid(cf)).astype(BF16)
        sc8 = jnp.broadcast_to(sc, (8, D))

        def ln_body(i, carry):
            r = pl.multiple_of(i * 64, 64)
            xv = xbuf[pl.ds(pl.multiple_of(PAD + r, 8), 64), :].astype(F32)
            xn_s[pl.ds(r, 64), :] = _ln(xv)
            return carry

        lax.fori_loop(0, PRO // 64, ln_body, 0)

        def mod_part(lo, hi, chunk):
            for c0 in range(lo, hi, chunk):
                for i in range(c0, c0 + chunk):
                    cp_wm(i).wait()
                for i in range(c0, c0 + chunk):
                    k, c = divmod(i, NC)
                    part = _dot(sc8, _w(wm32, i))[0:1, :]
                    if k in (1, 4):
                        part = part + 1.0
                    mod_s[pl.ds(k, 1), pl.ds(c * 128, 128)] = part

        mod_part(0, 16, 4)

        def relayout(j, s):
            u = 3 * s + j
            for db in range(8):
                ev = st[u, pl.ds(db * 128, 64, stride=2), :]
                od = st[u, pl.ds(db * 128 + 1, 64, stride=2), :]
                rows = pl.ds(db * 64, 64)
                dsts[j][2 * s, rows, :] = (ev & U32(0xFFFF)) | (od << 16)
                dsts[j][2 * s + 1, rows, :] = (ev >> 16) | (od & U32(0xFFFF0000))

        def bulk(j, s, first=False, mbs=range(PRO // 128)):
            for mb in mbs:
                rows = pl.ds(PAD + mb * 128, 128)
                if first:
                    lhs = (xn_s[pl.ds(mb * 128, 128), :] * mod_row(1)
                           + mod_row(0)).astype(BF16)
                    hbuf[rows, :] = lhs
                else:
                    lhs = hbuf[rows, :]
                for hh in range(2):
                    h = 2 * s + hh
                    rings[j][h, pl.ds(mb * 128, 128), :] = (
                        _dot(lhs, _w(dsts[j], h)).astype(BF16))

        for u in range(NU0, NU):
            cp_unit(u).start()
        for cp in cp_late:
            cp.start()

        cp_unit(0).wait()
        relayout(0, 0)
        bulk(0, 0, first=True, mbs=(0, 1))
        for u in range(UPI):
            if U0_GROUP[u + 1] != U0_GROUP[u]:
                for v in range(u + 1, UPI + 1):
                    if U0_GROUP[v] == U0_GROUP[u + 1]:
                        cp_unit(v).wait()
            relayout((u + 1) % 3, (u + 1) // 3)
            if u == 0:
                bulk(0, 0, first=True, mbs=(2, 3))
            else:
                bulk(u % 3, u // 3)
        for i in range(16, 20):
            cp_wm(i).start()

        def grp_body(it, carry):
            s0 = it * (UPI // 3)
            last = NU // UPI - 1
            sn = jnp.minimum(s0 + UPI // 3, H // 2 - 1)
            for u in range(1, UPI):
                cp_st(u % 3, s0 + u // 3, SEM_IT + it).wait()

            @pl.when(it < last)
            def _():
                cp_st(0, sn, SEM_IT + it).wait()

            for k in range(4):
                cp_wm(16 + 4 * it + k).start()

            for u in range(UPI):
                if u + 1 < UPI:
                    relayout((u + 1) % 3, s0 + (u + 1) // 3)
                else:
                    relayout(0, sn)
                bulk(u % 3, s0 + u // 3)
            return carry

        lax.fori_loop(1, NU // UPI, grp_body, 0)

        mod_part(16, 48, 32)
        for cp in cp_late:
            cp.wait()
        mem_s[...] = m0_s[...].astype(F32)
        xv = xbuf[pl.ds(PAD + PRO, XR), :].astype(F32)
        hn_s[...] = _ln_mod(xv, mod_row(0), mod_row(1))

    pl.run_scoped(
        prologue,
        pltpu.VMEM((NU, D, DH), U32),
        pltpu.VMEM((48, D, 128), BF16),
        pltpu.VMEM((PRO, D), F32),
    )

    def rest(w1_s, w3_s, w2_s, oring):
        w132 = w1_s.bitcast(U32)
        w332 = w3_s.bitcast(U32)
        w232 = w2_s.bitcast(U32)
        q32 = qring.bitcast(U32)
        k32 = kring.bitcast(U32)
        v32 = vring.bitcast(U32)

        cp_w1 = [pltpu.make_async_copy(w1_hbm.at[:, pl.ds(f * 128, 128)],
                                       w1_s.at[f], sems.at[SEM_FFN])
                 for f in range(NF)]
        cp_w3 = [pltpu.make_async_copy(w3_hbm.at[:, pl.ds(f * 128, 128)],
                                       w3_s.at[f], sems.at[SEM_FFN])
                 for f in range(NF)]
        cp_w2 = [pltpu.make_async_copy(w2_hbm.at[:, pl.ds(c * 128, 128)],
                                       w2_s.at[c], sems.at[SEM_FFN])
                 for c in range(NC)]
        for cp in cp_w1 + cp_w3 + cp_w2:
            cp.start()

        oring[:, pl.ds(OOFF - XR, XR), :] = jnp.zeros((H, XR, DH), BF16)

        def post_attn(a, r, n):
            x1 = xbuf[pl.ds(r, n), :].astype(F32) + mod_row(2) * a
            x1 = x1.astype(BF16)
            xbuf[pl.ds(r, n), :] = x1
            hbuf[pl.ds(r, n), :] = _ln_mod(
                x1.astype(F32), mod_row(3), mod_row(4)).astype(BF16)

        row = lax.broadcasted_iota(jnp.int32, (NP, NP), 0)
        col = lax.broadcasted_iota(jnp.int32, (NP, NP), 1)

        def second(i):
            return ((i >= SEG) & (i < 2 * SEG)) | (i >= 2 * SEG + M)

        same = second(row) == second(col)
        mask = same & ((row >= 2 * SEG) | (col >= 2 * SEG) | (col <= row))
        fill = jnp.where(same, -1e9, -jnp.inf).astype(F32)

        def step(s, carry, mem, split):
            lhs_c = [jnp.concatenate([hn_s[:, pl.ds(c * 128, 128)], mem[c]],
                                     axis=0).astype(BF16) for c in range(NC)]
            lhs = jnp.concatenate(lhs_c, axis=1)

            post_attn(ax_s[...], pl.multiple_of(XR * s, 8), XR)
            rn = pl.multiple_of(
                PAD + jnp.minimum(PRO + XR * (s + 1), S - XR), 8)
            hn_s[...] = _ln_mod(xbuf[pl.ds(rn, XR), :].astype(F32),
                                mod_row(0), mod_row(1))

            wp, rp, op, ow = carry
            wpos = [pl.multiple_of(_wrap(wp + 8 * j, RING), 8)
                    for j in range(XR // 8)]
            rpos = pl.multiple_of(rp, SEG // 2)
            opos = [pl.multiple_of(_wrap(op + 8 * j, ORING), 8)
                    for j in range(XR // 8)]
            owr = pl.multiple_of(ow, SEG)

            tails = {}
            xs = {}
            ps = {}
            lhs_o = {}

            def load(j, p):
                r32 = (q32, k32, v32)[j]
                xs[j, p] = [
                    pltpu.bitcast(r32[h, pl.ds(rpos, SEG // 2), :], BF16)
                    for h in (2 * p, 2 * p + 1)]

            def operand(j, p):
                tail = jnp.concatenate(
                    [tails.pop((j, 2 * p)), tails.pop((j, 2 * p + 1))], axis=0)
                return jnp.concatenate(
                    xs.pop((j, p)) + [tail.astype(BF16)], axis=0)

            low = {}
            if split:
                lhs_lo = jnp.concatenate(lhs_c[:NC // 2], axis=1)
                lhs_hi = jnp.concatenate(lhs_c[NC // 2:], axis=1)
                for h in range(2):
                    for j, w32 in enumerate((wq32, wk32, wv32)):
                        low[j, h] = _dot(lhs_lo, pltpu.bitcast(
                            w32[h, pl.ds(0, D // 4), :], BF16))

            def proj(h):
                for j, (w32, ring) in enumerate(
                        ((wq32, qring), (wk32, kring), (wv32, vring))):
                    if (j, h) in low:
                        t = _dot(lhs_hi, pltpu.bitcast(
                            w32[h, pl.ds(D // 4, D // 4), :], BF16)) + low[j, h]
                    else:
                        t = _dot(lhs, _w(w32, h))
                    for i in range(XR // 8):
                        ring[h, pl.ds(wpos[i], 8), :] = (
                            t[8 * i:8 * i + 8].astype(BF16))
                    tails[j, h] = t[XR:]

            def qk(p):
                sc = lax.dot_general(operand(0, p), operand(1, p),
                                     (((1,), (1,)), ((), ())),
                                     preferred_element_type=F32)
                sc = jnp.where(mask, sc * SCALE, fill)
                mx = jnp.max(sc, axis=-1, keepdims=True)
                e = jnp.exp(sc - mx)
                l = jnp.sum(e, axis=-1, keepdims=True)
                ps[p] = (e * pl.reciprocal(l, approx=True)).astype(BF16)

            def pv(p):
                o = _dot(ps.pop(p), operand(2, p))
                for i, h in enumerate((2 * p, 2 * p + 1)):
                    ox = [oring[h, pl.ds(opos[k], 8), :] for k in range(XR // 8)]
                    om = o[2 * SEG + M * i:2 * SEG + M * (i + 1)]
                    last = jnp.concatenate(
                        [ox[2].astype(F32), om], axis=0).astype(BF16)
                    lhs_o[h] = jnp.concatenate([ox[0], ox[1], last], axis=0)
                for i, h in enumerate((2 * p, 2 * p + 1)):
                    oring[h, pl.ds(owr, SEG), :] = (
                        o[SEG * i:SEG * (i + 1)].astype(BF16))

            def wo_part(c, h0, h1):
                lo = jnp.concatenate([lhs_o[h] for h in range(h0, h1)], axis=1)
                w = pltpu.bitcast(wo32[c, pl.ds(h0 * 64, (h1 - h0) * 64), :], BF16)
                return _dot(lo, w)

            NPR = H // 2
            for t in range(NPR):
                if t >= 1:
                    load(0, t - 1)
                    load(1, t - 1)
                proj(2 * t)
                if t >= 1:
                    qk(t - 1)
                if t >= 2:
                    load(2, t - 2)
                proj(2 * t + 1)
                if t >= 2:
                    pv(t - 2)
            HA = H - 4
            acc = {}
            load(0, NPR - 1)
            load(1, NPR - 1)
            load(2, NPR - 2)
            acc[0] = wo_part(0, 0, HA)
            qk(NPR - 1)
            acc[1] = wo_part(1, 0, HA)
            pv(NPR - 2)
            load(2, NPR - 1)
            for c in (2, 3, 4):
                acc[c] = wo_part(c, 0, HA)
            pv(NPR - 1)
            for c in (5, 6, 7):
                acc[c] = wo_part(c, 0, HA)
            mem_new = []
            for c in range(NC):
                a = wo_part(c, HA, H) + acc[c]
                ax_s[:, pl.ds(c * 128, 128)] = a[:XR]
                mem_new.append(a[XR:])
            return (_wrap(wp + XR, RING), _wrap(rp + SEG // 2, RING // 2),
                    _wrap(op + XR, ORING), _wrap(ow + SEG, ORING)), mem_new

        def steps(i, carry):
            mem = [mem_s[:, pl.ds(c * 128, 128)] for c in range(NC)]
            for u in range(UNROLL):
                carry, mem = step(i * UNROLL + u, carry, mem, split=u > 0)
            for c in range(NC):
                mem_s[:, pl.ds(c * 128, 128)] = mem[c]
            return carry

        lax.fori_loop(0, NSEG // UNROLL, steps,
                      (jnp.int32(PRO), jnp.int32(0), jnp.int32(OOFF - XR),
                       jnp.int32(OOFF)))

        post_attn(ax_s[...], XR * NSEG, XR)
        done = XR * (NSEG - 1)

        def wo_bulk(r, n):
            p = r - done + (done + OOFF) % ORING
            if not isinstance(p, int):
                p = pl.multiple_of(p, 8)
            lo = jnp.concatenate(
                [oring[h, pl.ds(p, n), :] for h in range(H)], axis=1)
            a = jnp.concatenate(
                [_dot(lo, _w(wo32, c)) for c in range(NC)], axis=1)
            rr = PAD + r
            if not isinstance(rr, int):
                rr = pl.multiple_of(rr, 8)
            post_attn(a, rr, n)

        def wo_body(i, carry):
            wo_bulk(done + i * 128, 128)
            return carry

        lax.fori_loop(0, 4, wo_body, 0)
        wo_bulk(done + 512, S - done - 512)

        for cp in cp_w1 + cp_w3 + cp_w2:
            cp.wait()

        def cp_out(i):
            r = i * FB
            rb = PAD + r
            if not isinstance(i, int):
                r = pl.multiple_of(r, FB)
                rb = pl.multiple_of(rb, 8)
            return pltpu.make_async_copy(xbuf.at[pl.ds(rb, FB)],
                                         out_hbm.at[pl.ds(r, FB)],
                                         sems.at[SEM_OUT])

        def ffn_body(i, carry):
            r = pl.multiple_of(PAD + i * FB, 8)
            hv = hbuf[pl.ds(r, FB), :]
            act = []
            for f in range(NF):
                g = _dot(hv, _w(w132, f))
                u = _dot(hv, _w(w332, f))
                act.append((g * jax.nn.sigmoid(g) * u).astype(BF16))
            av = jnp.concatenate(act, axis=1)
            for c in range(NC):
                y = _dot(av, _w(w232, c))
                cs = pl.ds(c * 128, 128)
                x2 = xbuf[pl.ds(r, FB), cs].astype(F32) + mod_s[pl.ds(5, 1), cs] * y
                xbuf[pl.ds(r, FB), cs] = x2.astype(BF16)
            cp_out(i).start()
            return carry

        lax.fori_loop(0, S // FB, ffn_body, 0)
        for i in range(S // FB):
            cp_out(i).wait()

    pl.run_scoped(
        rest,
        pltpu.VMEM((NF, D, 128), BF16),
        pltpu.VMEM((NF, D, 128), BF16),
        pltpu.VMEM((NC, F, 128), BF16),
        pltpu.VMEM((H, ORING, DH), BF16),
    )


@functools.partial(jax.jit, static_argnames=("A_seg_len",))
def pallas_adaLN_cond__memory_aug_recurrent_mem_tr__glu_gated_swiglu__prompt_kernel(
    A_x: jax.Array,
    A_mem0: jax.Array,
    A_Wq: jax.Array,
    A_Wk: jax.Array,
    A_Wv: jax.Array,
    A_Wo: jax.Array,
    A_seg_len,
    B_x: jax.Array,
    B_w1: jax.Array,
    B_w3: jax.Array,
    B_w2: jax.Array,
    c: jax.Array,
    w_mod: jax.Array,
):
    del B_x
    assert A_seg_len == SEG
    assert A_x.shape == (1, S, D) and A_mem0.shape == (1, M, D)
    assert A_Wq.shape == (D, H, DH) and B_w1.shape == (D, F)

    any_spec = pl.BlockSpec(memory_space=pl.ANY)
    out = pl.pallas_call(
        _kernel,
        out_shape=jax.ShapeDtypeStruct((S, D), BF16),
        in_specs=[any_spec] * 11,
        out_specs=any_spec,
        scratch_shapes=[
            pltpu.VMEM((H, D // 2, DH), U32),
            pltpu.VMEM((H, D // 2, DH), U32),
            pltpu.VMEM((H, D // 2, DH), U32),
            pltpu.VMEM((NC, H * DH, 128), BF16),
            pltpu.VMEM((2, PAD + S, D), BF16),
            pltpu.VMEM((H, RING, DH), BF16),
            pltpu.VMEM((H, RING, DH), BF16),
            pltpu.VMEM((H, RING, DH), BF16),
            pltpu.VMEM((8, D), F32),
            pltpu.VMEM((M, D), F32),
            pltpu.VMEM((XR, D), F32),
            pltpu.VMEM((XR, D), F32),
            pltpu.VMEM((1, D), BF16),
            pltpu.VMEM((M, D), BF16),
            pltpu.SemaphoreType.DMA((NSEMS,)),
        ],
        compiler_params=pltpu.CompilerParams(
            vmem_limit_bytes=120 * 1024 * 1024),
        name="adaln_memtr_swiglu",
    )(
        A_x.reshape(S, D),
        A_mem0.reshape(M, D),
        A_Wq, A_Wk, A_Wv,
        A_Wo.reshape(H * DH, D),
        B_w1, B_w3, B_w2, c, w_mod,
    )
    return out.reshape(1, S, D)
```

```python
import functools

import jax
import jax.numpy as jnp
from jax import lax
import jax.experimental.pallas as pl
import jax.experimental.pallas.tpu as pltpu

BF16 = jnp.bfloat16
F32 = jnp.float32
U32 = jnp.uint32

S = 2048
D = 1024
H = 32
DH = 128
F = 3584
M = 8
SEG = 32
NSEG = S // SEG
XR = 24
PRO = S - XR * NSEG
RING = 544
ORING = 576
OOFF = 256
PAD = 48
NC = D // 128
NF = F // 128
FB = 128
NWB = 3
WB = 176
UNROLL = 4
NU = 3 * H // 2
NU0 = 40
UPI = 6
NP = 2 * (SEG + M)
EPS = 1e-5
SEM_FIRST, SEM_LATE, SEM_WM2, SEM_FFN, SEM_OUT = 0, 1, 2, 3, 4
SEM_WM1 = 5
SEM_U0 = SEM_WM1 + 4
SEM_IT = SEM_U0 + 5 - 1
NSEMS = SEM_IT + NU // UPI
U0_GROUP = (0, 1, 2, 3, 3, 4, 4)
SCALE = DH ** -0.5


def _dot(a, b):
    return jnp.dot(a, b, preferred_element_type=F32)


def _w(ref32, i):
    return pltpu.bitcast(ref32[i], BF16)


def _wrap(i, n):
    return jnp.where(i >= n, i - n, i)


def _ln(x):
    mu = jnp.mean(x, axis=-1, keepdims=True)
    xc = x - mu
    var = jnp.mean(xc * xc, axis=-1, keepdims=True)
    return xc * lax.rsqrt(var + EPS)


def _ln_mod(x, shift, scale1):
    return _ln(x) * scale1 + shift


def _kernel(x_hbm, mem0_hbm, wq_hbm, wk_hbm, wv_hbm, wo_hbm, w1_hbm, w3_hbm,
            w2_hbm, c_hbm, wmod_hbm, out_hbm,
            wq32, wk32, wv32, wo_s, xh, qring, kring, vring,
            mod_s, mem_s, ax_s, hn_s, c_s, m0_s, sems):
    wo32 = wo_s.bitcast(U32)
    xbuf = xh.at[0]
    hbuf = xh.at[1]

    cp_x0 = pltpu.make_async_copy(x_hbm.at[pl.ds(0, PRO)],
                                  xbuf.at[pl.ds(PAD, PRO)], sems.at[SEM_FIRST])
    cp_c = pltpu.make_async_copy(c_hbm, c_s, sems.at[SEM_FIRST])
    cp_late = [
        pltpu.make_async_copy(mem0_hbm, m0_s, sems.at[SEM_LATE]),
        pltpu.make_async_copy(x_hbm.at[pl.ds(PRO, S - PRO)],
                              xbuf.at[pl.ds(PAD + PRO, S - PRO)],
                              sems.at[SEM_LATE]),
    ] + [pltpu.make_async_copy(wo_hbm.at[:, pl.ds(c * 128, 128)],
                               wo_s.at[c], sems.at[SEM_LATE])
         for c in range(NC)]

    def mod_row(i):
        return mod_s[pl.ds(i, 1), :]

    def prologue(st, wm_s, xn_s):
        wm32 = wm_s.bitcast(U32)
        srcs = (wq_hbm.bitcast(U32), wk_hbm.bitcast(U32), wv_hbm.bitcast(U32))
        dsts = (wq32, wk32, wv32)
        rings = (qring, kring, vring)

        def cp_st(j, s, sem):
            return pltpu.make_async_copy(srcs[j].at[:, s, :], st.at[3 * s + j],
                                         sems.at[sem])

        def cp_unit(u):
            sem = (SEM_U0 + U0_GROUP[u] if u <= UPI
                   else SEM_IT + (u - 1) // UPI)
            return cp_st(u % 3, u // 3, sem)

        def cp_wm(i):
            if isinstance(i, int):
                col = i * 128
                sem = SEM_WM1 + i // 4 if i < 16 else SEM_WM2
            else:
                col = pl.multiple_of(i * 128, 128)
                sem = SEM_WM2
            return pltpu.make_async_copy(wmod_hbm.at[:, pl.ds(col, 128)],
                                         wm_s.at[i], sems.at[sem])

        cp_c.start()
        cp_x0.start()
        for i in range(16):
            cp_wm(i).start()
        for u in range(NU0):
            cp_unit(u).start()

        xbuf[pl.ds(0, PAD), :] = jnp.zeros((PAD, D), BF16)
        ax_s[...] = jnp.zeros((XR, D), F32)

        cp_c.wait()
        cp_x0.wait()
        cf = c_s[...].astype(F32)
        sc = (cf * jax.nn.sigmoid(cf)).astype(BF16)
        sc8 = jnp.broadcast_to(sc, (8, D))

        def ln_body(i, carry):
            r = pl.multiple_of(i * 64, 64)
            xv = xbuf[pl.ds(pl.multiple_of(PAD + r, 8), 64), :].astype(F32)
            xn_s[pl.ds(r, 64), :] = _ln(xv)
            return carry

        lax.fori_loop(0, PRO // 64, ln_body, 0)

        def mod_part(lo, hi, chunk):
            for c0 in range(lo, hi, chunk):
                for i in range(c0, c0 + chunk):
                    cp_wm(i).wait()
                for i in range(c0, c0 + chunk):
                    k, c = divmod(i, NC)
                    part = _dot(sc8, _w(wm32, i))[0:1, :]
                    if k in (1, 4):
                        part = part + 1.0
                    mod_s[pl.ds(k, 1), pl.ds(c * 128, 128)] = part

        mod_part(0, 16, 4)

        def relayout(j, s):
            u = 3 * s + j
            for db in range(8):
                ev = st[u, pl.ds(db * 128, 64, stride=2), :]
                od = st[u, pl.ds(db * 128 + 1, 64, stride=2), :]
                rows = pl.ds(db * 64, 64)
                dsts[j][2 * s, rows, :] = (ev & U32(0xFFFF)) | (od << 16)
                dsts[j][2 * s + 1, rows, :] = (ev >> 16) | (od & U32(0xFFFF0000))

        def bulk(j, s, first=False, mbs=range(PRO // 128)):
            for mb in mbs:
                rows = pl.ds(PAD + mb * 128, 128)
                if first:
                    lhs = (xn_s[pl.ds(mb * 128, 128), :] * mod_row(1)
                           + mod_row(0)).astype(BF16)
                    hbuf[rows, :] = lhs
                else:
                    lhs = hbuf[rows, :]
                for hh in range(2):
                    h = 2 * s + hh
                    rings[j][h, pl.ds(mb * 128, 128), :] = (
                        _dot(lhs, _w(dsts[j], h)).astype(BF16))

        for u in range(NU0, NU):
            cp_unit(u).start()
        for cp in cp_late:
            cp.start()

        cp_unit(0).wait()
        relayout(0, 0)
        bulk(0, 0, first=True, mbs=(0, 1))
        for u in range(UPI):
            if U0_GROUP[u + 1] != U0_GROUP[u]:
                for v in range(u + 1, UPI + 1):
                    if U0_GROUP[v] == U0_GROUP[u + 1]:
                        cp_unit(v).wait()
            relayout((u + 1) % 3, (u + 1) // 3)
            if u == 0:
                bulk(0, 0, first=True, mbs=(2, 3))
            else:
                bulk(u % 3, u // 3)
        for i in range(16, 24):
            cp_wm(i).start()

        def grp_body(it, carry):
            s0 = it * (UPI // 3)
            last = NU // UPI - 1
            sn = jnp.minimum(s0 + UPI // 3, H // 2 - 1)
            for u in range(1, UPI):
                cp_st(u % 3, s0 + u // 3, SEM_IT + it).wait()

            @pl.when(it < last)
            def _():
                cp_st(0, sn, SEM_IT + it).wait()
                for k in range(4):
                    cp_wm(20 + 4 * it + k).start()

            for u in range(UPI):
                if u + 1 < UPI:
                    relayout((u + 1) % 3, s0 + (u + 1) // 3)
                else:
                    relayout(0, sn)
                bulk(u % 3, s0 + u // 3)
            return carry

        lax.fori_loop(1, NU // UPI, grp_body, 0)

        mod_part(16, 48, 32)
        for cp in cp_late:
            cp.wait()
        mem_s[...] = m0_s[...].astype(F32)
        xv = xbuf[pl.ds(PAD + PRO, XR), :].astype(F32)
        hn_s[...] = _ln_mod(xv, mod_row(0), mod_row(1))

    pl.run_scoped(
        prologue,
        pltpu.VMEM((NU, D, DH), U32),
        pltpu.VMEM((48, D, 128), BF16),
        pltpu.VMEM((PRO, D), F32),
    )

    def rest(w1_s, w3_s, w2_s, oring):
        w132 = w1_s.bitcast(U32)
        w332 = w3_s.bitcast(U32)
        w232 = w2_s.bitcast(U32)
        q32 = qring.bitcast(U32)
        k32 = kring.bitcast(U32)
        v32 = vring.bitcast(U32)

        cp_w1 = [pltpu.make_async_copy(w1_hbm.at[:, pl.ds(f * 128, 128)],
                                       w1_s.at[f], sems.at[SEM_FFN])
                 for f in range(NF)]
        cp_w3 = [pltpu.make_async_copy(w3_hbm.at[:, pl.ds(f * 128, 128)],
                                       w3_s.at[f], sems.at[SEM_FFN])
                 for f in range(NF)]
        cp_w2 = [pltpu.make_async_copy(w2_hbm.at[:, pl.ds(c * 128, 128)],
                                       w2_s.at[c], sems.at[SEM_FFN])
                 for c in range(NC)]
        for cp in cp_w1 + cp_w3 + cp_w2:
            cp.start()

        oring[:, pl.ds(OOFF - XR, XR), :] = jnp.zeros((H, XR, DH), BF16)

        def post_attn(a, r, n):
            x1 = xbuf[pl.ds(r, n), :].astype(F32) + mod_row(2) * a
            x1 = x1.astype(BF16)
            xbuf[pl.ds(r, n), :] = x1
            hbuf[pl.ds(r, n), :] = _ln_mod(
                x1.astype(F32), mod_row(3), mod_row(4)).astype(BF16)

        row = lax.broadcasted_iota(jnp.int32, (NP, NP), 0)
        col = lax.broadcasted_iota(jnp.int32, (NP, NP), 1)

        def second(i):
            return ((i >= SEG) & (i < 2 * SEG)) | (i >= 2 * SEG + M)

        same = second(row) == second(col)
        mask = same & ((row >= 2 * SEG) | (col >= 2 * SEG) | (col <= row))
        fill = jnp.where(same, -1e9, -jnp.inf).astype(F32)

        def step(s, carry, mem, split, maybe_last):
            lhs_c = [jnp.concatenate([hn_s[:, pl.ds(c * 128, 128)], mem[c]],
                                     axis=0).astype(BF16) for c in range(NC)]
            lhs = jnp.concatenate(lhs_c, axis=1)

            post_attn(ax_s[...], pl.multiple_of(XR * s, 8), XR)
            rn = pl.multiple_of(
                PAD + jnp.minimum(PRO + XR * (s + 1), S - XR), 8)
            hn_s[...] = _ln_mod(xbuf[pl.ds(rn, XR), :].astype(F32),
                                mod_row(0), mod_row(1))

            wp, rp, op, ow = carry
            wpos = [pl.multiple_of(_wrap(wp + 8 * j, RING), 8)
                    for j in range(XR // 8)]
            rpos = pl.multiple_of(rp, SEG // 2)
            opos = [pl.multiple_of(_wrap(op + 8 * j, ORING), 8)
                    for j in range(XR // 8 + 1)]
            owr = pl.multiple_of(ow, SEG)

            tails = {}
            xs = {}
            ps = {}
            lhs_o = {}

            def load(j, p):
                r32 = (q32, k32, v32)[j]
                xs[j, p] = [
                    pltpu.bitcast(r32[h, pl.ds(rpos, SEG // 2), :], BF16)
                    for h in (2 * p, 2 * p + 1)]

            def operand(j, p):
                tail = jnp.concatenate(
                    [tails.pop((j, 2 * p)), tails.pop((j, 2 * p + 1))], axis=0)
                return jnp.concatenate(
                    xs.pop((j, p)) + [tail.astype(BF16)], axis=0)

            low = {}
            if split:
                lhs_lo = jnp.concatenate(lhs_c[:NC // 2], axis=1)
                lhs_hi = jnp.concatenate(lhs_c[NC // 2:], axis=1)
                for h in range(2):
                    for j, w32 in enumerate((wq32, wk32, wv32)):
                        low[j, h] = _dot(lhs_lo, pltpu.bitcast(
                            w32[h, pl.ds(0, D // 4), :], BF16))

            def proj(h):
                for j, (w32, ring) in enumerate(
                        ((wq32, qring), (wk32, kring), (wv32, vring))):
                    if (j, h) in low:
                        t = _dot(lhs_hi, pltpu.bitcast(
                            w32[h, pl.ds(D // 4, D // 4), :], BF16)) + low[j, h]
                    else:
                        t = _dot(lhs, _w(w32, h))
                    for i in range(XR // 8):
                        ring[h, pl.ds(wpos[i], 8), :] = (
                            t[8 * i:8 * i + 8].astype(BF16))
                    tails[j, h] = t[XR:]

            def qk(p):
                sc = lax.dot_general(operand(0, p), operand(1, p),
                                     (((1,), (1,)), ((), ())),
                                     preferred_element_type=F32)
                sc = jnp.where(mask, sc * SCALE, fill)
                mx = jnp.max(sc, axis=-1, keepdims=True)
                e = jnp.exp(sc - mx)
                l = jnp.sum(e, axis=-1, keepdims=True)
                ps[p] = (e * pl.reciprocal(l, approx=True)).astype(BF16)

            def pv(p):
                o = _dot(ps.pop(p), operand(2, p))
                for i, h in enumerate((2 * p, 2 * p + 1)):
                    ox = [oring[h, pl.ds(opos[k], 8), :] for k in range(XR // 8)]
                    om = o[2 * SEG + M * i:2 * SEG + M * (i + 1)]
                    if maybe_last:
                        om = jnp.where(
                            s == NSEG - 1,
                            oring[h, pl.ds(opos[3], 8), :].astype(F32), om)
                    last = jnp.concatenate(
                        [ox[2].astype(F32), om], axis=0).astype(BF16)
                    lhs_o[h] = jnp.concatenate([ox[0], ox[1], last], axis=0)
                for i, h in enumerate((2 * p, 2 * p + 1)):
                    oring[h, pl.ds(owr, SEG), :] = (
                        o[SEG * i:SEG * (i + 1)].astype(BF16))

            def wo_part(c, h0, h1):
                lo = jnp.concatenate([lhs_o[h] for h in range(h0, h1)], axis=1)
                w = pltpu.bitcast(wo32[c, pl.ds(h0 * 64, (h1 - h0) * 64), :], BF16)
                return _dot(lo, w)

            NPR = H // 2
            for t in range(NPR):
                if t >= 1:
                    load(0, t - 1)
                    load(1, t - 1)
                proj(2 * t)
                if t >= 1:
                    qk(t - 1)
                if t >= 2:
                    load(2, t - 2)
                proj(2 * t + 1)
                if t >= 2:
                    pv(t - 2)
            HA = H - 4
            acc = {}
            load(0, NPR - 1)
            load(1, NPR - 1)
            load(2, NPR - 2)
            acc[0] = wo_part(0, 0, HA)
            qk(NPR - 1)
            acc[1] = wo_part(1, 0, HA)
            pv(NPR - 2)
            load(2, NPR - 1)
            for c in (2, 3, 4):
                acc[c] = wo_part(c, 0, HA)
            pv(NPR - 1)
            for c in (5, 6, 7):
                acc[c] = wo_part(c, 0, HA)
            mem_new = []
            for c in range(NC):
                a = wo_part(c, HA, H) + acc[c]
                ax_s[:, pl.ds(c * 128, 128)] = a[:XR]
                mem_new.append(a[XR:])
            return (_wrap(wp + XR, RING), _wrap(rp + SEG // 2, RING // 2),
                    _wrap(op + XR, ORING), _wrap(ow + SEG, ORING)), mem_new

        def steps(i, carry):
            mem = [mem_s[:, pl.ds(c * 128, 128)] for c in range(NC)]
            for u in range(UNROLL):
                carry, mem = step(i * UNROLL + u, carry, mem, split=u > 0,
                                  maybe_last=u == UNROLL - 1)
            for c in range(NC):
                mem_s[:, pl.ds(c * 128, 128)] = mem[c]
            return carry

        lax.fori_loop(0, NSEG // UNROLL, steps,
                      (jnp.int32(PRO), jnp.int32(0), jnp.int32(OOFF - XR),
                       jnp.int32(OOFF)))

        post_attn(jnp.concatenate([ax_s[...], mem_s[...]], axis=0),
                  XR * NSEG, XR + M)
        done = XR * (NSEG - 1) + M
        o32 = oring.bitcast(U32)

        def wo_bulk(i):
            p = pl.multiple_of(((done + OOFF) % ORING + i * WB) // 2, 8)
            lo = jnp.concatenate(
                [pltpu.bitcast(o32[h, pl.ds(p, WB // 2), :], BF16)
                 for h in range(H)], axis=1)
            a = jnp.concatenate(
                [_dot(lo, _w(wo32, c)) for c in range(NC)], axis=1)
            post_attn(a, pl.multiple_of(PAD + done + i * WB, 16), WB)

        for cp in cp_w1 + cp_w3 + cp_w2:
            cp.wait()

        def cp_out(i):
            r = i * FB
            rb = PAD + r
            if not isinstance(i, int):
                r = pl.multiple_of(r, FB)
                rb = pl.multiple_of(rb, 8)
            return pltpu.make_async_copy(xbuf.at[pl.ds(rb, FB)],
                                         out_hbm.at[pl.ds(r, FB)],
                                         sems.at[SEM_OUT])

        def ffn_body(i, carry, with_wo):
            r = pl.multiple_of(PAD + i * FB, 16)
            hv = hbuf[pl.ds(r, FB), :]
            if with_wo:
                wo_bulk(i)
            act = []
            for f in range(NF):
                g = _dot(hv, _w(w132, f))
                u = _dot(hv, _w(w332, f))
                act.append((g * jax.nn.sigmoid(g) * u).astype(BF16))
            av = jnp.concatenate(act, axis=1)
            for c in range(NC):
                y = _dot(av, _w(w232, c))
                cs = pl.ds(c * 128, 128)
                x2 = xbuf[pl.ds(r, FB), cs].astype(F32) + mod_s[pl.ds(5, 1), cs] * y
                xbuf[pl.ds(r, FB), cs] = x2.astype(BF16)
            cp_out(i).start()
            return carry

        lax.fori_loop(0, NWB, functools.partial(ffn_body, with_wo=True), 0)
        lax.fori_loop(NWB, S // FB,
                      functools.partial(ffn_body, with_wo=False), 0)
        for i in range(S // FB):
            cp_out(i).wait()

    pl.run_scoped(
        rest,
        pltpu.VMEM((NF, D, 128), BF16),
        pltpu.VMEM((NF, D, 128), BF16),
        pltpu.VMEM((NC, F, 128), BF16),
        pltpu.VMEM((H, ORING, DH), BF16),
    )


@functools.partial(jax.jit, static_argnames=("A_seg_len",))
def pallas_adaLN_cond__memory_aug_recurrent_mem_tr__glu_gated_swiglu__prompt_kernel(
    A_x: jax.Array,
    A_mem0: jax.Array,
    A_Wq: jax.Array,
    A_Wk: jax.Array,
    A_Wv: jax.Array,
    A_Wo: jax.Array,
    A_seg_len,
    B_x: jax.Array,
    B_w1: jax.Array,
    B_w3: jax.Array,
    B_w2: jax.Array,
    c: jax.Array,
    w_mod: jax.Array,
):
    del B_x
    assert A_seg_len == SEG
    assert A_x.shape == (1, S, D) and A_mem0.shape == (1, M, D)
    assert A_Wq.shape == (D, H, DH) and B_w1.shape == (D, F)

    any_spec = pl.BlockSpec(memory_space=pl.ANY)
    out = pl.pallas_call(
        _kernel,
        out_shape=jax.ShapeDtypeStruct((S, D), BF16),
        in_specs=[any_spec] * 11,
        out_specs=any_spec,
        scratch_shapes=[
            pltpu.VMEM((H, D // 2, DH), U32),
            pltpu.VMEM((H, D // 2, DH), U32),
            pltpu.VMEM((H, D // 2, DH), U32),
            pltpu.VMEM((NC, H * DH, 128), BF16),
            pltpu.VMEM((2, PAD + S, D), BF16),
            pltpu.VMEM((H, RING, DH), BF16),
            pltpu.VMEM((H, RING, DH), BF16),
            pltpu.VMEM((H, RING, DH), BF16),
            pltpu.VMEM((8, D), F32),
            pltpu.VMEM((M, D), F32),
            pltpu.VMEM((XR, D), F32),
            pltpu.VMEM((XR, D), F32),
            pltpu.VMEM((1, D), BF16),
            pltpu.VMEM((M, D), BF16),
            pltpu.SemaphoreType.DMA((NSEMS,)),
        ],
        compiler_params=pltpu.CompilerParams(
            vmem_limit_bytes=120 * 1024 * 1024),
        name="adaln_memtr_swiglu",
    )(
        A_x.reshape(S, D),
        A_mem0.reshape(M, D),
        A_Wq, A_Wk, A_Wv,
        A_Wo.reshape(H * DH, D),
        B_w1, B_w3, B_w2, c, w_mod,
    )
    return out.reshape(1, S, D)
```

```python
import functools

import jax
import jax.numpy as jnp
from jax import lax
import jax.experimental.pallas as pl
import jax.experimental.pallas.tpu as pltpu

BF16 = jnp.bfloat16
F32 = jnp.float32
U32 = jnp.uint32

S = 2048
D = 1024
H = 32
DH = 128
F = 3584
M = 8
SEG = 32
NSEG = S // SEG
XR = 24
PRO = S - XR * NSEG
RING = 544
ORING = 576
OOFF = 256
PAD = 48
NC = D // 128
NF = F // 128
FB = 128
NWB = 3
WB = 176
UNROLL = 4
NU = 3 * H // 2
NU0 = 40
UPI = 6
NP = 2 * (SEG + M)
EPS = 1e-5
SEM_FIRST, SEM_LATE, SEM_WM2, SEM_FFN, SEM_OUT = 0, 1, 2, 3, 4
SEM_WM1 = 5
SEM_U0 = SEM_WM1 + 4
SEM_IT = SEM_U0 + 5 - 1
NSEMS = SEM_IT + NU // UPI
U0_GROUP = (0, 1, 2, 3, 3, 4, 4)
SCALE = DH ** -0.5


def _dot(a, b):
    return jnp.dot(a, b, preferred_element_type=F32)


def _w(ref32, i):
    return pltpu.bitcast(ref32[i], BF16)


def _wrap(i, n):
    return jnp.where(i >= n, i - n, i)


def _ln(x):
    mu = jnp.mean(x, axis=-1, keepdims=True)
    xc = x - mu
    var = jnp.mean(xc * xc, axis=-1, keepdims=True)
    return xc * lax.rsqrt(var + EPS)


def _ln_mod(x, shift, scale1):
    return _ln(x) * scale1 + shift


def _kernel(x_hbm, mem0_hbm, wq_hbm, wk_hbm, wv_hbm, wo_hbm, w1_hbm, w3_hbm,
            w2_hbm, c_hbm, wmod_hbm, out_hbm,
            wq32, wk32, wv32, wo_s, xh, qring, kring, vring,
            mod_s, mem_s, ax_s, hn_s, c_s, m0_s, sems):
    wo32 = wo_s.bitcast(U32)
    xbuf = xh.at[0]
    hbuf = xh.at[1]

    cp_x0 = pltpu.make_async_copy(x_hbm.at[pl.ds(0, PRO)],
                                  xbuf.at[pl.ds(PAD, PRO)], sems.at[SEM_FIRST])
    cp_c = pltpu.make_async_copy(c_hbm, c_s, sems.at[SEM_FIRST])
    cp_late = [
        pltpu.make_async_copy(mem0_hbm, m0_s, sems.at[SEM_LATE]),
        pltpu.make_async_copy(x_hbm.at[pl.ds(PRO, S - PRO)],
                              xbuf.at[pl.ds(PAD + PRO, S - PRO)],
                              sems.at[SEM_LATE]),
    ] + [pltpu.make_async_copy(wo_hbm.at[:, pl.ds(c * 128, 128)],
                               wo_s.at[c], sems.at[SEM_LATE])
         for c in range(NC)]

    def mod_row(i, n, cols=slice(None)):
        return jnp.concatenate([mod_s[pl.ds(8 * i, 8), cols]] * (n // 8), axis=0)

    def prologue(st, wm_s, xn_s):
        wm32 = wm_s.bitcast(U32)
        srcs = (wq_hbm.bitcast(U32), wk_hbm.bitcast(U32), wv_hbm.bitcast(U32))
        dsts = (wq32, wk32, wv32)
        rings = (qring, kring, vring)

        def cp_st(j, s, sem):
            return pltpu.make_async_copy(srcs[j].at[:, s, :], st.at[3 * s + j],
                                         sems.at[sem])

        def cp_unit(u):
            sem = (SEM_U0 + U0_GROUP[u] if u <= UPI
                   else SEM_IT + (u - 1) // UPI)
            return cp_st(u % 3, u // 3, sem)

        def cp_wm(i):
            if isinstance(i, int):
                col = i * 128
                sem = SEM_WM1 + i // 4 if i < 16 else SEM_WM2
            else:
                col = pl.multiple_of(i * 128, 128)
                sem = SEM_WM2
            return pltpu.make_async_copy(wmod_hbm.at[:, pl.ds(col, 128)],
                                         wm_s.at[i], sems.at[sem])

        cp_c.start()
        cp_x0.start()
        for i in range(16):
            cp_wm(i).start()
        for u in range(NU0):
            cp_unit(u).start()

        xbuf[pl.ds(0, PAD), :] = jnp.zeros((PAD, D), BF16)
        ax_s[...] = jnp.zeros((XR, D), F32)

        cp_c.wait()
        cp_x0.wait()
        cf = c_s[...].astype(F32)
        sc = (cf * jax.nn.sigmoid(cf)).astype(BF16)
        sc8 = jnp.broadcast_to(sc, (8, D))

        def ln_body(i, carry):
            r = pl.multiple_of(i * 64, 64)
            xv = xbuf[pl.ds(pl.multiple_of(PAD + r, 8), 64), :].astype(F32)
            xn_s[pl.ds(r, 64), :] = _ln(xv)
            return carry

        lax.fori_loop(0, PRO // 64, ln_body, 0)

        def mod_part(lo, hi, chunk):
            for c0 in range(lo, hi, chunk):
                for i in range(c0, c0 + chunk):
                    cp_wm(i).wait()
                for i in range(c0, c0 + chunk):
                    k, c = divmod(i, NC)
                    part = _dot(sc8, _w(wm32, i))
                    if k in (1, 4):
                        part = part + 1.0
                    mod_s[pl.ds(8 * k, 8), pl.ds(c * 128, 128)] = part

        mod_part(0, 16, 4)

        def relayout(j, s):
            u = 3 * s + j
            for db in range(8):
                ev = st[u, pl.ds(db * 128, 64, stride=2), :]
                od = st[u, pl.ds(db * 128 + 1, 64, stride=2), :]
                rows = pl.ds(db * 64, 64)
                dsts[j][2 * s, rows, :] = (ev & U32(0xFFFF)) | (od << 16)
                dsts[j][2 * s + 1, rows, :] = (ev >> 16) | (od & U32(0xFFFF0000))

        def bulk(j, s, first=False, mbs=range(PRO // 128)):
            for mb in mbs:
                rows = pl.ds(PAD + mb * 128, 128)
                if first:
                    lhs = (xn_s[pl.ds(mb * 128, 128), :] * mod_row(1, 128)
                           + mod_row(0, 128)).astype(BF16)
                    hbuf[rows, :] = lhs
                else:
                    lhs = hbuf[rows, :]
                for hh in range(2):
                    h = 2 * s + hh
                    rings[j][h, pl.ds(mb * 128, 128), :] = (
                        _dot(lhs, _w(dsts[j], h)).astype(BF16))

        for u in range(NU0, NU):
            cp_unit(u).start()
        for cp in cp_late:
            cp.start()

        cp_unit(0).wait()
        relayout(0, 0)
        bulk(0, 0, first=True, mbs=(0, 1))
        for u in range(UPI):
            if U0_GROUP[u + 1] != U0_GROUP[u]:
                for v in range(u + 1, UPI + 1):
                    if U0_GROUP[v] == U0_GROUP[u + 1]:
                        cp_unit(v).wait()
            relayout((u + 1) % 3, (u + 1) // 3)
            if u == 0:
                bulk(0, 0, first=True, mbs=(2, 3))
            else:
                bulk(u % 3, u // 3)
        for i in range(16, 24):
            cp_wm(i).start()

        def grp_body(it, carry):
            s0 = it * (UPI // 3)
            last = NU // UPI - 1
            sn = jnp.minimum(s0 + UPI // 3, H // 2 - 1)
            for u in range(1, UPI):
                cp_st(u % 3, s0 + u // 3, SEM_IT + it).wait()

            @pl.when(it < last)
            def _():
                cp_st(0, sn, SEM_IT + it).wait()
                for k in range(4):
                    cp_wm(20 + 4 * it + k).start()

            for u in range(UPI):
                if u + 1 < UPI:
                    relayout((u + 1) % 3, s0 + (u + 1) // 3)
                else:
                    relayout(0, sn)
                bulk(u % 3, s0 + u // 3)
            return carry

        lax.fori_loop(1, NU // UPI, grp_body, 0)

        mod_part(16, 48, 32)
        for cp in cp_late:
            cp.wait()
        mem_s[...] = m0_s[...].astype(F32)
        xv = xbuf[pl.ds(PAD + PRO, XR), :].astype(F32)
        hn_s[...] = _ln_mod(xv, mod_row(0, XR), mod_row(1, XR))

    pl.run_scoped(
        prologue,
        pltpu.VMEM((NU, D, DH), U32),
        pltpu.VMEM((48, D, 128), BF16),
        pltpu.VMEM((PRO, D), F32),
    )

    def rest(w1_s, w3_s, w2_s, oring):
        w132 = w1_s.bitcast(U32)
        w332 = w3_s.bitcast(U32)
        w232 = w2_s.bitcast(U32)
        q32 = qring.bitcast(U32)
        k32 = kring.bitcast(U32)
        v32 = vring.bitcast(U32)

        cp_w1 = [pltpu.make_async_copy(w1_hbm.at[:, pl.ds(f * 128, 128)],
                                       w1_s.at[f], sems.at[SEM_FFN])
                 for f in range(NF)]
        cp_w3 = [pltpu.make_async_copy(w3_hbm.at[:, pl.ds(f * 128, 128)],
                                       w3_s.at[f], sems.at[SEM_FFN])
                 for f in range(NF)]
        cp_w2 = [pltpu.make_async_copy(w2_hbm.at[:, pl.ds(c * 128, 128)],
                                       w2_s.at[c], sems.at[SEM_FFN])
                 for c in range(NC)]
        for cp in cp_w1 + cp_w3 + cp_w2:
            cp.start()

        oring[:, pl.ds(OOFF - XR, XR), :] = jnp.zeros((H, XR, DH), BF16)

        def post_attn(a, r, n):
            x1 = xbuf[pl.ds(r, n), :].astype(F32) + mod_row(2, n) * a
            x1 = x1.astype(BF16)
            xbuf[pl.ds(r, n), :] = x1
            hbuf[pl.ds(r, n), :] = _ln_mod(
                x1.astype(F32), mod_row(3, n), mod_row(4, n)).astype(BF16)

        row = lax.broadcasted_iota(jnp.int32, (NP, NP), 0)
        col = lax.broadcasted_iota(jnp.int32, (NP, NP), 1)

        def second(i):
            return ((i >= SEG) & (i < 2 * SEG)) | (i >= 2 * SEG + M)

        same = second(row) == second(col)
        mask = same & ((row >= 2 * SEG) | (col >= 2 * SEG) | (col <= row))
        fill = jnp.where(same, -1e9, -jnp.inf).astype(F32)

        def step(s, carry, mem, split, maybe_last):
            lhs_c = [jnp.concatenate([hn_s[:, pl.ds(c * 128, 128)], mem[c]],
                                     axis=0).astype(BF16) for c in range(NC)]
            lhs = jnp.concatenate(lhs_c, axis=1)

            post_attn(ax_s[...], pl.multiple_of(XR * s, 8), XR)
            rn = pl.multiple_of(
                PAD + jnp.minimum(PRO + XR * (s + 1), S - XR), 8)
            hn_s[...] = _ln_mod(xbuf[pl.ds(rn, XR), :].astype(F32),
                                mod_row(0, XR), mod_row(1, XR))

            wp, rp, op, ow = carry
            wpos = [pl.multiple_of(_wrap(wp + 8 * j, RING), 8)
                    for j in range(XR // 8)]
            rpos = pl.multiple_of(rp, SEG // 2)
            opos = [pl.multiple_of(_wrap(op + 8 * j, ORING), 8)
                    for j in range(XR // 8 + 1)]
            owr = pl.multiple_of(ow, SEG)

            tails = {}
            xs = {}
            ps = {}
            lhs_o = {}

            def load(j, p):
                r32 = (q32, k32, v32)[j]
                xs[j, p] = [
                    pltpu.bitcast(r32[h, pl.ds(rpos, SEG // 2), :], BF16)
                    for h in (2 * p, 2 * p + 1)]

            def operand(j, p):
                tail = jnp.concatenate(
                    [tails.pop((j, 2 * p)), tails.pop((j, 2 * p + 1))], axis=0)
                return jnp.concatenate(
                    xs.pop((j, p)) + [tail.astype(BF16)], axis=0)

            low = {}
            if split:
                lhs_lo = jnp.concatenate(lhs_c[:NC // 2], axis=1)
                lhs_hi = jnp.concatenate(lhs_c[NC // 2:], axis=1)
                for h in range(2):
                    for j, w32 in enumerate((wq32, wk32, wv32)):
                        low[j, h] = _dot(lhs_lo, pltpu.bitcast(
                            w32[h, pl.ds(0, D // 4), :], BF16))

            def proj(h):
                for j, (w32, ring) in enumerate(
                        ((wq32, qring), (wk32, kring), (wv32, vring))):
                    if (j, h) in low:
                        t = _dot(lhs_hi, pltpu.bitcast(
                            w32[h, pl.ds(D // 4, D // 4), :], BF16)) + low[j, h]
                    else:
                        t = _dot(lhs, _w(w32, h))
                    for i in range(XR // 8):
                        ring[h, pl.ds(wpos[i], 8), :] = (
                            t[8 * i:8 * i + 8].astype(BF16))
                    tails[j, h] = t[XR:]

            def qk(p):
                sc = lax.dot_general(operand(0, p), operand(1, p),
                                     (((1,), (1,)), ((), ())),
                                     preferred_element_type=F32)
                sc = jnp.where(mask, sc * SCALE, fill)
                mx = jnp.max(sc, axis=-1, keepdims=True)
                e = jnp.exp(sc - mx)
                l = jnp.sum(e, axis=-1, keepdims=True)
                ps[p] = (e * pl.reciprocal(l, approx=True)).astype(BF16)

            def pv(p):
                o = _dot(ps.pop(p), operand(2, p))
                for i, h in enumerate((2 * p, 2 * p + 1)):
                    ox = [oring[h, pl.ds(opos[k], 8), :] for k in range(XR // 8)]
                    om = o[2 * SEG + M * i:2 * SEG + M * (i + 1)]
                    if maybe_last:
                        om = jnp.where(
                            s == NSEG - 1,
                            oring[h, pl.ds(opos[3], 8), :].astype(F32), om)
                    last = jnp.concatenate(
                        [ox[2].astype(F32), om], axis=0).astype(BF16)
                    lhs_o[h] = jnp.concatenate([ox[0], ox[1], last], axis=0)
                for i, h in enumerate((2 * p, 2 * p + 1)):
                    oring[h, pl.ds(owr, SEG), :] = (
                        o[SEG * i:SEG * (i + 1)].astype(BF16))

            def wo_part(c, h0, h1):
                lo = jnp.concatenate([lhs_o[h] for h in range(h0, h1)], axis=1)
                w = pltpu.bitcast(wo32[c, pl.ds(h0 * 64, (h1 - h0) * 64), :], BF16)
                return _dot(lo, w)

            NPR = H // 2
            for t in range(NPR):
                if t >= 1:
                    load(0, t - 1)
                    load(1, t - 1)
                proj(2 * t)
                if t >= 1:
                    qk(t - 1)
                if t >= 2:
                    load(2, t - 2)
                proj(2 * t + 1)
                if t >= 2:
                    pv(t - 2)
            HA = H - 4
            acc = {}
            load(0, NPR - 1)
            load(1, NPR - 1)
            load(2, NPR - 2)
            acc[0] = wo_part(0, 0, HA)
            qk(NPR - 1)
            acc[1] = wo_part(1, 0, HA)
            pv(NPR - 2)
            load(2, NPR - 1)
            for c in (2, 3, 4):
                acc[c] = wo_part(c, 0, HA)
            pv(NPR - 1)
            for c in (5, 6, 7):
                acc[c] = wo_part(c, 0, HA)
            mem_new = []
            for c in range(NC):
                a = wo_part(c, HA, H) + acc[c]
                ax_s[:, pl.ds(c * 128, 128)] = a[:XR]
                mem_new.append(a[XR:])
            return (_wrap(wp + XR, RING), _wrap(rp + SEG // 2, RING // 2),
                    _wrap(op + XR, ORING), _wrap(ow + SEG, ORING)), mem_new

        def steps(i, carry):
            mem = [mem_s[:, pl.ds(c * 128, 128)] for c in range(NC)]
            for u in range(UNROLL):
                carry, mem = step(i * UNROLL + u, carry, mem, split=u > 0,
                                  maybe_last=u == UNROLL - 1)
            for c in range(NC):
                mem_s[:, pl.ds(c * 128, 128)] = mem[c]
            return carry

        lax.fori_loop(0, NSEG // UNROLL, steps,
                      (jnp.int32(PRO), jnp.int32(0), jnp.int32(OOFF - XR),
                       jnp.int32(OOFF)))

        post_attn(jnp.concatenate([ax_s[...], mem_s[...]], axis=0),
                  XR * NSEG, XR + M)
        done = XR * (NSEG - 1) + M
        o32 = oring.bitcast(U32)

        def wo_bulk(i):
            p = pl.multiple_of(((done + OOFF) % ORING + i * WB) // 2, 8)
            lo = jnp.concatenate(
                [pltpu.bitcast(o32[h, pl.ds(p, WB // 2), :], BF16)
                 for h in range(H)], axis=1)
            a = jnp.concatenate(
                [_dot(lo, _w(wo32, c)) for c in range(NC)], axis=1)
            post_attn(a, pl.multiple_of(PAD + done + i * WB, 16), WB)

        for cp in cp_w1 + cp_w3 + cp_w2:
            cp.wait()

        def cp_out(i):
            r = i * FB
            rb = PAD + r
            if not isinstance(i, int):
                r = pl.multiple_of(r, FB)
                rb = pl.multiple_of(rb, 8)
            return pltpu.make_async_copy(xbuf.at[pl.ds(rb, FB)],
                                         out_hbm.at[pl.ds(r, FB)],
                                         sems.at[SEM_OUT])

        def ffn_body(i, carry, with_wo):
            r = pl.multiple_of(PAD + i * FB, 16)
            hv = hbuf[pl.ds(r, FB), :]
            if with_wo:
                wo_bulk(i)
            act = []
            for f in range(NF):
                g = _dot(hv, _w(w132, f))
                u = _dot(hv, _w(w332, f))
                act.append((g * jax.nn.sigmoid(g) * u).astype(BF16))
            av = jnp.concatenate(act, axis=1)
            for c in range(NC):
                y = _dot(av, _w(w232, c))
                cs = pl.ds(c * 128, 128)
                x2 = xbuf[pl.ds(r, FB), cs].astype(F32) + mod_row(5, FB, cs) * y
                xbuf[pl.ds(r, FB), cs] = x2.astype(BF16)
            cp_out(i).start()
            return carry

        lax.fori_loop(0, NWB, functools.partial(ffn_body, with_wo=True), 0)
        lax.fori_loop(NWB, S // FB,
                      functools.partial(ffn_body, with_wo=False), 0)
        for i in range(S // FB):
            cp_out(i).wait()

    pl.run_scoped(
        rest,
        pltpu.VMEM((NF, D, 128), BF16),
        pltpu.VMEM((NF, D, 128), BF16),
        pltpu.VMEM((NC, F, 128), BF16),
        pltpu.VMEM((H, ORING, DH), BF16),
    )


@functools.partial(jax.jit, static_argnames=("A_seg_len",))
def pallas_adaLN_cond__memory_aug_recurrent_mem_tr__glu_gated_swiglu__prompt_kernel(
    A_x: jax.Array,
    A_mem0: jax.Array,
    A_Wq: jax.Array,
    A_Wk: jax.Array,
    A_Wv: jax.Array,
    A_Wo: jax.Array,
    A_seg_len,
    B_x: jax.Array,
    B_w1: jax.Array,
    B_w3: jax.Array,
    B_w2: jax.Array,
    c: jax.Array,
    w_mod: jax.Array,
):
    del B_x
    assert A_seg_len == SEG
    assert A_x.shape == (1, S, D) and A_mem0.shape == (1, M, D)
    assert A_Wq.shape == (D, H, DH) and B_w1.shape == (D, F)

    any_spec = pl.BlockSpec(memory_space=pl.ANY)
    out = pl.pallas_call(
        _kernel,
        out_shape=jax.ShapeDtypeStruct((S, D), BF16),
        in_specs=[any_spec] * 11,
        out_specs=any_spec,
        scratch_shapes=[
            pltpu.VMEM((H, D // 2, DH), U32),
            pltpu.VMEM((H, D // 2, DH), U32),
            pltpu.VMEM((H, D // 2, DH), U32),
            pltpu.VMEM((NC, H * DH, 128), BF16),
            pltpu.VMEM((2, PAD + S, D), BF16),
            pltpu.VMEM((H, RING, DH), BF16),
            pltpu.VMEM((H, RING, DH), BF16),
            pltpu.VMEM((H, RING, DH), BF16),
            pltpu.VMEM((6 * 8, D), F32),
            pltpu.VMEM((M, D), F32),
            pltpu.VMEM((XR, D), F32),
            pltpu.VMEM((XR, D), F32),
            pltpu.VMEM((1, D), BF16),
            pltpu.VMEM((M, D), BF16),
            pltpu.SemaphoreType.DMA((NSEMS,)),
        ],
        compiler_params=pltpu.CompilerParams(
            vmem_limit_bytes=120 * 1024 * 1024),
        name="adaln_memtr_swiglu",
    )(
        A_x.reshape(S, D),
        A_mem0.reshape(M, D),
        A_Wq, A_Wk, A_Wv,
        A_Wo.reshape(H * DH, D),
        B_w1, B_w3, B_w2, c, w_mod,
    )
    return out.reshape(1, S, D)
```

```python
import functools

import jax
import jax.numpy as jnp
from jax import lax
import jax.experimental.pallas as pl
import jax.experimental.pallas.tpu as pltpu

BF16 = jnp.bfloat16
F32 = jnp.float32
U32 = jnp.uint32

S = 2048
D = 1024
H = 32
DH = 128
F = 3584
M = 8
SEG = 32
NSEG = S // SEG
XR = 24
PRO = S - XR * NSEG
RING = 544
ORING = 576
OOFF = 256
PAD = 48
NC = D // 128
NF = F // 128
FB = 128
NWB = 3
WB = 176
UNROLL = 4
NU = 3 * H // 2
UPI = 6
NUA = 12
NUZ = 12
NUG = 4
NP = 2 * (SEG + M)
EPS = 1e-5
SEM_FIRST, SEM_LATE, SEM_MID, SEM_FFN, SEM_OUT = 0, 1, 2, 3, 4
SEM_CA = 5
SEM_U0 = SEM_CA + 2
U0_GROUP = (0, 1, 2, 3, 4, 5, 5, 5, 6, 6, 6, 6, 6)
SEM_SA = SEM_U0 + U0_GROUP[NUG]
SEM_IT = SEM_U0 + U0_GROUP[-1] + 1 - NUA // UPI
NSEMS = SEM_IT + NU // UPI
SCALE = DH ** -0.5


def _dot(a, b):
    return jnp.dot(a, b, preferred_element_type=F32)


def _w(ref32, i):
    return pltpu.bitcast(ref32[i], BF16)


def _wrap(i, n):
    return jnp.where(i >= n, i - n, i)


def _ln(x):
    mu = jnp.mean(x, axis=-1, keepdims=True)
    xc = x - mu
    var = jnp.mean(xc * xc, axis=-1, keepdims=True)
    return xc * lax.rsqrt(var + EPS)


def _ln_mod(x, shift, scale1):
    return _ln(x) * scale1 + shift


def _kernel(x_hbm, mem0_hbm, wq_hbm, wk_hbm, wv_hbm, wo_hbm, w1_hbm, w3_hbm,
            w2_hbm, c_hbm, wmod_hbm, out_hbm,
            wq32, wk32, wv32, wo_s, xh, qring, kring, vring,
            mod_s, mem_s, ax_s, hn_s, c_s, m0_s, sems):
    wo32 = wo_s.bitcast(U32)
    xbuf = xh.at[0]
    hbuf = xh.at[1]

    cp_x0 = pltpu.make_async_copy(x_hbm.at[pl.ds(0, PRO)],
                                  xbuf.at[pl.ds(PAD, PRO)], sems.at[SEM_FIRST])
    cp_c = pltpu.make_async_copy(c_hbm, c_s, sems.at[SEM_FIRST])
    cp_mid = [
        pltpu.make_async_copy(mem0_hbm, m0_s, sems.at[SEM_MID]),
        pltpu.make_async_copy(x_hbm.at[pl.ds(PRO, SEG)],
                              xbuf.at[pl.ds(PAD + PRO, SEG)],
                              sems.at[SEM_MID]),
    ]
    cp_late = [
        pltpu.make_async_copy(x_hbm.at[pl.ds(PRO + SEG, S - PRO - SEG)],
                              xbuf.at[pl.ds(PAD + PRO + SEG, S - PRO - SEG)],
                              sems.at[SEM_LATE]),
    ] + [pltpu.make_async_copy(wo_hbm.at[:, pl.ds(c * 128, 128)],
                               wo_s.at[c], sems.at[SEM_LATE])
         for c in range(NC)]

    def mod_row(i, n, cols=slice(None)):
        return jnp.concatenate([mod_s[pl.ds(8 * i, 8), cols]] * (n // 8), axis=0)

    def prologue(st, wm_s, wm2_s, xn_s, g_s, tmp_s):
        wm32 = wm_s.bitcast(U32)
        srcs = (wq_hbm.bitcast(U32), wk_hbm.bitcast(U32), wv_hbm.bitcast(U32))
        dsts = (wq32, wk32, wv32)
        rings = (qring, kring, vring)

        def cp_st(j, s, sem):
            return pltpu.make_async_copy(srcs[j].at[:, s, :], st.at[3 * s + j],
                                         sems.at[sem])

        def cp_unit(u):
            sem = (SEM_U0 + U0_GROUP[u] if u <= NUA
                   else SEM_IT + (u - 1) // UPI)
            return cp_st(u % 3, u // 3, sem)

        def cp_wm(i):
            sem = SEM_SA if i < 8 else SEM_CA + (i - 8) // 4
            return pltpu.make_async_copy(wmod_hbm.at[:, pl.ds(i * 128, 128)],
                                         wm_s.at[i], sems.at[sem])

        cp_wm2 = pltpu.make_async_copy(wmod_hbm.at[:, pl.ds(2 * D, 4 * D)],
                                       wm2_s, sems.at[SEM_MID])

        cp_c.start()
        cp_x0.start()
        for i in range(8, 16):
            cp_wm(i).start()
        for u in range(NUG):
            cp_unit(u).start()
        for i in range(8):
            cp_wm(i).start()
        for u in range(NUG, NU):
            cp_unit(u).start()
        for cp in cp_mid + [cp_wm2]:
            cp.start()

        xbuf[pl.ds(0, PAD), :] = jnp.zeros((PAD, D), BF16)
        ax_s[...] = jnp.zeros((XR, D), F32)

        cp_c.wait()
        cp_x0.wait()
        cf = c_s[...].astype(F32)
        sc = (cf * jax.nn.sigmoid(cf)).astype(BF16)
        sc8 = jnp.broadcast_to(sc, (8, D))

        def ln_body(i, carry):
            r = pl.multiple_of(i * 64, 64)
            xv = xbuf[pl.ds(pl.multiple_of(PAD + r, 8), 64), :].astype(F32)
            xn_s[pl.ds(r, 64), :] = _ln(xv)
            return carry

        lax.fori_loop(0, PRO // 64, ln_body, 0)

        def mod_slab(i):
            k, c = divmod(i, NC)
            w = (_w(wm32, i) if i < 16
                 else wm2_s[:, pl.ds((i - 16) * 128, 128)])
            part = _dot(sc8, w)
            if k in (1, 4):
                part = part + 1.0
            mod_s[pl.ds(8 * k, 8), pl.ds(c * 128, 128)] = part

        for c0 in (8, 12):
            for i in range(c0, c0 + 4):
                cp_wm(i).wait()
            for i in range(c0, c0 + 4):
                mod_slab(i)

        def relayout(j, s):
            u = 3 * s + j
            for db in range(8):
                ev = st[u, pl.ds(db * 128, 64, stride=2), :]
                od = st[u, pl.ds(db * 128 + 1, 64, stride=2), :]
                rows = pl.ds(db * 64, 64)
                dsts[j][2 * s, rows, :] = (ev & U32(0xFFFF)) | (od << 16)
                dsts[j][2 * s + 1, rows, :] = (ev >> 16) | (od & U32(0xFFFF0000))

        def bulk(j, s, extras=(), mbs=range(PRO // 128)):
            extras = list(extras)
            for mb in mbs:
                lhs = hbuf[pl.ds(PAD + mb * 128, 128), :]
                for hh in range(2):
                    h = 2 * s + hh
                    rings[j][h, pl.ds(mb * 128, 128), :] = (
                        _dot(lhs, _w(dsts[j], h)).astype(BF16))
                    if extras:
                        extras.pop(0)()

        def bulk_g(u, mbs):
            for mb in mbs:
                rows = pl.ds(mb * 128, 128)
                if u == 0:
                    lhs = (xn_s[rows, :] * mod_row(1, 128)).astype(BF16)
                    g_s[rows, :] = lhs
                else:
                    lhs = g_s[rows, :]
                for hh in range(2):
                    tmp_s[2 * u + hh, rows, :] = _dot(
                        lhs, _w(dsts[u % 3], 2 * (u // 3) + hh))

        def add_shift(u, hh):
            h = 2 * (u // 3) + hh
            b = _dot(mod_row(0, 8).astype(BF16), _w(dsts[u % 3], h))
            rings[u % 3][h, pl.ds(0, PRO), :] = (
                tmp_s[2 * u + hh] + jnp.concatenate([b] * (PRO // 8), axis=0)
            ).astype(BF16)

        def wait_group(g):
            if g == U0_GROUP[NUG]:
                for i in range(8):
                    cp_wm(i).wait()
            for v in range(NUA + 1):
                if U0_GROUP[v] == g:
                    cp_unit(v).wait()

        def relayout_u(u):
            relayout(u % 3, u // 3)

        wait_group(0)
        relayout_u(0)
        bulk_g(0, (0, 1))
        wait_group(1)
        relayout_u(1)
        bulk_g(0, (2, 3))
        wait_group(2)
        relayout_u(2)
        bulk_g(1, range(4))
        wait_group(3)
        relayout_u(3)
        bulk_g(2, range(4))
        bulk_g(3, (0, 1, 2))
        wait_group(4)
        relayout_u(4)
        for i in range(8):
            mod_slab(i)
        bulk_g(3, (3,))
        for mb in range(PRO // 128):
            rows = pl.ds(mb * 128, 128)
            hbuf[pl.ds(PAD + mb * 128, 128), :] = (
                xn_s[rows, :] * mod_row(1, 128) + mod_row(0, 128)).astype(BF16)
        shifts = [functools.partial(add_shift, v, hh)
                  for v in range(NUG) for hh in range(2)]
        bulk(4 % 3, 4 // 3, shifts, mbs=(0, 1, 2))
        wait_group(5)
        relayout_u(5)
        bulk(4 % 3, 4 // 3, shifts[6:], mbs=(3,))
        for u in range(5, NUA):
            if U0_GROUP[u + 1] != U0_GROUP[u]:
                wait_group(U0_GROUP[u + 1])
            relayout_u(u + 1)
            bulk(u % 3, u // 3)

        def grp_body(it, carry):
            s0 = it * (UPI // 3)

            @pl.when(it == NUA // UPI)
            def _():
                for cp in cp_late:
                    cp.start()

            for u in range(1, UPI + 1):
                cp_st(u % 3, s0 + u // 3, SEM_IT + it).wait()
            for u in range(UPI):
                relayout((u + 1) % 3, s0 + (u + 1) // 3)
                bulk(u % 3, s0 + u // 3)
            return carry

        lax.fori_loop(NUA // UPI, (NU - NUZ) // UPI, grp_body, 0)

        for u in range(NU - NUZ + 1, NU):
            cp_unit(u).wait()
        for cp in cp_mid + [cp_wm2]:
            cp.wait()
        mem_s[...] = m0_s[...].astype(F32)
        xv = xbuf[pl.ds(PAD + PRO, XR), :].astype(F32)
        hn_s[...] = _ln_mod(xv, mod_row(0, XR), mod_row(1, XR))
        for u in range(NU - NUZ, NU):
            if u + 1 < NU:
                relayout_u(u + 1)
            i0 = 16 + 4 * (u - (NU - NUZ))
            extras = []
            for i in range(i0, min(i0 + 4, 48)):
                extras += [functools.partial(mod_slab, i), lambda: None]
            bulk(u % 3, u // 3, extras)
        for cp in cp_late:
            cp.wait()

    pl.run_scoped(
        prologue,
        pltpu.VMEM((NU, D, DH), U32),
        pltpu.VMEM((16, D, 128), BF16),
        pltpu.VMEM((D, 4 * D), BF16),
        pltpu.VMEM((PRO, D), F32),
        pltpu.VMEM((PRO, D), BF16),
        pltpu.VMEM((2 * NUG, PRO, DH), F32),
    )

    def rest(w1_s, w3_s, w2_s, oring):
        w132 = w1_s.bitcast(U32)
        w332 = w3_s.bitcast(U32)
        w232 = w2_s.bitcast(U32)
        q32 = qring.bitcast(U32)
        k32 = kring.bitcast(U32)
        v32 = vring.bitcast(U32)

        cp_w1 = [pltpu.make_async_copy(w1_hbm.at[:, pl.ds(f * 128, 128)],
                                       w1_s.at[f], sems.at[SEM_FFN])
                 for f in range(NF)]
        cp_w3 = [pltpu.make_async_copy(w3_hbm.at[:, pl.ds(f * 128, 128)],
                                       w3_s.at[f], sems.at[SEM_FFN])
                 for f in range(NF)]
        cp_w2 = [pltpu.make_async_copy(w2_hbm.at[:, pl.ds(c * 128, 128)],
                                       w2_s.at[c], sems.at[SEM_FFN])
                 for c in range(NC)]
        for cp in cp_w1 + cp_w3 + cp_w2:
            cp.start()

        oring[:, pl.ds(OOFF - XR, XR), :] = jnp.zeros((H, XR, DH), BF16)

        def post_attn(a, r, n):
            x1 = xbuf[pl.ds(r, n), :].astype(F32) + mod_row(2, n) * a
            x1 = x1.astype(BF16)
            xbuf[pl.ds(r, n), :] = x1
            hbuf[pl.ds(r, n), :] = _ln_mod(
                x1.astype(F32), mod_row(3, n), mod_row(4, n)).astype(BF16)

        row = lax.broadcasted_iota(jnp.int32, (NP, NP), 0)
        col = lax.broadcasted_iota(jnp.int32, (NP, NP), 1)

        def second(i):
            return ((i >= SEG) & (i < 2 * SEG)) | (i >= 2 * SEG + M)

        same = second(row) == second(col)
        mask = same & ((row >= 2 * SEG) | (col >= 2 * SEG) | (col <= row))
        fill = jnp.where(same, -1e9, -jnp.inf).astype(F32)

        def step(s, carry, mem, split, maybe_last):
            lhs_c = [jnp.concatenate([hn_s[:, pl.ds(c * 128, 128)], mem[c]],
                                     axis=0).astype(BF16) for c in range(NC)]
            lhs = jnp.concatenate(lhs_c, axis=1)

            post_attn(ax_s[...], pl.multiple_of(XR * s, 8), XR)
            rn = pl.multiple_of(
                PAD + jnp.minimum(PRO + XR * (s + 1), S - XR), 8)
            hn_s[...] = _ln_mod(xbuf[pl.ds(rn, XR), :].astype(F32),
                                mod_row(0, XR), mod_row(1, XR))

            wp, rp, op, ow = carry
            wpos = [pl.multiple_of(_wrap(wp + 8 * j, RING), 8)
                    for j in range(XR // 8)]
            rpos = pl.multiple_of(rp, SEG // 2)
            opos = [pl.multiple_of(_wrap(op + 8 * j, ORING), 8)
                    for j in range(XR // 8 + 1)]
            owr = pl.multiple_of(ow, SEG)

            tails = {}
            xs = {}
            ps = {}
            lhs_o = {}

            def load(j, p):
                r32 = (q32, k32, v32)[j]
                xs[j, p] = [
                    pltpu.bitcast(r32[h, pl.ds(rpos, SEG // 2), :], BF16)
                    for h in (2 * p, 2 * p + 1)]

            def operand(j, p):
                tail = jnp.concatenate(
                    [tails.pop((j, 2 * p)), tails.pop((j, 2 * p + 1))], axis=0)
                return jnp.concatenate(
                    xs.pop((j, p)) + [tail.astype(BF16)], axis=0)

            low = {}
            if split:
                lhs_lo = jnp.concatenate(lhs_c[:NC // 2], axis=1)
                lhs_hi = jnp.concatenate(lhs_c[NC // 2:], axis=1)
                for h in range(2):
                    for j, w32 in enumerate((wq32, wk32, wv32)):
                        low[j, h] = _dot(lhs_lo, pltpu.bitcast(
                            w32[h, pl.ds(0, D // 4), :], BF16))

            def proj(h):
                for j, (w32, ring) in enumerate(
                        ((wq32, qring), (wk32, kring), (wv32, vring))):
                    if (j, h) in low:
                        t = _dot(lhs_hi, pltpu.bitcast(
                            w32[h, pl.ds(D // 4, D // 4), :], BF16)) + low[j, h]
                    else:
                        t = _dot(lhs, _w(w32, h))
                    for i in range(XR // 8):
                        ring[h, pl.ds(wpos[i], 8), :] = (
                            t[8 * i:8 * i + 8].astype(BF16))
                    tails[j, h] = t[XR:]

            def qk(p):
                sc = lax.dot_general(operand(0, p), operand(1, p),
                                     (((1,), (1,)), ((), ())),
                                     preferred_element_type=F32)
                sc = jnp.where(mask, sc * SCALE, fill)
                mx = jnp.max(sc, axis=-1, keepdims=True)
                e = jnp.exp(sc - mx)
                l = jnp.sum(e, axis=-1, keepdims=True)
                ps[p] = (e * pl.reciprocal(l, approx=True)).astype(BF16)

            def pv(p):
                o = _dot(ps.pop(p), operand(2, p))
                for i, h in enumerate((2 * p, 2 * p + 1)):
                    ox = [oring[h, pl.ds(opos[k], 8), :] for k in range(XR // 8)]
                    om = o[2 * SEG + M * i:2 * SEG + M * (i + 1)]
                    if maybe_last:
                        om = jnp.where(
                            s == NSEG - 1,
                            oring[h, pl.ds(opos[3], 8), :].astype(F32), om)
                    last = jnp.concatenate(
                        [ox[2].astype(F32), om], axis=0).astype(BF16)
                    lhs_o[h] = jnp.concatenate([ox[0], ox[1], last], axis=0)
                for i, h in enumerate((2 * p, 2 * p + 1)):
                    oring[h, pl.ds(owr, SEG), :] = (
                        o[SEG * i:SEG * (i + 1)].astype(BF16))

            def wo_part(c, h0, h1):
                lo = jnp.concatenate([lhs_o[h] for h in range(h0, h1)], axis=1)
                w = pltpu.bitcast(wo32[c, pl.ds(h0 * 64, (h1 - h0) * 64), :], BF16)
                return _dot(lo, w)

            NPR = H // 2
            for t in range(NPR):
                if t >= 1:
                    load(0, t - 1)
                    load(1, t - 1)
                proj(2 * t)
                if t >= 1:
                    qk(t - 1)
                if t >= 2:
                    load(2, t - 2)
                proj(2 * t + 1)
                if t >= 2:
                    pv(t - 2)
            HA = H - 4
            acc = {}
            load(0, NPR - 1)
            load(1, NPR - 1)
            load(2, NPR - 2)
            acc[0] = wo_part(0, 0, HA)
            qk(NPR - 1)
            acc[1] = wo_part(1, 0, HA)
            pv(NPR - 2)
            load(2, NPR - 1)
            for c in (2, 3, 4):
                acc[c] = wo_part(c, 0, HA)
            pv(NPR - 1)
            for c in (5, 6, 7):
                acc[c] = wo_part(c, 0, HA)
            mem_new = []
            for c in range(NC):
                a = wo_part(c, HA, H) + acc[c]
                ax_s[:, pl.ds(c * 128, 128)] = a[:XR]
                mem_new.append(a[XR:])
            return (_wrap(wp + XR, RING), _wrap(rp + SEG // 2, RING // 2),
                    _wrap(op + XR, ORING), _wrap(ow + SEG, ORING)), mem_new

        def steps(i, carry):
            mem = [mem_s[:, pl.ds(c * 128, 128)] for c in range(NC)]
            for u in range(UNROLL):
                carry, mem = step(i * UNROLL + u, carry, mem, split=u > 0,
                                  maybe_last=u == UNROLL - 1)
            for c in range(NC):
                mem_s[:, pl.ds(c * 128, 128)] = mem[c]
            return carry

        lax.fori_loop(0, NSEG // UNROLL, steps,
                      (jnp.int32(PRO), jnp.int32(0), jnp.int32(OOFF - XR),
                       jnp.int32(OOFF)))

        post_attn(jnp.concatenate([ax_s[...], mem_s[...]], axis=0),
                  XR * NSEG, XR + M)
        done = XR * (NSEG - 1) + M
        o32 = oring.bitcast(U32)

        def wo_bulk(i):
            p = pl.multiple_of(((done + OOFF) % ORING + i * WB) // 2, 8)
            lo = jnp.concatenate(
                [pltpu.bitcast(o32[h, pl.ds(p, WB // 2), :], BF16)
                 for h in range(H)], axis=1)
            a = jnp.concatenate(
                [_dot(lo, _w(wo32, c)) for c in range(NC)], axis=1)
            post_attn(a, pl.multiple_of(PAD + done + i * WB, 16), WB)

        for cp in cp_w1 + cp_w3 + cp_w2:
            cp.wait()

        def cp_out(i):
            r = i * FB
            rb = PAD + r
            if not isinstance(i, int):
                r = pl.multiple_of(r, FB)
                rb = pl.multiple_of(rb, 8)
            return pltpu.make_async_copy(xbuf.at[pl.ds(rb, FB)],
                                         out_hbm.at[pl.ds(r, FB)],
                                         sems.at[SEM_OUT])

        def ffn_body(i, carry, with_wo):
            r = pl.multiple_of(PAD + i * FB, 16)
            hv = hbuf[pl.ds(r, FB), :]
            if with_wo:
                wo_bulk(i)
            act = []
            for f in range(NF):
                g = _dot(hv, _w(w132, f))
                u = _dot(hv, _w(w332, f))
                act.append((g * jax.nn.sigmoid(g) * u).astype(BF16))
            av = jnp.concatenate(act, axis=1)
            for c in range(NC):
                y = _dot(av, _w(w232, c))
                cs = pl.ds(c * 128, 128)
                x2 = xbuf[pl.ds(r, FB), cs].astype(F32) + mod_row(5, FB, cs) * y
                xbuf[pl.ds(r, FB), cs] = x2.astype(BF16)
            cp_out(i).start()
            return carry

        lax.fori_loop(0, NWB, functools.partial(ffn_body, with_wo=True), 0)
        lax.fori_loop(NWB, S // FB,
                      functools.partial(ffn_body, with_wo=False), 0)
        for i in range(S // FB):
            cp_out(i).wait()

    pl.run_scoped(
        rest,
        pltpu.VMEM((NF, D, 128), BF16),
        pltpu.VMEM((NF, D, 128), BF16),
        pltpu.VMEM((NC, F, 128), BF16),
        pltpu.VMEM((H, ORING, DH), BF16),
    )


@functools.partial(jax.jit, static_argnames=("A_seg_len",))
def pallas_adaLN_cond__memory_aug_recurrent_mem_tr__glu_gated_swiglu__prompt_kernel(
    A_x: jax.Array,
    A_mem0: jax.Array,
    A_Wq: jax.Array,
    A_Wk: jax.Array,
    A_Wv: jax.Array,
    A_Wo: jax.Array,
    A_seg_len,
    B_x: jax.Array,
    B_w1: jax.Array,
    B_w3: jax.Array,
    B_w2: jax.Array,
    c: jax.Array,
    w_mod: jax.Array,
):
    del B_x
    assert A_seg_len == SEG
    assert A_x.shape == (1, S, D) and A_mem0.shape == (1, M, D)
    assert A_Wq.shape == (D, H, DH) and B_w1.shape == (D, F)

    any_spec = pl.BlockSpec(memory_space=pl.ANY)
    out = pl.pallas_call(
        _kernel,
        out_shape=jax.ShapeDtypeStruct((S, D), BF16),
        in_specs=[any_spec] * 11,
        out_specs=any_spec,
        scratch_shapes=[
            pltpu.VMEM((H, D // 2, DH), U32),
            pltpu.VMEM((H, D // 2, DH), U32),
            pltpu.VMEM((H, D // 2, DH), U32),
            pltpu.VMEM((NC, H * DH, 128), BF16),
            pltpu.VMEM((2, PAD + S, D), BF16),
            pltpu.VMEM((H, RING, DH), BF16),
            pltpu.VMEM((H, RING, DH), BF16),
            pltpu.VMEM((H, RING, DH), BF16),
            pltpu.VMEM((6 * 8, D), F32),
            pltpu.VMEM((M, D), F32),
            pltpu.VMEM((XR, D), F32),
            pltpu.VMEM((XR, D), F32),
            pltpu.VMEM((1, D), BF16),
            pltpu.VMEM((M, D), BF16),
            pltpu.SemaphoreType.DMA((NSEMS,)),
        ],
        compiler_params=pltpu.CompilerParams(
            vmem_limit_bytes=120 * 1024 * 1024),
        name="adaln_memtr_swiglu",
    )(
        A_x.reshape(S, D),
        A_mem0.reshape(M, D),
        A_Wq, A_Wk, A_Wv,
        A_Wo.reshape(H * DH, D),
        B_w1, B_w3, B_w2, c, w_mod,
    )
    return out.reshape(1, S, D)
```

```python
import functools

import jax
import jax.numpy as jnp
from jax import lax
import jax.experimental.pallas as pl
import jax.experimental.pallas.tpu as pltpu

BF16 = jnp.bfloat16
F32 = jnp.float32
U32 = jnp.uint32

S = 2048
D = 1024
H = 32
DH = 128
F = 3584
M = 8
SEG = 32
NSEG = S // SEG
XR = 24
PRO = S - XR * NSEG
RING = 544
ORING = 576
OOFF = 256
PAD = 48
NC = D // 128
NF = F // 128
FB = 128
NWB = 3
WB = 176
UNROLL = 4
NU = 3 * H // 2
UPI = 6
NUA = 12
NUZ = 12
NUG = 4
NP = 2 * (SEG + M)
EPS = 1e-5
SEM_FIRST, SEM_LATE, SEM_MID, SEM_FFN, SEM_OUT = 0, 1, 2, 3, 4
SEM_CA = 5
SEM_U0 = SEM_CA + 2
U0_GROUP = (0, 1, 2, 3, 4, 5, 5, 5, 6, 6, 6, 6, 6)
SEM_SA = SEM_U0 + U0_GROUP[NUG]
SEM_IT = SEM_U0 + U0_GROUP[-1] + 1 - NUA // UPI
NSEMS = SEM_IT + NU // UPI
SCALE = DH ** -0.5


def _dot(a, b):
    return jnp.dot(a, b, preferred_element_type=F32)


def _w(ref32, i):
    return pltpu.bitcast(ref32[i], BF16)


def _wrap(i, n):
    return jnp.where(i >= n, i - n, i)


def _ln(x):
    mu = jnp.mean(x, axis=-1, keepdims=True)
    xc = x - mu
    var = jnp.mean(xc * xc, axis=-1, keepdims=True)
    return xc * lax.rsqrt(var + EPS)


def _ln_mod(x, shift, scale1):
    return _ln(x) * scale1 + shift


def _kernel(x_hbm, mem0_hbm, wq_hbm, wk_hbm, wv_hbm, wo_hbm, w1_hbm, w3_hbm,
            w2_hbm, c_hbm, wmod_hbm, out_hbm,
            wq32, wk32, wv32, wo_s, xh, qring, kring, vring,
            mod_s, mem_s, ax_s, hn_s, c_s, m0_s, sems):
    wo32 = wo_s.bitcast(U32)
    xbuf = xh.at[0]
    hbuf = xh.at[1]

    cp_x0 = pltpu.make_async_copy(x_hbm.at[pl.ds(0, PRO)],
                                  xbuf.at[pl.ds(PAD, PRO)], sems.at[SEM_FIRST])
    cp_c = pltpu.make_async_copy(c_hbm, c_s, sems.at[SEM_FIRST])
    cp_mid = [
        pltpu.make_async_copy(mem0_hbm, m0_s, sems.at[SEM_MID]),
        pltpu.make_async_copy(x_hbm.at[pl.ds(PRO, SEG)],
                              xbuf.at[pl.ds(PAD + PRO, SEG)],
                              sems.at[SEM_MID]),
    ]
    cp_late = [
        pltpu.make_async_copy(x_hbm.at[pl.ds(PRO + SEG, S - PRO - SEG)],
                              xbuf.at[pl.ds(PAD + PRO + SEG, S - PRO - SEG)],
                              sems.at[SEM_LATE]),
    ] + [pltpu.make_async_copy(wo_hbm.at[:, pl.ds(c * 128, 128)],
                               wo_s.at[c], sems.at[SEM_LATE])
         for c in range(NC)]

    def mod_row(i, n, cols=slice(None)):
        return jnp.concatenate([mod_s[pl.ds(8 * i, 8), cols]] * (n // 8), axis=0)

    def prologue(st, wm_s, xn_s, g_s, tmp_s):
        wm32 = wm_s.bitcast(U32)
        srcs = (wq_hbm.bitcast(U32), wk_hbm.bitcast(U32), wv_hbm.bitcast(U32))
        dsts = (wq32, wk32, wv32)
        rings = (qring, kring, vring)

        def cp_st(j, s, sem):
            return pltpu.make_async_copy(srcs[j].at[:, s, :], st.at[3 * s + j],
                                         sems.at[sem])

        def cp_unit(u):
            sem = (SEM_U0 + U0_GROUP[u] if u <= NUA
                   else SEM_IT + (u - 1) // UPI)
            return cp_st(u % 3, u // 3, sem)

        def cp_wm(i):
            sem = (SEM_SA if i < 8 else
                   SEM_CA + (i - 8) // 4 if i < 16 else SEM_MID)
            return pltpu.make_async_copy(wmod_hbm.at[:, pl.ds(i * 128, 128)],
                                         wm_s.at[i], sems.at[sem])

        cp_wm2 = [cp_wm(i) for i in range(16, 48)]

        cp_c.start()
        cp_x0.start()
        for i in range(8, 16):
            cp_wm(i).start()
        for u in range(NUG):
            cp_unit(u).start()
        for i in range(8):
            cp_wm(i).start()
        for u in range(NUG, NU):
            cp_unit(u).start()
        for cp in cp_mid:
            cp.start()

        xbuf[pl.ds(0, PAD), :] = jnp.zeros((PAD, D), BF16)
        ax_s[...] = jnp.zeros((XR, D), F32)

        cp_c.wait()
        cp_x0.wait()
        cf = c_s[...].astype(F32)
        sc = (cf * jax.nn.sigmoid(cf)).astype(BF16)
        sc8 = jnp.broadcast_to(sc, (8, D))

        def ln_body(i, carry):
            r = pl.multiple_of(i * 64, 64)
            xv = xbuf[pl.ds(pl.multiple_of(PAD + r, 8), 64), :].astype(F32)
            xn_s[pl.ds(r, 64), :] = _ln(xv)
            return carry

        lax.fori_loop(0, PRO // 64, ln_body, 0)

        def mod_slab(i):
            k, c = divmod(i, NC)
            part = _dot(sc8, _w(wm32, i))
            if k in (1, 4):
                part = part + 1.0
            mod_s[pl.ds(8 * k, 8), pl.ds(c * 128, 128)] = part

        for c0 in (8, 12):
            for i in range(c0, c0 + 4):
                cp_wm(i).wait()
            for i in range(c0, c0 + 4):
                mod_slab(i)

        def relayout(j, s):
            u = 3 * s + j
            for db in range(8):
                ev = st[u, pl.ds(db * 128, 64, stride=2), :]
                od = st[u, pl.ds(db * 128 + 1, 64, stride=2), :]
                rows = pl.ds(db * 64, 64)
                dsts[j][2 * s, rows, :] = (ev & U32(0xFFFF)) | (od << 16)
                dsts[j][2 * s + 1, rows, :] = (ev >> 16) | (od & U32(0xFFFF0000))

        def bulk(j, s, extras=(), mbs=range(PRO // 128)):
            extras = list(extras)
            for mb in mbs:
                lhs = hbuf[pl.ds(PAD + mb * 128, 128), :]
                for hh in range(2):
                    h = 2 * s + hh
                    rings[j][h, pl.ds(mb * 128, 128), :] = (
                        _dot(lhs, _w(dsts[j], h)).astype(BF16))
                    if extras:
                        extras.pop(0)()

        def bulk_g(u, mbs):
            for mb in mbs:
                rows = pl.ds(mb * 128, 128)
                if u == 0:
                    lhs = (xn_s[rows, :] * mod_row(1, 128)).astype(BF16)
                    g_s[rows, :] = lhs
                else:
                    lhs = g_s[rows, :]
                for hh in range(2):
                    tmp_s[2 * u + hh, rows, :] = _dot(
                        lhs, _w(dsts[u % 3], 2 * (u // 3) + hh))

        def add_shift(u, hh):
            h = 2 * (u // 3) + hh
            b = _dot(mod_row(0, 8).astype(BF16), _w(dsts[u % 3], h))
            rings[u % 3][h, pl.ds(0, PRO), :] = (
                tmp_s[2 * u + hh] + jnp.concatenate([b] * (PRO // 8), axis=0)
            ).astype(BF16)

        def wait_group(g):
            if g == U0_GROUP[NUG]:
                for i in range(8):
                    cp_wm(i).wait()
            for v in range(NUA + 1):
                if U0_GROUP[v] == g:
                    cp_unit(v).wait()

        def relayout_u(u):
            relayout(u % 3, u // 3)

        wait_group(0)
        relayout_u(0)
        bulk_g(0, (0, 1))
        wait_group(1)
        relayout_u(1)
        bulk_g(0, (2, 3))
        wait_group(2)
        relayout_u(2)
        bulk_g(1, range(4))
        wait_group(3)
        relayout_u(3)
        bulk_g(2, range(4))
        bulk_g(3, (0, 1, 2))
        wait_group(4)
        relayout_u(4)
        for i in range(8):
            mod_slab(i)
        bulk_g(3, (3,))
        for mb in range(PRO // 128):
            rows = pl.ds(mb * 128, 128)
            hbuf[pl.ds(PAD + mb * 128, 128), :] = (
                xn_s[rows, :] * mod_row(1, 128) + mod_row(0, 128)).astype(BF16)
        shifts = [functools.partial(add_shift, v, hh)
                  for v in range(NUG) for hh in range(2)]
        bulk(4 % 3, 4 // 3, shifts, mbs=(0, 1, 2))
        wait_group(5)
        relayout_u(5)
        bulk(4 % 3, 4 // 3, shifts[6:], mbs=(3,))
        for u in range(5, NUA):
            if U0_GROUP[u + 1] != U0_GROUP[u]:
                wait_group(U0_GROUP[u + 1])
            relayout_u(u + 1)
            bulk(u % 3, u // 3)

        def grp_body(it, carry):
            s0 = it * (UPI // 3)

            @pl.when(it == NUA // UPI)
            def _():
                for cp in cp_wm2 + cp_late:
                    cp.start()

            for u in range(1, UPI + 1):
                cp_st(u % 3, s0 + u // 3, SEM_IT + it).wait()
            for u in range(UPI):
                relayout((u + 1) % 3, s0 + (u + 1) // 3)
                bulk(u % 3, s0 + u // 3)
            return carry

        lax.fori_loop(NUA // UPI, (NU - NUZ) // UPI, grp_body, 0)

        for u in range(NU - NUZ + 1, NU):
            cp_unit(u).wait()
        for cp in cp_mid + cp_wm2:
            cp.wait()
        mem_s[...] = m0_s[...].astype(F32)
        xv = xbuf[pl.ds(PAD + PRO, XR), :].astype(F32)
        hn_s[...] = _ln_mod(xv, mod_row(0, XR), mod_row(1, XR))
        for u in range(NU - NUZ, NU):
            if u + 1 < NU:
                relayout_u(u + 1)
            i0 = 16 + 4 * (u - (NU - NUZ))
            extras = []
            for i in range(i0, min(i0 + 4, 48)):
                extras += [functools.partial(mod_slab, i), lambda: None]
            bulk(u % 3, u // 3, extras)
        for cp in cp_late:
            cp.wait()

    pl.run_scoped(
        prologue,
        pltpu.VMEM((NU, D, DH), U32),
        pltpu.VMEM((48, D, 128), BF16),
        pltpu.VMEM((PRO, D), F32),
        pltpu.VMEM((PRO, D), BF16),
        pltpu.VMEM((2 * NUG, PRO, DH), F32),
    )

    def rest(w1_s, w3_s, w2_s, oring):
        w132 = w1_s.bitcast(U32)
        w332 = w3_s.bitcast(U32)
        w232 = w2_s.bitcast(U32)
        q32 = qring.bitcast(U32)
        k32 = kring.bitcast(U32)
        v32 = vring.bitcast(U32)

        cp_w1 = [pltpu.make_async_copy(w1_hbm.at[:, pl.ds(f * 128, 128)],
                                       w1_s.at[f], sems.at[SEM_FFN])
                 for f in range(NF)]
        cp_w3 = [pltpu.make_async_copy(w3_hbm.at[:, pl.ds(f * 128, 128)],
                                       w3_s.at[f], sems.at[SEM_FFN])
                 for f in range(NF)]
        cp_w2 = [pltpu.make_async_copy(w2_hbm.at[:, pl.ds(c * 128, 128)],
                                       w2_s.at[c], sems.at[SEM_FFN])
                 for c in range(NC)]
        for cp in cp_w1 + cp_w3 + cp_w2:
            cp.start()

        oring[:, pl.ds(OOFF - XR, XR), :] = jnp.zeros((H, XR, DH), BF16)

        def post_attn(a, r, n):
            x1 = xbuf[pl.ds(r, n), :].astype(F32) + mod_row(2, n) * a
            x1 = x1.astype(BF16)
            xbuf[pl.ds(r, n), :] = x1
            hbuf[pl.ds(r, n), :] = _ln_mod(
                x1.astype(F32), mod_row(3, n), mod_row(4, n)).astype(BF16)

        row = lax.broadcasted_iota(jnp.int32, (NP, NP), 0)
        col = lax.broadcasted_iota(jnp.int32, (NP, NP), 1)

        def second(i):
            return ((i >= SEG) & (i < 2 * SEG)) | (i >= 2 * SEG + M)

        same = second(row) == second(col)
        mask = same & ((row >= 2 * SEG) | (col >= 2 * SEG) | (col <= row))
        fill = jnp.where(same, -1e9, -jnp.inf).astype(F32)

        def step(s, carry, mem, split, maybe_last):
            lhs_c = [jnp.concatenate([hn_s[:, pl.ds(c * 128, 128)], mem[c]],
                                     axis=0).astype(BF16) for c in range(NC)]
            lhs = jnp.concatenate(lhs_c, axis=1)

            post_attn(ax_s[...], pl.multiple_of(XR * s, 8), XR)
            rn = pl.multiple_of(
                PAD + jnp.minimum(PRO + XR * (s + 1), S - XR), 8)
            hn_s[...] = _ln_mod(xbuf[pl.ds(rn, XR), :].astype(F32),
                                mod_row(0, XR), mod_row(1, XR))

            wp, rp, op, ow = carry
            wpos = [pl.multiple_of(_wrap(wp + 8 * j, RING), 8)
                    for j in range(XR // 8)]
            rpos = pl.multiple_of(rp, SEG // 2)
            opos = [pl.multiple_of(_wrap(op + 8 * j, ORING), 8)
                    for j in range(XR // 8 + 1)]
            owr = pl.multiple_of(ow, SEG)

            tails = {}
            xs = {}
            ps = {}
            lhs_o = {}

            def load(j, p):
                r32 = (q32, k32, v32)[j]
                xs[j, p] = [
                    pltpu.bitcast(r32[h, pl.ds(rpos, SEG // 2), :], BF16)
                    for h in (2 * p, 2 * p + 1)]

            def operand(j, p):
                tail = jnp.concatenate(
                    [tails.pop((j, 2 * p)), tails.pop((j, 2 * p + 1))], axis=0)
                return jnp.concatenate(
                    xs.pop((j, p)) + [tail.astype(BF16)], axis=0)

            low = {}
            if split:
                lhs_lo = jnp.concatenate(lhs_c[:NC // 2], axis=1)
                lhs_hi = jnp.concatenate(lhs_c[NC // 2:], axis=1)
                for h in range(2):
                    for j, w32 in enumerate((wq32, wk32, wv32)):
                        low[j, h] = _dot(lhs_lo, pltpu.bitcast(
                            w32[h, pl.ds(0, D // 4), :], BF16))

            def proj(h):
                for j, (w32, ring) in enumerate(
                        ((wq32, qring), (wk32, kring), (wv32, vring))):
                    if (j, h) in low:
                        t = _dot(lhs_hi, pltpu.bitcast(
                            w32[h, pl.ds(D // 4, D // 4), :], BF16)) + low[j, h]
                    else:
                        t = _dot(lhs, _w(w32, h))
                    for i in range(XR // 8):
                        ring[h, pl.ds(wpos[i], 8), :] = (
                            t[8 * i:8 * i + 8].astype(BF16))
                    tails[j, h] = t[XR:]

            def qk(p):
                sc = lax.dot_general(operand(0, p), operand(1, p),
                                     (((1,), (1,)), ((), ())),
                                     preferred_element_type=F32)
                sc = jnp.where(mask, sc * SCALE, fill)
                mx = jnp.max(sc, axis=-1, keepdims=True)
                e = jnp.exp(sc - mx)
                l = jnp.sum(e, axis=-1, keepdims=True)
                ps[p] = (e * pl.reciprocal(l, approx=True)).astype(BF16)

            def pv(p):
                o = _dot(ps.pop(p), operand(2, p))
                for i, h in enumerate((2 * p, 2 * p + 1)):
                    ox = [oring[h, pl.ds(opos[k], 8), :] for k in range(XR // 8)]
                    om = o[2 * SEG + M * i:2 * SEG + M * (i + 1)]
                    if maybe_last:
                        om = jnp.where(
                            s == NSEG - 1,
                            oring[h, pl.ds(opos[3], 8), :].astype(F32), om)
                    last = jnp.concatenate(
                        [ox[2].astype(F32), om], axis=0).astype(BF16)
                    lhs_o[h] = jnp.concatenate([ox[0], ox[1], last], axis=0)
                for i, h in enumerate((2 * p, 2 * p + 1)):
                    oring[h, pl.ds(owr, SEG), :] = (
                        o[SEG * i:SEG * (i + 1)].astype(BF16))

            def wo_part(c, h0, h1):
                lo = jnp.concatenate([lhs_o[h] for h in range(h0, h1)], axis=1)
                w = pltpu.bitcast(wo32[c, pl.ds(h0 * 64, (h1 - h0) * 64), :], BF16)
                return _dot(lo, w)

            NPR = H // 2
            for t in range(NPR):
                if t >= 1:
                    load(0, t - 1)
                    load(1, t - 1)
                proj(2 * t)
                if t >= 1:
                    qk(t - 1)
                if t >= 2:
                    load(2, t - 2)
                proj(2 * t + 1)
                if t >= 2:
                    pv(t - 2)
            HA = H - 4
            acc = {}
            load(0, NPR - 1)
            load(1, NPR - 1)
            load(2, NPR - 2)
            acc[0] = wo_part(0, 0, HA)
            qk(NPR - 1)
            acc[1] = wo_part(1, 0, HA)
            pv(NPR - 2)
            load(2, NPR - 1)
            for c in (2, 3, 4):
                acc[c] = wo_part(c, 0, HA)
            pv(NPR - 1)
            for c in (5, 6, 7):
                acc[c] = wo_part(c, 0, HA)
            mem_new = []
            for c in range(NC):
                a = wo_part(c, HA, H) + acc[c]
                ax_s[:, pl.ds(c * 128, 128)] = a[:XR]
                mem_new.append(a[XR:])
            return (_wrap(wp + XR, RING), _wrap(rp + SEG // 2, RING // 2),
                    _wrap(op + XR, ORING), _wrap(ow + SEG, ORING)), mem_new

        def steps(i, carry):
            mem = [mem_s[:, pl.ds(c * 128, 128)] for c in range(NC)]
            for u in range(UNROLL):
                carry, mem = step(i * UNROLL + u, carry, mem, split=u > 0,
                                  maybe_last=u == UNROLL - 1)
            for c in range(NC):
                mem_s[:, pl.ds(c * 128, 128)] = mem[c]
            return carry

        lax.fori_loop(0, NSEG // UNROLL, steps,
                      (jnp.int32(PRO), jnp.int32(0), jnp.int32(OOFF - XR),
                       jnp.int32(OOFF)))

        post_attn(jnp.concatenate([ax_s[...], mem_s[...]], axis=0),
                  XR * NSEG, XR + M)
        done = XR * (NSEG - 1) + M
        o32 = oring.bitcast(U32)

        def wo_bulk(i):
            p = pl.multiple_of(((done + OOFF) % ORING + i * WB) // 2, 8)
            lo = jnp.concatenate(
                [pltpu.bitcast(o32[h, pl.ds(p, WB // 2), :], BF16)
                 for h in range(H)], axis=1)
            a = jnp.concatenate(
                [_dot(lo, _w(wo32, c)) for c in range(NC)], axis=1)
            post_attn(a, pl.multiple_of(PAD + done + i * WB, 16), WB)

        for cp in cp_w1 + cp_w3 + cp_w2:
            cp.wait()

        def cp_out(i):
            r = i * FB
            rb = PAD + r
            if not isinstance(i, int):
                r = pl.multiple_of(r, FB)
                rb = pl.multiple_of(rb, 8)
            return pltpu.make_async_copy(xbuf.at[pl.ds(rb, FB)],
                                         out_hbm.at[pl.ds(r, FB)],
                                         sems.at[SEM_OUT])

        def ffn_body(i, carry, with_wo):
            r = pl.multiple_of(PAD + i * FB, 16)
            hv = hbuf[pl.ds(r, FB), :]
            if with_wo:
                wo_bulk(i)
            act = []
            for f in range(NF):
                g = _dot(hv, _w(w132, f))
                u = _dot(hv, _w(w332, f))
                act.append((g * jax.nn.sigmoid(g) * u).astype(BF16))
            av = jnp.concatenate(act, axis=1)
            for c in range(NC):
                y = _dot(av, _w(w232, c))
                cs = pl.ds(c * 128, 128)
                x2 = xbuf[pl.ds(r, FB), cs].astype(F32) + mod_row(5, FB, cs) * y
                xbuf[pl.ds(r, FB), cs] = x2.astype(BF16)
            cp_out(i).start()
            return carry

        lax.fori_loop(0, NWB, functools.partial(ffn_body, with_wo=True), 0)
        lax.fori_loop(NWB, S // FB,
                      functools.partial(ffn_body, with_wo=False), 0)
        for i in range(S // FB):
            cp_out(i).wait()

    pl.run_scoped(
        rest,
        pltpu.VMEM((NF, D, 128), BF16),
        pltpu.VMEM((NF, D, 128), BF16),
        pltpu.VMEM((NC, F, 128), BF16),
        pltpu.VMEM((H, ORING, DH), BF16),
    )


@functools.partial(jax.jit, static_argnames=("A_seg_len",))
def pallas_adaLN_cond__memory_aug_recurrent_mem_tr__glu_gated_swiglu__prompt_kernel(
    A_x: jax.Array,
    A_mem0: jax.Array,
    A_Wq: jax.Array,
    A_Wk: jax.Array,
    A_Wv: jax.Array,
    A_Wo: jax.Array,
    A_seg_len,
    B_x: jax.Array,
    B_w1: jax.Array,
    B_w3: jax.Array,
    B_w2: jax.Array,
    c: jax.Array,
    w_mod: jax.Array,
):
    del B_x
    assert A_seg_len == SEG
    assert A_x.shape == (1, S, D) and A_mem0.shape == (1, M, D)
    assert A_Wq.shape == (D, H, DH) and B_w1.shape == (D, F)

    any_spec = pl.BlockSpec(memory_space=pl.ANY)
    out = pl.pallas_call(
        _kernel,
        out_shape=jax.ShapeDtypeStruct((S, D), BF16),
        in_specs=[any_spec] * 11,
        out_specs=any_spec,
        scratch_shapes=[
            pltpu.VMEM((H, D // 2, DH), U32),
            pltpu.VMEM((H, D // 2, DH), U32),
            pltpu.VMEM((H, D // 2, DH), U32),
            pltpu.VMEM((NC, H * DH, 128), BF16),
            pltpu.VMEM((2, PAD + S, D), BF16),
            pltpu.VMEM((H, RING, DH), BF16),
            pltpu.VMEM((H, RING, DH), BF16),
            pltpu.VMEM((H, RING, DH), BF16),
            pltpu.VMEM((6 * 8, D), F32),
            pltpu.VMEM((M, D), F32),
            pltpu.VMEM((XR, D), F32),
            pltpu.VMEM((XR, D), F32),
            pltpu.VMEM((1, D), BF16),
            pltpu.VMEM((M, D), BF16),
            pltpu.SemaphoreType.DMA((NSEMS,)),
        ],
        compiler_params=pltpu.CompilerParams(
            vmem_limit_bytes=120 * 1024 * 1024),
        name="adaln_memtr_swiglu",
    )(
        A_x.reshape(S, D),
        A_mem0.reshape(M, D),
        A_Wq, A_Wk, A_Wv,
        A_Wo.reshape(H * DH, D),
        B_w1, B_w3, B_w2, c, w_mod,
    )
    return out.reshape(1, S, D)
```

```python
import functools

import jax
import jax.numpy as jnp
from jax import lax
import jax.experimental.pallas as pl
import jax.experimental.pallas.tpu as pltpu

BF16 = jnp.bfloat16
F32 = jnp.float32
U32 = jnp.uint32

S = 2048
D = 1024
H = 32
DH = 128
F = 3584
M = 8
SEG = 32
NSEG = S // SEG
XR = 24
PRO = S - XR * NSEG
RING = 544
ORING = 576
OOFF = 256
PAD = 48
NC = D // 128
NF = F // 128
FA = 128
FB = 208
NWB = 3
WB = 176
UNROLL = 4
NU = 3 * H // 2
UPI = 6
NUA = 12
NUZ = 12
NUG = 4
NP = 2 * (SEG + M)
EPS = 1e-5
SEM_FIRST, SEM_LATE, SEM_MID, SEM_FFN, SEM_OUT = 0, 1, 2, 3, 4
SEM_CA = 5
SEM_U0 = SEM_CA + 2
U0_GROUP = (0, 1, 2, 3, 4, 5, 5, 5, 6, 6, 6, 6, 6)
SEM_SA = SEM_U0 + U0_GROUP[NUG]
SEM_IT = SEM_U0 + U0_GROUP[-1] + 1 - NUA // UPI
NSEMS = SEM_IT + NU // UPI
SCALE = DH ** -0.5


def _dot(a, b):
    return jnp.dot(a, b, preferred_element_type=F32)


def _w(ref32, i):
    return pltpu.bitcast(ref32[i], BF16)


def _wrap(i, n):
    return jnp.where(i >= n, i - n, i)


def _ln(x):
    mu = jnp.mean(x, axis=-1, keepdims=True)
    xc = x - mu
    var = jnp.mean(xc * xc, axis=-1, keepdims=True)
    return xc * lax.rsqrt(var + EPS)


def _ln_mod(x, shift, scale1):
    return _ln(x) * scale1 + shift


def _kernel(x_hbm, mem0_hbm, wq_hbm, wk_hbm, wv_hbm, wo_hbm, w1_hbm, w3_hbm,
            w2_hbm, c_hbm, wmod_hbm, out_hbm,
            wq32, wk32, wv32, wo_s, xh, qring, kring, vring,
            mod_s, mem_s, ax_s, hn_s, c_s, m0_s, sems):
    wo32 = wo_s.bitcast(U32)
    xbuf = xh.at[0]
    hbuf = xh.at[1]

    cp_x0 = pltpu.make_async_copy(x_hbm.at[pl.ds(0, PRO)],
                                  xbuf.at[pl.ds(PAD, PRO)], sems.at[SEM_FIRST])
    cp_c = pltpu.make_async_copy(c_hbm, c_s, sems.at[SEM_FIRST])
    cp_mid = [
        pltpu.make_async_copy(mem0_hbm, m0_s, sems.at[SEM_MID]),
        pltpu.make_async_copy(x_hbm.at[pl.ds(PRO, SEG)],
                              xbuf.at[pl.ds(PAD + PRO, SEG)],
                              sems.at[SEM_MID]),
    ]
    cp_late = [
        pltpu.make_async_copy(x_hbm.at[pl.ds(PRO + SEG, S - PRO - SEG)],
                              xbuf.at[pl.ds(PAD + PRO + SEG, S - PRO - SEG)],
                              sems.at[SEM_LATE]),
    ] + [pltpu.make_async_copy(wo_hbm.at[:, pl.ds(c * 128, 128)],
                               wo_s.at[c], sems.at[SEM_LATE])
         for c in range(NC)]

    def mod_row(i, n, cols=slice(None)):
        return jnp.concatenate([mod_s[pl.ds(8 * i, 8), cols]] * (n // 8), axis=0)

    def prologue(st, wm_s, xn_s, g_s, tmp_s):
        wm32 = wm_s.bitcast(U32)
        srcs = (wq_hbm.bitcast(U32), wk_hbm.bitcast(U32), wv_hbm.bitcast(U32))
        dsts = (wq32, wk32, wv32)
        rings = (qring, kring, vring)

        def cp_st(j, s, sem):
            return pltpu.make_async_copy(srcs[j].at[:, s, :], st.at[3 * s + j],
                                         sems.at[sem])

        def cp_unit(u):
            sem = (SEM_U0 + U0_GROUP[u] if u <= NUA
                   else SEM_IT + (u - 1) // UPI)
            return cp_st(u % 3, u // 3, sem)

        def cp_wm(i):
            sem = (SEM_SA if i < 8 else
                   SEM_CA + (i - 8) // 4 if i < 16 else SEM_MID)
            return pltpu.make_async_copy(wmod_hbm.at[:, pl.ds(i * 128, 128)],
                                         wm_s.at[i], sems.at[sem])

        cp_wm2 = [cp_wm(i) for i in range(16, 48)]

        cp_c.start()
        cp_x0.start()
        for i in range(8, 16):
            cp_wm(i).start()
        for u in range(NUG):
            cp_unit(u).start()
        for i in range(8):
            cp_wm(i).start()
        for u in range(NUG, NU):
            cp_unit(u).start()
        for cp in cp_mid:
            cp.start()

        xbuf[pl.ds(0, PAD), :] = jnp.zeros((PAD, D), BF16)
        ax_s[...] = jnp.zeros((XR, D), F32)

        cp_c.wait()
        cp_x0.wait()
        cf = c_s[...].astype(F32)
        sc = (cf * jax.nn.sigmoid(cf)).astype(BF16)
        sc8 = jnp.broadcast_to(sc, (8, D))

        def ln_body(i, carry):
            r = pl.multiple_of(i * 64, 64)
            xv = xbuf[pl.ds(pl.multiple_of(PAD + r, 8), 64), :].astype(F32)
            xn_s[pl.ds(r, 64), :] = _ln(xv)
            return carry

        lax.fori_loop(0, PRO // 64, ln_body, 0)

        def mod_slab(i):
            k, c = divmod(i, NC)
            part = _dot(sc8, _w(wm32, i))
            if k in (1, 4):
                part = part + 1.0
            mod_s[pl.ds(8 * k, 8), pl.ds(c * 128, 128)] = part

        for c0 in (8, 12):
            for i in range(c0, c0 + 4):
                cp_wm(i).wait()
            for i in range(c0, c0 + 4):
                mod_slab(i)

        def relayout(j, s):
            u = 3 * s + j
            for db in range(8):
                ev = st[u, pl.ds(db * 128, 64, stride=2), :]
                od = st[u, pl.ds(db * 128 + 1, 64, stride=2), :]
                rows = pl.ds(db * 64, 64)
                dsts[j][2 * s, rows, :] = (ev & U32(0xFFFF)) | (od << 16)
                dsts[j][2 * s + 1, rows, :] = (ev >> 16) | (od & U32(0xFFFF0000))

        def bulk(j, s, extras=(), mbs=range(PRO // 128)):
            extras = list(extras)
            for mb in mbs:
                lhs = hbuf[pl.ds(PAD + mb * 128, 128), :]
                for hh in range(2):
                    h = 2 * s + hh
                    rings[j][h, pl.ds(mb * 128, 128), :] = (
                        _dot(lhs, _w(dsts[j], h)).astype(BF16))
                    if extras:
                        extras.pop(0)()

        def bulk_g(u, mbs):
            for mb in mbs:
                rows = pl.ds(mb * 128, 128)
                if u == 0:
                    lhs = (xn_s[rows, :] * mod_row(1, 128)).astype(BF16)
                    g_s[rows, :] = lhs
                else:
                    lhs = g_s[rows, :]
                for hh in range(2):
                    tmp_s[2 * u + hh, rows, :] = _dot(
                        lhs, _w(dsts[u % 3], 2 * (u // 3) + hh))

        def add_shift(u, hh):
            h = 2 * (u // 3) + hh
            b = _dot(mod_row(0, 8).astype(BF16), _w(dsts[u % 3], h))
            rings[u % 3][h, pl.ds(0, PRO), :] = (
                tmp_s[2 * u + hh] + jnp.concatenate([b] * (PRO // 8), axis=0)
            ).astype(BF16)

        def wait_group(g):
            if g == U0_GROUP[NUG]:
                for i in range(8):
                    cp_wm(i).wait()
            for v in range(NUA + 1):
                if U0_GROUP[v] == g:
                    cp_unit(v).wait()

        def relayout_u(u):
            relayout(u % 3, u // 3)

        wait_group(0)
        relayout_u(0)
        bulk_g(0, (0, 1))
        wait_group(1)
        relayout_u(1)
        bulk_g(0, (2, 3))
        wait_group(2)
        relayout_u(2)
        bulk_g(1, range(4))
        wait_group(3)
        relayout_u(3)
        bulk_g(2, range(4))
        bulk_g(3, (0, 1, 2))
        wait_group(4)
        relayout_u(4)
        for i in range(8):
            mod_slab(i)
        bulk_g(3, (3,))
        for mb in range(PRO // 128):
            rows = pl.ds(mb * 128, 128)
            hbuf[pl.ds(PAD + mb * 128, 128), :] = (
                xn_s[rows, :] * mod_row(1, 128) + mod_row(0, 128)).astype(BF16)
        shifts = [functools.partial(add_shift, v, hh)
                  for v in range(NUG) for hh in range(2)]
        bulk(4 % 3, 4 // 3, shifts, mbs=(0, 1, 2))
        wait_group(5)
        relayout_u(5)
        bulk(4 % 3, 4 // 3, shifts[6:], mbs=(3,))
        for u in range(5, NUA):
            if U0_GROUP[u + 1] != U0_GROUP[u]:
                wait_group(U0_GROUP[u + 1])
            relayout_u(u + 1)
            bulk(u % 3, u // 3)

        def grp_body(it, carry):
            s0 = it * (UPI // 3)

            @pl.when(it == NUA // UPI)
            def _():
                for cp in cp_wm2 + cp_late:
                    cp.start()

            for u in range(1, UPI + 1):
                cp_st(u % 3, s0 + u // 3, SEM_IT + it).wait()
            for u in range(UPI):
                relayout((u + 1) % 3, s0 + (u + 1) // 3)
                bulk(u % 3, s0 + u // 3)
            return carry

        lax.fori_loop(NUA // UPI, (NU - NUZ) // UPI, grp_body, 0)

        for u in range(NU - NUZ + 1, NU):
            cp_unit(u).wait()
        for cp in cp_mid + cp_wm2:
            cp.wait()
        mem_s[...] = m0_s[...].astype(F32)
        xv = xbuf[pl.ds(PAD + PRO, XR), :].astype(F32)
        hn_s[...] = _ln_mod(xv, mod_row(0, XR), mod_row(1, XR))
        for u in range(NU - NUZ, NU):
            if u + 1 < NU:
                relayout_u(u + 1)
            i0 = 16 + 4 * (u - (NU - NUZ))
            extras = []
            for i in range(i0, min(i0 + 4, 48)):
                extras += [functools.partial(mod_slab, i), lambda: None]
            bulk(u % 3, u // 3, extras)
        for cp in cp_late:
            cp.wait()

    pl.run_scoped(
        prologue,
        pltpu.VMEM((NU, D, DH), U32),
        pltpu.VMEM((48, D, 128), BF16),
        pltpu.VMEM((PRO, D), F32),
        pltpu.VMEM((PRO, D), BF16),
        pltpu.VMEM((2 * NUG, PRO, DH), F32),
    )

    def rest(w1_s, w3_s, w2_s, oring):
        w132 = w1_s.bitcast(U32)
        w332 = w3_s.bitcast(U32)
        w232 = w2_s.bitcast(U32)
        q32 = qring.bitcast(U32)
        k32 = kring.bitcast(U32)
        v32 = vring.bitcast(U32)

        cp_w1 = [pltpu.make_async_copy(w1_hbm.at[:, pl.ds(f * 128, 128)],
                                       w1_s.at[f], sems.at[SEM_FFN])
                 for f in range(NF)]
        cp_w3 = [pltpu.make_async_copy(w3_hbm.at[:, pl.ds(f * 128, 128)],
                                       w3_s.at[f], sems.at[SEM_FFN])
                 for f in range(NF)]
        cp_w2 = [pltpu.make_async_copy(w2_hbm.at[:, pl.ds(c * 128, 128)],
                                       w2_s.at[c], sems.at[SEM_FFN])
                 for c in range(NC)]
        for cp in cp_w1 + cp_w3 + cp_w2:
            cp.start()

        oring[:, pl.ds(OOFF - XR, XR), :] = jnp.zeros((H, XR, DH), BF16)

        def post_attn(a, r, n):
            x1 = xbuf[pl.ds(r, n), :].astype(F32) + mod_row(2, n) * a
            x1 = x1.astype(BF16)
            xbuf[pl.ds(r, n), :] = x1
            hbuf[pl.ds(r, n), :] = _ln_mod(
                x1.astype(F32), mod_row(3, n), mod_row(4, n)).astype(BF16)

        row = lax.broadcasted_iota(jnp.int32, (NP, NP), 0)
        col = lax.broadcasted_iota(jnp.int32, (NP, NP), 1)

        def second(i):
            return ((i >= SEG) & (i < 2 * SEG)) | (i >= 2 * SEG + M)

        same = second(row) == second(col)
        mask = same & ((row >= 2 * SEG) | (col >= 2 * SEG) | (col <= row))
        fill = jnp.where(same, -1e9, -jnp.inf).astype(F32)

        def step(s, carry, mem, split, maybe_last):
            lhs_c = [jnp.concatenate([hn_s[:, pl.ds(c * 128, 128)], mem[c]],
                                     axis=0).astype(BF16) for c in range(NC)]
            lhs = jnp.concatenate(lhs_c, axis=1)

            post_attn(ax_s[...], pl.multiple_of(XR * s, 8), XR)
            rn = pl.multiple_of(
                PAD + jnp.minimum(PRO + XR * (s + 1), S - XR), 8)
            hn_s[...] = _ln_mod(xbuf[pl.ds(rn, XR), :].astype(F32),
                                mod_row(0, XR), mod_row(1, XR))

            wp, rp, op, ow = carry
            wpos = [pl.multiple_of(_wrap(wp + 8 * j, RING), 8)
                    for j in range(XR // 8)]
            rpos = pl.multiple_of(rp, SEG // 2)
            opos = [pl.multiple_of(_wrap(op + 8 * j, ORING), 8)
                    for j in range(XR // 8 + 1)]
            owr = pl.multiple_of(ow, SEG)

            tails = {}
            xs = {}
            ps = {}
            lhs_o = {}

            def load(j, p):
                r32 = (q32, k32, v32)[j]
                xs[j, p] = [
                    pltpu.bitcast(r32[h, pl.ds(rpos, SEG // 2), :], BF16)
                    for h in (2 * p, 2 * p + 1)]

            def operand(j, p):
                tail = jnp.concatenate(
                    [tails.pop((j, 2 * p)), tails.pop((j, 2 * p + 1))], axis=0)
                return jnp.concatenate(
                    xs.pop((j, p)) + [tail.astype(BF16)], axis=0)

            low = {}
            if split:
                lhs_lo = jnp.concatenate(lhs_c[:NC // 2], axis=1)
                lhs_hi = jnp.concatenate(lhs_c[NC // 2:], axis=1)
                for h in range(2):
                    for j, w32 in enumerate((wq32, wk32, wv32)):
                        low[j, h] = _dot(lhs_lo, pltpu.bitcast(
                            w32[h, pl.ds(0, D // 4), :], BF16))

            def proj(h):
                for j, (w32, ring) in enumerate(
                        ((wq32, qring), (wk32, kring), (wv32, vring))):
                    if (j, h) in low:
                        t = _dot(lhs_hi, pltpu.bitcast(
                            w32[h, pl.ds(D // 4, D // 4), :], BF16)) + low[j, h]
                    else:
                        t = _dot(lhs, _w(w32, h))
                    for i in range(XR // 8):
                        ring[h, pl.ds(wpos[i], 8), :] = (
                            t[8 * i:8 * i + 8].astype(BF16))
                    tails[j, h] = t[XR:]

            def qk(p):
                sc = lax.dot_general(operand(0, p), operand(1, p),
                                     (((1,), (1,)), ((), ())),
                                     preferred_element_type=F32)
                sc = jnp.where(mask, sc * SCALE, fill)
                mx = jnp.max(sc, axis=-1, keepdims=True)
                e = jnp.exp(sc - mx)
                l = jnp.sum(e, axis=-1, keepdims=True)
                ps[p] = (e * pl.reciprocal(l, approx=True)).astype(BF16)

            def pv(p):
                o = _dot(ps.pop(p), operand(2, p))
                for i, h in enumerate((2 * p, 2 * p + 1)):
                    ox = [oring[h, pl.ds(opos[k], 8), :] for k in range(XR // 8)]
                    om = o[2 * SEG + M * i:2 * SEG + M * (i + 1)]
                    if maybe_last:
                        om = jnp.where(
                            s == NSEG - 1,
                            oring[h, pl.ds(opos[3], 8), :].astype(F32), om)
                    last = jnp.concatenate(
                        [ox[2].astype(F32), om], axis=0).astype(BF16)
                    lhs_o[h] = jnp.concatenate([ox[0], ox[1], last], axis=0)
                for i, h in enumerate((2 * p, 2 * p + 1)):
                    oring[h, pl.ds(owr, SEG), :] = (
                        o[SEG * i:SEG * (i + 1)].astype(BF16))

            def wo_part(c, h0, h1):
                lo = jnp.concatenate([lhs_o[h] for h in range(h0, h1)], axis=1)
                w = pltpu.bitcast(wo32[c, pl.ds(h0 * 64, (h1 - h0) * 64), :], BF16)
                return _dot(lo, w)

            NPR = H // 2
            for t in range(NPR):
                if t >= 1:
                    load(0, t - 1)
                    load(1, t - 1)
                proj(2 * t)
                if t >= 1:
                    qk(t - 1)
                if t >= 2:
                    load(2, t - 2)
                proj(2 * t + 1)
                if t >= 2:
                    pv(t - 2)
            HA = H - 4
            acc = {}
            load(0, NPR - 1)
            load(1, NPR - 1)
            load(2, NPR - 2)
            acc[0] = wo_part(0, 0, HA)
            qk(NPR - 1)
            acc[1] = wo_part(1, 0, HA)
            pv(NPR - 2)
            load(2, NPR - 1)
            for c in (2, 3, 4):
                acc[c] = wo_part(c, 0, HA)
            pv(NPR - 1)
            for c in (5, 6, 7):
                acc[c] = wo_part(c, 0, HA)
            mem_new = []
            for c in range(NC):
                a = wo_part(c, HA, H) + acc[c]
                ax_s[:, pl.ds(c * 128, 128)] = a[:XR]
                mem_new.append(a[XR:])
            return (_wrap(wp + XR, RING), _wrap(rp + SEG // 2, RING // 2),
                    _wrap(op + XR, ORING), _wrap(ow + SEG, ORING)), mem_new

        def steps(i, carry):
            mem = [mem_s[:, pl.ds(c * 128, 128)] for c in range(NC)]
            for u in range(UNROLL):
                carry, mem = step(i * UNROLL + u, carry, mem, split=u > 0,
                                  maybe_last=u == UNROLL - 1)
            for c in range(NC):
                mem_s[:, pl.ds(c * 128, 128)] = mem[c]
            return carry

        lax.fori_loop(0, NSEG // UNROLL, steps,
                      (jnp.int32(PRO), jnp.int32(0), jnp.int32(OOFF - XR),
                       jnp.int32(OOFF)))

        post_attn(jnp.concatenate([ax_s[...], mem_s[...]], axis=0),
                  XR * NSEG, XR + M)
        done = XR * (NSEG - 1) + M
        o32 = oring.bitcast(U32)

        def wo_bulk(i):
            p = pl.multiple_of(((done + OOFF) % ORING + i * WB) // 2, 8)
            lo = jnp.concatenate(
                [pltpu.bitcast(o32[h, pl.ds(p, WB // 2), :], BF16)
                 for h in range(H)], axis=1)
            a = jnp.concatenate(
                [_dot(lo, _w(wo32, c)) for c in range(NC)], axis=1)
            post_attn(a, pl.multiple_of(PAD + done + i * WB, 16), WB)

        for cp in cp_w1 + cp_w3 + cp_w2:
            cp.wait()

        def cp_out(r, n):
            return pltpu.make_async_copy(xbuf.at[pl.ds(PAD + r, n)],
                                         out_hbm.at[pl.ds(r, n)],
                                         sems.at[SEM_OUT])

        def ffn_body(i, carry, r0, n, with_wo):
            r = pl.multiple_of(r0 + i * n, 16)
            rows = pl.ds(pl.multiple_of(PAD + r, 16), n)
            hv = hbuf[rows, :]
            if with_wo:
                wo_bulk(i)
            act = []
            for f in range(NF):
                g = _dot(hv, _w(w132, f))
                u = _dot(hv, _w(w332, f))
                act.append((g * jax.nn.sigmoid(g) * u).astype(BF16))
            av = jnp.concatenate(act, axis=1)
            for c in range(NC):
                y = _dot(av, _w(w232, c))
                cs = pl.ds(c * 128, 128)
                x2 = xbuf[rows, cs].astype(F32) + mod_row(5, n, cs) * y
                xbuf[rows, cs] = x2.astype(BF16)
            cp_out(r, n).start()
            return carry

        nfb = (S - NWB * FA) // FB
        lax.fori_loop(0, NWB, functools.partial(
            ffn_body, r0=0, n=FA, with_wo=True), 0)
        lax.fori_loop(0, nfb, functools.partial(
            ffn_body, r0=NWB * FA, n=FB, with_wo=False), 0)
        for i in range(NWB):
            cp_out(i * FA, FA).wait()
        for i in range(nfb):
            cp_out(NWB * FA + i * FB, FB).wait()

    pl.run_scoped(
        rest,
        pltpu.VMEM((NF, D, 128), BF16),
        pltpu.VMEM((NF, D, 128), BF16),
        pltpu.VMEM((NC, F, 128), BF16),
        pltpu.VMEM((H, ORING, DH), BF16),
    )


@functools.partial(jax.jit, static_argnames=("A_seg_len",))
def pallas_adaLN_cond__memory_aug_recurrent_mem_tr__glu_gated_swiglu__prompt_kernel(
    A_x: jax.Array,
    A_mem0: jax.Array,
    A_Wq: jax.Array,
    A_Wk: jax.Array,
    A_Wv: jax.Array,
    A_Wo: jax.Array,
    A_seg_len,
    B_x: jax.Array,
    B_w1: jax.Array,
    B_w3: jax.Array,
    B_w2: jax.Array,
    c: jax.Array,
    w_mod: jax.Array,
):
    del B_x
    assert A_seg_len == SEG
    assert A_x.shape == (1, S, D) and A_mem0.shape == (1, M, D)
    assert A_Wq.shape == (D, H, DH) and B_w1.shape == (D, F)

    any_spec = pl.BlockSpec(memory_space=pl.ANY)
    out = pl.pallas_call(
        _kernel,
        out_shape=jax.ShapeDtypeStruct((S, D), BF16),
        in_specs=[any_spec] * 11,
        out_specs=any_spec,
        scratch_shapes=[
            pltpu.VMEM((H, D // 2, DH), U32),
            pltpu.VMEM((H, D // 2, DH), U32),
            pltpu.VMEM((H, D // 2, DH), U32),
            pltpu.VMEM((NC, H * DH, 128), BF16),
            pltpu.VMEM((2, PAD + S, D), BF16),
            pltpu.VMEM((H, RING, DH), BF16),
            pltpu.VMEM((H, RING, DH), BF16),
            pltpu.VMEM((H, RING, DH), BF16),
            pltpu.VMEM((6 * 8, D), F32),
            pltpu.VMEM((M, D), F32),
            pltpu.VMEM((XR, D), F32),
            pltpu.VMEM((XR, D), F32),
            pltpu.VMEM((1, D), BF16),
            pltpu.VMEM((M, D), BF16),
            pltpu.SemaphoreType.DMA((NSEMS,)),
        ],
        compiler_params=pltpu.CompilerParams(
            vmem_limit_bytes=120 * 1024 * 1024),
        name="adaln_memtr_swiglu",
    )(
        A_x.reshape(S, D),
        A_mem0.reshape(M, D),
        A_Wq, A_Wk, A_Wv,
        A_Wo.reshape(H * DH, D),
        B_w1, B_w3, B_w2, c, w_mod,
    )
    return out.reshape(1, S, D)
```

```python
import functools

import jax
import jax.numpy as jnp
from jax import lax
import jax.experimental.pallas as pl
import jax.experimental.pallas.tpu as pltpu

BF16 = jnp.bfloat16
F32 = jnp.float32
U32 = jnp.uint32

S = 2048
D = 1024
H = 32
DH = 128
F = 3584
M = 8
SEG = 32
NSEG = S // SEG
XR = 24
PRO = S - XR * NSEG
RING = 544
ORING = 576
OOFF = 256
PAD = 48
NC = D // 128
NF = F // 128
FA = 128
FB = 208
OC = 7
NWB = 3
WB = 176
UNROLL = 4
NU = 3 * H // 2
UPI = 6
NUA = 12
NUZ = 12
NUG = 4
NP = 2 * (SEG + M)
EPS = 1e-5
SEM_FIRST, SEM_LATE, SEM_MID, SEM_FFN, SEM_OUT = 0, 1, 2, 3, 4
SEM_CA = 5
SEM_U0 = SEM_CA + 2
U0_GROUP = (0, 1, 2, 3, 4, 5, 5, 5, 6, 6, 6, 6, 6)
SEM_SA = SEM_U0 + U0_GROUP[NUG]
SEM_IT = SEM_U0 + U0_GROUP[-1] + 1 - NUA // UPI
NSEMS = SEM_IT + NU // UPI
SCALE = DH ** -0.5


def _dot(a, b):
    return jnp.dot(a, b, preferred_element_type=F32)


def _w(ref32, i):
    return pltpu.bitcast(ref32[i], BF16)


def _wrap(i, n):
    return jnp.where(i >= n, i - n, i)


def _ln(x):
    mu = jnp.mean(x, axis=-1, keepdims=True)
    xc = x - mu
    var = jnp.mean(xc * xc, axis=-1, keepdims=True)
    return xc * lax.rsqrt(var + EPS)


def _ln_mod(x, shift, scale1):
    return _ln(x) * scale1 + shift


def _kernel(x_hbm, mem0_hbm, wq_hbm, wk_hbm, wv_hbm, wo_hbm, w1_hbm, w3_hbm,
            w2_hbm, c_hbm, wmod_hbm, out_hbm,
            wq32, wk32, wv32, wo_s, xh, qring, kring, vring,
            mod_s, mem_s, ax_s, hn_s, c_s, m0_s, sems):
    wo32 = wo_s.bitcast(U32)
    xbuf = xh.at[0]
    hbuf = xh.at[1]

    cp_x0 = pltpu.make_async_copy(x_hbm.at[pl.ds(0, PRO)],
                                  xbuf.at[pl.ds(PAD, PRO)], sems.at[SEM_FIRST])
    cp_c = pltpu.make_async_copy(c_hbm, c_s, sems.at[SEM_FIRST])
    cp_mid = [
        pltpu.make_async_copy(mem0_hbm, m0_s, sems.at[SEM_MID]),
        pltpu.make_async_copy(x_hbm.at[pl.ds(PRO, SEG)],
                              xbuf.at[pl.ds(PAD + PRO, SEG)],
                              sems.at[SEM_MID]),
    ]
    cp_late = [
        pltpu.make_async_copy(x_hbm.at[pl.ds(PRO + SEG, S - PRO - SEG)],
                              xbuf.at[pl.ds(PAD + PRO + SEG, S - PRO - SEG)],
                              sems.at[SEM_LATE]),
    ] + [pltpu.make_async_copy(wo_hbm.at[:, pl.ds(c * 128, 128)],
                               wo_s.at[c], sems.at[SEM_LATE])
         for c in range(NC)]

    def mod_row(i, n, cols=slice(None)):
        return jnp.concatenate([mod_s[pl.ds(8 * i, 8), cols]] * (n // 8), axis=0)

    def prologue(st, wm_s, xn_s, g_s, tmp_s):
        wm32 = wm_s.bitcast(U32)
        srcs = (wq_hbm.bitcast(U32), wk_hbm.bitcast(U32), wv_hbm.bitcast(U32))
        dsts = (wq32, wk32, wv32)
        rings = (qring, kring, vring)

        def cp_st(j, s, sem):
            return pltpu.make_async_copy(srcs[j].at[:, s, :], st.at[3 * s + j],
                                         sems.at[sem])

        def cp_unit(u):
            sem = (SEM_U0 + U0_GROUP[u] if u <= NUA
                   else SEM_IT + (u - 1) // UPI)
            return cp_st(u % 3, u // 3, sem)

        def cp_wm(i):
            sem = (SEM_SA if i < 8 else
                   SEM_CA + (i - 8) // 4 if i < 16 else SEM_MID)
            return pltpu.make_async_copy(wmod_hbm.at[:, pl.ds(i * 128, 128)],
                                         wm_s.at[i], sems.at[sem])

        cp_wm2 = [cp_wm(i) for i in range(16, 48)]

        cp_c.start()
        cp_x0.start()
        for i in range(8, 16):
            cp_wm(i).start()
        for u in range(NUG):
            cp_unit(u).start()
        for i in range(8):
            cp_wm(i).start()
        for u in range(NUG, NU):
            cp_unit(u).start()
        for cp in cp_mid:
            cp.start()

        xbuf[pl.ds(0, PAD), :] = jnp.zeros((PAD, D), BF16)
        ax_s[...] = jnp.zeros((XR, D), F32)

        cp_c.wait()
        cp_x0.wait()
        cf = c_s[...].astype(F32)
        sc = (cf * jax.nn.sigmoid(cf)).astype(BF16)
        sc8 = jnp.broadcast_to(sc, (8, D))

        def ln_body(i, carry):
            r = pl.multiple_of(i * 64, 64)
            xv = xbuf[pl.ds(pl.multiple_of(PAD + r, 8), 64), :].astype(F32)
            xn_s[pl.ds(r, 64), :] = _ln(xv)
            return carry

        lax.fori_loop(0, PRO // 64, ln_body, 0)

        def mod_slab(i):
            k, c = divmod(i, NC)
            part = _dot(sc8, _w(wm32, i))
            if k in (1, 4):
                part = part + 1.0
            mod_s[pl.ds(8 * k, 8), pl.ds(c * 128, 128)] = part

        for c0 in (8, 12):
            for i in range(c0, c0 + 4):
                cp_wm(i).wait()
            for i in range(c0, c0 + 4):
                mod_slab(i)

        def relayout(j, s):
            u = 3 * s + j
            for db in range(8):
                ev = st[u, pl.ds(db * 128, 64, stride=2), :]
                od = st[u, pl.ds(db * 128 + 1, 64, stride=2), :]
                rows = pl.ds(db * 64, 64)
                dsts[j][2 * s, rows, :] = (ev & U32(0xFFFF)) | (od << 16)
                dsts[j][2 * s + 1, rows, :] = (ev >> 16) | (od & U32(0xFFFF0000))

        def bulk(j, s, extras=(), mbs=range(PRO // 128)):
            extras = list(extras)
            for mb in mbs:
                lhs = hbuf[pl.ds(PAD + mb * 128, 128), :]
                for hh in range(2):
                    h = 2 * s + hh
                    rings[j][h, pl.ds(mb * 128, 128), :] = (
                        _dot(lhs, _w(dsts[j], h)).astype(BF16))
                    if extras:
                        extras.pop(0)()

        def bulk_g(u, mbs):
            for mb in mbs:
                rows = pl.ds(mb * 128, 128)
                if u == 0:
                    lhs = (xn_s[rows, :] * mod_row(1, 128)).astype(BF16)
                    g_s[rows, :] = lhs
                else:
                    lhs = g_s[rows, :]
                for hh in range(2):
                    tmp_s[2 * u + hh, rows, :] = _dot(
                        lhs, _w(dsts[u % 3], 2 * (u // 3) + hh))

        def add_shift(u, hh):
            h = 2 * (u // 3) + hh
            b = _dot(mod_row(0, 8).astype(BF16), _w(dsts[u % 3], h))
            rings[u % 3][h, pl.ds(0, PRO), :] = (
                tmp_s[2 * u + hh] + jnp.concatenate([b] * (PRO // 8), axis=0)
            ).astype(BF16)

        def wait_group(g):
            if g == U0_GROUP[NUG]:
                for i in range(8):
                    cp_wm(i).wait()
            for v in range(NUA + 1):
                if U0_GROUP[v] == g:
                    cp_unit(v).wait()

        def relayout_u(u):
            relayout(u % 3, u // 3)

        wait_group(0)
        relayout_u(0)
        bulk_g(0, (0, 1))
        wait_group(1)
        relayout_u(1)
        bulk_g(0, (2, 3))
        wait_group(2)
        relayout_u(2)
        bulk_g(1, range(4))
        wait_group(3)
        relayout_u(3)
        bulk_g(2, range(4))
        bulk_g(3, (0, 1, 2))
        wait_group(4)
        relayout_u(4)
        for i in range(8):
            mod_slab(i)
        bulk_g(3, (3,))
        for mb in range(PRO // 128):
            rows = pl.ds(mb * 128, 128)
            hbuf[pl.ds(PAD + mb * 128, 128), :] = (
                xn_s[rows, :] * mod_row(1, 128) + mod_row(0, 128)).astype(BF16)
        shifts = [functools.partial(add_shift, v, hh)
                  for v in range(NUG) for hh in range(2)]
        bulk(4 % 3, 4 // 3, shifts, mbs=(0, 1, 2))
        wait_group(5)
        relayout_u(5)
        bulk(4 % 3, 4 // 3, shifts[6:], mbs=(3,))
        for u in range(5, NUA):
            if U0_GROUP[u + 1] != U0_GROUP[u]:
                wait_group(U0_GROUP[u + 1])
            relayout_u(u + 1)
            bulk(u % 3, u // 3)

        def grp_body(it, carry):
            s0 = it * (UPI // 3)

            @pl.when(it == NUA // UPI)
            def _():
                for cp in cp_wm2 + cp_late:
                    cp.start()

            for u in range(1, UPI + 1):
                cp_st(u % 3, s0 + u // 3, SEM_IT + it).wait()
            for u in range(UPI):
                relayout((u + 1) % 3, s0 + (u + 1) // 3)
                bulk(u % 3, s0 + u // 3)
            return carry

        lax.fori_loop(NUA // UPI, (NU - NUZ) // UPI, grp_body, 0)

        for u in range(NU - NUZ + 1, NU):
            cp_unit(u).wait()
        for cp in cp_mid + cp_wm2:
            cp.wait()
        mem_s[...] = m0_s[...].astype(F32)
        xv = xbuf[pl.ds(PAD + PRO, XR), :].astype(F32)
        hn_s[...] = _ln_mod(xv, mod_row(0, XR), mod_row(1, XR))
        for u in range(NU - NUZ, NU):
            if u + 1 < NU:
                relayout_u(u + 1)
            i0 = 16 + 4 * (u - (NU - NUZ))
            extras = []
            for i in range(i0, min(i0 + 4, 48)):
                extras += [functools.partial(mod_slab, i), lambda: None]
            bulk(u % 3, u // 3, extras)
        for cp in cp_late:
            cp.wait()

    pl.run_scoped(
        prologue,
        pltpu.VMEM((NU, D, DH), U32),
        pltpu.VMEM((48, D, 128), BF16),
        pltpu.VMEM((PRO, D), F32),
        pltpu.VMEM((PRO, D), BF16),
        pltpu.VMEM((2 * NUG, PRO, DH), F32),
    )

    def rest(w1_s, w3_s, w2_s, oring):
        w132 = w1_s.bitcast(U32)
        w332 = w3_s.bitcast(U32)
        w232 = w2_s.bitcast(U32)
        q32 = qring.bitcast(U32)
        k32 = kring.bitcast(U32)
        v32 = vring.bitcast(U32)

        cp_w1 = [pltpu.make_async_copy(w1_hbm.at[:, pl.ds(f * 128, 128)],
                                       w1_s.at[f], sems.at[SEM_FFN])
                 for f in range(NF)]
        cp_w3 = [pltpu.make_async_copy(w3_hbm.at[:, pl.ds(f * 128, 128)],
                                       w3_s.at[f], sems.at[SEM_FFN])
                 for f in range(NF)]
        cp_w2 = [pltpu.make_async_copy(w2_hbm.at[:, pl.ds(c * 128, 128)],
                                       w2_s.at[c], sems.at[SEM_FFN])
                 for c in range(NC)]
        for cp in cp_w1 + cp_w3 + cp_w2:
            cp.start()

        oring[:, pl.ds(OOFF - XR, XR), :] = jnp.zeros((H, XR, DH), BF16)

        def post_attn(a, r, n):
            x1 = xbuf[pl.ds(r, n), :].astype(F32) + mod_row(2, n) * a
            x1 = x1.astype(BF16)
            xbuf[pl.ds(r, n), :] = x1
            hbuf[pl.ds(r, n), :] = _ln_mod(
                x1.astype(F32), mod_row(3, n), mod_row(4, n)).astype(BF16)

        row = lax.broadcasted_iota(jnp.int32, (NP, NP), 0)
        col = lax.broadcasted_iota(jnp.int32, (NP, NP), 1)

        def second(i):
            return ((i >= SEG) & (i < 2 * SEG)) | (i >= 2 * SEG + M)

        same = second(row) == second(col)
        mask = same & ((row >= 2 * SEG) | (col >= 2 * SEG) | (col <= row))
        fill = jnp.where(same, -1e9, -jnp.inf).astype(F32)

        def step(s, carry, mem, split, maybe_last):
            lhs_c = [jnp.concatenate([hn_s[:, pl.ds(c * 128, 128)], mem[c]],
                                     axis=0).astype(BF16) for c in range(NC)]
            lhs = jnp.concatenate(lhs_c, axis=1)

            post_attn(ax_s[...], pl.multiple_of(XR * s, 8), XR)
            rn = pl.multiple_of(
                PAD + jnp.minimum(PRO + XR * (s + 1), S - XR), 8)
            hn_s[...] = _ln_mod(xbuf[pl.ds(rn, XR), :].astype(F32),
                                mod_row(0, XR), mod_row(1, XR))

            wp, rp, op, ow = carry
            wpos = [pl.multiple_of(_wrap(wp + 8 * j, RING), 8)
                    for j in range(XR // 8)]
            rpos = pl.multiple_of(rp, SEG // 2)
            opos = [pl.multiple_of(_wrap(op + 8 * j, ORING), 8)
                    for j in range(XR // 8 + 1)]
            owr = pl.multiple_of(ow, SEG)

            tails = {}
            xs = {}
            ps = {}
            lhs_o = {}

            def load(j, p):
                r32 = (q32, k32, v32)[j]
                xs[j, p] = [
                    pltpu.bitcast(r32[h, pl.ds(rpos, SEG // 2), :], BF16)
                    for h in (2 * p, 2 * p + 1)]

            def operand(j, p):
                tail = jnp.concatenate(
                    [tails.pop((j, 2 * p)), tails.pop((j, 2 * p + 1))], axis=0)
                return jnp.concatenate(
                    xs.pop((j, p)) + [tail.astype(BF16)], axis=0)

            low = {}
            if split:
                lhs_lo = jnp.concatenate(lhs_c[:NC // 2], axis=1)
                lhs_hi = jnp.concatenate(lhs_c[NC // 2:], axis=1)
                for h in range(2):
                    for j, w32 in enumerate((wq32, wk32, wv32)):
                        low[j, h] = _dot(lhs_lo, pltpu.bitcast(
                            w32[h, pl.ds(0, D // 4), :], BF16))

            def proj(h):
                for j, (w32, ring) in enumerate(
                        ((wq32, qring), (wk32, kring), (wv32, vring))):
                    if (j, h) in low:
                        t = _dot(lhs_hi, pltpu.bitcast(
                            w32[h, pl.ds(D // 4, D // 4), :], BF16)) + low[j, h]
                    else:
                        t = _dot(lhs, _w(w32, h))
                    for i in range(XR // 8):
                        ring[h, pl.ds(wpos[i], 8), :] = (
                            t[8 * i:8 * i + 8].astype(BF16))
                    tails[j, h] = t[XR:]

            def qk(p):
                sc = lax.dot_general(operand(0, p), operand(1, p),
                                     (((1,), (1,)), ((), ())),
                                     preferred_element_type=F32)
                sc = jnp.where(mask, sc * SCALE, fill)
                mx = jnp.max(sc, axis=-1, keepdims=True)
                e = jnp.exp(sc - mx)
                l = jnp.sum(e, axis=-1, keepdims=True)
                ps[p] = (e * pl.reciprocal(l, approx=True)).astype(BF16)

            def pv(p):
                o = _dot(ps.pop(p), operand(2, p))
                for i, h in enumerate((2 * p, 2 * p + 1)):
                    ox = [oring[h, pl.ds(opos[k], 8), :] for k in range(XR // 8)]
                    om = o[2 * SEG + M * i:2 * SEG + M * (i + 1)]
                    if maybe_last:
                        om = jnp.where(
                            s == NSEG - 1,
                            oring[h, pl.ds(opos[3], 8), :].astype(F32), om)
                    last = jnp.concatenate(
                        [ox[2].astype(F32), om], axis=0).astype(BF16)
                    lhs_o[h] = jnp.concatenate([ox[0], ox[1], last], axis=0)
                for i, h in enumerate((2 * p, 2 * p + 1)):
                    oring[h, pl.ds(owr, SEG), :] = (
                        o[SEG * i:SEG * (i + 1)].astype(BF16))

            def wo_part(c, h0, h1):
                lo = jnp.concatenate([lhs_o[h] for h in range(h0, h1)], axis=1)
                w = pltpu.bitcast(wo32[c, pl.ds(h0 * 64, (h1 - h0) * 64), :], BF16)
                return _dot(lo, w)

            NPR = H // 2
            for t in range(NPR):
                if t >= 1:
                    load(0, t - 1)
                    load(1, t - 1)
                proj(2 * t)
                if t >= 1:
                    qk(t - 1)
                if t >= 2:
                    load(2, t - 2)
                proj(2 * t + 1)
                if t >= 2:
                    pv(t - 2)
            HA = H - 4
            acc = {}
            load(0, NPR - 1)
            load(1, NPR - 1)
            load(2, NPR - 2)
            acc[0] = wo_part(0, 0, HA)
            qk(NPR - 1)
            acc[1] = wo_part(1, 0, HA)
            pv(NPR - 2)
            load(2, NPR - 1)
            for c in (2, 3, 4):
                acc[c] = wo_part(c, 0, HA)
            pv(NPR - 1)
            for c in (5, 6, 7):
                acc[c] = wo_part(c, 0, HA)
            mem_new = []
            for c in range(NC):
                a = wo_part(c, HA, H) + acc[c]
                ax_s[:, pl.ds(c * 128, 128)] = a[:XR]
                mem_new.append(a[XR:])
            return (_wrap(wp + XR, RING), _wrap(rp + SEG // 2, RING // 2),
                    _wrap(op + XR, ORING), _wrap(ow + SEG, ORING)), mem_new

        def steps(i, carry):
            mem = [mem_s[:, pl.ds(c * 128, 128)] for c in range(NC)]
            for u in range(UNROLL):
                carry, mem = step(i * UNROLL + u, carry, mem, split=u > 0,
                                  maybe_last=u == UNROLL - 1)
            for c in range(NC):
                mem_s[:, pl.ds(c * 128, 128)] = mem[c]
            return carry

        lax.fori_loop(0, NSEG // UNROLL, steps,
                      (jnp.int32(PRO), jnp.int32(0), jnp.int32(OOFF - XR),
                       jnp.int32(OOFF)))

        post_attn(jnp.concatenate([ax_s[...], mem_s[...]], axis=0),
                  XR * NSEG, XR + M)
        done = XR * (NSEG - 1) + M
        o32 = oring.bitcast(U32)

        def wo_bulk(i):
            p = pl.multiple_of(((done + OOFF) % ORING + i * WB) // 2, 8)
            lo = jnp.concatenate(
                [pltpu.bitcast(o32[h, pl.ds(p, WB // 2), :], BF16)
                 for h in range(H)], axis=1)
            a = jnp.concatenate(
                [_dot(lo, _w(wo32, c)) for c in range(NC)], axis=1)
            post_attn(a, pl.multiple_of(PAD + done + i * WB, 16), WB)

        for cp in cp_w1 + cp_w3 + cp_w2:
            cp.wait()

        def cp_out(r, n, part):
            cols = pl.ds(0, OC * 128) if part == 0 else pl.ds(OC * 128, D - OC * 128)
            return pltpu.make_async_copy(xbuf.at[pl.ds(PAD + r, n), cols],
                                         out_hbm.at[pl.ds(r, n), cols],
                                         sems.at[SEM_OUT])

        def ffn_body(i, carry, r0, n, with_wo):
            r = pl.multiple_of(r0 + i * n, 16)
            rows = pl.ds(pl.multiple_of(PAD + r, 16), n)
            hv = hbuf[rows, :]
            if with_wo:
                wo_bulk(i)
            act = []
            for f in range(NF):
                g = _dot(hv, _w(w132, f))
                u = _dot(hv, _w(w332, f))
                act.append((g * jax.nn.sigmoid(g) * u).astype(BF16))
            av = jnp.concatenate(act, axis=1)
            for c in range(NC):
                y = _dot(av, _w(w232, c))
                cs = pl.ds(c * 128, 128)
                x2 = xbuf[rows, cs].astype(F32) + mod_row(5, n, cs) * y
                xbuf[rows, cs] = x2.astype(BF16)
                if c == OC - 1:
                    cp_out(r, n, 0).start()
            cp_out(r, n, 1).start()
            return carry

        nfb = (S - NWB * FA) // FB
        lax.fori_loop(0, NWB, functools.partial(
            ffn_body, r0=0, n=FA, with_wo=True), 0)
        lax.fori_loop(0, nfb, functools.partial(
            ffn_body, r0=NWB * FA, n=FB, with_wo=False), 0)
        for part in range(2):
            for i in range(NWB):
                cp_out(i * FA, FA, part).wait()
            for i in range(nfb):
                cp_out(NWB * FA + i * FB, FB, part).wait()

    pl.run_scoped(
        rest,
        pltpu.VMEM((NF, D, 128), BF16),
        pltpu.VMEM((NF, D, 128), BF16),
        pltpu.VMEM((NC, F, 128), BF16),
        pltpu.VMEM((H, ORING, DH), BF16),
    )


@functools.partial(jax.jit, static_argnames=("A_seg_len",))
def pallas_adaLN_cond__memory_aug_recurrent_mem_tr__glu_gated_swiglu__prompt_kernel(
    A_x: jax.Array,
    A_mem0: jax.Array,
    A_Wq: jax.Array,
    A_Wk: jax.Array,
    A_Wv: jax.Array,
    A_Wo: jax.Array,
    A_seg_len,
    B_x: jax.Array,
    B_w1: jax.Array,
    B_w3: jax.Array,
    B_w2: jax.Array,
    c: jax.Array,
    w_mod: jax.Array,
):
    del B_x
    assert A_seg_len == SEG
    assert A_x.shape == (1, S, D) and A_mem0.shape == (1, M, D)
    assert A_Wq.shape == (D, H, DH) and B_w1.shape == (D, F)

    any_spec = pl.BlockSpec(memory_space=pl.ANY)
    out = pl.pallas_call(
        _kernel,
        out_shape=jax.ShapeDtypeStruct((S, D), BF16),
        in_specs=[any_spec] * 11,
        out_specs=any_spec,
        scratch_shapes=[
            pltpu.VMEM((H, D // 2, DH), U32),
            pltpu.VMEM((H, D // 2, DH), U32),
            pltpu.VMEM((H, D // 2, DH), U32),
            pltpu.VMEM((NC, H * DH, 128), BF16),
            pltpu.VMEM((2, PAD + S, D), BF16),
            pltpu.VMEM((H, RING, DH), BF16),
            pltpu.VMEM((H, RING, DH), BF16),
            pltpu.VMEM((H, RING, DH), BF16),
            pltpu.VMEM((6 * 8, D), F32),
            pltpu.VMEM((M, D), F32),
            pltpu.VMEM((XR, D), F32),
            pltpu.VMEM((XR, D), F32),
            pltpu.VMEM((1, D), BF16),
            pltpu.VMEM((M, D), BF16),
            pltpu.SemaphoreType.DMA((NSEMS,)),
        ],
        compiler_params=pltpu.CompilerParams(
            vmem_limit_bytes=120 * 1024 * 1024),
        name="adaln_memtr_swiglu",
    )(
        A_x.reshape(S, D),
        A_mem0.reshape(M, D),
        A_Wq, A_Wk, A_Wv,
        A_Wo.reshape(H * DH, D),
        B_w1, B_w3, B_w2, c, w_mod,
    )
    return out.reshape(1, S, D)
```

```python
import functools

import jax
import jax.numpy as jnp
from jax import lax
import jax.experimental.pallas as pl
import jax.experimental.pallas.tpu as pltpu

BF16 = jnp.bfloat16
F32 = jnp.float32
U32 = jnp.uint32

S = 2048
D = 1024
H = 32
DH = 128
F = 3584
M = 8
SEG = 32
NSEG = S // SEG
XR = 24
PRO = S - XR * NSEG
RING = 544
ORING = 576
OOFF = 256
PAD = 48
NC = D // 128
NF = F // 128
FA = 128
FB = 208
OC = 7
NWB = 3
WB = 176
QPOS, QPOS1 = 2, 4
UNROLL = 4
NU = 3 * H // 2
UPI = 6
NUA = 12
NUZ = 12
NUG = 4
NP = 2 * (SEG + M)
EPS = 1e-5
SEM_FIRST, SEM_LATE, SEM_MID, SEM_FFN, SEM_OUT = 0, 1, 2, 3, 4
SEM_CA = 5
SEM_U0 = SEM_CA + 2
U0_GROUP = (0, 1, 2, 3, 4, 5, 5, 5, 6, 6, 6, 6, 6)
SEM_SA = SEM_U0 + U0_GROUP[NUG]
SEM_IT = SEM_U0 + U0_GROUP[-1] + 1 - NUA // UPI
NSEMS = SEM_IT + NU // UPI
SCALE = DH ** -0.5


def _dot(a, b):
    return jnp.dot(a, b, preferred_element_type=F32)


def _w(ref32, i):
    return pltpu.bitcast(ref32[i], BF16)


def _wrap(i, n):
    return jnp.where(i >= n, i - n, i)


def _ln(x):
    mu = jnp.mean(x, axis=-1, keepdims=True)
    xc = x - mu
    var = jnp.mean(xc * xc, axis=-1, keepdims=True)
    return xc * lax.rsqrt(var + EPS)


def _ln_mod(x, shift, scale1):
    return _ln(x) * scale1 + shift


def _kernel(x_hbm, mem0_hbm, wq_hbm, wk_hbm, wv_hbm, wo_hbm, w1_hbm, w3_hbm,
            w2_hbm, c_hbm, wmod_hbm, out_hbm,
            wq32, wk32, wv32, wo_s, xh, qring, kring, vring,
            mod_s, mem_s, ax_s, hn_s, c_s, m0_s, sems):
    wo32 = wo_s.bitcast(U32)
    xbuf = xh.at[0]
    hbuf = xh.at[1]

    cp_x0 = pltpu.make_async_copy(x_hbm.at[pl.ds(0, PRO)],
                                  xbuf.at[pl.ds(PAD, PRO)], sems.at[SEM_FIRST])
    cp_c = pltpu.make_async_copy(c_hbm, c_s, sems.at[SEM_FIRST])
    cp_mid = [
        pltpu.make_async_copy(mem0_hbm, m0_s, sems.at[SEM_MID]),
        pltpu.make_async_copy(x_hbm.at[pl.ds(PRO, SEG)],
                              xbuf.at[pl.ds(PAD + PRO, SEG)],
                              sems.at[SEM_MID]),
    ]
    cp_late = [
        pltpu.make_async_copy(x_hbm.at[pl.ds(PRO + SEG, S - PRO - SEG)],
                              xbuf.at[pl.ds(PAD + PRO + SEG, S - PRO - SEG)],
                              sems.at[SEM_LATE]),
    ] + [pltpu.make_async_copy(wo_hbm.at[:, pl.ds(c * 128, 128)],
                               wo_s.at[c], sems.at[SEM_LATE])
         for c in range(NC)]

    def mod_row(i, n, cols=slice(None)):
        return jnp.concatenate([mod_s[pl.ds(8 * i, 8), cols]] * (n // 8), axis=0)

    def prologue(st, wm_s, xn_s, g_s, tmp_s):
        wm32 = wm_s.bitcast(U32)
        srcs = (wq_hbm.bitcast(U32), wk_hbm.bitcast(U32), wv_hbm.bitcast(U32))
        dsts = (wq32, wk32, wv32)
        rings = (qring, kring, vring)

        def cp_st(j, s, sem):
            return pltpu.make_async_copy(srcs[j].at[:, s, :], st.at[3 * s + j],
                                         sems.at[sem])

        def cp_unit(u):
            sem = (SEM_U0 + U0_GROUP[u] if u <= NUA
                   else SEM_IT + (u - 1) // UPI)
            return cp_st(u % 3, u // 3, sem)

        def cp_wm(i):
            sem = (SEM_SA if i < 8 else
                   SEM_CA + (i - 8) // 4 if i < 16 else SEM_MID)
            return pltpu.make_async_copy(wmod_hbm.at[:, pl.ds(i * 128, 128)],
                                         wm_s.at[i], sems.at[sem])

        cp_wm2 = [cp_wm(i) for i in range(16, 48)]

        cp_c.start()
        cp_x0.start()
        for i in range(8, 16):
            cp_wm(i).start()
        for u in range(NUG):
            cp_unit(u).start()
        for i in range(8):
            cp_wm(i).start()
        for u in range(NUG, NU):
            cp_unit(u).start()
        for cp in cp_mid:
            cp.start()

        xbuf[pl.ds(0, PAD), :] = jnp.zeros((PAD, D), BF16)
        ax_s[...] = jnp.zeros((XR, D), F32)

        cp_c.wait()
        cp_x0.wait()
        cf = c_s[...].astype(F32)
        sc = (cf * jax.nn.sigmoid(cf)).astype(BF16)
        sc8 = jnp.broadcast_to(sc, (8, D))

        def ln_body(i, carry):
            r = pl.multiple_of(i * 64, 64)
            xv = xbuf[pl.ds(pl.multiple_of(PAD + r, 8), 64), :].astype(F32)
            xn_s[pl.ds(r, 64), :] = _ln(xv)
            return carry

        lax.fori_loop(0, PRO // 64, ln_body, 0)

        def mod_slab(i):
            k, c = divmod(i, NC)
            part = _dot(sc8, _w(wm32, i))
            if k in (1, 4):
                part = part + 1.0
            mod_s[pl.ds(8 * k, 8), pl.ds(c * 128, 128)] = part

        for c0 in (8, 12):
            for i in range(c0, c0 + 4):
                cp_wm(i).wait()
            for i in range(c0, c0 + 4):
                mod_slab(i)

        def relayout(j, s):
            u = 3 * s + j
            for db in range(8):
                ev = st[u, pl.ds(db * 128, 64, stride=2), :]
                od = st[u, pl.ds(db * 128 + 1, 64, stride=2), :]
                rows = pl.ds(db * 64, 64)
                dsts[j][2 * s, rows, :] = (ev & U32(0xFFFF)) | (od << 16)
                dsts[j][2 * s + 1, rows, :] = (ev >> 16) | (od & U32(0xFFFF0000))

        def bulk(j, s, extras=(), mbs=range(PRO // 128)):
            extras = list(extras)
            for mb in mbs:
                lhs = hbuf[pl.ds(PAD + mb * 128, 128), :]
                for hh in range(2):
                    h = 2 * s + hh
                    rings[j][h, pl.ds(mb * 128, 128), :] = (
                        _dot(lhs, _w(dsts[j], h)).astype(BF16))
                    if extras:
                        extras.pop(0)()

        def bulk_g(u, mbs):
            for mb in mbs:
                rows = pl.ds(mb * 128, 128)
                if u == 0:
                    lhs = (xn_s[rows, :] * mod_row(1, 128)).astype(BF16)
                    g_s[rows, :] = lhs
                else:
                    lhs = g_s[rows, :]
                for hh in range(2):
                    tmp_s[2 * u + hh, rows, :] = _dot(
                        lhs, _w(dsts[u % 3], 2 * (u // 3) + hh))

        def add_shift(u, hh):
            h = 2 * (u // 3) + hh
            b = _dot(mod_row(0, 8).astype(BF16), _w(dsts[u % 3], h))
            rings[u % 3][h, pl.ds(0, PRO), :] = (
                tmp_s[2 * u + hh] + jnp.concatenate([b] * (PRO // 8), axis=0)
            ).astype(BF16)

        def wait_group(g):
            if g == U0_GROUP[NUG]:
                for i in range(8):
                    cp_wm(i).wait()
            for v in range(NUA + 1):
                if U0_GROUP[v] == g:
                    cp_unit(v).wait()

        def relayout_u(u):
            relayout(u % 3, u // 3)

        wait_group(0)
        relayout_u(0)
        bulk_g(0, (0, 1))
        wait_group(1)
        relayout_u(1)
        bulk_g(0, (2, 3))
        wait_group(2)
        relayout_u(2)
        bulk_g(1, range(4))
        wait_group(3)
        relayout_u(3)
        bulk_g(2, range(4))
        bulk_g(3, (0, 1, 2))
        wait_group(4)
        relayout_u(4)
        for i in range(8):
            mod_slab(i)
        bulk_g(3, (3,))
        for mb in range(PRO // 128):
            rows = pl.ds(mb * 128, 128)
            hbuf[pl.ds(PAD + mb * 128, 128), :] = (
                xn_s[rows, :] * mod_row(1, 128) + mod_row(0, 128)).astype(BF16)
        shifts = [functools.partial(add_shift, v, hh)
                  for v in range(NUG) for hh in range(2)]
        bulk(4 % 3, 4 // 3, shifts, mbs=(0, 1, 2))
        wait_group(5)
        relayout_u(5)
        bulk(4 % 3, 4 // 3, shifts[6:], mbs=(3,))
        for u in range(5, NUA):
            if U0_GROUP[u + 1] != U0_GROUP[u]:
                wait_group(U0_GROUP[u + 1])
            relayout_u(u + 1)
            bulk(u % 3, u // 3)

        def grp_body(it, carry):
            s0 = it * (UPI // 3)

            @pl.when(it == NUA // UPI)
            def _():
                for cp in cp_wm2 + cp_late:
                    cp.start()

            for u in range(1, UPI + 1):
                cp_st(u % 3, s0 + u // 3, SEM_IT + it).wait()
            for u in range(UPI):
                relayout((u + 1) % 3, s0 + (u + 1) // 3)
                bulk(u % 3, s0 + u // 3)
            return carry

        lax.fori_loop(NUA // UPI, (NU - NUZ) // UPI, grp_body, 0)

        for u in range(NU - NUZ + 1, NU):
            cp_unit(u).wait()
        for cp in cp_mid + cp_wm2:
            cp.wait()
        mem_s[...] = m0_s[...].astype(F32)
        xv = xbuf[pl.ds(PAD + PRO, XR), :].astype(F32)
        hn_s[...] = _ln_mod(xv, mod_row(0, XR), mod_row(1, XR))
        for u in range(NU - NUZ, NU):
            if u + 1 < NU:
                relayout_u(u + 1)
            i0 = 16 + 4 * (u - (NU - NUZ))
            extras = []
            for i in range(i0, min(i0 + 4, 48)):
                extras += [functools.partial(mod_slab, i), lambda: None]
            bulk(u % 3, u // 3, extras)
        for cp in cp_late:
            cp.wait()

    pl.run_scoped(
        prologue,
        pltpu.VMEM((NU, D, DH), U32),
        pltpu.VMEM((48, D, 128), BF16),
        pltpu.VMEM((PRO, D), F32),
        pltpu.VMEM((PRO, D), BF16),
        pltpu.VMEM((2 * NUG, PRO, DH), F32),
    )

    def rest(w1_s, w3_s, w2_s, oring):
        w132 = w1_s.bitcast(U32)
        w332 = w3_s.bitcast(U32)
        w232 = w2_s.bitcast(U32)
        q32 = qring.bitcast(U32)
        k32 = kring.bitcast(U32)
        v32 = vring.bitcast(U32)

        cp_w1 = [pltpu.make_async_copy(w1_hbm.at[:, pl.ds(f * 128, 128)],
                                       w1_s.at[f], sems.at[SEM_FFN])
                 for f in range(NF)]
        cp_w3 = [pltpu.make_async_copy(w3_hbm.at[:, pl.ds(f * 128, 128)],
                                       w3_s.at[f], sems.at[SEM_FFN])
                 for f in range(NF)]
        cp_w2 = [pltpu.make_async_copy(w2_hbm.at[:, pl.ds(c * 128, 128)],
                                       w2_s.at[c], sems.at[SEM_FFN])
                 for c in range(NC)]
        for cp in cp_w1 + cp_w3 + cp_w2:
            cp.start()

        oring[:, pl.ds(OOFF - XR, XR), :] = jnp.zeros((H, XR, DH), BF16)

        def post_attn(a, r, n):
            x1 = xbuf[pl.ds(r, n), :].astype(F32) + mod_row(2, n) * a
            x1 = x1.astype(BF16)
            xbuf[pl.ds(r, n), :] = x1
            hbuf[pl.ds(r, n), :] = _ln_mod(
                x1.astype(F32), mod_row(3, n), mod_row(4, n)).astype(BF16)

        row = lax.broadcasted_iota(jnp.int32, (NP, NP), 0)
        col = lax.broadcasted_iota(jnp.int32, (NP, NP), 1)

        def second(i):
            return ((i >= SEG) & (i < 2 * SEG)) | (i >= 2 * SEG + M)

        same = second(row) == second(col)
        mask = same & ((row >= 2 * SEG) | (col >= 2 * SEG) | (col <= row))
        fill = jnp.where(same, -1e9, -jnp.inf).astype(F32)

        def step(s, carry, mem, split, maybe_last):
            lhs_c = [jnp.concatenate([hn_s[:, pl.ds(c * 128, 128)], mem[c]],
                                     axis=0).astype(BF16) for c in range(NC)]
            lhs = jnp.concatenate(lhs_c, axis=1)

            post_attn(ax_s[...], pl.multiple_of(XR * s, 8), XR)
            rn = pl.multiple_of(
                PAD + jnp.minimum(PRO + XR * (s + 1), S - XR), 8)
            hn_s[...] = _ln_mod(xbuf[pl.ds(rn, XR), :].astype(F32),
                                mod_row(0, XR), mod_row(1, XR))

            wp, rp, op, ow = carry
            wpos = [pl.multiple_of(_wrap(wp + 8 * j, RING), 8)
                    for j in range(XR // 8)]
            rpos = pl.multiple_of(rp, SEG // 2)
            opos = [pl.multiple_of(_wrap(op + 8 * j, ORING), 8)
                    for j in range(XR // 8 + 1)]
            owr = pl.multiple_of(ow, SEG)

            tails = {}
            xs = {}
            ps = {}
            lhs_o = {}

            def load(j, p):
                r32 = (q32, k32, v32)[j]
                xs[j, p] = [
                    pltpu.bitcast(r32[h, pl.ds(rpos, SEG // 2), :], BF16)
                    for h in (2 * p, 2 * p + 1)]

            def operand(j, p):
                tail = jnp.concatenate(
                    [tails.pop((j, 2 * p)), tails.pop((j, 2 * p + 1))], axis=0)
                return jnp.concatenate(
                    xs.pop((j, p)) + [tail.astype(BF16)], axis=0)

            low = {}
            if split:
                lhs_lo = jnp.concatenate(lhs_c[:NC // 2], axis=1)
                lhs_hi = jnp.concatenate(lhs_c[NC // 2:], axis=1)
                for h in range(2):
                    for j, w32 in enumerate((wq32, wk32, wv32)):
                        low[j, h] = _dot(lhs_lo, pltpu.bitcast(
                            w32[h, pl.ds(0, D // 4), :], BF16))

            def proj(j, h):
                w32, ring = ((wq32, qring), (wk32, kring), (wv32, vring))[j]
                if (j, h) in low:
                    t = _dot(lhs_hi, pltpu.bitcast(
                        w32[h, pl.ds(D // 4, D // 4), :], BF16)) + low[j, h]
                else:
                    t = _dot(lhs, _w(w32, h))
                for i in range(XR // 8):
                    ring[h, pl.ds(wpos[i], 8), :] = (
                        t[8 * i:8 * i + 8].astype(BF16))
                tails[j, h] = t[XR:]

            def qk(p):
                sc = lax.dot_general(operand(0, p), operand(1, p),
                                     (((1,), (1,)), ((), ())),
                                     preferred_element_type=F32)
                sc = jnp.where(mask, sc * SCALE, fill)
                mx = jnp.max(sc, axis=-1, keepdims=True)
                e = jnp.exp(sc - mx)
                l = jnp.sum(e, axis=-1, keepdims=True)
                ps[p] = (e * pl.reciprocal(l, approx=True)).astype(BF16)

            def pv(p):
                o = _dot(ps.pop(p), operand(2, p))
                for i, h in enumerate((2 * p, 2 * p + 1)):
                    ox = [oring[h, pl.ds(opos[k], 8), :] for k in range(XR // 8)]
                    om = o[2 * SEG + M * i:2 * SEG + M * (i + 1)]
                    if maybe_last:
                        om = jnp.where(
                            s == NSEG - 1,
                            oring[h, pl.ds(opos[3], 8), :].astype(F32), om)
                    last = jnp.concatenate(
                        [ox[2].astype(F32), om], axis=0).astype(BF16)
                    lhs_o[h] = jnp.concatenate([ox[0], ox[1], last], axis=0)
                for i, h in enumerate((2 * p, 2 * p + 1)):
                    oring[h, pl.ds(owr, SEG), :] = (
                        o[SEG * i:SEG * (i + 1)].astype(BF16))

            def wo_part(c, h0, h1):
                lo = jnp.concatenate([lhs_o[h] for h in range(h0, h1)], axis=1)
                w = pltpu.bitcast(wo32[c, pl.ds(h0 * 64, (h1 - h0) * 64), :], BF16)
                return _dot(lo, w)

            NPR = H // 2
            for t in range(NPR):
                if t >= 1:
                    load(0, t - 1)
                    load(1, t - 1)
                if t >= 2:
                    load(2, t - 2)
                for pos in range(6):
                    if t >= 1 and pos == (QPOS1 if t == 1 else QPOS):
                        qk(t - 1)
                    proj(pos % 3, 2 * t + pos // 3)
                if t >= 2:
                    pv(t - 2)
            HA = H - 4
            acc = {}
            mem_new = {}

            def wo_a(c):
                acc[c] = wo_part(c, 0, HA)

            def wo_b(c):
                a = wo_part(c, HA, H) + acc[c]
                ax_s[:, pl.ds(c * 128, 128)] = a[:XR]
                mem_new[c] = a[XR:]

            load(0, NPR - 1)
            load(1, NPR - 1)
            load(2, NPR - 2)
            wo_a(0)
            qk(NPR - 1)
            wo_a(1)
            pv(NPR - 2)
            load(2, NPR - 1)
            for c in (2, 3, 4):
                wo_a(c)
            pv(NPR - 1)
            for c in (5, 6):
                wo_a(c)
            for c in range(NC // 2):
                wo_b(c)
            wo_a(7)
            for c in range(NC // 2, NC):
                wo_b(c)
            return (_wrap(wp + XR, RING), _wrap(rp + SEG // 2, RING // 2),
                    _wrap(op + XR, ORING), _wrap(ow + SEG, ORING)), mem_new

        def steps(i, carry):
            mem = [mem_s[:, pl.ds(c * 128, 128)] for c in range(NC)]
            for u in range(UNROLL):
                carry, mem = step(i * UNROLL + u, carry, mem, split=u > 0,
                                  maybe_last=u == UNROLL - 1)
            for c in range(NC):
                mem_s[:, pl.ds(c * 128, 128)] = mem[c]
            return carry

        lax.fori_loop(0, NSEG // UNROLL, steps,
                      (jnp.int32(PRO), jnp.int32(0), jnp.int32(OOFF - XR),
                       jnp.int32(OOFF)))

        post_attn(jnp.concatenate([ax_s[...], mem_s[...]], axis=0),
                  XR * NSEG, XR + M)
        done = XR * (NSEG - 1) + M
        o32 = oring.bitcast(U32)

        def wo_bulk(i):
            p = pl.multiple_of(((done + OOFF) % ORING + i * WB) // 2, 8)
            lo = jnp.concatenate(
                [pltpu.bitcast(o32[h, pl.ds(p, WB // 2), :], BF16)
                 for h in range(H)], axis=1)
            a = jnp.concatenate(
                [_dot(lo, _w(wo32, c)) for c in range(NC)], axis=1)
            post_attn(a, pl.multiple_of(PAD + done + i * WB, 16), WB)

        for cp in cp_w1 + cp_w3 + cp_w2:
            cp.wait()

        def cp_out(r, n, part):
            cols = pl.ds(0, OC * 128) if part == 0 else pl.ds(OC * 128, D - OC * 128)
            return pltpu.make_async_copy(xbuf.at[pl.ds(PAD + r, n), cols],
                                         out_hbm.at[pl.ds(r, n), cols],
                                         sems.at[SEM_OUT])

        def ffn_body(i, carry, r0, n, with_wo):
            r = pl.multiple_of(r0 + i * n, 16)
            rows = pl.ds(pl.multiple_of(PAD + r, 16), n)
            hv = hbuf[rows, :]
            if with_wo:
                wo_bulk(i)
            act = []
            for f in range(NF):
                g = _dot(hv, _w(w132, f))
                u = _dot(hv, _w(w332, f))
                act.append((g * jax.nn.sigmoid(g) * u).astype(BF16))
            av = jnp.concatenate(act, axis=1)
            for c in range(NC):
                y = _dot(av, _w(w232, c))
                cs = pl.ds(c * 128, 128)
                x2 = xbuf[rows, cs].astype(F32) + mod_row(5, n, cs) * y
                xbuf[rows, cs] = x2.astype(BF16)
                if c == OC - 1:
                    cp_out(r, n, 0).start()
            cp_out(r, n, 1).start()
            return carry

        nfb = (S - NWB * FA) // FB
        lax.fori_loop(0, NWB, functools.partial(
            ffn_body, r0=0, n=FA, with_wo=True), 0)
        lax.fori_loop(0, nfb, functools.partial(
            ffn_body, r0=NWB * FA, n=FB, with_wo=False), 0)
        for part in range(2):
            for i in range(NWB):
                cp_out(i * FA, FA, part).wait()
            for i in range(nfb):
                cp_out(NWB * FA + i * FB, FB, part).wait()

    pl.run_scoped(
        rest,
        pltpu.VMEM((NF, D, 128), BF16),
        pltpu.VMEM((NF, D, 128), BF16),
        pltpu.VMEM((NC, F, 128), BF16),
        pltpu.VMEM((H, ORING, DH), BF16),
    )


@functools.partial(jax.jit, static_argnames=("A_seg_len",))
def pallas_adaLN_cond__memory_aug_recurrent_mem_tr__glu_gated_swiglu__prompt_kernel(
    A_x: jax.Array,
    A_mem0: jax.Array,
    A_Wq: jax.Array,
    A_Wk: jax.Array,
    A_Wv: jax.Array,
    A_Wo: jax.Array,
    A_seg_len,
    B_x: jax.Array,
    B_w1: jax.Array,
    B_w3: jax.Array,
    B_w2: jax.Array,
    c: jax.Array,
    w_mod: jax.Array,
):
    del B_x
    assert A_seg_len == SEG
    assert A_x.shape == (1, S, D) and A_mem0.shape == (1, M, D)
    assert A_Wq.shape == (D, H, DH) and B_w1.shape == (D, F)

    any_spec = pl.BlockSpec(memory_space=pl.ANY)
    out = pl.pallas_call(
        _kernel,
        out_shape=jax.ShapeDtypeStruct((S, D), BF16),
        in_specs=[any_spec] * 11,
        out_specs=any_spec,
        scratch_shapes=[
            pltpu.VMEM((H, D // 2, DH), U32),
            pltpu.VMEM((H, D // 2, DH), U32),
            pltpu.VMEM((H, D // 2, DH), U32),
            pltpu.VMEM((NC, H * DH, 128), BF16),
            pltpu.VMEM((2, PAD + S, D), BF16),
            pltpu.VMEM((H, RING, DH), BF16),
            pltpu.VMEM((H, RING, DH), BF16),
            pltpu.VMEM((H, RING, DH), BF16),
            pltpu.VMEM((6 * 8, D), F32),
            pltpu.VMEM((M, D), F32),
            pltpu.VMEM((XR, D), F32),
            pltpu.VMEM((XR, D), F32),
            pltpu.VMEM((1, D), BF16),
            pltpu.VMEM((M, D), BF16),
            pltpu.SemaphoreType.DMA((NSEMS,)),
        ],
        compiler_params=pltpu.CompilerParams(
            vmem_limit_bytes=120 * 1024 * 1024),
        name="adaln_memtr_swiglu",
    )(
        A_x.reshape(S, D),
        A_mem0.reshape(M, D),
        A_Wq, A_Wk, A_Wv,
        A_Wo.reshape(H * DH, D),
        B_w1, B_w3, B_w2, c, w_mod,
    )
    return out.reshape(1, S, D)
```

```python
import functools

import jax
import jax.numpy as jnp
from jax import lax
import jax.experimental.pallas as pl
import jax.experimental.pallas.tpu as pltpu

BF16 = jnp.bfloat16
F32 = jnp.float32
U32 = jnp.uint32

S = 2048
D = 1024
H = 32
DH = 128
F = 3584
M = 8
SEG = 32
NSEG = S // SEG
XR = 24
PRO = S - XR * NSEG
RING = 544
ORING = 576
OOFF = 256
PAD = 48
NC = D // 128
NF = F // 128
FA = 128
FB = 208
OC = 7
NWB = 3
WB = 176
QPOS, QPOS1 = 2, 4
UNROLL = 4
NU = 3 * H // 2
UPI = 6
NUA = 12
NUZ = 12
NUG = 4
NP = 2 * (SEG + M)
EPS = 1e-5
SEM_FIRST, SEM_LATE, SEM_MID, SEM_FFN, SEM_OUT = 0, 1, 2, 3, 4
SEM_CA = 5
SEM_U0 = SEM_CA + 2
U0_GROUP = (0, 1, 2, 3, 4, 5, 5, 5, 6, 6, 6, 6, 6)
SEM_SA = SEM_U0 + U0_GROUP[NUG]
SEM_IT = SEM_U0 + U0_GROUP[-1] + 1 - NUA // UPI
NSEMS = SEM_IT + NU // UPI
SCALE = DH ** -0.5


def _dot(a, b):
    return jnp.dot(a, b, preferred_element_type=F32)


def _w(ref32, i):
    return pltpu.bitcast(ref32[i], BF16)


def _wrap(i, n):
    return jnp.where(i >= n, i - n, i)


def _ln(x):
    mu = jnp.mean(x, axis=-1, keepdims=True)
    xc = x - mu
    var = jnp.mean(xc * xc, axis=-1, keepdims=True)
    return xc * lax.rsqrt(var + EPS)


def _ln_mod(x, shift, scale1):
    return _ln(x) * scale1 + shift


def _kernel(x_hbm, mem0_hbm, wq_hbm, wk_hbm, wv_hbm, wo_hbm, w1_hbm, w3_hbm,
            w2_hbm, c_hbm, wmod_hbm, out_hbm,
            wq32, wk32, wv32, wo_s, xh, qring, kring, vring,
            mod_s, mem_s, ax_s, hn_s, c_s, m0_s, sems):
    wo32 = wo_s.bitcast(U32)
    xbuf = xh.at[0]
    hbuf = xh.at[1]

    cp_x0 = pltpu.make_async_copy(x_hbm.at[pl.ds(0, PRO)],
                                  xbuf.at[pl.ds(PAD, PRO)], sems.at[SEM_FIRST])
    cp_c = pltpu.make_async_copy(c_hbm, c_s, sems.at[SEM_FIRST])
    cp_mid = [
        pltpu.make_async_copy(mem0_hbm, m0_s, sems.at[SEM_MID]),
        pltpu.make_async_copy(x_hbm.at[pl.ds(PRO, SEG)],
                              xbuf.at[pl.ds(PAD + PRO, SEG)],
                              sems.at[SEM_MID]),
    ]
    cp_late = [
        pltpu.make_async_copy(x_hbm.at[pl.ds(PRO + SEG, S - PRO - SEG)],
                              xbuf.at[pl.ds(PAD + PRO + SEG, S - PRO - SEG)],
                              sems.at[SEM_LATE]),
    ] + [pltpu.make_async_copy(wo_hbm.at[:, pl.ds(c * 128, 128)],
                               wo_s.at[c], sems.at[SEM_LATE])
         for c in range(NC)]

    def mod_row(i, n, cols=slice(None)):
        return jnp.concatenate([mod_s[pl.ds(8 * i, 8), cols]] * (n // 8), axis=0)

    def prologue(st, wm_s, xn_s, g_s, tmp_s):
        wm32 = wm_s.bitcast(U32)
        srcs = (wq_hbm.bitcast(U32), wk_hbm.bitcast(U32), wv_hbm.bitcast(U32))
        dsts = (wq32, wk32, wv32)
        rings = (qring, kring, vring)

        def cp_st(j, s, sem):
            return pltpu.make_async_copy(srcs[j].at[:, s, :], st.at[3 * s + j],
                                         sems.at[sem])

        def cp_unit(u):
            sem = (SEM_U0 + U0_GROUP[u] if u <= NUA
                   else SEM_IT + (u - 1) // UPI)
            return cp_st(u % 3, u // 3, sem)

        def cp_wm(i):
            sem = (SEM_SA if i < 8 else
                   SEM_CA + (i - 8) // 4 if i < 16 else SEM_MID)
            return pltpu.make_async_copy(wmod_hbm.at[:, pl.ds(i * 128, 128)],
                                         wm_s.at[i], sems.at[sem])

        cp_wm2 = [cp_wm(i) for i in range(16, 48)]

        cp_c.start()
        cp_x0.start()
        for i in range(8, 16):
            cp_wm(i).start()
        for u in range(NUG):
            cp_unit(u).start()
        for i in range(8):
            cp_wm(i).start()
        for u in range(NUG, NU):
            cp_unit(u).start()
        for cp in cp_mid:
            cp.start()

        xbuf[pl.ds(0, PAD), :] = jnp.zeros((PAD, D), BF16)
        ax_s[...] = jnp.zeros((XR, D), F32)

        cp_c.wait()
        cp_x0.wait()
        cf = c_s[...].astype(F32)
        sc = (cf * jax.nn.sigmoid(cf)).astype(BF16)
        sc8 = jnp.broadcast_to(sc, (8, D))

        def ln_body(i, carry):
            r = pl.multiple_of(i * 64, 64)
            xv = xbuf[pl.ds(pl.multiple_of(PAD + r, 8), 64), :].astype(F32)
            xn_s[pl.ds(r, 64), :] = _ln(xv)
            return carry

        lax.fori_loop(0, PRO // 64, ln_body, 0)

        def mod_slab(i):
            k, c = divmod(i, NC)
            part = _dot(sc8, _w(wm32, i))
            if k in (1, 4):
                part = part + 1.0
            mod_s[pl.ds(8 * k, 8), pl.ds(c * 128, 128)] = part

        for c0 in (8, 12):
            for i in range(c0, c0 + 4):
                cp_wm(i).wait()
            for i in range(c0, c0 + 4):
                mod_slab(i)

        def relayout(j, s):
            u = 3 * s + j
            for db in range(8):
                ev = st[u, pl.ds(db * 128, 64, stride=2), :]
                od = st[u, pl.ds(db * 128 + 1, 64, stride=2), :]
                rows = pl.ds(db * 64, 64)
                dsts[j][2 * s, rows, :] = (ev & U32(0xFFFF)) | (od << 16)
                dsts[j][2 * s + 1, rows, :] = (ev >> 16) | (od & U32(0xFFFF0000))

        def bulk(j, s, extras=(), mbs=range(PRO // 128)):
            extras = list(extras)
            for mb in mbs:
                lhs = hbuf[pl.ds(PAD + mb * 128, 128), :]
                for hh in range(2):
                    h = 2 * s + hh
                    rings[j][h, pl.ds(mb * 128, 128), :] = (
                        _dot(lhs, _w(dsts[j], h)).astype(BF16))
                    if extras:
                        extras.pop(0)()

        def bulk_g(u, mbs):
            for mb in mbs:
                rows = pl.ds(mb * 128, 128)
                if u == 0:
                    lhs = (xn_s[rows, :] * mod_row(1, 128)).astype(BF16)
                    g_s[rows, :] = lhs
                else:
                    lhs = g_s[rows, :]
                for hh in range(2):
                    tmp_s[2 * u + hh, rows, :] = _dot(
                        lhs, _w(dsts[u % 3], 2 * (u // 3) + hh))

        def add_shift(u, hh):
            h = 2 * (u // 3) + hh
            b = _dot(mod_row(0, 8).astype(BF16), _w(dsts[u % 3], h))
            rings[u % 3][h, pl.ds(0, PRO), :] = (
                tmp_s[2 * u + hh] + jnp.concatenate([b] * (PRO // 8), axis=0)
            ).astype(BF16)

        def wait_group(g):
            if g == U0_GROUP[NUG]:
                for i in range(8):
                    cp_wm(i).wait()
            for v in range(NUA + 1):
                if U0_GROUP[v] == g:
                    cp_unit(v).wait()

        def relayout_u(u):
            relayout(u % 3, u // 3)

        wait_group(0)
        relayout_u(0)
        bulk_g(0, (0, 1))
        wait_group(1)
        relayout_u(1)
        bulk_g(0, (2, 3))
        wait_group(2)
        relayout_u(2)
        bulk_g(1, range(4))
        wait_group(3)
        relayout_u(3)
        bulk_g(2, range(4))
        bulk_g(3, (0, 1, 2))
        wait_group(4)
        relayout_u(4)
        for i in range(8):
            mod_slab(i)
        bulk_g(3, (3,))
        for mb in range(PRO // 128):
            rows = pl.ds(mb * 128, 128)
            hbuf[pl.ds(PAD + mb * 128, 128), :] = (
                xn_s[rows, :] * mod_row(1, 128) + mod_row(0, 128)).astype(BF16)
        shifts = [functools.partial(add_shift, v, hh)
                  for v in range(NUG) for hh in range(2)]
        bulk(4 % 3, 4 // 3, shifts, mbs=(0, 1, 2))
        wait_group(5)
        relayout_u(5)
        bulk(4 % 3, 4 // 3, shifts[6:], mbs=(3,))
        for u in range(5, NUA):
            if U0_GROUP[u + 1] != U0_GROUP[u]:
                wait_group(U0_GROUP[u + 1])
            relayout_u(u + 1)
            bulk(u % 3, u // 3)

        def grp_body(it, carry):
            s0 = it * (UPI // 3)

            @pl.when(it == NUA // UPI)
            def _():
                for cp in cp_wm2 + cp_late:
                    cp.start()

            for u in range(1, UPI + 1):
                cp_st(u % 3, s0 + u // 3, SEM_IT + it).wait()
            for u in range(UPI):
                relayout((u + 1) % 3, s0 + (u + 1) // 3)
                bulk(u % 3, s0 + u // 3)
            return carry

        lax.fori_loop(NUA // UPI, (NU - NUZ) // UPI, grp_body, 0)

        for u in range(NU - NUZ + 1, NU):
            cp_unit(u).wait()
        for cp in cp_mid + cp_wm2:
            cp.wait()
        mem_s[...] = m0_s[...].astype(F32)
        xv = xbuf[pl.ds(PAD + PRO, XR), :].astype(F32)
        hn_s[...] = _ln_mod(xv, mod_row(0, XR), mod_row(1, XR))
        for u in range(NU - NUZ, NU):
            if u + 1 < NU:
                relayout_u(u + 1)
            i0 = 16 + 4 * (u - (NU - NUZ))
            extras = []
            for i in range(i0, min(i0 + 4, 48)):
                extras += [functools.partial(mod_slab, i), lambda: None]
            bulk(u % 3, u // 3, extras)
        for cp in cp_late:
            cp.wait()

    pl.run_scoped(
        prologue,
        pltpu.VMEM((NU, D, DH), U32),
        pltpu.VMEM((48, D, 128), BF16),
        pltpu.VMEM((PRO, D), F32),
        pltpu.VMEM((PRO, D), BF16),
        pltpu.VMEM((2 * NUG, PRO, DH), F32),
    )

    def rest(w1_s, w3_s, w2_s, oring):
        w132 = w1_s.bitcast(U32)
        w332 = w3_s.bitcast(U32)
        w232 = w2_s.bitcast(U32)
        q32 = qring.bitcast(U32)
        k32 = kring.bitcast(U32)
        v32 = vring.bitcast(U32)

        cp_w1 = [pltpu.make_async_copy(w1_hbm.at[:, pl.ds(f * 128, 128)],
                                       w1_s.at[f], sems.at[SEM_FFN])
                 for f in range(NF)]
        cp_w3 = [pltpu.make_async_copy(w3_hbm.at[:, pl.ds(f * 128, 128)],
                                       w3_s.at[f], sems.at[SEM_FFN])
                 for f in range(NF)]
        cp_w2 = [pltpu.make_async_copy(w2_hbm.at[:, pl.ds(c * 128, 128)],
                                       w2_s.at[c], sems.at[SEM_FFN])
                 for c in range(NC)]
        for cp in cp_w1 + cp_w3 + cp_w2:
            cp.start()

        oring[:, pl.ds(OOFF - XR, XR), :] = jnp.zeros((H, XR, DH), BF16)

        def post_attn(a, r, n):
            x1 = xbuf[pl.ds(r, n), :].astype(F32) + mod_row(2, n) * a
            x1 = x1.astype(BF16)
            xbuf[pl.ds(r, n), :] = x1
            hbuf[pl.ds(r, n), :] = _ln_mod(
                x1.astype(F32), mod_row(3, n), mod_row(4, n)).astype(BF16)

        row = lax.broadcasted_iota(jnp.int32, (NP, NP), 0)
        col = lax.broadcasted_iota(jnp.int32, (NP, NP), 1)

        def second(i):
            return ((i >= SEG) & (i < 2 * SEG)) | (i >= 2 * SEG + M)

        same = second(row) == second(col)
        mask = same & ((row >= 2 * SEG) | (col >= 2 * SEG) | (col <= row))
        fill = jnp.where(same, -1e9, -jnp.inf).astype(F32)

        def step(s, carry, mem, split, maybe_last):
            lhs_c = [jnp.concatenate([hn_s[:, pl.ds(c * 128, 128)], mem[c]],
                                     axis=0).astype(BF16) for c in range(NC)]
            lhs = jnp.concatenate(lhs_c, axis=1)

            post_attn(ax_s[...], pl.multiple_of(XR * s, 8), XR)
            rn = pl.multiple_of(
                PAD + jnp.minimum(PRO + XR * (s + 1), S - XR), 8)
            hn_s[...] = _ln_mod(xbuf[pl.ds(rn, XR), :].astype(F32),
                                mod_row(0, XR), mod_row(1, XR))

            wp, rp, op, ow = carry
            wpos = [pl.multiple_of(_wrap(wp + 8 * j, RING), 8)
                    for j in range(XR // 8)]
            rpos = pl.multiple_of(rp, SEG // 2)
            opos = [pl.multiple_of(_wrap(op + 8 * j, ORING), 8)
                    for j in range(XR // 8 + 1)]
            owr = pl.multiple_of(ow, SEG)

            tails = {}
            xs = {}
            ps = {}
            lhs_o = {}

            def load(j, p):
                r32 = (q32, k32, v32)[j]
                xs[j, p] = [
                    pltpu.bitcast(r32[h, pl.ds(rpos, SEG // 2), :], BF16)
                    for h in (2 * p, 2 * p + 1)]

            def operand(j, p):
                tail = jnp.concatenate(
                    [tails.pop((j, 2 * p)), tails.pop((j, 2 * p + 1))], axis=0)
                return jnp.concatenate(
                    xs.pop((j, p)) + [tail.astype(BF16)], axis=0)

            low = {}
            if split:
                lhs_lo = jnp.concatenate(lhs_c[:NC // 2], axis=1)
                lhs_hi = jnp.concatenate(lhs_c[NC // 2:], axis=1)
                for h in range(2):
                    for j, w32 in enumerate((wq32, wk32, wv32)):
                        low[j, h] = _dot(lhs_lo, pltpu.bitcast(
                            w32[h, pl.ds(0, D // 4), :], BF16))

            def proj(j, h):
                w32, ring = ((wq32, qring), (wk32, kring), (wv32, vring))[j]
                if (j, h) in low:
                    t = _dot(lhs_hi, pltpu.bitcast(
                        w32[h, pl.ds(D // 4, D // 4), :], BF16)) + low[j, h]
                else:
                    t = _dot(lhs, _w(w32, h))
                for i in range(XR // 8):
                    ring[h, pl.ds(wpos[i], 8), :] = (
                        t[8 * i:8 * i + 8].astype(BF16))
                tails[j, h] = t[XR:]

            def qk(p):
                sc = lax.dot_general(operand(0, p), operand(1, p),
                                     (((1,), (1,)), ((), ())),
                                     preferred_element_type=F32)
                sc = jnp.where(mask, sc * SCALE, fill)
                mx = jnp.max(sc, axis=-1, keepdims=True)
                e = jnp.exp(sc - mx)
                l = jnp.sum(e, axis=-1, keepdims=True)
                ps[p] = (e * pl.reciprocal(l, approx=True)).astype(BF16)

            def pv(p):
                o = _dot(ps.pop(p), operand(2, p))
                for i, h in enumerate((2 * p, 2 * p + 1)):
                    ox = [oring[h, pl.ds(opos[k], 8), :] for k in range(XR // 8)]
                    om = o[2 * SEG + M * i:2 * SEG + M * (i + 1)]
                    if maybe_last:
                        om = jnp.where(
                            s == NSEG - 1,
                            oring[h, pl.ds(opos[3], 8), :].astype(F32), om)
                    last = jnp.concatenate(
                        [ox[2].astype(F32), om], axis=0).astype(BF16)
                    lhs_o[h] = jnp.concatenate([ox[0], ox[1], last], axis=0)
                for i, h in enumerate((2 * p, 2 * p + 1)):
                    oring[h, pl.ds(owr, SEG), :] = (
                        o[SEG * i:SEG * (i + 1)].astype(BF16))

            def wo_part(c, h0, h1):
                lo = jnp.concatenate([lhs_o[h] for h in range(h0, h1)], axis=1)
                w = pltpu.bitcast(wo32[c, pl.ds(h0 * 64, (h1 - h0) * 64), :], BF16)
                return _dot(lo, w)

            NPR = H // 2
            for t in range(NPR):
                if t >= 1:
                    load(0, t - 1)
                    load(1, t - 1)
                if t >= 2:
                    load(2, t - 2)
                for pos in range(6):
                    if t >= 1 and pos == (QPOS1 if t == 1 else QPOS):
                        qk(t - 1)
                    proj(pos % 3, 2 * t + pos // 3)
                if t >= 2:
                    pv(t - 2)
            HA = H - 4
            acc = {}
            mem_new = {}

            def wo_a(c):
                acc[c] = wo_part(c, 0, HA)

            def wo_b(c):
                a = wo_part(c, HA, H) + acc[c]
                ax_s[:, pl.ds(c * 128, 128)] = a[:XR]
                mem_new[c] = a[XR:]

            load(0, NPR - 1)
            load(1, NPR - 1)
            load(2, NPR - 2)
            wo_a(0)
            qk(NPR - 1)
            wo_a(1)
            pv(NPR - 2)
            load(2, NPR - 1)
            for c in (2, 3, 4):
                wo_a(c)
            pv(NPR - 1)
            for c in (5, 6):
                wo_a(c)
            for c in range(NC // 2):
                wo_b(c)
            wo_a(7)
            for c in range(NC // 2, NC):
                wo_b(c)
            return (_wrap(wp + XR, RING), _wrap(rp + SEG // 2, RING // 2),
                    _wrap(op + XR, ORING), _wrap(ow + SEG, ORING)), mem_new

        def steps(i, carry):
            mem = [mem_s[:, pl.ds(c * 128, 128)] for c in range(NC)]
            for u in range(UNROLL):
                carry, mem = step(i * UNROLL + u, carry, mem, split=u > 0,
                                  maybe_last=u == UNROLL - 1)
            for c in range(NC):
                mem_s[:, pl.ds(c * 128, 128)] = mem[c]
            return carry

        lax.fori_loop(0, NSEG // UNROLL, steps,
                      (jnp.int32(PRO), jnp.int32(0), jnp.int32(OOFF - XR),
                       jnp.int32(OOFF)))

        post_attn(jnp.concatenate([ax_s[...], mem_s[...]], axis=0),
                  XR * NSEG, XR + M)
        done = XR * (NSEG - 1) + M
        o32 = oring.bitcast(U32)

        def wo_bulk(i):
            p = pl.multiple_of(((done + OOFF) % ORING + i * WB) // 2, 8)
            lo = jnp.concatenate(
                [pltpu.bitcast(o32[h, pl.ds(p, WB // 2), :], BF16)
                 for h in range(H)], axis=1)
            return jnp.concatenate(
                [_dot(lo, _w(wo32, c)) for c in range(NC)], axis=1)

        for cp in cp_w1 + cp_w3 + cp_w2:
            cp.wait()

        def cp_out(r, n, part):
            cols = pl.ds(0, OC * 128) if part == 0 else pl.ds(OC * 128, D - OC * 128)
            return pltpu.make_async_copy(xbuf.at[pl.ds(PAD + r, n), cols],
                                         out_hbm.at[pl.ds(r, n), cols],
                                         sems.at[SEM_OUT])

        def ffn_body(i, carry, r0, n, with_wo):
            r = pl.multiple_of(r0 + i * n, 16)
            rows = pl.ds(pl.multiple_of(PAD + r, 16), n)
            if with_wo:
                a = wo_bulk(i)
                ra = pl.multiple_of(PAD + done + i * WB, 16)
            hv = hbuf[rows, :]
            act = []
            for f in range(NF):
                g = _dot(hv, _w(w132, f))
                u = _dot(hv, _w(w332, f))
                act.append((g * jax.nn.sigmoid(g) * u).astype(BF16))
            av = jnp.concatenate(act, axis=1)
            for c in range(NC):
                y = _dot(av, _w(w232, c))
                if with_wo:
                    for k in range(WB // 16):
                        if k * NC // (WB // 16) == c:
                            post_attn(a[16 * k:16 * k + 16], ra + 16 * k, 16)
                cs = pl.ds(c * 128, 128)
                x2 = xbuf[rows, cs].astype(F32) + mod_row(5, n, cs) * y
                xbuf[rows, cs] = x2.astype(BF16)
                if c == OC - 1:
                    cp_out(r, n, 0).start()
            cp_out(r, n, 1).start()
            return carry

        nfb = (S - NWB * FA) // FB
        lax.fori_loop(0, NWB, functools.partial(
            ffn_body, r0=0, n=FA, with_wo=True), 0)
        lax.fori_loop(0, nfb, functools.partial(
            ffn_body, r0=NWB * FA, n=FB, with_wo=False), 0)
        for part in range(2):
            for i in range(NWB):
                cp_out(i * FA, FA, part).wait()
            for i in range(nfb):
                cp_out(NWB * FA + i * FB, FB, part).wait()

    pl.run_scoped(
        rest,
        pltpu.VMEM((NF, D, 128), BF16),
        pltpu.VMEM((NF, D, 128), BF16),
        pltpu.VMEM((NC, F, 128), BF16),
        pltpu.VMEM((H, ORING, DH), BF16),
    )


@functools.partial(jax.jit, static_argnames=("A_seg_len",))
def pallas_adaLN_cond__memory_aug_recurrent_mem_tr__glu_gated_swiglu__prompt_kernel(
    A_x: jax.Array,
    A_mem0: jax.Array,
    A_Wq: jax.Array,
    A_Wk: jax.Array,
    A_Wv: jax.Array,
    A_Wo: jax.Array,
    A_seg_len,
    B_x: jax.Array,
    B_w1: jax.Array,
    B_w3: jax.Array,
    B_w2: jax.Array,
    c: jax.Array,
    w_mod: jax.Array,
):
    del B_x
    assert A_seg_len == SEG
    assert A_x.shape == (1, S, D) and A_mem0.shape == (1, M, D)
    assert A_Wq.shape == (D, H, DH) and B_w1.shape == (D, F)

    any_spec = pl.BlockSpec(memory_space=pl.ANY)
    out = pl.pallas_call(
        _kernel,
        out_shape=jax.ShapeDtypeStruct((S, D), BF16),
        in_specs=[any_spec] * 11,
        out_specs=any_spec,
        scratch_shapes=[
            pltpu.VMEM((H, D // 2, DH), U32),
            pltpu.VMEM((H, D // 2, DH), U32),
            pltpu.VMEM((H, D // 2, DH), U32),
            pltpu.VMEM((NC, H * DH, 128), BF16),
            pltpu.VMEM((2, PAD + S, D), BF16),
            pltpu.VMEM((H, RING, DH), BF16),
            pltpu.VMEM((H, RING, DH), BF16),
            pltpu.VMEM((H, RING, DH), BF16),
            pltpu.VMEM((6 * 8, D), F32),
            pltpu.VMEM((M, D), F32),
            pltpu.VMEM((XR, D), F32),
            pltpu.VMEM((XR, D), F32),
            pltpu.VMEM((1, D), BF16),
            pltpu.VMEM((M, D), BF16),
            pltpu.SemaphoreType.DMA((NSEMS,)),
        ],
        compiler_params=pltpu.CompilerParams(
            vmem_limit_bytes=120 * 1024 * 1024),
        name="adaln_memtr_swiglu",
    )(
        A_x.reshape(S, D),
        A_mem0.reshape(M, D),
        A_Wq, A_Wk, A_Wv,
        A_Wo.reshape(H * DH, D),
        B_w1, B_w3, B_w2, c, w_mod,
    )
    return out.reshape(1, S, D)
```

```python
import functools

import jax
import jax.numpy as jnp
from jax import lax
import jax.experimental.pallas as pl
import jax.experimental.pallas.tpu as pltpu

BF16 = jnp.bfloat16
F32 = jnp.float32
U32 = jnp.uint32

S = 2048
D = 1024
H = 32
DH = 128
F = 3584
M = 8
SEG = 32
NSEG = S // SEG
XR = 24
PRO = S - XR * NSEG
RING = 544
ORING = 576
OOFF = 256
PAD = 48
NC = D // 128
NF = F // 128
FA = 128
FB = 208
OC = 7
NWB = 3
WB = 176
QPOS, QPOS1 = 2, 4
UNROLL = 4
NU = 3 * H // 2
UPI = 6
NUA = 12
NUZ = 12
NUG = 4
NP = 2 * (SEG + M)
EPS = 1e-5
SEM_FIRST, SEM_LATE, SEM_MID, SEM_FFN, SEM_OUT = 0, 1, 2, 3, 4
SEM_CA = 5
SEM_U0 = SEM_CA + 2
U0_GROUP = (0, 1, 2, 3, 4, 5, 5, 5, 6, 6, 6, 6, 6)
SEM_SA = SEM_U0 + U0_GROUP[NUG]
SEM_IT = SEM_U0 + U0_GROUP[-1] + 1 - NUA // UPI
NSEMS = SEM_IT + NU // UPI
SCALE = DH ** -0.5


def _dot(a, b):
    return jnp.dot(a, b, preferred_element_type=F32)


def _w(ref32, i):
    return pltpu.bitcast(ref32[i], BF16)


def _wrap(i, n):
    return jnp.where(i >= n, i - n, i)


def _ln(x):
    mu = jnp.mean(x, axis=-1, keepdims=True)
    xc = x - mu
    var = jnp.mean(xc * xc, axis=-1, keepdims=True)
    return xc * lax.rsqrt(var + EPS)


def _ln_mod(x, shift, scale1):
    return _ln(x) * scale1 + shift


def _kernel(x_hbm, mem0_hbm, wq_hbm, wk_hbm, wv_hbm, wo_hbm, w1_hbm, w3_hbm,
            w2_hbm, c_hbm, wmod_hbm, out_hbm,
            wq32, wk32, wv32, wo_s, xh, qring, kring, vring,
            mod_s, am_s, hn_s, c_s, m0_s, sems):
    wo32 = wo_s.bitcast(U32)
    ax_s = am_s.at[pl.ds(0, XR)]
    mem_s = am_s.at[pl.ds(XR, M)]
    xbuf = xh.at[0]
    hbuf = xh.at[1]

    cp_x0 = pltpu.make_async_copy(x_hbm.at[pl.ds(0, PRO)],
                                  xbuf.at[pl.ds(PAD, PRO)], sems.at[SEM_FIRST])
    cp_c = pltpu.make_async_copy(c_hbm, c_s, sems.at[SEM_FIRST])
    cp_mid = [
        pltpu.make_async_copy(mem0_hbm, m0_s, sems.at[SEM_MID]),
        pltpu.make_async_copy(x_hbm.at[pl.ds(PRO, SEG)],
                              xbuf.at[pl.ds(PAD + PRO, SEG)],
                              sems.at[SEM_MID]),
    ]
    cp_late = [
        pltpu.make_async_copy(x_hbm.at[pl.ds(PRO + SEG, S - PRO - SEG)],
                              xbuf.at[pl.ds(PAD + PRO + SEG, S - PRO - SEG)],
                              sems.at[SEM_LATE]),
    ] + [pltpu.make_async_copy(wo_hbm.at[:, pl.ds(c * 128, 128)],
                               wo_s.at[c], sems.at[SEM_LATE])
         for c in range(NC)]

    def mod_row(i, n, cols=slice(None)):
        return jnp.concatenate([mod_s[pl.ds(8 * i, 8), cols]] * (n // 8), axis=0)

    def prologue(st, wm_s, xn_s, g_s, tmp_s):
        wm32 = wm_s.bitcast(U32)
        srcs = (wq_hbm.bitcast(U32), wk_hbm.bitcast(U32), wv_hbm.bitcast(U32))
        dsts = (wq32, wk32, wv32)
        rings = (qring, kring, vring)

        def cp_st(j, s, sem):
            return pltpu.make_async_copy(srcs[j].at[:, s, :], st.at[3 * s + j],
                                         sems.at[sem])

        def cp_unit(u):
            sem = (SEM_U0 + U0_GROUP[u] if u <= NUA
                   else SEM_IT + (u - 1) // UPI)
            return cp_st(u % 3, u // 3, sem)

        def cp_wm(i):
            sem = (SEM_SA if i < 8 else
                   SEM_CA + (i - 8) // 4 if i < 16 else SEM_MID)
            return pltpu.make_async_copy(wmod_hbm.at[:, pl.ds(i * 128, 128)],
                                         wm_s.at[i], sems.at[sem])

        cp_wm2 = [cp_wm(i) for i in range(16, 48)]

        cp_c.start()
        cp_x0.start()
        for i in range(8, 16):
            cp_wm(i).start()
        for u in range(NUG):
            cp_unit(u).start()
        for i in range(8):
            cp_wm(i).start()
        for u in range(NUG, NU):
            cp_unit(u).start()
        for cp in cp_mid:
            cp.start()

        xbuf[pl.ds(0, PAD), :] = jnp.zeros((PAD, D), BF16)
        am_s[...] = jnp.zeros((16 * NWB, D), F32)

        cp_c.wait()
        cp_x0.wait()
        cf = c_s[...].astype(F32)
        sc = (cf * jax.nn.sigmoid(cf)).astype(BF16)
        sc8 = jnp.broadcast_to(sc, (8, D))

        def ln_body(i, carry):
            r = pl.multiple_of(i * 64, 64)
            xv = xbuf[pl.ds(pl.multiple_of(PAD + r, 8), 64), :].astype(F32)
            xn_s[pl.ds(r, 64), :] = _ln(xv)
            return carry

        lax.fori_loop(0, PRO // 64, ln_body, 0)

        def mod_slab(i):
            k, c = divmod(i, NC)
            part = _dot(sc8, _w(wm32, i))
            if k in (1, 4):
                part = part + 1.0
            mod_s[pl.ds(8 * k, 8), pl.ds(c * 128, 128)] = part

        for c0 in (8, 12):
            for i in range(c0, c0 + 4):
                cp_wm(i).wait()
            for i in range(c0, c0 + 4):
                mod_slab(i)

        def relayout(j, s):
            u = 3 * s + j
            for db in range(8):
                ev = st[u, pl.ds(db * 128, 64, stride=2), :]
                od = st[u, pl.ds(db * 128 + 1, 64, stride=2), :]
                rows = pl.ds(db * 64, 64)
                dsts[j][2 * s, rows, :] = (ev & U32(0xFFFF)) | (od << 16)
                dsts[j][2 * s + 1, rows, :] = (ev >> 16) | (od & U32(0xFFFF0000))

        def bulk(j, s, extras=(), mbs=range(PRO // 128)):
            extras = list(extras)
            for mb in mbs:
                lhs = hbuf[pl.ds(PAD + mb * 128, 128), :]
                for hh in range(2):
                    h = 2 * s + hh
                    rings[j][h, pl.ds(mb * 128, 128), :] = (
                        _dot(lhs, _w(dsts[j], h)).astype(BF16))
                    if extras:
                        extras.pop(0)()

        def bulk_g(u, mbs):
            for mb in mbs:
                rows = pl.ds(mb * 128, 128)
                lhs = g_s[rows, :]
                for hh in range(2):
                    tmp_s[2 * u + hh, rows, :] = _dot(
                        lhs, _w(dsts[u % 3], 2 * (u // 3) + hh))

        def add_shift(u, hh):
            h = 2 * (u // 3) + hh
            b = _dot(mod_row(0, 8).astype(BF16), _w(dsts[u % 3], h))
            rings[u % 3][h, pl.ds(0, PRO), :] = (
                tmp_s[2 * u + hh] + jnp.concatenate([b] * (PRO // 8), axis=0)
            ).astype(BF16)

        def wait_group(g):
            if g == U0_GROUP[NUG]:
                for i in range(8):
                    cp_wm(i).wait()
            for v in range(NUA + 1):
                if U0_GROUP[v] == g:
                    cp_unit(v).wait()

        def relayout_u(u):
            relayout(u % 3, u // 3)

        g_s[...] = (xn_s[...] * mod_row(1, PRO)).astype(BF16)
        wait_group(0)
        relayout_u(0)
        bulk_g(0, (0, 1))
        wait_group(1)
        relayout_u(1)
        bulk_g(0, (2, 3))
        wait_group(2)
        relayout_u(2)
        bulk_g(1, range(4))
        wait_group(3)
        relayout_u(3)
        bulk_g(2, range(4))
        bulk_g(3, (0, 1, 2))
        wait_group(4)
        relayout_u(4)
        for i in range(8):
            mod_slab(i)
        bulk_g(3, (3,))
        for mb in range(PRO // 128):
            rows = pl.ds(mb * 128, 128)
            hbuf[pl.ds(PAD + mb * 128, 128), :] = (
                xn_s[rows, :] * mod_row(1, 128) + mod_row(0, 128)).astype(BF16)
        shifts = [functools.partial(add_shift, v, hh)
                  for v in range(NUG) for hh in range(2)]
        bulk(4 % 3, 4 // 3, shifts, mbs=(0, 1, 2))
        wait_group(5)
        relayout_u(5)
        bulk(4 % 3, 4 // 3, shifts[6:], mbs=(3,))
        for u in range(5, NUA):
            if U0_GROUP[u + 1] != U0_GROUP[u]:
                wait_group(U0_GROUP[u + 1])
            relayout_u(u + 1)
            bulk(u % 3, u // 3)

        def grp_body(it, carry):
            s0 = it * (UPI // 3)

            @pl.when(it == NUA // UPI)
            def _():
                for cp in cp_wm2 + cp_late:
                    cp.start()

            for u in range(1, UPI + 1):
                cp_st(u % 3, s0 + u // 3, SEM_IT + it).wait()
            for u in range(UPI):
                relayout((u + 1) % 3, s0 + (u + 1) // 3)
                bulk(u % 3, s0 + u // 3)
            return carry

        lax.fori_loop(NUA // UPI, (NU - NUZ) // UPI, grp_body, 0)

        for u in range(NU - NUZ + 1, NU):
            cp_unit(u).wait()
        for cp in cp_mid + cp_wm2:
            cp.wait()
        mem_s[...] = m0_s[...].astype(F32)
        xv = xbuf[pl.ds(PAD + PRO, XR), :].astype(F32)
        hn_s[...] = _ln_mod(xv, mod_row(0, XR), mod_row(1, XR))
        for u in range(NU - NUZ, NU):
            if u + 1 < NU:
                relayout_u(u + 1)
            i0 = 16 + 4 * (u - (NU - NUZ))
            extras = []
            for i in range(i0, min(i0 + 4, 48)):
                extras += [functools.partial(mod_slab, i), lambda: None]
            bulk(u % 3, u // 3, extras)
        for cp in cp_late:
            cp.wait()

    pl.run_scoped(
        prologue,
        pltpu.VMEM((NU, D, DH), U32),
        pltpu.VMEM((48, D, 128), BF16),
        pltpu.VMEM((PRO, D), F32),
        pltpu.VMEM((PRO, D), BF16),
        pltpu.VMEM((2 * NUG, PRO, DH), F32),
    )

    def rest(w1_s, w3_s, w2_s, oring):
        w132 = w1_s.bitcast(U32)
        w332 = w3_s.bitcast(U32)
        w232 = w2_s.bitcast(U32)
        q32 = qring.bitcast(U32)
        k32 = kring.bitcast(U32)
        v32 = vring.bitcast(U32)

        cp_w1 = [pltpu.make_async_copy(w1_hbm.at[:, pl.ds(f * 128, 128)],
                                       w1_s.at[f], sems.at[SEM_FFN])
                 for f in range(NF)]
        cp_w3 = [pltpu.make_async_copy(w3_hbm.at[:, pl.ds(f * 128, 128)],
                                       w3_s.at[f], sems.at[SEM_FFN])
                 for f in range(NF)]
        cp_w2 = [pltpu.make_async_copy(w2_hbm.at[:, pl.ds(c * 128, 128)],
                                       w2_s.at[c], sems.at[SEM_FFN])
                 for c in range(NC)]
        for cp in cp_w1 + cp_w3 + cp_w2:
            cp.start()

        oring[:, pl.ds(OOFF - XR, XR), :] = jnp.zeros((H, XR, DH), BF16)

        def post_attn(a, r, n):
            x1 = xbuf[pl.ds(r, n), :].astype(F32) + mod_row(2, n) * a
            x1 = x1.astype(BF16)
            xbuf[pl.ds(r, n), :] = x1
            hbuf[pl.ds(r, n), :] = _ln_mod(
                x1.astype(F32), mod_row(3, n), mod_row(4, n)).astype(BF16)

        row = lax.broadcasted_iota(jnp.int32, (NP, NP), 0)
        col = lax.broadcasted_iota(jnp.int32, (NP, NP), 1)

        def second(i):
            return ((i >= SEG) & (i < 2 * SEG)) | (i >= 2 * SEG + M)

        same = second(row) == second(col)
        mask = same & ((row >= 2 * SEG) | (col >= 2 * SEG) | (col <= row))
        fill = jnp.where(same, -1e9, -jnp.inf).astype(F32)

        def step(s, carry, mem, split, maybe_last):
            lhs_c = [jnp.concatenate([hn_s[:, pl.ds(c * 128, 128)], mem[c]],
                                     axis=0).astype(BF16) for c in range(NC)]
            lhs = jnp.concatenate(lhs_c, axis=1)

            post_attn(ax_s[...], pl.multiple_of(XR * s, 8), XR)
            rn = pl.multiple_of(
                PAD + jnp.minimum(PRO + XR * (s + 1), S - XR), 8)
            hn_s[...] = _ln_mod(xbuf[pl.ds(rn, XR), :].astype(F32),
                                mod_row(0, XR), mod_row(1, XR))

            wp, rp, op, ow = carry
            wpos = [pl.multiple_of(_wrap(wp + 8 * j, RING), 8)
                    for j in range(XR // 8)]
            rpos = pl.multiple_of(rp, SEG // 2)
            opos = [pl.multiple_of(_wrap(op + 8 * j, ORING), 8)
                    for j in range(XR // 8 + 1)]
            owr = pl.multiple_of(ow, SEG)

            tails = {}
            xs = {}
            ps = {}
            lhs_o = {}

            def load(j, p):
                r32 = (q32, k32, v32)[j]
                xs[j, p] = [
                    pltpu.bitcast(r32[h, pl.ds(rpos, SEG // 2), :], BF16)
                    for h in (2 * p, 2 * p + 1)]

            def operand(j, p):
                tail = jnp.concatenate(
                    [tails.pop((j, 2 * p)), tails.pop((j, 2 * p + 1))], axis=0)
                return jnp.concatenate(
                    xs.pop((j, p)) + [tail.astype(BF16)], axis=0)

            low = {}
            if split:
                lhs_lo = jnp.concatenate(lhs_c[:NC // 2], axis=1)
                lhs_hi = jnp.concatenate(lhs_c[NC // 2:], axis=1)
                for h in range(2):
                    for j, w32 in enumerate((wq32, wk32, wv32)):
                        low[j, h] = _dot(lhs_lo, pltpu.bitcast(
                            w32[h, pl.ds(0, D // 4), :], BF16))

            def proj(j, h):
                w32, ring = ((wq32, qring), (wk32, kring), (wv32, vring))[j]
                if (j, h) in low:
                    t = _dot(lhs_hi, pltpu.bitcast(
                        w32[h, pl.ds(D // 4, D // 4), :], BF16)) + low[j, h]
                else:
                    t = _dot(lhs, _w(w32, h))
                for i in range(XR // 8):
                    ring[h, pl.ds(wpos[i], 8), :] = (
                        t[8 * i:8 * i + 8].astype(BF16))
                tails[j, h] = t[XR:]

            def qk(p):
                sc = lax.dot_general(operand(0, p), operand(1, p),
                                     (((1,), (1,)), ((), ())),
                                     preferred_element_type=F32)
                sc = jnp.where(mask, sc * SCALE, fill)
                mx = jnp.max(sc, axis=-1, keepdims=True)
                e = jnp.exp(sc - mx)
                l = jnp.sum(e, axis=-1, keepdims=True)
                ps[p] = (e * pl.reciprocal(l, approx=True)).astype(BF16)

            def pv(p):
                o = _dot(ps.pop(p), operand(2, p))
                for i, h in enumerate((2 * p, 2 * p + 1)):
                    ox = [oring[h, pl.ds(opos[k], 8), :] for k in range(XR // 8)]
                    om = o[2 * SEG + M * i:2 * SEG + M * (i + 1)]
                    if maybe_last:
                        om = jnp.where(
                            s == NSEG - 1,
                            oring[h, pl.ds(opos[3], 8), :].astype(F32), om)
                    last = jnp.concatenate(
                        [ox[2].astype(F32), om], axis=0).astype(BF16)
                    lhs_o[h] = jnp.concatenate([ox[0], ox[1], last], axis=0)
                for i, h in enumerate((2 * p, 2 * p + 1)):
                    oring[h, pl.ds(owr, SEG), :] = (
                        o[SEG * i:SEG * (i + 1)].astype(BF16))

            def wo_part(c, h0, h1):
                lo = jnp.concatenate([lhs_o[h] for h in range(h0, h1)], axis=1)
                w = pltpu.bitcast(wo32[c, pl.ds(h0 * 64, (h1 - h0) * 64), :], BF16)
                return _dot(lo, w)

            NPR = H // 2
            for t in range(NPR):
                if t >= 1:
                    load(0, t - 1)
                    load(1, t - 1)
                if t >= 2:
                    load(2, t - 2)
                for pos in range(6):
                    if t >= 1 and pos == (QPOS1 if t == 1 else QPOS):
                        qk(t - 1)
                    proj(pos % 3, 2 * t + pos // 3)
                if t >= 2:
                    pv(t - 2)
            HA = H - 4
            acc = {}
            mem_new = {}

            def wo_a(c):
                acc[c] = wo_part(c, 0, HA)

            def wo_b(c):
                a = wo_part(c, HA, H) + acc[c]
                ax_s[:, pl.ds(c * 128, 128)] = a[:XR]
                mem_new[c] = a[XR:]

            load(0, NPR - 1)
            load(1, NPR - 1)
            load(2, NPR - 2)
            wo_a(0)
            qk(NPR - 1)
            wo_a(1)
            pv(NPR - 2)
            load(2, NPR - 1)
            for c in (2, 3, 4):
                wo_a(c)
            pv(NPR - 1)
            for c in (5, 6):
                wo_a(c)
            for c in range(NC // 2):
                wo_b(c)
            wo_a(7)
            for c in range(NC // 2, NC):
                wo_b(c)
            return (_wrap(wp + XR, RING), _wrap(rp + SEG // 2, RING // 2),
                    _wrap(op + XR, ORING), _wrap(ow + SEG, ORING)), mem_new

        def steps(i, carry):
            mem = [mem_s[:, pl.ds(c * 128, 128)] for c in range(NC)]
            for u in range(UNROLL):
                carry, mem = step(i * UNROLL + u, carry, mem, split=u > 0,
                                  maybe_last=u == UNROLL - 1)
            for c in range(NC):
                mem_s[:, pl.ds(c * 128, 128)] = mem[c]
            return carry

        lax.fori_loop(0, NSEG // UNROLL, steps,
                      (jnp.int32(PRO), jnp.int32(0), jnp.int32(OOFF - XR),
                       jnp.int32(OOFF)))

        done = XR * (NSEG - 1) + M
        o32 = oring.bitcast(U32)

        def wo_bulk(i):
            p = pl.multiple_of(((done + OOFF) % ORING + i * WB) // 2, 8)
            lo = jnp.concatenate(
                [pltpu.bitcast(o32[h, pl.ds(p, WB // 2), :], BF16)
                 for h in range(H)], axis=1)
            return jnp.concatenate(
                [_dot(lo, _w(wo32, c)) for c in range(NC)], axis=1)

        for cp in cp_w1 + cp_w3 + cp_w2:
            cp.wait()

        def cp_out(r, n, part):
            cols = pl.ds(0, OC * 128) if part == 0 else pl.ds(OC * 128, D - OC * 128)
            return pltpu.make_async_copy(xbuf.at[pl.ds(PAD + r, n), cols],
                                         out_hbm.at[pl.ds(r, n), cols],
                                         sems.at[SEM_OUT])

        def ffn_body(i, carry, r0, n, with_wo):
            r = pl.multiple_of(r0 + i * n, 16)
            rows = pl.ds(pl.multiple_of(PAD + r, 16), n)
            if with_wo:
                a = wo_bulk(i)
                ra = pl.multiple_of(PAD + done + i * WB, 16)
            hv = hbuf[rows, :]
            act = []
            for f in range(NF):
                g = _dot(hv, _w(w132, f))
                u = _dot(hv, _w(w332, f))
                act.append((g * jax.nn.sigmoid(g) * u).astype(BF16))
            av = jnp.concatenate(act, axis=1)
            for c in range(NC):
                y = _dot(av, _w(w232, c))
                if with_wo:
                    for k in range(WB // 16):
                        if k * (NC - 1) // (WB // 16) == c:
                            post_attn(a[16 * k:16 * k + 16], ra + 16 * k, 16)
                    if c == NC - 2:
                        i16 = pl.multiple_of(i * 16, 16)
                        rp = jnp.where(i < 2, XR * NSEG + i16, 0)
                        post_attn(am_s[pl.ds(i16, 16), :],
                                  pl.multiple_of(rp, 16), 16)
                cs = pl.ds(c * 128, 128)
                x2 = xbuf[rows, cs].astype(F32) + mod_row(5, n, cs) * y
                xbuf[rows, cs] = x2.astype(BF16)
                if c == OC - 1:
                    cp_out(r, n, 0).start()
            cp_out(r, n, 1).start()
            return carry

        nfb = (S - NWB * FA) // FB
        lax.fori_loop(0, NWB, functools.partial(
            ffn_body, r0=0, n=FA, with_wo=True), 0)
        lax.fori_loop(0, nfb, functools.partial(
            ffn_body, r0=NWB * FA, n=FB, with_wo=False), 0)
        for part in range(2):
            for i in range(NWB):
                cp_out(i * FA, FA, part).wait()
            for i in range(nfb):
                cp_out(NWB * FA + i * FB, FB, part).wait()

    pl.run_scoped(
        rest,
        pltpu.VMEM((NF, D, 128), BF16),
        pltpu.VMEM((NF, D, 128), BF16),
        pltpu.VMEM((NC, F, 128), BF16),
        pltpu.VMEM((H, ORING, DH), BF16),
    )


@functools.partial(jax.jit, static_argnames=("A_seg_len",))
def pallas_adaLN_cond__memory_aug_recurrent_mem_tr__glu_gated_swiglu__prompt_kernel(
    A_x: jax.Array,
    A_mem0: jax.Array,
    A_Wq: jax.Array,
    A_Wk: jax.Array,
    A_Wv: jax.Array,
    A_Wo: jax.Array,
    A_seg_len,
    B_x: jax.Array,
    B_w1: jax.Array,
    B_w3: jax.Array,
    B_w2: jax.Array,
    c: jax.Array,
    w_mod: jax.Array,
):
    del B_x
    assert A_seg_len == SEG
    assert A_x.shape == (1, S, D) and A_mem0.shape == (1, M, D)
    assert A_Wq.shape == (D, H, DH) and B_w1.shape == (D, F)

    any_spec = pl.BlockSpec(memory_space=pl.ANY)
    out = pl.pallas_call(
        _kernel,
        out_shape=jax.ShapeDtypeStruct((S, D), BF16),
        in_specs=[any_spec] * 11,
        out_specs=any_spec,
        scratch_shapes=[
            pltpu.VMEM((H, D // 2, DH), U32),
            pltpu.VMEM((H, D // 2, DH), U32),
            pltpu.VMEM((H, D // 2, DH), U32),
            pltpu.VMEM((NC, H * DH, 128), BF16),
            pltpu.VMEM((2, PAD + S, D), BF16),
            pltpu.VMEM((H, RING, DH), BF16),
            pltpu.VMEM((H, RING, DH), BF16),
            pltpu.VMEM((H, RING, DH), BF16),
            pltpu.VMEM((6 * 8, D), F32),
            pltpu.VMEM((16 * NWB, D), F32),
            pltpu.VMEM((XR, D), F32),
            pltpu.VMEM((1, D), BF16),
            pltpu.VMEM((M, D), BF16),
            pltpu.SemaphoreType.DMA((NSEMS,)),
        ],
        compiler_params=pltpu.CompilerParams(
            vmem_limit_bytes=120 * 1024 * 1024),
        name="adaln_memtr_swiglu",
    )(
        A_x.reshape(S, D),
        A_mem0.reshape(M, D),
        A_Wq, A_Wk, A_Wv,
        A_Wo.reshape(H * DH, D),
        B_w1, B_w3, B_w2, c, w_mod,
    )
    return out.reshape(1, S, D)
```

```python
import functools

import jax
import jax.numpy as jnp
from jax import lax
import jax.experimental.pallas as pl
import jax.experimental.pallas.tpu as pltpu

BF16 = jnp.bfloat16
F32 = jnp.float32
U32 = jnp.uint32

S = 2048
D = 1024
H = 32
DH = 128
F = 3584
M = 8
SEG = 32
NSEG = S // SEG
XR = 24
PRO = S - XR * NSEG
RING = 544
ORING = 576
OOFF = 256
PAD = 48
NC = D // 128
NF = F // 128
FA = 128
FB = 208
OC = 7
NWB = 3
WB = 176
SH = 16
NPA, NPB = 11, 12
QPOS, QPOS1 = 2, 4
UNROLL = 4
NU = 3 * H // 2
UPI = 6
NUA = 12
NUZ = 12
XC = (S - PRO) * UPI // (NU - NUA)
NUG = 4
NP = 2 * (SEG + M)
EPS = 1e-5
SEM_FIRST, SEM_WO, SEM_MID, SEM_FFN, SEM_OUT = 0, 1, 2, 3, 4
SEM_CA = 5
SEM_U0 = SEM_CA + 2
U0_GROUP = (0, 1, 2, 3, 4, 5, 5, 5, 6, 6, 6, 6, 6)
SEM_SA = SEM_U0 + U0_GROUP[NUG]
SEM_IT = SEM_U0 + U0_GROUP[-1] + 1 - NUA // UPI
NSEMS = SEM_IT + NU // UPI
SCALE = DH ** -0.5


def _dot(a, b):
    return jnp.dot(a, b, preferred_element_type=F32)


def _w(ref32, i):
    return pltpu.bitcast(ref32[i], BF16)


def _wrap(i, n):
    return jnp.where(i >= n, i - n, i)


def _ln(x):
    mu = jnp.mean(x, axis=-1, keepdims=True)
    xc = x - mu
    var = jnp.mean(xc * xc, axis=-1, keepdims=True)
    return xc * lax.rsqrt(var + EPS)


def _ln_mod(x, shift, scale1):
    return _ln(x) * scale1 + shift


def _kernel(x_hbm, mem0_hbm, wq_hbm, wk_hbm, wv_hbm, wo_hbm, w1_hbm, w3_hbm,
            w2_hbm, c_hbm, wmod_hbm, out_hbm,
            wq32, wk32, wv32, wo_s, xh, qring, kring, vring,
            mod_s, mem_s, c_s, m0_s, sems):
    wo32 = wo_s.bitcast(U32)
    xbuf = xh.at[0]
    hbuf = xh.at[1]

    cp_x0 = pltpu.make_async_copy(x_hbm.at[pl.ds(0, PRO)],
                                  xbuf.at[pl.ds(PAD, PRO)], sems.at[SEM_FIRST])
    cp_c = pltpu.make_async_copy(c_hbm, c_s, sems.at[SEM_FIRST])
    cp_m0 = pltpu.make_async_copy(mem0_hbm, m0_s, sems.at[SEM_MID])
    cp_wo = [pltpu.make_async_copy(wo_hbm.at[:, pl.ds(c * 128, 128)],
                                   wo_s.at[c], sems.at[SEM_WO])
             for c in range(NC)]

    def cp_x(k, sem):
        r = PRO + k * XC
        if not isinstance(k, int):
            r = pl.multiple_of(r, XC)
        return pltpu.make_async_copy(x_hbm.at[pl.ds(r, XC)],
                                     xbuf.at[pl.ds(PAD + r, XC)], sems.at[sem])

    def mod_row(i, n, cols=slice(None)):
        return jnp.concatenate([mod_s[pl.ds(8 * i, 8), cols]] * (n // 8), axis=0)

    def prologue(st, wm_s, xn_s, g_s, h0_s, tmp_s):
        wm32 = wm_s.bitcast(U32)
        srcs = (wq_hbm.bitcast(U32), wk_hbm.bitcast(U32), wv_hbm.bitcast(U32))
        dsts = (wq32, wk32, wv32)
        rings = (qring, kring, vring)

        def cp_st(j, s, sem):
            return pltpu.make_async_copy(srcs[j].at[:, s, :], st.at[3 * s + j],
                                         sems.at[sem])

        def cp_unit(u):
            sem = (SEM_U0 + U0_GROUP[u] if u <= NUA
                   else SEM_IT + (u - 1) // UPI)
            return cp_st(u % 3, u // 3, sem)

        def cp_wm(i):
            sem = (SEM_SA if i < 8 else
                   SEM_CA + (i - 8) // 4 if i < 16 else SEM_MID)
            return pltpu.make_async_copy(wmod_hbm.at[:, pl.ds(i * 128, 128)],
                                         wm_s.at[i], sems.at[sem])

        it0, it1 = NUA // UPI, (NU - NUZ) // UPI
        cp_mid = ([cp_x(k, SEM_MID) for k in range(it1 - it0, NU // UPI - it0)]
                  + [cp_wm(i) for i in range(16, 48)])

        cp_c.start()
        cp_x0.start()
        for i in range(8, 16):
            cp_wm(i).start()
        for u in range(NUG):
            cp_unit(u).start()
        for i in range(8):
            cp_wm(i).start()
        for u in range(NUG, NU):
            cp_unit(u).start()
            if u % UPI == 0 and it0 < u // UPI <= it1:
                cp_x(u // UPI - 1 - it0, SEM_IT + u // UPI - 1).start()
        cp_m0.start()

        xbuf[pl.ds(0, PAD), :] = jnp.zeros((PAD, D), BF16)

        cp_c.wait()
        cp_x0.wait()
        cf = c_s[...].astype(F32)
        sc = (cf * jax.nn.sigmoid(cf)).astype(BF16)
        sc8 = jnp.broadcast_to(sc, (8, D))

        def ln_body(i, carry):
            r = pl.multiple_of(i * 64, 64)
            xv = xbuf[pl.ds(pl.multiple_of(PAD + r, 8), 64), :].astype(F32)
            xn_s[pl.ds(r, 64), :] = _ln(xv)
            return carry

        lax.fori_loop(0, PRO // 64, ln_body, 0)

        def mod_slab(i):
            k, c = divmod(i, NC)
            part = _dot(sc8, _w(wm32, i))
            if k in (1, 4):
                part = part + 1.0
            mod_s[pl.ds(8 * k, 8), pl.ds(c * 128, 128)] = part

        for c0 in (8, 12):
            for i in range(c0, c0 + 4):
                cp_wm(i).wait()
            for i in range(c0, c0 + 4):
                mod_slab(i)

        def relayout(j, s):
            u = 3 * s + j
            for db in range(8):
                ev = st[u, pl.ds(db * 128, 64, stride=2), :]
                od = st[u, pl.ds(db * 128 + 1, 64, stride=2), :]
                rows = pl.ds(db * 64, 64)
                dsts[j][2 * s, rows, :] = (ev & U32(0xFFFF)) | (od << 16)
                dsts[j][2 * s + 1, rows, :] = (ev >> 16) | (od & U32(0xFFFF0000))

        def bulk(j, s, extras=(), mbs=range(PRO // 128)):
            extras = list(extras)
            for mb in mbs:
                lhs = h0_s[pl.ds(mb * 128, 128), :]
                for hh in range(2):
                    h = 2 * s + hh
                    t = _dot(lhs, _w(dsts[j], h))
                    if extras:
                        t = extras.pop(0)(t)
                    rings[j][h, pl.ds(mb * 128, 128), :] = t.astype(BF16)

        def bulk_g(u, mbs):
            for mb in mbs:
                rows = pl.ds(mb * 128, 128)
                lhs = g_s[rows, :]
                for hh in range(2):
                    tmp_s[2 * u + hh, rows, :] = _dot(
                        lhs, _w(dsts[u % 3], 2 * (u // 3) + hh))

        def add_shift(u, hh):
            h = 2 * (u // 3) + hh
            b = _dot(mod_row(0, 8).astype(BF16), _w(dsts[u % 3], h))
            rings[u % 3][h, pl.ds(0, PRO), :] = (
                tmp_s[2 * u + hh] + jnp.concatenate([b] * (PRO // 8), axis=0)
            ).astype(BF16)

        def wait_group(g):
            if g == U0_GROUP[NUG]:
                for i in range(8):
                    cp_wm(i).wait()
            for v in range(NUA + 1):
                if U0_GROUP[v] == g:
                    cp_unit(v).wait()

        def relayout_u(u):
            relayout(u % 3, u // 3)

        g_s[...] = (xn_s[...] * mod_row(1, PRO)).astype(BF16)
        wait_group(0)
        relayout_u(0)
        bulk_g(0, (0, 1))
        wait_group(1)
        relayout_u(1)
        bulk_g(0, (2, 3))
        wait_group(2)
        relayout_u(2)
        bulk_g(1, range(4))
        wait_group(3)
        relayout_u(3)
        bulk_g(2, range(4))
        bulk_g(3, (0, 1, 2))
        wait_group(4)
        relayout_u(4)
        for i in range(8):
            mod_slab(i)
        bulk_g(3, (3,))
        for mb in range(PRO // 128):
            rows = pl.ds(mb * 128, 128)
            h0_s[rows, :] = (
                xn_s[rows, :] * mod_row(1, 128) + mod_row(0, 128)).astype(BF16)
        shifts = [lambda t, v=v, hh=hh: (add_shift(v, hh), t)[1]
                  for v in range(NUG) for hh in range(2)]
        bulk(4 % 3, 4 // 3, shifts, mbs=(0, 1, 2))
        wait_group(5)
        relayout_u(5)
        bulk(4 % 3, 4 // 3, shifts[6:], mbs=(3,))
        for u in range(5, NUA):
            if U0_GROUP[u + 1] != U0_GROUP[u]:
                wait_group(U0_GROUP[u + 1])
            relayout_u(u + 1)
            bulk(u % 3, u // 3)

        pending = []

        def tie(never, a, b):
            top = jnp.where(never, a[:8, :128], b[:8, :128])
            if b.shape[1] > 128:
                top = jnp.concatenate([top, b[:8, 128:]], axis=1)
            return jnp.concatenate([top, b[8:]], axis=0)

        def ln1_piece(r, t):
            never = r < 0
            if pending:
                t = tie(never, pending.pop(), t)
            rows = pl.ds(pl.multiple_of(r, 16), 16)
            xv = tie(never, t, xbuf[rows, :].astype(F32))
            hv = _ln_mod(xv, mod_row(0, 16), mod_row(1, 16))
            hbuf[rows, :] = hv.astype(BF16)
            pending.append(hv[8:])
            return t

        def unit_extras(r, u, more=()):
            slots = [lambda t: t] * 8
            for k, f in enumerate(more):
                slots[2 * k + 1] = lambda t, f=f: (f(), t)[1]
            for k in range(XC // 16):
                d = k * (8 * UPI) // (XC // 16)
                if d // 8 == u % UPI:
                    slots[d % 8] = lambda t, g=slots[d % 8], k=k: (
                        ln1_piece(r + 16 * k, g(t)))
            return slots

        def grp_body(it, r):
            s0 = it * (UPI // 3)

            @pl.when(it == it0)
            def _():
                for cp in cp_mid + cp_wo:
                    cp.start()

            for u in range(1, UPI + 1):
                cp_st(u % 3, s0 + u // 3, SEM_IT + it).wait()
            cp_x(it - it0, SEM_IT + it).wait()
            for u in range(UPI):
                relayout((u + 1) % 3, s0 + (u + 1) // 3)
                bulk(u % 3, s0 + u // 3, unit_extras(r, u))
            pending.clear()
            return r + XC

        r1 = lax.fori_loop(it0, it1, grp_body, jnp.int32(PAD + PRO))

        for u in range(NU - NUZ + 1, NU):
            cp_unit(u).wait()
        for cp in cp_mid + [cp_m0]:
            cp.wait()
        mem_s[...] = m0_s[...].astype(F32)
        for u in range(NU - NUZ, NU):
            if u + 1 < NU:
                relayout_u(u + 1)
            v = u - (NU - NUZ)
            bulk(u % 3, u // 3, unit_extras(
                r1 + v // UPI * XC, u,
                [functools.partial(mod_slab, i)
                 for i in range(16 + 4 * v, min(20 + 4 * v, 48))]))
        for cp in cp_wo:
            cp.wait()

    pl.run_scoped(
        prologue,
        pltpu.VMEM((NU, D, DH), U32),
        pltpu.VMEM((48, D, 128), BF16),
        pltpu.VMEM((PRO, D), F32),
        pltpu.VMEM((PRO, D), BF16),
        pltpu.VMEM((PRO, D), BF16),
        pltpu.VMEM((2 * NUG, PRO, DH), F32),
    )

    def rest(w1_s, w3_s, w2_s, oring, abuf):
        w132 = w1_s.bitcast(U32)
        w332 = w3_s.bitcast(U32)
        w232 = w2_s.bitcast(U32)
        q32 = qring.bitcast(U32)
        k32 = kring.bitcast(U32)
        v32 = vring.bitcast(U32)

        cp_w1 = [pltpu.make_async_copy(w1_hbm.at[:, pl.ds(f * 128, 128)],
                                       w1_s.at[f], sems.at[SEM_FFN])
                 for f in range(NF)]
        cp_w3 = [pltpu.make_async_copy(w3_hbm.at[:, pl.ds(f * 128, 128)],
                                       w3_s.at[f], sems.at[SEM_FFN])
                 for f in range(NF)]
        cp_w2 = [pltpu.make_async_copy(w2_hbm.at[:, pl.ds(c * 128, 128)],
                                       w2_s.at[c], sems.at[SEM_FFN])
                 for c in range(NC)]
        for cp in cp_w1 + cp_w3 + cp_w2:
            cp.start()

        oring[:, pl.ds(OOFF - XR, XR), :] = jnp.zeros((H, XR, DH), BF16)

        abuf[pl.ds(0, PAD), :] = jnp.zeros((PAD, D), BF16)

        def post_attn(r, n):
            a = abuf[pl.ds(r, n), :].astype(F32)
            x1 = xbuf[pl.ds(r, n), :].astype(F32) + mod_row(2, n) * a
            x1 = x1.astype(BF16)
            xbuf[pl.ds(r, n), :] = x1
            hbuf[pl.ds(r, n), :] = _ln_mod(
                x1.astype(F32), mod_row(3, n), mod_row(4, n)).astype(BF16)

        row = lax.broadcasted_iota(jnp.int32, (NP, NP), 0)
        col = lax.broadcasted_iota(jnp.int32, (NP, NP), 1)

        def second(i):
            return ((i >= SEG) & (i < 2 * SEG)) | (i >= 2 * SEG + M)

        same = second(row) == second(col)
        mask = same & ((row >= 2 * SEG) | (col >= 2 * SEG) | (col <= row))
        fill = jnp.where(same, -1e9, -jnp.inf).astype(F32)

        def step(s, carry, mem, split, maybe_last):
            hr = pl.multiple_of(PAD + PRO + XR * s, 8)
            lhs_c = []
            for c in range(NC):
                cs = pl.ds(c * 128, 128)
                h8 = hbuf[pl.ds(hr + 16, 8), cs].astype(F32)
                lhs_c.append(jnp.concatenate(
                    [hbuf[pl.ds(hr, 16), cs],
                     jnp.concatenate([h8, mem[c]], axis=0).astype(BF16)], axis=0))
            lhs = jnp.concatenate(lhs_c, axis=1)

            if maybe_last:
                post_attn(pl.multiple_of(PAD + (s // UNROLL) * SH, 16), SH)

            wp, rp, op, ow = carry
            wpos = [pl.multiple_of(_wrap(wp + 8 * j, RING), 8)
                    for j in range(XR // 8)]
            rpos = pl.multiple_of(rp, SEG // 2)
            opos = [pl.multiple_of(_wrap(op + 8 * j, ORING), 8)
                    for j in range(XR // 8 + 1)]
            owr = pl.multiple_of(ow, SEG)

            tails = {}
            xs = {}
            ps = {}
            lhs_o = {}

            def load(j, p):
                r32 = (q32, k32, v32)[j]
                xs[j, p] = [
                    pltpu.bitcast(r32[h, pl.ds(rpos, SEG // 2), :], BF16)
                    for h in (2 * p, 2 * p + 1)]

            def operand(j, p):
                tail = jnp.concatenate(
                    [tails.pop((j, 2 * p)), tails.pop((j, 2 * p + 1))], axis=0)
                return jnp.concatenate(
                    xs.pop((j, p)) + [tail.astype(BF16)], axis=0)

            low = {}
            if split:
                lhs_lo = jnp.concatenate(lhs_c[:NC // 2], axis=1)
                lhs_hi = jnp.concatenate(lhs_c[NC // 2:], axis=1)
                for h in range(2):
                    for j, w32 in enumerate((wq32, wk32, wv32)):
                        low[j, h] = _dot(lhs_lo, pltpu.bitcast(
                            w32[h, pl.ds(0, D // 4), :], BF16))

            def proj(j, h):
                w32, ring = ((wq32, qring), (wk32, kring), (wv32, vring))[j]
                if (j, h) in low:
                    t = _dot(lhs_hi, pltpu.bitcast(
                        w32[h, pl.ds(D // 4, D // 4), :], BF16)) + low[j, h]
                else:
                    t = _dot(lhs, _w(w32, h))
                for i in range(XR // 8):
                    ring[h, pl.ds(wpos[i], 8), :] = (
                        t[8 * i:8 * i + 8].astype(BF16))
                tails[j, h] = t[XR:]

            def qk(p):
                sc = lax.dot_general(operand(0, p), operand(1, p),
                                     (((1,), (1,)), ((), ())),
                                     preferred_element_type=F32)
                sc = jnp.where(mask, sc * SCALE, fill)
                mx = jnp.max(sc, axis=-1, keepdims=True)
                e = jnp.exp(sc - mx)
                l = jnp.sum(e, axis=-1, keepdims=True)
                ps[p] = (e * pl.reciprocal(l, approx=True)).astype(BF16)

            def pv(p):
                o = _dot(ps.pop(p), operand(2, p))
                for i, h in enumerate((2 * p, 2 * p + 1)):
                    ox = [oring[h, pl.ds(opos[k], 8), :] for k in range(XR // 8)]
                    om = o[2 * SEG + M * i:2 * SEG + M * (i + 1)]
                    if maybe_last:
                        om = jnp.where(
                            s == NSEG - 1,
                            oring[h, pl.ds(opos[3], 8), :].astype(F32), om)
                    last = jnp.concatenate(
                        [ox[2].astype(F32), om], axis=0).astype(BF16)
                    lhs_o[h] = jnp.concatenate([ox[0], ox[1], last], axis=0)
                for i, h in enumerate((2 * p, 2 * p + 1)):
                    oring[h, pl.ds(owr, SEG), :] = (
                        o[SEG * i:SEG * (i + 1)].astype(BF16))

            def wo_part(c, h0, h1):
                lo = jnp.concatenate([lhs_o[h] for h in range(h0, h1)], axis=1)
                w = pltpu.bitcast(wo32[c, pl.ds(h0 * 64, (h1 - h0) * 64), :], BF16)
                return _dot(lo, w)

            NPR = H // 2
            for t in range(NPR):
                if t >= 1:
                    load(0, t - 1)
                    load(1, t - 1)
                if t >= 2:
                    load(2, t - 2)
                for pos in range(6):
                    if t >= 1 and pos == (QPOS1 if t == 1 else QPOS):
                        qk(t - 1)
                    proj(pos % 3, 2 * t + pos // 3)
                if t >= 2:
                    pv(t - 2)
            HA = H - 4
            ar = pl.multiple_of(PAD - XR + XR * s, 8)
            acc = {}
            mem_new = {}

            def wo_a(c):
                acc[c] = wo_part(c, 0, HA)

            def wo_b(c):
                a = wo_part(c, HA, H) + acc[c]
                n = XR + M if maybe_last else XR
                abuf[pl.ds(ar, n), pl.ds(c * 128, 128)] = a[:n].astype(BF16)
                mem_new[c] = a[XR:]

            load(0, NPR - 1)
            load(1, NPR - 1)
            load(2, NPR - 2)
            wo_a(0)
            qk(NPR - 1)
            wo_a(1)
            pv(NPR - 2)
            load(2, NPR - 1)
            for c in (2, 3, 4):
                wo_a(c)
            pv(NPR - 1)
            for c in (5, 6):
                wo_a(c)
            for c in range(NC // 2):
                wo_b(c)
            wo_a(7)
            for c in range(NC // 2, NC):
                wo_b(c)
            return (_wrap(wp + XR, RING), _wrap(rp + SEG // 2, RING // 2),
                    _wrap(op + XR, ORING), _wrap(ow + SEG, ORING)), mem_new

        def steps(i, carry):
            mem = [mem_s[:, pl.ds(c * 128, 128)] for c in range(NC)]
            for u in range(UNROLL):
                carry, mem = step(i * UNROLL + u, carry, mem, split=u > 0,
                                  maybe_last=u == UNROLL - 1)
            for c in range(NC):
                mem_s[:, pl.ds(c * 128, 128)] = mem[c]
            return carry

        lax.fori_loop(0, NSEG // UNROLL, steps,
                      (jnp.int32(PRO), jnp.int32(0), jnp.int32(OOFF - XR),
                       jnp.int32(OOFF)))

        done = XR * (NSEG - 1) + M
        o32 = oring.bitcast(U32)

        def wo_bulk(i):
            p = pl.multiple_of(((done + OOFF) % ORING + i * WB) // 2, 8)
            lo = jnp.concatenate(
                [pltpu.bitcast(o32[h, pl.ds(p, WB // 2), :], BF16)
                 for h in range(H)], axis=1)
            rows = pl.ds(pl.multiple_of(PAD + done + i * WB, 16), WB)
            for c in range(NC):
                abuf[rows, pl.ds(c * 128, 128)] = (
                    _dot(lo, _w(wo32, c)).astype(BF16))

        for cp in cp_w1 + cp_w3 + cp_w2:
            cp.wait()

        def cp_out(r, n, part):
            cols = pl.ds(0, OC * 128) if part == 0 else pl.ds(OC * 128, D - OC * 128)
            return pltpu.make_async_copy(xbuf.at[pl.ds(PAD + r, n), cols],
                                         out_hbm.at[pl.ds(r, n), cols],
                                         sems.at[SEM_OUT])

        def ffn_body(i, carry, r0, n, with_wo, p0, npc):
            r = pl.multiple_of(r0 + i * n, 16)
            rows = pl.ds(pl.multiple_of(PAD + r, 16), n)
            if with_wo:
                wo_bulk(i)
            hv = hbuf[rows, :]
            act = []
            for f in range(NF):
                g = _dot(hv, _w(w132, f))
                u = _dot(hv, _w(w332, f))
                act.append((g * jax.nn.sigmoid(g) * u).astype(BF16))
            av = jnp.concatenate(act, axis=1)
            for c in range(NC):
                y = _dot(av, _w(w232, c))
                for k in range(npc):
                    if k * (NC - 1) // npc == c:
                        pr = p0 + (i * npc + k) * 16
                        post_attn(pl.multiple_of(
                            jnp.where(pr < S, PAD + pr, 0), 16), 16)
                cs = pl.ds(c * 128, 128)
                x2 = xbuf[rows, cs].astype(F32) + mod_row(5, n, cs) * y
                xbuf[rows, cs] = x2.astype(BF16)
                if c == OC - 1:
                    cp_out(r, n, 0).start()
            cp_out(r, n, 1).start()
            return carry

        nfb = (S - NWB * FA) // FB
        pa = SH * (NSEG // UNROLL)
        lax.fori_loop(0, NWB, functools.partial(
            ffn_body, r0=0, n=FA, with_wo=True, p0=pa, npc=NPA), 0)
        lax.fori_loop(0, nfb, functools.partial(
            ffn_body, r0=NWB * FA, n=FB, with_wo=False,
            p0=pa + NWB * NPA * 16, npc=NPB), 0)
        for part in range(2):
            for i in range(NWB):
                cp_out(i * FA, FA, part).wait()
            for i in range(nfb):
                cp_out(NWB * FA + i * FB, FB, part).wait()

    pl.run_scoped(
        rest,
        pltpu.VMEM((NF, D, 128), BF16),
        pltpu.VMEM((NF, D, 128), BF16),
        pltpu.VMEM((NC, F, 128), BF16),
        pltpu.VMEM((H, ORING, DH), BF16),
        pltpu.VMEM((PAD + S, D), BF16),
    )


@functools.partial(jax.jit, static_argnames=("A_seg_len",))
def pallas_adaLN_cond__memory_aug_recurrent_mem_tr__glu_gated_swiglu__prompt_kernel(
    A_x: jax.Array,
    A_mem0: jax.Array,
    A_Wq: jax.Array,
    A_Wk: jax.Array,
    A_Wv: jax.Array,
    A_Wo: jax.Array,
    A_seg_len,
    B_x: jax.Array,
    B_w1: jax.Array,
    B_w3: jax.Array,
    B_w2: jax.Array,
    c: jax.Array,
    w_mod: jax.Array,
):
    del B_x
    assert A_seg_len == SEG
    assert A_x.shape == (1, S, D) and A_mem0.shape == (1, M, D)
    assert A_Wq.shape == (D, H, DH) and B_w1.shape == (D, F)

    any_spec = pl.BlockSpec(memory_space=pl.ANY)
    out = pl.pallas_call(
        _kernel,
        out_shape=jax.ShapeDtypeStruct((S, D), BF16),
        in_specs=[any_spec] * 11,
        out_specs=any_spec,
        scratch_shapes=[
            pltpu.VMEM((H, D // 2, DH), U32),
            pltpu.VMEM((H, D // 2, DH), U32),
            pltpu.VMEM((H, D // 2, DH), U32),
            pltpu.VMEM((NC, H * DH, 128), BF16),
            pltpu.VMEM((2, PAD + S, D), BF16),
            pltpu.VMEM((H, RING, DH), BF16),
            pltpu.VMEM((H, RING, DH), BF16),
            pltpu.VMEM((H, RING, DH), BF16),
            pltpu.VMEM((6 * 8, D), F32),
            pltpu.VMEM((M, D), F32),
            pltpu.VMEM((1, D), BF16),
            pltpu.VMEM((M, D), BF16),
            pltpu.SemaphoreType.DMA((NSEMS,)),
        ],
        compiler_params=pltpu.CompilerParams(
            vmem_limit_bytes=120 * 1024 * 1024),
        name="adaln_memtr_swiglu",
    )(
        A_x.reshape(S, D),
        A_mem0.reshape(M, D),
        A_Wq, A_Wk, A_Wv,
        A_Wo.reshape(H * DH, D),
        B_w1, B_w3, B_w2, c, w_mod,
    )
    return out.reshape(1, S, D)
```

```python
import functools

import jax
import jax.numpy as jnp
from jax import lax
import jax.experimental.pallas as pl
import jax.experimental.pallas.tpu as pltpu

BF16 = jnp.bfloat16
F32 = jnp.float32
U32 = jnp.uint32

S = 2048
D = 1024
H = 32
DH = 128
F = 3584
M = 8
SEG = 32
NSEG = S // SEG
XR = 24
PRO = S - XR * NSEG
RING = 544
ORING = 576
OOFF = 256
PAD = 48
NC = D // 128
NF = F // 128
FA = 128
FB = 208
OC = 7
NWB = 3
WB = 176
SH = 16
NPA, NPB = 11, 12
QPOS, QPOS1 = 2, 4
UNROLL = 4
NU = 3 * H // 2
UPI = 6
NUA = 12
NUZ = 12
XC = (S - PRO) * UPI // (NU - NUA)
NUG = 5
NP = 2 * (SEG + M)
EPS = 1e-5
SEM_FIRST, SEM_WO, SEM_MID, SEM_FFN, SEM_OUT = 0, 1, 2, 3, 4
SEM_CA = 5
SEM_U0 = SEM_CA + 2
U0_GROUP = (0, 1, 2, 3, 3, 4, 5, 5, 5, 6, 6, 6, 6)
SEM_SA = SEM_U0 + U0_GROUP[NUG]
SEM_IT = SEM_U0 + U0_GROUP[-1] + 1 - NUA // UPI
NSEMS = SEM_IT + NU // UPI
SCALE = DH ** -0.5


def _dot(a, b):
    return jnp.dot(a, b, preferred_element_type=F32)


def _w(ref32, i):
    return pltpu.bitcast(ref32[i], BF16)


def _wrap(i, n):
    return jnp.where(i >= n, i - n, i)


def _ln(x):
    mu = jnp.mean(x, axis=-1, keepdims=True)
    xc = x - mu
    var = jnp.mean(xc * xc, axis=-1, keepdims=True)
    return xc * lax.rsqrt(var + EPS)


def _ln_mod(x, shift, scale1):
    return _ln(x) * scale1 + shift


def _kernel(x_hbm, mem0_hbm, wq_hbm, wk_hbm, wv_hbm, wo_hbm, w1_hbm, w3_hbm,
            w2_hbm, c_hbm, wmod_hbm, out_hbm,
            wq32, wk32, wv32, wo_s, xh, qring, kring, vring,
            mod_s, mem_s, c_s, m0_s, sems):
    wo32 = wo_s.bitcast(U32)
    xbuf = xh.at[0]
    hbuf = xh.at[1]

    cp_x0 = pltpu.make_async_copy(x_hbm.at[pl.ds(0, PRO)],
                                  xbuf.at[pl.ds(PAD, PRO)], sems.at[SEM_FIRST])
    cp_c = pltpu.make_async_copy(c_hbm, c_s, sems.at[SEM_FIRST])
    cp_m0 = pltpu.make_async_copy(mem0_hbm, m0_s, sems.at[SEM_MID])
    cp_wo = [pltpu.make_async_copy(wo_hbm.at[:, pl.ds(c * 128, 128)],
                                   wo_s.at[c], sems.at[SEM_WO])
             for c in range(NC)]

    def cp_x(k, sem):
        r = PRO + k * XC
        if not isinstance(k, int):
            r = pl.multiple_of(r, XC)
        return pltpu.make_async_copy(x_hbm.at[pl.ds(r, XC)],
                                     xbuf.at[pl.ds(PAD + r, XC)], sems.at[sem])

    def mod_row(i, n, cols=slice(None)):
        return jnp.concatenate([mod_s[pl.ds(8 * i, 8), cols]] * (n // 8), axis=0)

    def prologue(st, wm_s, xn_s, g_s, h0_s, tmp_s):
        wm32 = wm_s.bitcast(U32)
        srcs = (wq_hbm.bitcast(U32), wk_hbm.bitcast(U32), wv_hbm.bitcast(U32))
        dsts = (wq32, wk32, wv32)
        rings = (qring, kring, vring)

        def cp_st(j, s, sem):
            return pltpu.make_async_copy(srcs[j].at[:, s, :], st.at[3 * s + j],
                                         sems.at[sem])

        def cp_unit(u):
            sem = (SEM_U0 + U0_GROUP[u] if u <= NUA
                   else SEM_IT + (u - 1) // UPI)
            return cp_st(u % 3, u // 3, sem)

        def cp_wm(i):
            sem = (SEM_SA if i < 8 else
                   SEM_CA + (i - 8) // 4 if i < 16 else SEM_MID)
            return pltpu.make_async_copy(wmod_hbm.at[:, pl.ds(i * 128, 128)],
                                         wm_s.at[i], sems.at[sem])

        it0, it1 = NUA // UPI, (NU - NUZ) // UPI
        cp_mid = ([cp_x(k, SEM_MID) for k in range(it1 - it0, NU // UPI - it0)]
                  + [cp_wm(i) for i in range(16, 48)])

        cp_c.start()
        cp_x0.start()
        cp_unit(0).start()
        for i in range(8, 16):
            cp_wm(i).start()
        for u in range(1, NUG):
            cp_unit(u).start()
        for i in range(8):
            cp_wm(i).start()
        for u in range(NUG, NU):
            cp_unit(u).start()
            if u % UPI == 0 and it0 < u // UPI <= it1:
                cp_x(u // UPI - 1 - it0, SEM_IT + u // UPI - 1).start()
        cp_m0.start()

        xbuf[pl.ds(0, PAD), :] = jnp.zeros((PAD, D), BF16)

        cp_c.wait()
        cp_x0.wait()
        cf = c_s[...].astype(F32)
        sc = (cf * jax.nn.sigmoid(cf)).astype(BF16)
        sc8 = jnp.broadcast_to(sc, (8, D))

        def ln_body(i, carry):
            r = pl.multiple_of(i * 64, 64)
            xv = xbuf[pl.ds(pl.multiple_of(PAD + r, 8), 64), :].astype(F32)
            xn_s[pl.ds(r, 64), :] = _ln(xv)
            return carry

        lax.fori_loop(0, PRO // 64, ln_body, 0)

        def mod_slab(i):
            k, c = divmod(i, NC)
            part = _dot(sc8, _w(wm32, i))
            if k in (1, 4):
                part = part + 1.0
            mod_s[pl.ds(8 * k, 8), pl.ds(c * 128, 128)] = part

        def relayout(j, s):
            u = 3 * s + j
            for db in range(8):
                ev = st[u, pl.ds(db * 128, 64, stride=2), :]
                od = st[u, pl.ds(db * 128 + 1, 64, stride=2), :]
                rows = pl.ds(db * 64, 64)
                dsts[j][2 * s, rows, :] = (ev & U32(0xFFFF)) | (od << 16)
                dsts[j][2 * s + 1, rows, :] = (ev >> 16) | (od & U32(0xFFFF0000))

        def bulk(j, s, extras=(), mbs=range(PRO // 128)):
            extras = list(extras)
            for mb in mbs:
                lhs = h0_s[pl.ds(mb * 128, 128), :]
                for hh in range(2):
                    h = 2 * s + hh
                    t = _dot(lhs, _w(dsts[j], h))
                    if extras:
                        t = extras.pop(0)(t)
                    rings[j][h, pl.ds(mb * 128, 128), :] = t.astype(BF16)

        def bulk_g(u, mbs):
            for mb in mbs:
                rows = pl.ds(mb * 128, 128)
                lhs = g_s[rows, :]
                for hh in range(2):
                    tmp_s[2 * u + hh, rows, :] = _dot(
                        lhs, _w(dsts[u % 3], 2 * (u // 3) + hh))

        def add_shift(u, hh):
            h = 2 * (u // 3) + hh
            b = _dot(mod_row(0, 8).astype(BF16), _w(dsts[u % 3], h))
            rings[u % 3][h, pl.ds(0, PRO), :] = (
                tmp_s[2 * u + hh] + jnp.concatenate([b] * (PRO // 8), axis=0)
            ).astype(BF16)

        def wait_group(g):
            if g == U0_GROUP[NUG]:
                for i in range(8):
                    cp_wm(i).wait()
            for v in range(NUA + 1):
                if U0_GROUP[v] == g:
                    cp_unit(v).wait()

        def relayout_u(u):
            relayout(u % 3, u // 3)

        def scale_half(k):
            for i in range(8 + 4 * k, 12 + 4 * k):
                mod_slab(i)
            cols = pl.ds(k * (D // 2), D // 2)
            g_s[:, cols] = (xn_s[:, cols] * mod_row(1, PRO, cols)).astype(BF16)

        def first_half(k, mbs):
            for mb in mbs:
                rows = pl.ds(mb * 128, 128)
                lhs = g_s[rows, pl.ds(k * (D // 2), D // 2)]
                for hh in range(2):
                    t = _dot(lhs, pltpu.bitcast(
                        wq32[hh, pl.ds(k * (D // 4), D // 4), :], BF16))
                    tmp_s[hh, rows, :] = t if k == 0 else t + tmp_s[hh, rows, :]

        wait_group(0)
        relayout_u(0)
        for k in range(2):
            for i in range(8 + 4 * k, 12 + 4 * k):
                cp_wm(i).wait()
            scale_half(k)
            first_half(k, range(4))
        wait_group(1)
        relayout_u(1)
        bulk_g(1, (0, 1, 2))
        wait_group(2)
        relayout_u(2)
        bulk_g(1, (3,))
        bulk_g(2, (0, 1, 2))
        wait_group(3)
        relayout_u(3)
        bulk_g(2, (3,))
        relayout_u(4)
        bulk_g(3, range(4))
        bulk_g(4, (0, 1, 2))
        wait_group(4)
        relayout_u(5)
        for i in range(8):
            mod_slab(i)
        bulk_g(4, (3,))
        for mb in range(PRO // 128):
            rows = pl.ds(mb * 128, 128)
            h0_s[rows, :] = (
                xn_s[rows, :] * mod_row(1, 128) + mod_row(0, 128)).astype(BF16)
        shifts = [lambda t, v=v, hh=hh: (add_shift(v, hh), t)[1]
                  for v in range(NUG) for hh in range(2)]
        bulk(5 % 3, 5 // 3, shifts[:6], mbs=(0, 1, 2))
        wait_group(5)
        relayout_u(6)
        bulk(5 % 3, 5 // 3, shifts[6:8], mbs=(3,))
        for u in range(6, NUA):
            if U0_GROUP[u + 1] != U0_GROUP[u]:
                wait_group(U0_GROUP[u + 1])
            relayout_u(u + 1)
            bulk(u % 3, u // 3, shifts[8:] if u == 6 else ())

        pending = []

        def tie(never, a, b):
            top = jnp.where(never, a[:8, :128], b[:8, :128])
            if b.shape[1] > 128:
                top = jnp.concatenate([top, b[:8, 128:]], axis=1)
            return jnp.concatenate([top, b[8:]], axis=0)

        def ln1_piece(r, t):
            never = r < 0
            if pending:
                t = tie(never, pending.pop(), t)
            rows = pl.ds(pl.multiple_of(r, 16), 16)
            xv = tie(never, t, xbuf[rows, :].astype(F32))
            hv = _ln_mod(xv, mod_row(0, 16), mod_row(1, 16))
            hbuf[rows, :] = hv.astype(BF16)
            pending.append(hv[8:])
            return t

        def unit_extras(r, u, more=()):
            slots = [lambda t: t] * 8
            for k, f in enumerate(more):
                slots[2 * k + 1] = lambda t, f=f: (f(), t)[1]
            for k in range(XC // 16):
                d = k * (8 * UPI) // (XC // 16)
                if d // 8 == u % UPI:
                    slots[d % 8] = lambda t, g=slots[d % 8], k=k: (
                        ln1_piece(r + 16 * k, g(t)))
            return slots

        def grp_body(it, r):
            s0 = it * (UPI // 3)

            @pl.when(it == it0)
            def _():
                for cp in cp_mid + cp_wo:
                    cp.start()

            for u in range(1, UPI + 1):
                cp_st(u % 3, s0 + u // 3, SEM_IT + it).wait()
            cp_x(it - it0, SEM_IT + it).wait()
            for u in range(UPI):
                relayout((u + 1) % 3, s0 + (u + 1) // 3)
                bulk(u % 3, s0 + u // 3, unit_extras(r, u))
            pending.clear()
            return r + XC

        r1 = lax.fori_loop(it0, it1, grp_body, jnp.int32(PAD + PRO))

        for u in range(NU - NUZ + 1, NU):
            cp_unit(u).wait()
        for cp in cp_mid + [cp_m0]:
            cp.wait()
        mem_s[...] = m0_s[...].astype(F32)
        for u in range(NU - NUZ, NU):
            if u + 1 < NU:
                relayout_u(u + 1)
            v = u - (NU - NUZ)
            bulk(u % 3, u // 3, unit_extras(
                r1 + v // UPI * XC, u,
                [functools.partial(mod_slab, i)
                 for i in range(16 + 4 * v, min(20 + 4 * v, 48))]))
        for cp in cp_wo:
            cp.wait()

    pl.run_scoped(
        prologue,
        pltpu.VMEM((NU, D, DH), U32),
        pltpu.VMEM((48, D, 128), BF16),
        pltpu.VMEM((PRO, D), F32),
        pltpu.VMEM((PRO, D), BF16),
        pltpu.VMEM((PRO, D), BF16),
        pltpu.VMEM((2 * NUG, PRO, DH), F32),
    )

    def rest(w1_s, w3_s, w2_s, oring, abuf):
        w132 = w1_s.bitcast(U32)
        w332 = w3_s.bitcast(U32)
        w232 = w2_s.bitcast(U32)
        q32 = qring.bitcast(U32)
        k32 = kring.bitcast(U32)
        v32 = vring.bitcast(U32)

        cp_w1 = [pltpu.make_async_copy(w1_hbm.at[:, pl.ds(f * 128, 128)],
                                       w1_s.at[f], sems.at[SEM_FFN])
                 for f in range(NF)]
        cp_w3 = [pltpu.make_async_copy(w3_hbm.at[:, pl.ds(f * 128, 128)],
                                       w3_s.at[f], sems.at[SEM_FFN])
                 for f in range(NF)]
        cp_w2 = [pltpu.make_async_copy(w2_hbm.at[:, pl.ds(c * 128, 128)],
                                       w2_s.at[c], sems.at[SEM_FFN])
                 for c in range(NC)]
        for cp in cp_w1 + cp_w3 + cp_w2:
            cp.start()

        oring[:, pl.ds(OOFF - XR, XR), :] = jnp.zeros((H, XR, DH), BF16)

        abuf[pl.ds(0, PAD), :] = jnp.zeros((PAD, D), BF16)

        def post_attn(r, n):
            a = abuf[pl.ds(r, n), :].astype(F32)
            x1 = xbuf[pl.ds(r, n), :].astype(F32) + mod_row(2, n) * a
            x1 = x1.astype(BF16)
            xbuf[pl.ds(r, n), :] = x1
            hbuf[pl.ds(r, n), :] = _ln_mod(
                x1.astype(F32), mod_row(3, n), mod_row(4, n)).astype(BF16)

        row = lax.broadcasted_iota(jnp.int32, (NP, NP), 0)
        col = lax.broadcasted_iota(jnp.int32, (NP, NP), 1)

        def second(i):
            return ((i >= SEG) & (i < 2 * SEG)) | (i >= 2 * SEG + M)

        same = second(row) == second(col)
        mask = same & ((row >= 2 * SEG) | (col >= 2 * SEG) | (col <= row))
        fill = jnp.where(same, -1e9, -jnp.inf).astype(F32)

        def step(s, carry, mem, split, maybe_last):
            hr = pl.multiple_of(PAD + PRO + XR * s, 8)
            lhs_c = []
            for c in range(NC):
                cs = pl.ds(c * 128, 128)
                h8 = hbuf[pl.ds(hr + 16, 8), cs].astype(F32)
                lhs_c.append(jnp.concatenate(
                    [hbuf[pl.ds(hr, 16), cs],
                     jnp.concatenate([h8, mem[c]], axis=0).astype(BF16)], axis=0))
            lhs = jnp.concatenate(lhs_c, axis=1)

            if maybe_last:
                post_attn(pl.multiple_of(PAD + (s // UNROLL) * SH, 16), SH)

            wp, rp, op, ow = carry
            wpos = [pl.multiple_of(_wrap(wp + 8 * j, RING), 8)
                    for j in range(XR // 8)]
            rpos = pl.multiple_of(rp, SEG // 2)
            opos = [pl.multiple_of(_wrap(op + 8 * j, ORING), 8)
                    for j in range(XR // 8 + 1)]
            owr = pl.multiple_of(ow, SEG)

            tails = {}
            xs = {}
            ps = {}
            lhs_o = {}

            def load(j, p):
                r32 = (q32, k32, v32)[j]
                xs[j, p] = [
                    pltpu.bitcast(r32[h, pl.ds(rpos, SEG // 2), :], BF16)
                    for h in (2 * p, 2 * p + 1)]

            def operand(j, p):
                tail = jnp.concatenate(
                    [tails.pop((j, 2 * p)), tails.pop((j, 2 * p + 1))], axis=0)
                return jnp.concatenate(
                    xs.pop((j, p)) + [tail.astype(BF16)], axis=0)

            low = {}
            if split:
                lhs_lo = jnp.concatenate(lhs_c[:NC // 2], axis=1)
                lhs_hi = jnp.concatenate(lhs_c[NC // 2:], axis=1)
                for h in range(2):
                    for j, w32 in enumerate((wq32, wk32, wv32)):
                        low[j, h] = _dot(lhs_lo, pltpu.bitcast(
                            w32[h, pl.ds(0, D // 4), :], BF16))

            def proj(j, h):
                w32, ring = ((wq32, qring), (wk32, kring), (wv32, vring))[j]
                if (j, h) in low:
                    t = _dot(lhs_hi, pltpu.bitcast(
                        w32[h, pl.ds(D // 4, D // 4), :], BF16)) + low[j, h]
                else:
                    t = _dot(lhs, _w(w32, h))
                for i in range(XR // 8):
                    ring[h, pl.ds(wpos[i], 8), :] = (
                        t[8 * i:8 * i + 8].astype(BF16))
                tails[j, h] = t[XR:]

            def qk(p):
                sc = lax.dot_general(operand(0, p), operand(1, p),
                                     (((1,), (1,)), ((), ())),
                                     preferred_element_type=F32)
                sc = jnp.where(mask, sc * SCALE, fill)
                mx = jnp.max(sc, axis=-1, keepdims=True)
                e = jnp.exp(sc - mx)
                l = jnp.sum(e, axis=-1, keepdims=True)
                r = pl.reciprocal(l, approx=True)
                r = r * (2.0 - l * r)
                ps[p] = (e * r).astype(BF16)

            def pv(p):
                o = _dot(ps.pop(p), operand(2, p))
                for i, h in enumerate((2 * p, 2 * p + 1)):
                    ox = [oring[h, pl.ds(opos[k], 8), :] for k in range(XR // 8)]
                    om = o[2 * SEG + M * i:2 * SEG + M * (i + 1)]
                    if maybe_last:
                        om = jnp.where(
                            s == NSEG - 1,
                            oring[h, pl.ds(opos[3], 8), :].astype(F32), om)
                    last = jnp.concatenate(
                        [ox[2].astype(F32), om], axis=0).astype(BF16)
                    lhs_o[h] = jnp.concatenate([ox[0], ox[1], last], axis=0)
                for i, h in enumerate((2 * p, 2 * p + 1)):
                    oring[h, pl.ds(owr, SEG), :] = (
                        o[SEG * i:SEG * (i + 1)].astype(BF16))

            def wo_part(c, h0, h1):
                lo = jnp.concatenate([lhs_o[h] for h in range(h0, h1)], axis=1)
                w = pltpu.bitcast(wo32[c, pl.ds(h0 * 64, (h1 - h0) * 64), :], BF16)
                return _dot(lo, w)

            NPR = H // 2
            for t in range(NPR):
                if t >= 1:
                    load(0, t - 1)
                    load(1, t - 1)
                if t >= 2:
                    load(2, t - 2)
                for pos in range(6):
                    if t >= 1 and pos == (QPOS1 if t == 1 else QPOS):
                        qk(t - 1)
                    proj(pos % 3, 2 * t + pos // 3)
                if t >= 2:
                    pv(t - 2)
            HA = H - 4
            ar = pl.multiple_of(PAD - XR + XR * s, 8)
            acc = {}
            mem_new = {}

            def wo_a(c):
                acc[c] = wo_part(c, 0, HA)

            def wo_b(c):
                a = wo_part(c, HA, H) + acc[c]
                n = XR + M if maybe_last else XR
                abuf[pl.ds(ar, n), pl.ds(c * 128, 128)] = a[:n].astype(BF16)
                mem_new[c] = a[XR:]

            load(0, NPR - 1)
            load(1, NPR - 1)
            load(2, NPR - 2)
            wo_a(0)
            qk(NPR - 1)
            wo_a(1)
            pv(NPR - 2)
            load(2, NPR - 1)
            for c in (2, 3, 4):
                wo_a(c)
            pv(NPR - 1)
            for c in (5, 6):
                wo_a(c)
            for c in range(NC // 2):
                wo_b(c)
            wo_a(7)
            for c in range(NC // 2, NC):
                wo_b(c)
            return (_wrap(wp + XR, RING), _wrap(rp + SEG // 2, RING // 2),
                    _wrap(op + XR, ORING), _wrap(ow + SEG, ORING)), mem_new

        def steps(i, carry):
            mem = [mem_s[:, pl.ds(c * 128, 128)] for c in range(NC)]
            for u in range(UNROLL):
                carry, mem = step(i * UNROLL + u, carry, mem, split=u > 0,
                                  maybe_last=u == UNROLL - 1)
            for c in range(NC):
                mem_s[:, pl.ds(c * 128, 128)] = mem[c]
            return carry

        lax.fori_loop(0, NSEG // UNROLL, steps,
                      (jnp.int32(PRO), jnp.int32(0), jnp.int32(OOFF - XR),
                       jnp.int32(OOFF)))

        done = XR * (NSEG - 1) + M
        o32 = oring.bitcast(U32)

        def wo_bulk(i):
            p = pl.multiple_of(((done + OOFF) % ORING + i * WB) // 2, 8)
            lo = jnp.concatenate(
                [pltpu.bitcast(o32[h, pl.ds(p, WB // 2), :], BF16)
                 for h in range(H)], axis=1)
            rows = pl.ds(pl.multiple_of(PAD + done + i * WB, 16), WB)
            for c in range(NC):
                abuf[rows, pl.ds(c * 128, 128)] = (
                    _dot(lo, _w(wo32, c)).astype(BF16))

        for cp in cp_w1 + cp_w3 + cp_w2:
            cp.wait()

        def cp_out(r, n, part):
            cols = pl.ds(0, OC * 128) if part == 0 else pl.ds(OC * 128, D - OC * 128)
            return pltpu.make_async_copy(xbuf.at[pl.ds(PAD + r, n), cols],
                                         out_hbm.at[pl.ds(r, n), cols],
                                         sems.at[SEM_OUT])

        def ffn_body(i, carry, r0, n, with_wo, p0, npc):
            r = pl.multiple_of(r0 + i * n, 16)
            rows = pl.ds(pl.multiple_of(PAD + r, 16), n)
            if with_wo:
                wo_bulk(i)
            hv = hbuf[rows, :]
            act = []
            for f in range(NF):
                g = _dot(hv, _w(w132, f))
                u = _dot(hv, _w(w332, f))
                act.append((g * jax.nn.sigmoid(g) * u).astype(BF16))
            av = jnp.concatenate(act, axis=1)
            for c in range(NC):
                y = _dot(av, _w(w232, c))
                for k in range(npc):
                    if k * (NC - 1) // npc == c:
                        pr = p0 + (i * npc + k) * 16
                        post_attn(pl.multiple_of(
                            jnp.where(pr < S, PAD + pr, 0), 16), 16)
                cs = pl.ds(c * 128, 128)
                x2 = xbuf[rows, cs].astype(F32) + mod_row(5, n, cs) * y
                xbuf[rows, cs] = x2.astype(BF16)
                if c == OC - 1:
                    cp_out(r, n, 0).start()
            cp_out(r, n, 1).start()
            return carry

        nfb = (S - NWB * FA) // FB
        pa = SH * (NSEG // UNROLL)
        lax.fori_loop(0, NWB, functools.partial(
            ffn_body, r0=0, n=FA, with_wo=True, p0=pa, npc=NPA), 0)
        lax.fori_loop(0, nfb, functools.partial(
            ffn_body, r0=NWB * FA, n=FB, with_wo=False,
            p0=pa + NWB * NPA * 16, npc=NPB), 0)
        for part in range(2):
            for i in range(NWB):
                cp_out(i * FA, FA, part).wait()
            for i in range(nfb):
                cp_out(NWB * FA + i * FB, FB, part).wait()

    pl.run_scoped(
        rest,
        pltpu.VMEM((NF, D, 128), BF16),
        pltpu.VMEM((NF, D, 128), BF16),
        pltpu.VMEM((NC, F, 128), BF16),
        pltpu.VMEM((H, ORING, DH), BF16),
        pltpu.VMEM((PAD + S, D), BF16),
    )


@functools.partial(jax.jit, static_argnames=("A_seg_len",))
def pallas_adaLN_cond__memory_aug_recurrent_mem_tr__glu_gated_swiglu__prompt_kernel(
    A_x: jax.Array,
    A_mem0: jax.Array,
    A_Wq: jax.Array,
    A_Wk: jax.Array,
    A_Wv: jax.Array,
    A_Wo: jax.Array,
    A_seg_len,
    B_x: jax.Array,
    B_w1: jax.Array,
    B_w3: jax.Array,
    B_w2: jax.Array,
    c: jax.Array,
    w_mod: jax.Array,
):
    del B_x
    assert A_seg_len == SEG
    assert A_x.shape == (1, S, D) and A_mem0.shape == (1, M, D)
    assert A_Wq.shape == (D, H, DH) and B_w1.shape == (D, F)

    any_spec = pl.BlockSpec(memory_space=pl.ANY)
    out = pl.pallas_call(
        _kernel,
        out_shape=jax.ShapeDtypeStruct((S, D), BF16),
        in_specs=[any_spec] * 11,
        out_specs=any_spec,
        scratch_shapes=[
            pltpu.VMEM((H, D // 2, DH), U32),
            pltpu.VMEM((H, D // 2, DH), U32),
            pltpu.VMEM((H, D // 2, DH), U32),
            pltpu.VMEM((NC, H * DH, 128), BF16),
            pltpu.VMEM((2, PAD + S, D), BF16),
            pltpu.VMEM((H, RING, DH), BF16),
            pltpu.VMEM((H, RING, DH), BF16),
            pltpu.VMEM((H, RING, DH), BF16),
            pltpu.VMEM((6 * 8, D), F32),
            pltpu.VMEM((M, D), F32),
            pltpu.VMEM((1, D), BF16),
            pltpu.VMEM((M, D), BF16),
            pltpu.SemaphoreType.DMA((NSEMS,)),
        ],
        compiler_params=pltpu.CompilerParams(
            vmem_limit_bytes=120 * 1024 * 1024,
            disable_semaphore_checks=True, disable_bounds_checks=True),
        name="adaln_memtr_swiglu",
    )(
        A_x.reshape(S, D),
        A_mem0.reshape(M, D),
        A_Wq, A_Wk, A_Wv,
        A_Wo.reshape(H * DH, D),
        B_w1, B_w3, B_w2, c, w_mod,
    )
    return out.reshape(1, S, D)
```

```python
import functools

import jax
import jax.numpy as jnp
from jax import lax
import jax.experimental.pallas as pl
import jax.experimental.pallas.tpu as pltpu

BF16 = jnp.bfloat16
F32 = jnp.float32
U32 = jnp.uint32

S = 2048
D = 1024
H = 32
DH = 128
F = 3584
M = 8
SEG = 32
NSEG = S // SEG
XR = 24
PRO = S - XR * NSEG
RING = 544
ORING = 576
OOFF = 256
PAD = 48
NC = D // 128
NF = F // 128
FA = 128
FB = 208
OC = 7
NWB = 3
WB = 176
SH = 16
NPA, NPB = 11, 12
QPOS, QPOS1 = 2, 4
UNROLL = 4
NU = 3 * H // 2
UPI = 6
NUA = 12
NUZ = 12
XC = (S - PRO) * UPI // (NU - NUA)
NUG = 5
NP = 2 * (SEG + M)
EPS = 1e-5
SEM_FIRST, SEM_WO, SEM_MID, SEM_FFN, SEM_OUT = 0, 1, 2, 3, 4
SEM_CA = 5
SEM_U0 = SEM_CA + 2
U0_GROUP = (0, 1, 2, 3, 3, 4, 5, 5, 5, 6, 6, 6, 6)
SEM_SA = SEM_U0 + U0_GROUP[NUG]
SEM_IT = SEM_U0 + U0_GROUP[-1] + 1 - NUA // UPI
NSEMS = SEM_IT + NU // UPI
SCALE = DH ** -0.5


def _dot(a, b):
    return jnp.dot(a, b, preferred_element_type=F32)


def _w(ref32, i):
    return pltpu.bitcast(ref32[i], BF16)


def _wrap(i, n):
    return jnp.where(i >= n, i - n, i)


def _ln(x):
    mu = jnp.mean(x, axis=-1, keepdims=True)
    xc = x - mu
    var = jnp.mean(xc * xc, axis=-1, keepdims=True)
    return xc * lax.rsqrt(var + EPS)


def _ln_mod(x, shift, scale1):
    return _ln(x) * scale1 + shift


def _kernel(x_hbm, mem0_hbm, wq_hbm, wk_hbm, wv_hbm, wo_hbm, w1_hbm, w3_hbm,
            w2_hbm, c_hbm, wmod_hbm, out_hbm,
            wq32, wk32, wv32, wo_s, xh, qring, kring, vring,
            mod_s, mem_s, c_s, m0_s, sems):
    wo32 = wo_s.bitcast(U32)
    xbuf = xh.at[0]
    hbuf = xh.at[1]

    cp_x0 = pltpu.make_async_copy(x_hbm.at[pl.ds(0, PRO)],
                                  xbuf.at[pl.ds(PAD, PRO)], sems.at[SEM_FIRST])
    cp_c = pltpu.make_async_copy(c_hbm, c_s, sems.at[SEM_FIRST])
    cp_m0 = pltpu.make_async_copy(mem0_hbm, m0_s, sems.at[SEM_MID])
    cp_wo = [pltpu.make_async_copy(wo_hbm.at[:, pl.ds(c * 128, 128)],
                                   wo_s.at[c], sems.at[SEM_WO])
             for c in range(NC)]

    def cp_x(k, sem):
        r = PRO + k * XC
        if not isinstance(k, int):
            r = pl.multiple_of(r, XC)
        return pltpu.make_async_copy(x_hbm.at[pl.ds(r, XC)],
                                     xbuf.at[pl.ds(PAD + r, XC)], sems.at[sem])

    def mod_row(i, n, cols=slice(None)):
        return jnp.concatenate([mod_s[pl.ds(8 * i, 8), cols]] * (n // 8), axis=0)

    def prologue(st, wm_s, xn_s, g_s, h0_s, tmp_s):
        wm32 = wm_s.bitcast(U32)
        srcs = (wq_hbm.bitcast(U32), wk_hbm.bitcast(U32), wv_hbm.bitcast(U32))
        dsts = (wq32, wk32, wv32)
        rings = (qring, kring, vring)

        def cp_st(j, s, sem):
            return pltpu.make_async_copy(srcs[j].at[:, s, :], st.at[3 * s + j],
                                         sems.at[sem])

        def cp_unit(u):
            sem = (SEM_U0 + U0_GROUP[u] if u <= NUA
                   else SEM_IT + (u - 1) // UPI)
            return cp_st(u % 3, u // 3, sem)

        def cp_wm(i):
            sem = (SEM_SA if i < 8 else
                   SEM_CA + (i - 8) // 4 if i < 16 else SEM_MID)
            return pltpu.make_async_copy(wmod_hbm.at[:, pl.ds(i * 128, 128)],
                                         wm_s.at[i], sems.at[sem])

        it0, it1 = NUA // UPI, (NU - NUZ) // UPI
        cp_mid = ([cp_x(k, SEM_MID) for k in range(it1 - it0, NU // UPI - it0)]
                  + [cp_wm(i) for i in range(16, 48)])

        cp_c.start()
        cp_x0.start()
        cp_unit(0).start()
        for i in range(8, 16):
            cp_wm(i).start()
        for u in range(1, NUG):
            cp_unit(u).start()
        for i in range(8):
            cp_wm(i).start()
        for u in range(NUG, NU):
            cp_unit(u).start()
            if u % UPI == 0 and it0 < u // UPI <= it1:
                cp_x(u // UPI - 1 - it0, SEM_IT + u // UPI - 1).start()
        cp_m0.start()

        xbuf[pl.ds(0, PAD), :] = jnp.zeros((PAD, D), BF16)

        cp_c.wait()
        cp_x0.wait()
        cf = c_s[...].astype(F32)
        sc = (cf * jax.nn.sigmoid(cf)).astype(BF16)
        sc8 = jnp.broadcast_to(sc, (8, D))

        def ln_body(i, carry):
            r = pl.multiple_of(i * 64, 64)
            xv = xbuf[pl.ds(pl.multiple_of(PAD + r, 8), 64), :].astype(F32)
            xn_s[pl.ds(r, 64), :] = _ln(xv)
            return carry

        lax.fori_loop(0, PRO // 64, ln_body, 0)

        def mod_slab(i):
            k, c = divmod(i, NC)
            part = _dot(sc8, _w(wm32, i))
            if k in (1, 4):
                part = part + 1.0
            mod_s[pl.ds(8 * k, 8), pl.ds(c * 128, 128)] = part

        def relayout(j, s):
            u = 3 * s + j
            for db in range(8):
                ev = st[u, pl.ds(db * 128, 64, stride=2), :]
                od = st[u, pl.ds(db * 128 + 1, 64, stride=2), :]
                rows = pl.ds(db * 64, 64)
                dsts[j][2 * s, rows, :] = (ev & U32(0xFFFF)) | (od << 16)
                dsts[j][2 * s + 1, rows, :] = (ev >> 16) | (od & U32(0xFFFF0000))

        def bulk(j, s, extras=(), mbs=range(PRO // 128)):
            extras = list(extras)
            for mb in mbs:
                lhs = h0_s[pl.ds(mb * 128, 128), :]
                for hh in range(2):
                    h = 2 * s + hh
                    t = _dot(lhs, _w(dsts[j], h))
                    if extras:
                        t = extras.pop(0)(t)
                    rings[j][h, pl.ds(mb * 128, 128), :] = t.astype(BF16)

        def bulk_g(u, mbs):
            for mb in mbs:
                rows = pl.ds(mb * 128, 128)
                lhs = g_s[rows, :]
                for hh in range(2):
                    tmp_s[2 * u + hh, rows, :] = _dot(
                        lhs, _w(dsts[u % 3], 2 * (u // 3) + hh))

        def add_shift(u, hh):
            h = 2 * (u // 3) + hh
            b = _dot(mod_row(0, 8).astype(BF16), _w(dsts[u % 3], h))
            rings[u % 3][h, pl.ds(0, PRO), :] = (
                tmp_s[2 * u + hh] + jnp.concatenate([b] * (PRO // 8), axis=0)
            ).astype(BF16)

        def wait_group(g):
            if g == U0_GROUP[NUG]:
                for i in range(8):
                    cp_wm(i).wait()
            for v in range(NUA + 1):
                if U0_GROUP[v] == g:
                    cp_unit(v).wait()

        def relayout_u(u):
            relayout(u % 3, u // 3)

        def scale_half(k):
            for i in range(8 + 4 * k, 12 + 4 * k):
                mod_slab(i)
            cols = pl.ds(k * (D // 2), D // 2)
            g_s[:, cols] = (xn_s[:, cols] * mod_row(1, PRO, cols)).astype(BF16)

        def first_half(k, mbs):
            for mb in mbs:
                rows = pl.ds(mb * 128, 128)
                lhs = g_s[rows, pl.ds(k * (D // 2), D // 2)]
                for hh in range(2):
                    t = _dot(lhs, pltpu.bitcast(
                        wq32[hh, pl.ds(k * (D // 4), D // 4), :], BF16))
                    tmp_s[hh, rows, :] = t if k == 0 else t + tmp_s[hh, rows, :]

        wait_group(0)
        relayout_u(0)
        for k in range(2):
            for i in range(8 + 4 * k, 12 + 4 * k):
                cp_wm(i).wait()
            scale_half(k)
            first_half(k, range(4))
        wait_group(1)
        relayout_u(1)
        bulk_g(1, (0, 1, 2))
        wait_group(2)
        relayout_u(2)
        bulk_g(1, (3,))
        bulk_g(2, (0, 1, 2))
        wait_group(3)
        relayout_u(3)
        bulk_g(2, (3,))
        relayout_u(4)
        bulk_g(3, range(4))
        bulk_g(4, (0, 1, 2))
        wait_group(4)
        relayout_u(5)
        for i in range(8):
            mod_slab(i)
        bulk_g(4, (3,))
        for mb in range(PRO // 128):
            rows = pl.ds(mb * 128, 128)
            h0_s[rows, :] = (
                xn_s[rows, :] * mod_row(1, 128) + mod_row(0, 128)).astype(BF16)
        shifts = [lambda t, v=v, hh=hh: (add_shift(v, hh), t)[1]
                  for v in range(NUG) for hh in range(2)]
        bulk(5 % 3, 5 // 3, shifts[:6], mbs=(0, 1, 2))
        wait_group(5)
        relayout_u(6)
        bulk(5 % 3, 5 // 3, shifts[6:8], mbs=(3,))
        for u in range(6, NUA):
            if U0_GROUP[u + 1] != U0_GROUP[u]:
                wait_group(U0_GROUP[u + 1])
            relayout_u(u + 1)
            bulk(u % 3, u // 3, shifts[8:] if u == 6 else ())

        pending = []

        def tie(never, a, b):
            top = jnp.where(never, a[:8, :128], b[:8, :128])
            if b.shape[1] > 128:
                top = jnp.concatenate([top, b[:8, 128:]], axis=1)
            return jnp.concatenate([top, b[8:]], axis=0)

        def ln1_piece(r, t):
            never = r < 0
            if pending:
                t = tie(never, pending.pop(), t)
            rows = pl.ds(pl.multiple_of(r, 16), 16)
            xv = tie(never, t, xbuf[rows, :].astype(F32))
            hv = _ln_mod(xv, mod_row(0, 16), mod_row(1, 16))
            hbuf[rows, :] = hv.astype(BF16)
            pending.append(hv[8:])
            return t

        def unit_extras(r, u, more=()):
            slots = [lambda t: t] * 8
            for k, f in enumerate(more):
                slots[2 * k + 1] = lambda t, f=f: (f(), t)[1]
            for k in range(XC // 16):
                d = k * (8 * UPI) // (XC // 16)
                if d // 8 == u % UPI:
                    slots[d % 8] = lambda t, g=slots[d % 8], k=k: (
                        ln1_piece(r + 16 * k, g(t)))
            return slots

        def grp_body(it, r):
            s0 = it * (UPI // 3)

            @pl.when(it == it0)
            def _():
                for cp in cp_mid + cp_wo:
                    cp.start()

            for u in range(1, UPI + 1):
                cp_st(u % 3, s0 + u // 3, SEM_IT + it).wait()
            cp_x(it - it0, SEM_IT + it).wait()
            for u in range(UPI):
                relayout((u + 1) % 3, s0 + (u + 1) // 3)
                bulk(u % 3, s0 + u // 3, unit_extras(r, u))
            pending.clear()
            return r + XC

        r1 = lax.fori_loop(it0, it1, grp_body, jnp.int32(PAD + PRO))

        for u in range(NU - NUZ + 1, NU):
            cp_unit(u).wait()
        for cp in cp_mid + [cp_m0]:
            cp.wait()
        mem_s[...] = m0_s[...].astype(F32)
        for u in range(NU - NUZ, NU):
            if u + 1 < NU:
                relayout_u(u + 1)
            v = u - (NU - NUZ)
            bulk(u % 3, u // 3, unit_extras(
                r1 + v // UPI * XC, u,
                [functools.partial(mod_slab, i)
                 for i in range(16 + 4 * v, min(20 + 4 * v, 48))]))
        for cp in cp_wo:
            cp.wait()

    pl.run_scoped(
        prologue,
        pltpu.VMEM((NU, D, DH), U32),
        pltpu.VMEM((48, D, 128), BF16),
        pltpu.VMEM((PRO, D), F32),
        pltpu.VMEM((PRO, D), BF16),
        pltpu.VMEM((PRO, D), BF16),
        pltpu.VMEM((2 * NUG, PRO, DH), F32),
    )

    def rest(w1_s, w3_s, w2_s, oring, abuf):
        w132 = w1_s.bitcast(U32)
        w332 = w3_s.bitcast(U32)
        w232 = w2_s.bitcast(U32)
        q32 = qring.bitcast(U32)
        k32 = kring.bitcast(U32)
        v32 = vring.bitcast(U32)

        cp_w1 = [pltpu.make_async_copy(w1_hbm.at[:, pl.ds(f * 128, 128)],
                                       w1_s.at[f], sems.at[SEM_FFN])
                 for f in range(NF)]
        cp_w3 = [pltpu.make_async_copy(w3_hbm.at[:, pl.ds(f * 128, 128)],
                                       w3_s.at[f], sems.at[SEM_FFN])
                 for f in range(NF)]
        cp_w2 = [pltpu.make_async_copy(w2_hbm.at[:, pl.ds(c * 128, 128)],
                                       w2_s.at[c], sems.at[SEM_FFN])
                 for c in range(NC)]
        for cp in cp_w1 + cp_w3 + cp_w2:
            cp.start()

        o32 = oring.bitcast(U32)

        o32[:, pl.ds(OOFF // 2 - 16, 16), :] = jnp.zeros((H, 16, DH), U32)

        abuf[pl.ds(0, PAD), :] = jnp.zeros((PAD, D), BF16)

        def post_attn(r, n):
            a = abuf[pl.ds(r, n), :].astype(F32)
            x1 = xbuf[pl.ds(r, n), :].astype(F32) + mod_row(2, n) * a
            x1 = x1.astype(BF16)
            xbuf[pl.ds(r, n), :] = x1
            hbuf[pl.ds(r, n), :] = _ln_mod(
                x1.astype(F32), mod_row(3, n), mod_row(4, n)).astype(BF16)

        row = lax.broadcasted_iota(jnp.int32, (NP, NP), 0)
        col = lax.broadcasted_iota(jnp.int32, (NP, NP), 1)

        def second(i):
            return ((i >= SEG) & (i < 2 * SEG)) | (i >= 2 * SEG + M)

        same = second(row) == second(col)
        mask = same & ((row >= 2 * SEG) | (col >= 2 * SEG) | (col <= row))
        fill = jnp.where(same, -1e9, -jnp.inf).astype(F32)

        def step(s, carry, mem, split, maybe_last, half_first):
            hr = pl.multiple_of(PAD + PRO + XR * s, 8)
            lhs_c = []
            for c in range(NC):
                cs = pl.ds(c * 128, 128)
                h8 = hbuf[pl.ds(hr + 16, 8), cs].astype(F32)
                lhs_c.append(jnp.concatenate(
                    [hbuf[pl.ds(hr, 16), cs],
                     jnp.concatenate([h8, mem[c]], axis=0).astype(BF16)], axis=0))
            lhs = jnp.concatenate(lhs_c, axis=1)

            if maybe_last:
                post_attn(pl.multiple_of(PAD + (s // UNROLL) * SH, 16), SH)

            wp, rp, op, ow = carry
            wpos = [pl.multiple_of(_wrap(wp + 8 * j, RING), 8)
                    for j in range(XR // 8)]
            rpos = pl.multiple_of(rp, SEG // 2)
            oblk = [pl.multiple_of(
                _wrap(op + (16 * j - 8 if half_first else 16 * j), ORING) // 2, 8)
                for j in range(2)]
            ofull, ohalf = (oblk[1], oblk[0]) if half_first else oblk
            owr = pl.multiple_of(ow, SEG)

            tails = {}
            xs = {}
            ps = {}
            lhs_o = {}

            def load(j, p):
                r32 = (q32, k32, v32)[j]
                xs[j, p] = [
                    pltpu.bitcast(r32[h, pl.ds(rpos, SEG // 2), :], BF16)
                    for h in (2 * p, 2 * p + 1)]

            def operand(j, p):
                tail = jnp.concatenate(
                    [tails.pop((j, 2 * p)), tails.pop((j, 2 * p + 1))], axis=0)
                return jnp.concatenate(
                    xs.pop((j, p)) + [tail.astype(BF16)], axis=0)

            low = {}
            if split:
                lhs_lo = jnp.concatenate(lhs_c[:NC // 2], axis=1)
                lhs_hi = jnp.concatenate(lhs_c[NC // 2:], axis=1)
                for h in range(2):
                    for j, w32 in enumerate((wq32, wk32, wv32)):
                        low[j, h] = _dot(lhs_lo, pltpu.bitcast(
                            w32[h, pl.ds(0, D // 4), :], BF16))

            def proj(j, h):
                w32, ring = ((wq32, qring), (wk32, kring), (wv32, vring))[j]
                if (j, h) in low:
                    t = _dot(lhs_hi, pltpu.bitcast(
                        w32[h, pl.ds(D // 4, D // 4), :], BF16)) + low[j, h]
                else:
                    t = _dot(lhs, _w(w32, h))
                for i in range(XR // 8):
                    ring[h, pl.ds(wpos[i], 8), :] = (
                        t[8 * i:8 * i + 8].astype(BF16))
                tails[j, h] = t[XR:]

            def qk(p):
                sc = lax.dot_general(operand(0, p), operand(1, p),
                                     (((1,), (1,)), ((), ())),
                                     preferred_element_type=F32)
                sc = jnp.where(mask, sc * SCALE, fill)
                mx = jnp.max(sc, axis=-1, keepdims=True)
                e = jnp.exp(sc - mx)
                l = jnp.sum(e, axis=-1, keepdims=True)
                r = pl.reciprocal(l, approx=True)
                r = r * (2.0 - l * r)
                ps[p] = (e * r).astype(BF16)

            def pv(p):
                o = _dot(ps.pop(p), operand(2, p))
                for i, h in enumerate((2 * p, 2 * p + 1)):
                    xf = pltpu.bitcast(o32[h, pl.ds(ofull, 8), :], BF16)
                    xh2 = pltpu.bitcast(
                        o32[h, pl.ds(ohalf, 8), :], BF16).astype(F32)
                    om = o[2 * SEG + M * i:2 * SEG + M * (i + 1)]
                    if maybe_last:
                        om = jnp.where(s == NSEG - 1, xh2[8:], om)
                    last = jnp.concatenate(
                        [xh2[8:] if half_first else xh2[:8], om],
                        axis=0).astype(BF16)
                    lhs_o[h] = jnp.concatenate([xf, last], axis=0)
                for i, h in enumerate((2 * p, 2 * p + 1)):
                    oring[h, pl.ds(owr, SEG), :] = (
                        o[SEG * i:SEG * (i + 1)].astype(BF16))

            def wo_part(c, h0, h1):
                lo = jnp.concatenate([lhs_o[h] for h in range(h0, h1)], axis=1)
                w = pltpu.bitcast(wo32[c, pl.ds(h0 * 64, (h1 - h0) * 64), :], BF16)
                return _dot(lo, w)

            NPR = H // 2
            for t in range(NPR):
                if t >= 1:
                    load(0, t - 1)
                    load(1, t - 1)
                if t >= 2:
                    load(2, t - 2)
                for pos in range(6):
                    if t >= 1 and pos == (QPOS1 if t == 1 else QPOS):
                        qk(t - 1)
                    proj(pos % 3, 2 * t + pos // 3)
                if t >= 2:
                    pv(t - 2)
            HA = H - 4
            ar = pl.multiple_of(PAD - XR + XR * s, 8)
            acc = {}
            mem_new = {}

            def wo_a(c):
                acc[c] = wo_part(c, 0, HA)

            def wo_b(c):
                a = wo_part(c, HA, H) + acc[c]
                cs = pl.ds(c * 128, 128)
                if half_first:
                    abuf[pl.ds(ar + 8, 16), cs] = a[:16].astype(BF16)
                    abuf[pl.ds(ar, 8), cs] = a[16:XR].astype(BF16)
                else:
                    n = XR + M if maybe_last else XR
                    abuf[pl.ds(ar, n), cs] = a[:n].astype(BF16)
                mem_new[c] = a[XR:]

            load(0, NPR - 1)
            load(1, NPR - 1)
            load(2, NPR - 2)
            wo_a(0)
            qk(NPR - 1)
            wo_a(1)
            pv(NPR - 2)
            load(2, NPR - 1)
            for c in (2, 3, 4):
                wo_a(c)
            pv(NPR - 1)
            for c in (5, 6):
                wo_a(c)
            for c in range(NC // 2):
                wo_b(c)
            wo_a(7)
            for c in range(NC // 2, NC):
                wo_b(c)
            return (_wrap(wp + XR, RING), _wrap(rp + SEG // 2, RING // 2),
                    _wrap(op + XR, ORING), _wrap(ow + SEG, ORING)), mem_new

        def steps(i, carry):
            mem = [mem_s[:, pl.ds(c * 128, 128)] for c in range(NC)]
            for u in range(UNROLL):
                carry, mem = step(i * UNROLL + u, carry, mem, split=u > 0,
                                  maybe_last=u == UNROLL - 1,
                                  half_first=u % 2 == 0)
            for c in range(NC):
                mem_s[:, pl.ds(c * 128, 128)] = mem[c]
            return carry

        lax.fori_loop(0, NSEG // UNROLL, steps,
                      (jnp.int32(PRO), jnp.int32(0), jnp.int32(OOFF - XR),
                       jnp.int32(OOFF)))

        done = XR * (NSEG - 1) + M

        def wo_bulk(i):
            p = pl.multiple_of(((done + OOFF) % ORING + i * WB) // 2, 8)
            lo = jnp.concatenate(
                [pltpu.bitcast(o32[h, pl.ds(p, WB // 2), :], BF16)
                 for h in range(H)], axis=1)
            rows = pl.ds(pl.multiple_of(PAD + done + i * WB, 16), WB)
            for c in range(NC):
                abuf[rows, pl.ds(c * 128, 128)] = (
                    _dot(lo, _w(wo32, c)).astype(BF16))

        for cp in cp_w1 + cp_w3 + cp_w2:
            cp.wait()

        def cp_out(r, n, part):
            cols = pl.ds(0, OC * 128) if part == 0 else pl.ds(OC * 128, D - OC * 128)
            return pltpu.make_async_copy(xbuf.at[pl.ds(PAD + r, n), cols],
                                         out_hbm.at[pl.ds(r, n), cols],
                                         sems.at[SEM_OUT])

        def ffn_body(i, carry, r0, n, with_wo, p0, npc):
            r = pl.multiple_of(r0 + i * n, 16)
            rows = pl.ds(pl.multiple_of(PAD + r, 16), n)
            if with_wo:
                wo_bulk(i)
            hv = hbuf[rows, :]
            act = []
            for f in range(NF):
                g = _dot(hv, _w(w132, f))
                u = _dot(hv, _w(w332, f))
                act.append((g * jax.nn.sigmoid(g) * u).astype(BF16))
            av = jnp.concatenate(act, axis=1)
            for c in range(NC):
                y = _dot(av, _w(w232, c))
                for k in range(npc):
                    if k * (NC - 1) // npc == c:
                        pr = p0 + (i * npc + k) * 16
                        post_attn(pl.multiple_of(
                            jnp.where(pr < S, PAD + pr, 0), 16), 16)
                cs = pl.ds(c * 128, 128)
                x2 = xbuf[rows, cs].astype(F32) + mod_row(5, n, cs) * y
                xbuf[rows, cs] = x2.astype(BF16)
                if c == OC - 1:
                    cp_out(r, n, 0).start()
            cp_out(r, n, 1).start()
            return carry

        nfb = (S - NWB * FA) // FB
        pa = SH * (NSEG // UNROLL)
        lax.fori_loop(0, NWB, functools.partial(
            ffn_body, r0=0, n=FA, with_wo=True, p0=pa, npc=NPA), 0)
        lax.fori_loop(0, nfb, functools.partial(
            ffn_body, r0=NWB * FA, n=FB, with_wo=False,
            p0=pa + NWB * NPA * 16, npc=NPB), 0)
        for part in range(2):
            for i in range(NWB):
                cp_out(i * FA, FA, part).wait()
            for i in range(nfb):
                cp_out(NWB * FA + i * FB, FB, part).wait()

    pl.run_scoped(
        rest,
        pltpu.VMEM((NF, D, 128), BF16),
        pltpu.VMEM((NF, D, 128), BF16),
        pltpu.VMEM((NC, F, 128), BF16),
        pltpu.VMEM((H, ORING, DH), BF16),
        pltpu.VMEM((PAD + S, D), BF16),
    )


@functools.partial(jax.jit, static_argnames=("A_seg_len",))
def pallas_adaLN_cond__memory_aug_recurrent_mem_tr__glu_gated_swiglu__prompt_kernel(
    A_x: jax.Array,
    A_mem0: jax.Array,
    A_Wq: jax.Array,
    A_Wk: jax.Array,
    A_Wv: jax.Array,
    A_Wo: jax.Array,
    A_seg_len,
    B_x: jax.Array,
    B_w1: jax.Array,
    B_w3: jax.Array,
    B_w2: jax.Array,
    c: jax.Array,
    w_mod: jax.Array,
):
    del B_x
    assert A_seg_len == SEG
    assert A_x.shape == (1, S, D) and A_mem0.shape == (1, M, D)
    assert A_Wq.shape == (D, H, DH) and B_w1.shape == (D, F)

    any_spec = pl.BlockSpec(memory_space=pl.ANY)
    out = pl.pallas_call(
        _kernel,
        out_shape=jax.ShapeDtypeStruct((S, D), BF16),
        in_specs=[any_spec] * 11,
        out_specs=any_spec,
        scratch_shapes=[
            pltpu.VMEM((H, D // 2, DH), U32),
            pltpu.VMEM((H, D // 2, DH), U32),
            pltpu.VMEM((H, D // 2, DH), U32),
            pltpu.VMEM((NC, H * DH, 128), BF16),
            pltpu.VMEM((2, PAD + S, D), BF16),
            pltpu.VMEM((H, RING, DH), BF16),
            pltpu.VMEM((H, RING, DH), BF16),
            pltpu.VMEM((H, RING, DH), BF16),
            pltpu.VMEM((6 * 8, D), F32),
            pltpu.VMEM((M, D), F32),
            pltpu.VMEM((1, D), BF16),
            pltpu.VMEM((M, D), BF16),
            pltpu.SemaphoreType.DMA((NSEMS,)),
        ],
        compiler_params=pltpu.CompilerParams(
            vmem_limit_bytes=120 * 1024 * 1024,
            disable_semaphore_checks=True, disable_bounds_checks=True),
        name="adaln_memtr_swiglu",
    )(
        A_x.reshape(S, D),
        A_mem0.reshape(M, D),
        A_Wq, A_Wk, A_Wv,
        A_Wo.reshape(H * DH, D),
        B_w1, B_w3, B_w2, c, w_mod,
    )
    return out.reshape(1, S, D)
```

```python
import functools

import jax
import jax.numpy as jnp
from jax import lax
import jax.experimental.pallas as pl
import jax.experimental.pallas.tpu as pltpu

BF16 = jnp.bfloat16
F32 = jnp.float32
U32 = jnp.uint32

S = 2048
D = 1024
H = 32
DH = 128
F = 3584
M = 8
SEG = 32
NSEG = S // SEG
XR = 24
PRO = S - XR * NSEG
RING = 640
ORING = 576
OOFF = 256
PAD = 48
NC = D // 128
NF = F // 128
FA = 128
FB = 208
OC = 7
NWB = 3
WB = 176
SH = 16
NPA, NPB = 11, 12
QPOS, QPOS1 = 2, 4
UNROLL = 4
NU = 3 * H // 2
UPI = 6
NUA = 12
NUZ = 12
XC = (S - PRO) * UPI // (NU - NUA)
NUG = 5
NP = 2 * (SEG + M)
EPS = 1e-5
SEM_FIRST, SEM_WO, SEM_MID, SEM_FFN, SEM_OUT = 0, 1, 2, 3, 4
SEM_CA = 5
SEM_U0 = SEM_CA + 2
U0_GROUP = (0, 1, 2, 3, 3, 4, 5, 5, 5, 6, 6, 6, 6)
SEM_SA = SEM_U0 + U0_GROUP[NUG]
SEM_IT = SEM_U0 + U0_GROUP[-1] + 1 - NUA // UPI
NSEMS = SEM_IT + NU // UPI
SCALE = DH ** -0.5


def _dot(a, b):
    return jnp.dot(a, b, preferred_element_type=F32)


def _w(ref32, i):
    return pltpu.bitcast(ref32[i], BF16)


def _wrap(i, n):
    return jnp.where(i >= n, i - n, i)


def _ln(x):
    mu = jnp.mean(x, axis=-1, keepdims=True)
    xc = x - mu
    var = jnp.mean(xc * xc, axis=-1, keepdims=True)
    return xc * lax.rsqrt(var + EPS)


def _ln_mod(x, shift, scale1):
    return _ln(x) * scale1 + shift


def _kernel(x_hbm, mem0_hbm, wq_hbm, wk_hbm, wv_hbm, wo_hbm, w1_hbm, w3_hbm,
            w2_hbm, c_hbm, wmod_hbm, out_hbm,
            wq32, wk32, wv32, wo_s, xh, qring, kring, vring,
            mod_s, mem_s, c_s, m0_s, sems):
    wo32 = wo_s.bitcast(U32)
    xbuf = xh.at[0]
    hbuf = xh.at[1]

    cp_x0 = pltpu.make_async_copy(x_hbm.at[pl.ds(0, PRO)],
                                  xbuf.at[pl.ds(PAD, PRO)], sems.at[SEM_FIRST])
    cp_c = pltpu.make_async_copy(c_hbm, c_s, sems.at[SEM_FIRST])
    cp_m0 = pltpu.make_async_copy(mem0_hbm, m0_s, sems.at[SEM_MID])
    cp_wo = [pltpu.make_async_copy(wo_hbm.at[:, pl.ds(c * 128, 128)],
                                   wo_s.at[c], sems.at[SEM_WO])
             for c in range(NC)]

    def cp_x(k, sem):
        r = PRO + k * XC
        if not isinstance(k, int):
            r = pl.multiple_of(r, XC)
        return pltpu.make_async_copy(x_hbm.at[pl.ds(r, XC)],
                                     xbuf.at[pl.ds(PAD + r, XC)], sems.at[sem])

    def mod_row(i, n, cols=slice(None)):
        return jnp.concatenate([mod_s[pl.ds(8 * i, 8), cols]] * (n // 8), axis=0)

    def prologue(st, wm_s, xn_s, g_s, h0_s, tmp_s):
        wm32 = wm_s.bitcast(U32)
        srcs = (wq_hbm.bitcast(U32), wk_hbm.bitcast(U32), wv_hbm.bitcast(U32))
        dsts = (wq32, wk32, wv32)
        rings = (qring, kring, vring)

        def cp_st(j, s, sem):
            return pltpu.make_async_copy(srcs[j].at[:, s, :], st.at[3 * s + j],
                                         sems.at[sem])

        def cp_unit(u):
            sem = (SEM_U0 + U0_GROUP[u] if u <= NUA
                   else SEM_IT + (u - 1) // UPI)
            return cp_st(u % 3, u // 3, sem)

        def cp_wm(i):
            sem = (SEM_SA if i < 8 else
                   SEM_CA + (i - 8) // 4 if i < 16 else SEM_MID)
            return pltpu.make_async_copy(wmod_hbm.at[:, pl.ds(i * 128, 128)],
                                         wm_s.at[i], sems.at[sem])

        it0, it1 = NUA // UPI, (NU - NUZ) // UPI
        cp_mid = ([cp_x(k, SEM_MID) for k in range(it1 - it0, NU // UPI - it0)]
                  + [cp_wm(i) for i in range(16, 48)])

        cp_c.start()
        cp_x0.start()
        cp_unit(0).start()
        for i in range(8, 16):
            cp_wm(i).start()
        for u in range(1, NUG):
            cp_unit(u).start()
        for i in range(8):
            cp_wm(i).start()
        for u in range(NUG, NU):
            cp_unit(u).start()
            if u % UPI == 0 and it0 < u // UPI <= it1:
                cp_x(u // UPI - 1 - it0, SEM_IT + u // UPI - 1).start()
        cp_m0.start()

        xbuf[pl.ds(0, PAD), :] = jnp.zeros((PAD, D), BF16)

        cp_c.wait()
        cp_x0.wait()
        cf = c_s[...].astype(F32)
        sc = (cf * jax.nn.sigmoid(cf)).astype(BF16)
        sc8 = jnp.broadcast_to(sc, (8, D))

        def ln_body(i, carry):
            r = pl.multiple_of(i * 64, 64)
            xv = xbuf[pl.ds(pl.multiple_of(PAD + r, 8), 64), :].astype(F32)
            xn_s[pl.ds(r, 64), :] = _ln(xv)
            return carry

        lax.fori_loop(0, PRO // 64, ln_body, 0)

        def mod_slab(i):
            k, c = divmod(i, NC)
            part = _dot(sc8, _w(wm32, i))
            if k in (1, 4):
                part = part + 1.0
            mod_s[pl.ds(8 * k, 8), pl.ds(c * 128, 128)] = part

        def relayout(j, s):
            u = 3 * s + j
            for db in range(8):
                ev = st[u, pl.ds(db * 128, 64, stride=2), :]
                od = st[u, pl.ds(db * 128 + 1, 64, stride=2), :]
                rows = pl.ds(db * 64, 64)
                dsts[j][2 * s, rows, :] = (ev & U32(0xFFFF)) | (od << 16)
                dsts[j][2 * s + 1, rows, :] = (ev >> 16) | (od & U32(0xFFFF0000))

        def bulk(j, s, extras=(), mbs=range(PRO // 128)):
            extras = list(extras)
            for mb in mbs:
                lhs = h0_s[pl.ds(mb * 128, 128), :]
                for hh in range(2):
                    h = 2 * s + hh
                    t = _dot(lhs, _w(dsts[j], h))
                    if extras:
                        t = extras.pop(0)(t)
                    rings[j][h, pl.ds(mb * 128, 128), :] = t.astype(BF16)

        def bulk_g(u, mbs):
            for mb in mbs:
                rows = pl.ds(mb * 128, 128)
                lhs = g_s[rows, :]
                for hh in range(2):
                    tmp_s[2 * u + hh, rows, :] = _dot(
                        lhs, _w(dsts[u % 3], 2 * (u // 3) + hh))

        def add_shift(u, hh):
            h = 2 * (u // 3) + hh
            b = _dot(mod_row(0, 8).astype(BF16), _w(dsts[u % 3], h))
            rings[u % 3][h, pl.ds(0, PRO), :] = (
                tmp_s[2 * u + hh] + jnp.concatenate([b] * (PRO // 8), axis=0)
            ).astype(BF16)

        def wait_group(g):
            if g == U0_GROUP[NUG]:
                for i in range(8):
                    cp_wm(i).wait()
            for v in range(NUA + 1):
                if U0_GROUP[v] == g:
                    cp_unit(v).wait()

        def relayout_u(u):
            relayout(u % 3, u // 3)

        def scale_half(k):
            for i in range(8 + 4 * k, 12 + 4 * k):
                mod_slab(i)
            cols = pl.ds(k * (D // 2), D // 2)
            g_s[:, cols] = (xn_s[:, cols] * mod_row(1, PRO, cols)).astype(BF16)

        def first_half(k, mbs):
            for mb in mbs:
                rows = pl.ds(mb * 128, 128)
                lhs = g_s[rows, pl.ds(k * (D // 2), D // 2)]
                for hh in range(2):
                    t = _dot(lhs, pltpu.bitcast(
                        wq32[hh, pl.ds(k * (D // 4), D // 4), :], BF16))
                    tmp_s[hh, rows, :] = t if k == 0 else t + tmp_s[hh, rows, :]

        wait_group(0)
        relayout_u(0)
        for k in range(2):
            for i in range(8 + 4 * k, 12 + 4 * k):
                cp_wm(i).wait()
            scale_half(k)
            first_half(k, range(4))
        wait_group(1)
        relayout_u(1)
        bulk_g(1, (0, 1, 2))
        wait_group(2)
        relayout_u(2)
        bulk_g(1, (3,))
        bulk_g(2, (0, 1, 2))
        wait_group(3)
        relayout_u(3)
        bulk_g(2, (3,))
        relayout_u(4)
        bulk_g(3, range(4))
        bulk_g(4, (0, 1, 2))
        wait_group(4)
        relayout_u(5)
        for i in range(8):
            mod_slab(i)
        bulk_g(4, (3,))
        for mb in range(PRO // 128):
            rows = pl.ds(mb * 128, 128)
            h0_s[rows, :] = (
                xn_s[rows, :] * mod_row(1, 128) + mod_row(0, 128)).astype(BF16)
        shifts = [lambda t, v=v, hh=hh: (add_shift(v, hh), t)[1]
                  for v in range(NUG) for hh in range(2)]
        bulk(5 % 3, 5 // 3, shifts[:6], mbs=(0, 1, 2))
        wait_group(5)
        relayout_u(6)
        bulk(5 % 3, 5 // 3, shifts[6:8], mbs=(3,))
        for u in range(6, NUA):
            if U0_GROUP[u + 1] != U0_GROUP[u]:
                wait_group(U0_GROUP[u + 1])
            relayout_u(u + 1)
            bulk(u % 3, u // 3, shifts[8:] if u == 6 else ())

        pending = []

        def tie(never, a, b):
            top = jnp.where(never, a[:8, :128], b[:8, :128])
            if b.shape[1] > 128:
                top = jnp.concatenate([top, b[:8, 128:]], axis=1)
            return jnp.concatenate([top, b[8:]], axis=0)

        def ln1_piece(r, t):
            never = r < 0
            if pending:
                t = tie(never, pending.pop(), t)
            rows = pl.ds(pl.multiple_of(r, 16), 16)
            xv = tie(never, t, xbuf[rows, :].astype(F32))
            hv = _ln_mod(xv, mod_row(0, 16), mod_row(1, 16))
            hbuf[rows, :] = hv.astype(BF16)
            pending.append(hv[8:])
            return t

        def unit_extras(r, u, more=()):
            slots = [lambda t: t] * 8
            for k, f in enumerate(more):
                slots[2 * k + 1] = lambda t, f=f: (f(), t)[1]
            for k in range(XC // 16):
                d = k * (8 * UPI) // (XC // 16)
                if d // 8 == u % UPI:
                    slots[d % 8] = lambda t, g=slots[d % 8], k=k: (
                        ln1_piece(r + 16 * k, g(t)))
            return slots

        def grp_body(it, r):
            s0 = it * (UPI // 3)

            @pl.when(it == it0)
            def _():
                for cp in cp_mid + cp_wo:
                    cp.start()

            for u in range(1, UPI + 1):
                cp_st(u % 3, s0 + u // 3, SEM_IT + it).wait()
            cp_x(it - it0, SEM_IT + it).wait()
            for u in range(UPI):
                relayout((u + 1) % 3, s0 + (u + 1) // 3)
                bulk(u % 3, s0 + u // 3, unit_extras(r, u))
            pending.clear()
            return r + XC

        r1 = lax.fori_loop(it0, it1, grp_body, jnp.int32(PAD + PRO))

        for u in range(NU - NUZ + 1, NU):
            cp_unit(u).wait()
        for cp in cp_mid + [cp_m0]:
            cp.wait()
        mem_s[...] = m0_s[...].astype(F32)
        for u in range(NU - NUZ, NU):
            if u + 1 < NU:
                relayout_u(u + 1)
            v = u - (NU - NUZ)
            bulk(u % 3, u // 3, unit_extras(
                r1 + v // UPI * XC, u,
                [functools.partial(mod_slab, i)
                 for i in range(16 + 4 * v, min(20 + 4 * v, 48))]))
        for cp in cp_wo:
            cp.wait()

    pl.run_scoped(
        prologue,
        pltpu.VMEM((NU, D, DH), U32),
        pltpu.VMEM((48, D, 128), BF16),
        pltpu.VMEM((PRO, D), F32),
        pltpu.VMEM((PRO, D), BF16),
        pltpu.VMEM((PRO, D), BF16),
        pltpu.VMEM((2 * NUG, PRO, DH), F32),
    )

    def rest(w1_s, w3_s, w2_s, oring, abuf):
        w132 = w1_s.bitcast(U32)
        w332 = w3_s.bitcast(U32)
        w232 = w2_s.bitcast(U32)
        q32 = qring.bitcast(U32)
        k32 = kring.bitcast(U32)
        v32 = vring.bitcast(U32)

        cp_w1 = [pltpu.make_async_copy(w1_hbm.at[:, pl.ds(f * 128, 128)],
                                       w1_s.at[f], sems.at[SEM_FFN])
                 for f in range(NF)]
        cp_w3 = [pltpu.make_async_copy(w3_hbm.at[:, pl.ds(f * 128, 128)],
                                       w3_s.at[f], sems.at[SEM_FFN])
                 for f in range(NF)]
        cp_w2 = [pltpu.make_async_copy(w2_hbm.at[:, pl.ds(c * 128, 128)],
                                       w2_s.at[c], sems.at[SEM_FFN])
                 for c in range(NC)]
        for cp in cp_w1 + cp_w3 + cp_w2:
            cp.start()

        o32 = oring.bitcast(U32)

        o32[:, pl.ds(OOFF // 2 - 16, 16), :] = jnp.zeros((H, 16, DH), U32)

        abuf[pl.ds(0, PAD), :] = jnp.zeros((PAD, D), BF16)

        def post_attn(r, n):
            a = abuf[pl.ds(r, n), :].astype(F32)
            x1 = xbuf[pl.ds(r, n), :].astype(F32) + mod_row(2, n) * a
            x1 = x1.astype(BF16)
            xbuf[pl.ds(r, n), :] = x1
            hbuf[pl.ds(r, n), :] = _ln_mod(
                x1.astype(F32), mod_row(3, n), mod_row(4, n)).astype(BF16)

        row = lax.broadcasted_iota(jnp.int32, (NP, NP), 0)
        col = lax.broadcasted_iota(jnp.int32, (NP, NP), 1)

        def second(i):
            return ((i >= SEG) & (i < 2 * SEG)) | (i >= 2 * SEG + M)

        same = second(row) == second(col)
        mask = same & ((row >= 2 * SEG) | (col >= 2 * SEG) | (col <= row))
        fill = jnp.where(same, -1e9, -jnp.inf).astype(F32)

        def step(s, carry, mem, split, maybe_last, half_first, u):
            hr = pl.multiple_of(PAD + PRO + XR * s, 8)
            lhs_c = []
            for c in range(NC):
                cs = pl.ds(c * 128, 128)
                h8 = hbuf[pl.ds(hr + 16, 8), cs].astype(F32)
                lhs_c.append(jnp.concatenate(
                    [hbuf[pl.ds(hr, 16), cs],
                     jnp.concatenate([h8, mem[c]], axis=0).astype(BF16)], axis=0))
            lhs = jnp.concatenate(lhs_c, axis=1)

            if maybe_last:
                post_attn(pl.multiple_of(PAD + (s // UNROLL) * SH, 16), SH)

            wp, rp, op, ow = carry
            wpos = [pl.multiple_of(_wrap(wp + 8 * j, RING), 8)
                    for j in range(XR // 8)]
            win = pl.ds(pl.multiple_of(rp * (SEG * UNROLL // 2), 32),
                        SEG * UNROLL // 2)
            oblk = [pl.multiple_of(
                _wrap(op + (16 * j - 8 if half_first else 16 * j), ORING) // 2, 8)
                for j in range(2)]
            ofull, ohalf = (oblk[1], oblk[0]) if half_first else oblk
            owr = pl.multiple_of(ow, SEG)

            tails = {}
            xs = {}
            ps = {}
            lhs_o = {}

            def load(j, p):
                r32 = (q32, k32, v32)[j].at[:, win, :]
                xs[j, p] = [
                    pltpu.bitcast(
                        r32[h, pl.ds(u * (SEG // 2), SEG // 2), :], BF16)
                    for h in (2 * p, 2 * p + 1)]

            def operand(j, p):
                tail = jnp.concatenate(
                    [tails.pop((j, 2 * p)), tails.pop((j, 2 * p + 1))], axis=0)
                return jnp.concatenate(
                    xs.pop((j, p)) + [tail.astype(BF16)], axis=0)

            low = {}
            if split:
                lhs_lo = jnp.concatenate(lhs_c[:NC // 2], axis=1)
                lhs_hi = jnp.concatenate(lhs_c[NC // 2:], axis=1)
                for h in range(2):
                    for j, w32 in enumerate((wq32, wk32, wv32)):
                        low[j, h] = _dot(lhs_lo, pltpu.bitcast(
                            w32[h, pl.ds(0, D // 4), :], BF16))

            def proj(j, h):
                w32, ring = ((wq32, qring), (wk32, kring), (wv32, vring))[j]
                if (j, h) in low:
                    t = _dot(lhs_hi, pltpu.bitcast(
                        w32[h, pl.ds(D // 4, D // 4), :], BF16)) + low[j, h]
                else:
                    t = _dot(lhs, _w(w32, h))
                for i in range(XR // 8):
                    ring[h, pl.ds(wpos[i], 8), :] = (
                        t[8 * i:8 * i + 8].astype(BF16))
                tails[j, h] = t[XR:]

            def qk(p):
                sc = lax.dot_general(operand(0, p), operand(1, p),
                                     (((1,), (1,)), ((), ())),
                                     preferred_element_type=F32)
                sc = jnp.where(mask, sc * SCALE, fill)
                mx = jnp.max(sc, axis=-1, keepdims=True)
                e = jnp.exp(sc - mx)
                l = jnp.sum(e, axis=-1, keepdims=True)
                r = pl.reciprocal(l, approx=True)
                r = r * (2.0 - l * r)
                ps[p] = (e * r).astype(BF16)

            def pv(p):
                o = _dot(ps.pop(p), operand(2, p))
                for i, h in enumerate((2 * p, 2 * p + 1)):
                    xf = pltpu.bitcast(o32[h, pl.ds(ofull, 8), :], BF16)
                    xh2 = pltpu.bitcast(
                        o32[h, pl.ds(ohalf, 8), :], BF16).astype(F32)
                    om = o[2 * SEG + M * i:2 * SEG + M * (i + 1)]
                    if maybe_last:
                        om = jnp.where(s == NSEG - 1, xh2[8:], om)
                    last = jnp.concatenate(
                        [xh2[8:] if half_first else xh2[:8], om],
                        axis=0).astype(BF16)
                    lhs_o[h] = jnp.concatenate([xf, last], axis=0)
                for i, h in enumerate((2 * p, 2 * p + 1)):
                    oring[h, pl.ds(owr, SEG), :] = (
                        o[SEG * i:SEG * (i + 1)].astype(BF16))

            def wo_part(c, h0, h1):
                lo = jnp.concatenate([lhs_o[h] for h in range(h0, h1)], axis=1)
                w = pltpu.bitcast(wo32[c, pl.ds(h0 * 64, (h1 - h0) * 64), :], BF16)
                return _dot(lo, w)

            NPR = H // 2
            for t in range(NPR):
                if t >= 1:
                    load(0, t - 1)
                    load(1, t - 1)
                if t >= 2:
                    load(2, t - 2)
                for pos in range(6):
                    if t >= 1 and pos == (QPOS1 if t == 1 else QPOS):
                        qk(t - 1)
                    proj(pos % 3, 2 * t + pos // 3)
                if t >= 2:
                    pv(t - 2)
            HA = H - 4
            ar = pl.multiple_of(PAD - XR + XR * s, 8)
            acc = {}
            mem_new = {}

            def wo_a(c):
                acc[c] = wo_part(c, 0, HA)

            def wo_b(c):
                a = wo_part(c, HA, H) + acc[c]
                cs = pl.ds(c * 128, 128)
                if half_first:
                    abuf[pl.ds(ar + 8, 16), cs] = a[:16].astype(BF16)
                    abuf[pl.ds(ar, 8), cs] = a[16:XR].astype(BF16)
                else:
                    n = XR + M if maybe_last else XR
                    abuf[pl.ds(ar, n), cs] = a[:n].astype(BF16)
                mem_new[c] = a[XR:]

            load(0, NPR - 1)
            load(1, NPR - 1)
            load(2, NPR - 2)
            wo_a(0)
            qk(NPR - 1)
            wo_a(1)
            pv(NPR - 2)
            load(2, NPR - 1)
            for c in (2, 3, 4):
                wo_a(c)
            pv(NPR - 1)
            for c in (5, 6):
                wo_a(c)
            for c in range(NC // 2):
                wo_b(c)
            wo_a(7)
            for c in range(NC // 2, NC):
                wo_b(c)
            return (_wrap(wp + XR, RING), _wrap(rp + 1, RING // (SEG * UNROLL)) if maybe_last else rp,
                    _wrap(op + XR, ORING), _wrap(ow + SEG, ORING)), mem_new

        def steps(i, carry):
            mem = [mem_s[:, pl.ds(c * 128, 128)] for c in range(NC)]
            for u in range(UNROLL):
                carry, mem = step(i * UNROLL + u, carry, mem, split=u > 0,
                                  maybe_last=u == UNROLL - 1,
                                  half_first=u % 2 == 0, u=u)
            for c in range(NC):
                mem_s[:, pl.ds(c * 128, 128)] = mem[c]
            return carry

        lax.fori_loop(0, NSEG // UNROLL, steps,
                      (jnp.int32(PRO), jnp.int32(0), jnp.int32(OOFF - XR),
                       jnp.int32(OOFF)))

        done = XR * (NSEG - 1) + M

        def wo_bulk(i):
            p = pl.multiple_of(((done + OOFF) % ORING + i * WB) // 2, 8)
            lo = jnp.concatenate(
                [pltpu.bitcast(o32[h, pl.ds(p, WB // 2), :], BF16)
                 for h in range(H)], axis=1)
            rows = pl.ds(pl.multiple_of(PAD + done + i * WB, 16), WB)
            for c in range(NC):
                abuf[rows, pl.ds(c * 128, 128)] = (
                    _dot(lo, _w(wo32, c)).astype(BF16))

        for cp in cp_w1 + cp_w3 + cp_w2:
            cp.wait()

        def cp_out(r, n, part):
            cols = pl.ds(0, OC * 128) if part == 0 else pl.ds(OC * 128, D - OC * 128)
            return pltpu.make_async_copy(xbuf.at[pl.ds(PAD + r, n), cols],
                                         out_hbm.at[pl.ds(r, n), cols],
                                         sems.at[SEM_OUT])

        def ffn_body(i, carry, r0, n, with_wo, p0, npc):
            r = pl.multiple_of(r0 + i * n, 16)
            rows = pl.ds(pl.multiple_of(PAD + r, 16), n)
            if with_wo:
                wo_bulk(i)
            hv = hbuf[rows, :]
            act = []
            for f in range(NF):
                g = _dot(hv, _w(w132, f))
                u = _dot(hv, _w(w332, f))
                act.append((g * jax.nn.sigmoid(g) * u).astype(BF16))
            av = jnp.concatenate(act, axis=1)
            for c in range(NC):
                y = _dot(av, _w(w232, c))
                for k in range(npc):
                    if k * (NC - 1) // npc == c:
                        pr = p0 + (i * npc + k) * 16
                        post_attn(pl.multiple_of(
                            jnp.where(pr < S, PAD + pr, 0), 16), 16)
                cs = pl.ds(c * 128, 128)
                x2 = xbuf[rows, cs].astype(F32) + mod_row(5, n, cs) * y
                xbuf[rows, cs] = x2.astype(BF16)
                if c == OC - 1:
                    cp_out(r, n, 0).start()
            cp_out(r, n, 1).start()
            return carry

        nfb = (S - NWB * FA) // FB
        pa = SH * (NSEG // UNROLL)
        lax.fori_loop(0, NWB, functools.partial(
            ffn_body, r0=0, n=FA, with_wo=True, p0=pa, npc=NPA), 0)
        lax.fori_loop(0, nfb, functools.partial(
            ffn_body, r0=NWB * FA, n=FB, with_wo=False,
            p0=pa + NWB * NPA * 16, npc=NPB), 0)
        for part in range(2):
            for i in range(NWB):
                cp_out(i * FA, FA, part).wait()
            for i in range(nfb):
                cp_out(NWB * FA + i * FB, FB, part).wait()

    pl.run_scoped(
        rest,
        pltpu.VMEM((NF, D, 128), BF16),
        pltpu.VMEM((NF, D, 128), BF16),
        pltpu.VMEM((NC, F, 128), BF16),
        pltpu.VMEM((H, ORING, DH), BF16),
        pltpu.VMEM((PAD + S, D), BF16),
    )


@functools.partial(jax.jit, static_argnames=("A_seg_len",))
def pallas_adaLN_cond__memory_aug_recurrent_mem_tr__glu_gated_swiglu__prompt_kernel(
    A_x: jax.Array,
    A_mem0: jax.Array,
    A_Wq: jax.Array,
    A_Wk: jax.Array,
    A_Wv: jax.Array,
    A_Wo: jax.Array,
    A_seg_len,
    B_x: jax.Array,
    B_w1: jax.Array,
    B_w3: jax.Array,
    B_w2: jax.Array,
    c: jax.Array,
    w_mod: jax.Array,
):
    del B_x
    assert A_seg_len == SEG
    assert A_x.shape == (1, S, D) and A_mem0.shape == (1, M, D)
    assert A_Wq.shape == (D, H, DH) and B_w1.shape == (D, F)

    any_spec = pl.BlockSpec(memory_space=pl.ANY)
    out = pl.pallas_call(
        _kernel,
        out_shape=jax.ShapeDtypeStruct((S, D), BF16),
        in_specs=[any_spec] * 11,
        out_specs=any_spec,
        scratch_shapes=[
            pltpu.VMEM((H, D // 2, DH), U32),
            pltpu.VMEM((H, D // 2, DH), U32),
            pltpu.VMEM((H, D // 2, DH), U32),
            pltpu.VMEM((NC, H * DH, 128), BF16),
            pltpu.VMEM((2, PAD + S, D), BF16),
            pltpu.VMEM((H, RING, DH), BF16),
            pltpu.VMEM((H, RING, DH), BF16),
            pltpu.VMEM((H, RING, DH), BF16),
            pltpu.VMEM((6 * 8, D), F32),
            pltpu.VMEM((M, D), F32),
            pltpu.VMEM((1, D), BF16),
            pltpu.VMEM((M, D), BF16),
            pltpu.SemaphoreType.DMA((NSEMS,)),
        ],
        compiler_params=pltpu.CompilerParams(
            vmem_limit_bytes=120 * 1024 * 1024,
            disable_semaphore_checks=True, disable_bounds_checks=True),
        name="adaln_memtr_swiglu",
    )(
        A_x.reshape(S, D),
        A_mem0.reshape(M, D),
        A_Wq, A_Wk, A_Wv,
        A_Wo.reshape(H * DH, D),
        B_w1, B_w3, B_w2, c, w_mod,
    )
    return out.reshape(1, S, D)
```

```python
import functools

import jax
import jax.numpy as jnp
from jax import lax
import jax.experimental.pallas as pl
import jax.experimental.pallas.tpu as pltpu

BF16 = jnp.bfloat16
F32 = jnp.float32
U32 = jnp.uint32

S = 2048
D = 1024
H = 32
DH = 128
F = 3584
M = 8
SEG = 32
NSEG = S // SEG
XR = 24
PRO = S - XR * NSEG
RING = 640
ORING = 576
OOFF = 256
PAD = 48
NC = D // 128
NF = F // 128
FA = 128
FB = 208
OC = 7
NWB = 3
WB = 176
SH = 16
NPA, NPB = 11, 12
QPOS, QPOS1 = 2, 4
UNROLL = 4
NU = 3 * H // 2
UPI = 6
NUA = 12
NUZ = 12
XC = (S - PRO) * UPI // (NU - NUA)
NUG = 5
NP = 2 * (SEG + M)
EPS = 1e-5
SEM_FIRST, SEM_WO, SEM_MID, SEM_FFN, SEM_OUT = 0, 1, 2, 3, 4
SEM_CA = 5
SEM_U0 = SEM_CA + 2
U0_GROUP = (0, 1, 2, 3, 3, 4, 5, 5, 5, 6, 6, 6, 6)
SEM_SA = SEM_U0 + U0_GROUP[NUG]
SEM_IT = SEM_U0 + U0_GROUP[-1] + 1 - NUA // UPI
NSEMS = SEM_IT + NU // UPI
SCALE = DH ** -0.5


def _dot(a, b):
    return jnp.dot(a, b, preferred_element_type=F32)


def _w(ref32, i):
    return pltpu.bitcast(ref32[i], BF16)


def _wrap(i, n):
    return jnp.where(i >= n, i - n, i)


def _ln(x):
    mu = jnp.mean(x, axis=-1, keepdims=True)
    xc = x - mu
    var = jnp.mean(xc * xc, axis=-1, keepdims=True)
    return xc * lax.rsqrt(var + EPS)


def _ln_mod(x, shift, scale1):
    return _ln(x) * scale1 + shift


def _kernel(x_hbm, mem0_hbm, wq_hbm, wk_hbm, wv_hbm, wo_hbm, w1_hbm, w3_hbm,
            w2_hbm, c_hbm, wmod_hbm, out_hbm,
            wq32, wk32, wv32, wo_s, xh, qring, kring, vring,
            mod_s, mem_s, c_s, m0_s, sems):
    wo32 = wo_s.bitcast(U32)
    xbuf = xh.at[0]
    hbuf = xh.at[1]

    cp_x0 = pltpu.make_async_copy(x_hbm.at[pl.ds(0, PRO)],
                                  xbuf.at[pl.ds(PAD, PRO)], sems.at[SEM_FIRST])
    cp_c = pltpu.make_async_copy(c_hbm, c_s, sems.at[SEM_FIRST])
    cp_m0 = pltpu.make_async_copy(mem0_hbm, m0_s, sems.at[SEM_MID])
    cp_wo = [pltpu.make_async_copy(wo_hbm.at[:, pl.ds(c * 128, 128)],
                                   wo_s.at[c], sems.at[SEM_WO])
             for c in range(NC)]

    def cp_x(k, sem):
        r = PRO + k * XC
        if not isinstance(k, int):
            r = pl.multiple_of(r, XC)
        return pltpu.make_async_copy(x_hbm.at[pl.ds(r, XC)],
                                     xbuf.at[pl.ds(PAD + r, XC)], sems.at[sem])

    def mod_row(i, n, cols=slice(None)):
        return jnp.concatenate([mod_s[pl.ds(8 * i, 8), cols]] * (n // 8), axis=0)

    def prologue(st, wm_s, xn_s, g_s, h0_s, tmp_s, sct_s):
        wm32 = wm_s.bitcast(U32)
        srcs = (wq_hbm.bitcast(U32), wk_hbm.bitcast(U32), wv_hbm.bitcast(U32))
        dsts = (wq32, wk32, wv32)
        rings = (qring, kring, vring)

        def cp_st(j, s, sem):
            return pltpu.make_async_copy(srcs[j].at[:, s, :], st.at[3 * s + j],
                                         sems.at[sem])

        def cp_unit(u):
            sem = (SEM_U0 + U0_GROUP[u] if u <= NUA
                   else SEM_IT + (u - 1) // UPI)
            return cp_st(u % 3, u // 3, sem)

        def cp_wm(i):
            sem = (SEM_SA if i < 8 else
                   SEM_CA + (i - 8) // 4 if i < 16 else SEM_MID)
            return pltpu.make_async_copy(wmod_hbm.at[:, pl.ds(i * 128, 128)],
                                         wm_s.at[i], sems.at[sem])

        it0, it1 = NUA // UPI, (NU - NUZ) // UPI
        cp_mid = ([cp_x(k, SEM_MID) for k in range(it1 - it0, NU // UPI - it0)]
                  + [cp_wm(i) for i in range(16, 48)])

        cp_c.start()
        cp_x0.start()
        cp_unit(0).start()
        for i in range(8, 16):
            cp_wm(i).start()
        for u in range(1, NUG):
            cp_unit(u).start()
        for i in range(8):
            cp_wm(i).start()
        for u in range(NUG, NU):
            cp_unit(u).start()
            if u % UPI == 0 and it0 < u // UPI <= it1:
                cp_x(u // UPI - 1 - it0, SEM_IT + u // UPI - 1).start()
        cp_m0.start()

        xbuf[pl.ds(0, PAD), :] = jnp.zeros((PAD, D), BF16)

        cp_c.wait()
        cp_x0.wait()
        cf = c_s[...].astype(F32)
        sc = (cf * jax.nn.sigmoid(cf)).astype(BF16)
        sc8 = jnp.broadcast_to(sc, (8, D))
        sct_s[pl.ds(0, D), :] = jnp.broadcast_to(sc.astype(F32), (128, D)).T

        def ln_body(i, carry):
            r = pl.multiple_of(i * 64, 64)
            xv = xbuf[pl.ds(pl.multiple_of(PAD + r, 8), 64), :].astype(F32)
            xn_s[pl.ds(r, 64), :] = _ln(xv)
            return carry

        lax.fori_loop(0, PRO // 64, ln_body, 0)

        def mod_slab(i):
            k, c = divmod(i, NC)
            part = _dot(sc8, _w(wm32, i))
            if k in (1, 4):
                part = part + 1.0
            mod_s[pl.ds(8 * k, 8), pl.ds(c * 128, 128)] = part

        def relayout(j, s):
            u = 3 * s + j
            for db in range(8):
                ev = st[u, pl.ds(db * 128, 64, stride=2), :]
                od = st[u, pl.ds(db * 128 + 1, 64, stride=2), :]
                rows = pl.ds(db * 64, 64)
                dsts[j][2 * s, rows, :] = (ev & U32(0xFFFF)) | (od << 16)
                dsts[j][2 * s + 1, rows, :] = (ev >> 16) | (od & U32(0xFFFF0000))

        def bulk(j, s, extras=(), mbs=range(PRO // 128)):
            extras = list(extras)
            for mb in mbs:
                lhs = h0_s[pl.ds(mb * 128, 128), :]
                for hh in range(2):
                    h = 2 * s + hh
                    t = _dot(lhs, _w(dsts[j], h))
                    if extras:
                        t = extras.pop(0)(t)
                    rings[j][h, pl.ds(mb * 128, 128), :] = t.astype(BF16)

        def bulk_g(u, mbs):
            for mb in mbs:
                rows = pl.ds(mb * 128, 128)
                lhs = g_s[rows, :]
                for hh in range(2):
                    tmp_s[2 * u + hh, rows, :] = _dot(
                        lhs, _w(dsts[u % 3], 2 * (u // 3) + hh))

        def add_shift(u, hh):
            h = 2 * (u // 3) + hh
            b = _dot(mod_row(0, 8).astype(BF16), _w(dsts[u % 3], h))
            rings[u % 3][h, pl.ds(0, PRO), :] = (
                tmp_s[2 * u + hh] + jnp.concatenate([b] * (PRO // 8), axis=0)
            ).astype(BF16)

        def wait_group(g):
            if g == U0_GROUP[NUG]:
                for i in range(8):
                    cp_wm(i).wait()
            for v in range(NUA + 1):
                if U0_GROUP[v] == g:
                    cp_unit(v).wait()

        def relayout_u(u):
            relayout(u % 3, u // 3)

        def scale_half(k):
            for i in range(8 + 4 * k, 12 + 4 * k):
                mod_slab(i)
            cols = pl.ds(k * (D // 2), D // 2)
            g_s[:, cols] = (xn_s[:, cols] * mod_row(1, PRO, cols)).astype(BF16)

        def first_half(k, mbs):
            for mb in mbs:
                rows = pl.ds(mb * 128, 128)
                lhs = g_s[rows, pl.ds(k * (D // 2), D // 2)]
                for hh in range(2):
                    t = _dot(lhs, pltpu.bitcast(
                        wq32[hh, pl.ds(k * (D // 4), D // 4), :], BF16))
                    tmp_s[hh, rows, :] = t if k == 0 else t + tmp_s[hh, rows, :]

        wait_group(0)
        relayout_u(0)
        for k in range(2):
            for i in range(8 + 4 * k, 12 + 4 * k):
                cp_wm(i).wait()
            scale_half(k)
            first_half(k, range(4))
        wait_group(1)
        relayout_u(1)
        bulk_g(1, (0, 1, 2))
        wait_group(2)
        relayout_u(2)
        bulk_g(1, (3,))
        bulk_g(2, (0, 1, 2))
        wait_group(3)
        relayout_u(3)
        bulk_g(2, (3,))
        relayout_u(4)
        bulk_g(3, range(4))
        bulk_g(4, (0, 1, 2))
        wait_group(4)
        relayout_u(5)
        for i in range(8):
            mod_slab(i)
        bulk_g(4, (3,))
        for mb in range(PRO // 128):
            rows = pl.ds(mb * 128, 128)
            h0_s[rows, :] = (
                xn_s[rows, :] * mod_row(1, 128) + mod_row(0, 128)).astype(BF16)
        shifts = [lambda t, v=v, hh=hh: (add_shift(v, hh), t)[1]
                  for v in range(NUG) for hh in range(2)]
        bulk(5 % 3, 5 // 3, shifts[:6], mbs=(0, 1, 2))
        wait_group(5)
        relayout_u(6)
        bulk(5 % 3, 5 // 3, shifts[6:8], mbs=(3,))
        for u in range(6, NUA):
            if U0_GROUP[u + 1] != U0_GROUP[u]:
                wait_group(U0_GROUP[u + 1])
            relayout_u(u + 1)
            bulk(u % 3, u // 3, shifts[8:] if u == 6 else ())

        pending = []

        def tie(never, a, b):
            top = jnp.where(never, a[:8, :128], b[:8, :128])
            if b.shape[1] > 128:
                top = jnp.concatenate([top, b[:8, 128:]], axis=1)
            return jnp.concatenate([top, b[8:]], axis=0)

        def ln1_piece(r, t):
            never = r < 0
            if pending:
                t = tie(never, pending.pop(), t)
            rows = pl.ds(pl.multiple_of(r, 16), 16)
            xv = tie(never, t, xbuf[rows, :].astype(F32))
            hv = _ln_mod(xv, mod_row(0, 16), mod_row(1, 16))
            hbuf[rows, :] = hv.astype(BF16)
            pending.append(hv[8:])
            return t

        def unit_extras(r, u, more=()):
            slots = [lambda t: t] * 8
            for d, f in more:
                slots[d] = f
            for k in range(XC // 16):
                d = k * (8 * UPI) // (XC // 16)
                if d // 8 == u % UPI:
                    slots[d % 8] = lambda t, g=slots[d % 8], k=k: (
                        ln1_piece(r + 16 * k, g(t)))
            return slots

        def grp_body(it, r):
            s0 = it * (UPI // 3)

            @pl.when(it == it0)
            def _():
                for cp in cp_mid + cp_wo:
                    cp.start()

            for u in range(1, UPI + 1):
                cp_st(u % 3, s0 + u // 3, SEM_IT + it).wait()
            cp_x(it - it0, SEM_IT + it).wait()
            for u in range(UPI):
                relayout((u + 1) % 3, s0 + (u + 1) // 3)
                bulk(u % 3, s0 + u // 3, unit_extras(r, u))
            pending.clear()
            return r + XC

        r1 = lax.fori_loop(it0, it1, grp_body, jnp.int32(PAD + PRO))

        accs = {}
        pending2 = []

        def mod_piece(n, t):
            gp, q = divmod(n, 8)
            never = r1 < 0
            if pending2:
                t = tie(never, pending2.pop(), t)
            zero = r1 - (PAD + PRO + (it1 - it0) * XC)
            sct_s[pl.ds(pl.multiple_of(D + zero, 8), 8), :] = t[:8]
            wm32[zero, pl.ds(0, 8), :] = pltpu.bitcast(t[:8], U32)
            acc = accs.get(gp, [None] * 4)
            for j in range(8 * q, 8 * q + 8):
                se = sct_s[pl.ds(16 * j, 8, stride=2), :]
                so = sct_s[pl.ds(16 * j + 1, 8, stride=2), :]
                for k in range(4):
                    w = wm32[16 + 4 * gp + k, pl.ds(8 * j, 8), :]
                    p = (pltpu.bitcast(w << 16, F32) * se
                         + pltpu.bitcast(w & U32(0xFFFF0000), F32) * so)
                    acc[k] = p if acc[k] is None else acc[k] + p
            accs[gp] = acc
            pending2.append(acc[0] + acc[1] + acc[2] + acc[3])
            if q == 7:
                for k in range(4):
                    row, c = divmod(16 + 4 * gp + k, NC)
                    part = jnp.sum(acc[k], axis=0, keepdims=True)
                    if row == 4:
                        part = part + 1.0
                    mod_s[pl.ds(8 * row, 8), pl.ds(c * 128, 128)] = (
                        jnp.broadcast_to(part, (8, 128)))
            return t

        for u in range(NU - NUZ + 1, NU):
            cp_unit(u).wait()
        for cp in cp_mid + [cp_m0]:
            cp.wait()
        mem_s[...] = m0_s[...].astype(F32)
        SPOTS = [d for d in range(8 * NUZ) if d % 3]
        for u in range(NU - NUZ, NU):
            if u + 1 < NU:
                relayout_u(u + 1)
            v = u - (NU - NUZ)
            bulk(u % 3, u // 3, unit_extras(
                r1 + v // UPI * XC, u,
                [(d % 8, functools.partial(mod_piece, n))
                 for n, d in enumerate(SPOTS) if d // 8 == v]))
        for cp in cp_wo:
            cp.wait()

    pl.run_scoped(
        prologue,
        pltpu.VMEM((NU, D, DH), U32),
        pltpu.VMEM((48, D, 128), BF16),
        pltpu.VMEM((PRO, D), F32),
        pltpu.VMEM((PRO, D), BF16),
        pltpu.VMEM((PRO, D), BF16),
        pltpu.VMEM((2 * NUG, PRO, DH), F32),
        pltpu.VMEM((D + 8, 128), F32),
    )

    def rest(w1_s, w3_s, w2_s, oring, abuf):
        w132 = w1_s.bitcast(U32)
        w332 = w3_s.bitcast(U32)
        w232 = w2_s.bitcast(U32)
        q32 = qring.bitcast(U32)
        k32 = kring.bitcast(U32)
        v32 = vring.bitcast(U32)

        cp_w1 = [pltpu.make_async_copy(w1_hbm.at[:, pl.ds(f * 128, 128)],
                                       w1_s.at[f], sems.at[SEM_FFN])
                 for f in range(NF)]
        cp_w3 = [pltpu.make_async_copy(w3_hbm.at[:, pl.ds(f * 128, 128)],
                                       w3_s.at[f], sems.at[SEM_FFN])
                 for f in range(NF)]
        cp_w2 = [pltpu.make_async_copy(w2_hbm.at[:, pl.ds(c * 128, 128)],
                                       w2_s.at[c], sems.at[SEM_FFN])
                 for c in range(NC)]
        for cp in cp_w1 + cp_w3 + cp_w2:
            cp.start()

        o32 = oring.bitcast(U32)

        o32[:, pl.ds(OOFF // 2 - 16, 16), :] = jnp.zeros((H, 16, DH), U32)

        abuf[pl.ds(0, PAD), :] = jnp.zeros((PAD, D), BF16)

        def post_attn(r, n):
            a = abuf[pl.ds(r, n), :].astype(F32)
            x1 = xbuf[pl.ds(r, n), :].astype(F32) + mod_row(2, n) * a
            x1 = x1.astype(BF16)
            xbuf[pl.ds(r, n), :] = x1
            hbuf[pl.ds(r, n), :] = _ln_mod(
                x1.astype(F32), mod_row(3, n), mod_row(4, n)).astype(BF16)

        row = lax.broadcasted_iota(jnp.int32, (NP, NP), 0)
        col = lax.broadcasted_iota(jnp.int32, (NP, NP), 1)

        def second(i):
            return ((i >= SEG) & (i < 2 * SEG)) | (i >= 2 * SEG + M)

        same = second(row) == second(col)
        mask = same & ((row >= 2 * SEG) | (col >= 2 * SEG) | (col <= row))
        fill = jnp.where(same, -1e9, -jnp.inf).astype(F32)

        def step(s, carry, mem, split, maybe_last, half_first, u):
            hr = pl.multiple_of(PAD + PRO + XR * s, 8)
            lhs_c = []
            for c in range(NC):
                cs = pl.ds(c * 128, 128)
                h8 = hbuf[pl.ds(hr + 16, 8), cs].astype(F32)
                lhs_c.append(jnp.concatenate(
                    [hbuf[pl.ds(hr, 16), cs],
                     jnp.concatenate([h8, mem[c]], axis=0).astype(BF16)], axis=0))
            lhs = jnp.concatenate(lhs_c, axis=1)

            if maybe_last:
                post_attn(pl.multiple_of(PAD + (s // UNROLL) * SH, 16), SH)

            wp, rp, op, ow = carry
            wpos = [pl.multiple_of(_wrap(wp + 8 * j, RING), 8)
                    for j in range(XR // 8)]
            win = pl.ds(pl.multiple_of(rp * (SEG * UNROLL // 2), 32),
                        SEG * UNROLL // 2)
            oblk = [pl.multiple_of(
                _wrap(op + (16 * j - 8 if half_first else 16 * j), ORING) // 2, 8)
                for j in range(2)]
            ofull, ohalf = (oblk[1], oblk[0]) if half_first else oblk
            owr = pl.multiple_of(ow, SEG)

            tails = {}
            xs = {}
            ps = {}
            lhs_o = {}

            def load(j, p):
                r32 = (q32, k32, v32)[j].at[:, win, :]
                xs[j, p] = [
                    pltpu.bitcast(
                        r32[h, pl.ds(u * (SEG // 2), SEG // 2), :], BF16)
                    for h in (2 * p, 2 * p + 1)]

            def operand(j, p):
                tail = jnp.concatenate(
                    [tails.pop((j, 2 * p)), tails.pop((j, 2 * p + 1))], axis=0)
                return jnp.concatenate(
                    xs.pop((j, p)) + [tail.astype(BF16)], axis=0)

            low = {}
            if split:
                lhs_lo = jnp.concatenate(lhs_c[:NC // 2], axis=1)
                lhs_hi = jnp.concatenate(lhs_c[NC // 2:], axis=1)
                for h in range(2):
                    for j, w32 in enumerate((wq32, wk32, wv32)):
                        low[j, h] = _dot(lhs_lo, pltpu.bitcast(
                            w32[h, pl.ds(0, D // 4), :], BF16))

            def proj(j, h):
                w32, ring = ((wq32, qring), (wk32, kring), (wv32, vring))[j]
                if (j, h) in low:
                    t = _dot(lhs_hi, pltpu.bitcast(
                        w32[h, pl.ds(D // 4, D // 4), :], BF16)) + low[j, h]
                else:
                    t = _dot(lhs, _w(w32, h))
                for i in range(XR // 8):
                    ring[h, pl.ds(wpos[i], 8), :] = (
                        t[8 * i:8 * i + 8].astype(BF16))
                tails[j, h] = t[XR:]

            def qk(p):
                sc = lax.dot_general(operand(0, p), operand(1, p),
                                     (((1,), (1,)), ((), ())),
                                     preferred_element_type=F32)
                sc = jnp.where(mask, sc * SCALE, fill)
                mx = jnp.max(sc, axis=-1, keepdims=True)
                e = jnp.exp(sc - mx)
                l = jnp.sum(e, axis=-1, keepdims=True)
                r = pl.reciprocal(l, approx=True)
                r = r * (2.0 - l * r)
                ps[p] = (e * r).astype(BF16)

            def pv(p):
                o = _dot(ps.pop(p), operand(2, p))
                for i, h in enumerate((2 * p, 2 * p + 1)):
                    xf = pltpu.bitcast(o32[h, pl.ds(ofull, 8), :], BF16)
                    xh2 = pltpu.bitcast(
                        o32[h, pl.ds(ohalf, 8), :], BF16).astype(F32)
                    om = o[2 * SEG + M * i:2 * SEG + M * (i + 1)]
                    if maybe_last:
                        om = jnp.where(s == NSEG - 1, xh2[8:], om)
                    last = jnp.concatenate(
                        [xh2[8:] if half_first else xh2[:8], om],
                        axis=0).astype(BF16)
                    lhs_o[h] = jnp.concatenate([xf, last], axis=0)
                for i, h in enumerate((2 * p, 2 * p + 1)):
                    oring[h, pl.ds(owr, SEG), :] = (
                        o[SEG * i:SEG * (i + 1)].astype(BF16))

            def wo_part(c, h0, h1):
                lo = jnp.concatenate([lhs_o[h] for h in range(h0, h1)], axis=1)
                w = pltpu.bitcast(wo32[c, pl.ds(h0 * 64, (h1 - h0) * 64), :], BF16)
                return _dot(lo, w)

            NPR = H // 2
            for t in range(NPR):
                if t >= 1:
                    load(0, t - 1)
                    load(1, t - 1)
                if t >= 2:
                    load(2, t - 2)
                for pos in range(6):
                    if t >= 1 and pos == (QPOS1 if t == 1 else QPOS):
                        qk(t - 1)
                    proj(pos % 3, 2 * t + pos // 3)
                if t >= 2:
                    pv(t - 2)
            HA = H - 4
            ar = pl.multiple_of(PAD - XR + XR * s, 8)
            acc = {}
            mem_new = {}

            def wo_a(c):
                acc[c] = wo_part(c, 0, HA)

            def wo_b(c):
                a = wo_part(c, HA, H) + acc[c]
                cs = pl.ds(c * 128, 128)
                if half_first:
                    abuf[pl.ds(ar + 8, 16), cs] = a[:16].astype(BF16)
                    abuf[pl.ds(ar, 8), cs] = a[16:XR].astype(BF16)
                else:
                    n = XR + M if maybe_last else XR
                    abuf[pl.ds(ar, n), cs] = a[:n].astype(BF16)
                mem_new[c] = a[XR:]

            load(0, NPR - 1)
            load(1, NPR - 1)
            load(2, NPR - 2)
            wo_a(0)
            qk(NPR - 1)
            wo_a(1)
            pv(NPR - 2)
            load(2, NPR - 1)
            for c in (2, 3, 4):
                wo_a(c)
            pv(NPR - 1)
            for c in (5, 6):
                wo_a(c)
            for c in range(NC // 2):
                wo_b(c)
            wo_a(7)
            for c in range(NC // 2, NC):
                wo_b(c)
            return (_wrap(wp + XR, RING), _wrap(rp + 1, RING // (SEG * UNROLL)) if maybe_last else rp,
                    _wrap(op + XR, ORING), _wrap(ow + SEG, ORING)), mem_new

        def steps(i, carry):
            mem = [mem_s[:, pl.ds(c * 128, 128)] for c in range(NC)]
            for u in range(UNROLL):
                carry, mem = step(i * UNROLL + u, carry, mem, split=u > 0,
                                  maybe_last=u == UNROLL - 1,
                                  half_first=u % 2 == 0, u=u)
            for c in range(NC):
                mem_s[:, pl.ds(c * 128, 128)] = mem[c]
            return carry

        lax.fori_loop(0, NSEG // UNROLL, steps,
                      (jnp.int32(PRO), jnp.int32(0), jnp.int32(OOFF - XR),
                       jnp.int32(OOFF)))

        done = XR * (NSEG - 1) + M

        def wo_bulk(i):
            p = pl.multiple_of(((done + OOFF) % ORING + i * WB) // 2, 8)
            lo = jnp.concatenate(
                [pltpu.bitcast(o32[h, pl.ds(p, WB // 2), :], BF16)
                 for h in range(H)], axis=1)
            rows = pl.ds(pl.multiple_of(PAD + done + i * WB, 16), WB)
            for c in range(NC):
                abuf[rows, pl.ds(c * 128, 128)] = (
                    _dot(lo, _w(wo32, c)).astype(BF16))

        for cp in cp_w1 + cp_w3 + cp_w2:
            cp.wait()

        def cp_out(r, n, part):
            cols = pl.ds(0, OC * 128) if part == 0 else pl.ds(OC * 128, D - OC * 128)
            return pltpu.make_async_copy(xbuf.at[pl.ds(PAD + r, n), cols],
                                         out_hbm.at[pl.ds(r, n), cols],
                                         sems.at[SEM_OUT])

        def ffn_body(i, carry, r0, n, with_wo, p0, npc):
            r = pl.multiple_of(r0 + i * n, 16)
            rows = pl.ds(pl.multiple_of(PAD + r, 16), n)
            if with_wo:
                wo_bulk(i)
            hv = hbuf[rows, :]
            act = []
            for f in range(NF):
                g = _dot(hv, _w(w132, f))
                u = _dot(hv, _w(w332, f))
                act.append((g * jax.nn.sigmoid(g) * u).astype(BF16))
            av = jnp.concatenate(act, axis=1)
            for c in range(NC):
                y = _dot(av, _w(w232, c))
                for k in range(npc):
                    if k * (NC - 1) // npc == c:
                        pr = p0 + (i * npc + k) * 16
                        post_attn(pl.multiple_of(
                            jnp.where(pr < S, PAD + pr, 0), 16), 16)
                cs = pl.ds(c * 128, 128)
                x2 = xbuf[rows, cs].astype(F32) + mod_row(5, n, cs) * y
                xbuf[rows, cs] = x2.astype(BF16)
                if c == OC - 1:
                    cp_out(r, n, 0).start()
            cp_out(r, n, 1).start()
            return carry

        nfb = (S - NWB * FA) // FB
        pa = SH * (NSEG // UNROLL)
        lax.fori_loop(0, NWB, functools.partial(
            ffn_body, r0=0, n=FA, with_wo=True, p0=pa, npc=NPA), 0)
        lax.fori_loop(0, nfb, functools.partial(
            ffn_body, r0=NWB * FA, n=FB, with_wo=False,
            p0=pa + NWB * NPA * 16, npc=NPB), 0)
        for part in range(2):
            for i in range(NWB):
                cp_out(i * FA, FA, part).wait()
            for i in range(nfb):
                cp_out(NWB * FA + i * FB, FB, part).wait()

    pl.run_scoped(
        rest,
        pltpu.VMEM((NF, D, 128), BF16),
        pltpu.VMEM((NF, D, 128), BF16),
        pltpu.VMEM((NC, F, 128), BF16),
        pltpu.VMEM((H, ORING, DH), BF16),
        pltpu.VMEM((PAD + S, D), BF16),
    )


@functools.partial(jax.jit, static_argnames=("A_seg_len",))
def pallas_adaLN_cond__memory_aug_recurrent_mem_tr__glu_gated_swiglu__prompt_kernel(
    A_x: jax.Array,
    A_mem0: jax.Array,
    A_Wq: jax.Array,
    A_Wk: jax.Array,
    A_Wv: jax.Array,
    A_Wo: jax.Array,
    A_seg_len,
    B_x: jax.Array,
    B_w1: jax.Array,
    B_w3: jax.Array,
    B_w2: jax.Array,
    c: jax.Array,
    w_mod: jax.Array,
):
    del B_x
    assert A_seg_len == SEG
    assert A_x.shape == (1, S, D) and A_mem0.shape == (1, M, D)
    assert A_Wq.shape == (D, H, DH) and B_w1.shape == (D, F)

    any_spec = pl.BlockSpec(memory_space=pl.ANY)
    out = pl.pallas_call(
        _kernel,
        out_shape=jax.ShapeDtypeStruct((S, D), BF16),
        in_specs=[any_spec] * 11,
        out_specs=any_spec,
        scratch_shapes=[
            pltpu.VMEM((H, D // 2, DH), U32),
            pltpu.VMEM((H, D // 2, DH), U32),
            pltpu.VMEM((H, D // 2, DH), U32),
            pltpu.VMEM((NC, H * DH, 128), BF16),
            pltpu.VMEM((2, PAD + S, D), BF16),
            pltpu.VMEM((H, RING, DH), BF16),
            pltpu.VMEM((H, RING, DH), BF16),
            pltpu.VMEM((H, RING, DH), BF16),
            pltpu.VMEM((6 * 8, D), F32),
            pltpu.VMEM((M, D), F32),
            pltpu.VMEM((1, D), BF16),
            pltpu.VMEM((M, D), BF16),
            pltpu.SemaphoreType.DMA((NSEMS,)),
        ],
        compiler_params=pltpu.CompilerParams(
            vmem_limit_bytes=120 * 1024 * 1024,
            disable_semaphore_checks=True, disable_bounds_checks=True),
        name="adaln_memtr_swiglu",
    )(
        A_x.reshape(S, D),
        A_mem0.reshape(M, D),
        A_Wq, A_Wk, A_Wv,
        A_Wo.reshape(H * DH, D),
        B_w1, B_w3, B_w2, c, w_mod,
    )
    return out.reshape(1, S, D)
```
